```python
import jax
import jax.numpy as jnp

def _softmax(x, axis=-1):
    return jax.nn.softmax(x, axis=axis)

def _gelu(x):
    return jax.nn.gelu(x, approximate=True)

def _silu(x):
    return jax.nn.silu(x)

def _sigmoid(x):
    return jax.nn.sigmoid(x)

def _layernorm(x, axis=-1, eps=1e-05):
    m = jnp.mean(x, axis=axis, keepdims=True)
    v = jnp.var(x, axis=axis, keepdims=True)
    return (x - m) / jnp.sqrt(v + eps)

def _scatter_add(tgt, idx, src, axis=0):
    return tgt.at[idx].add(src)

def _segment_sum(src, seg, n):
    return jax.ops.segment_sum(src, seg, n)

class _Rng:

    def __init__(self, key):
        self._k = key

    def _next(self):
        self._k, sub = jax.random.split(self._k)
        return sub

    def normal(self, shape):
        return jax.random.normal(self._next(), shape, dtype=jnp.bfloat16)

    def randint(self, lo, hi, shape):
        return jax.random.randint(self._next(), shape, lo, hi, dtype=jnp.int32)

    def uniform(self, shape, lo=0.0, hi=1.0):
        return jax.random.uniform(self._next(), shape, jnp.bfloat16, lo, hi)

    def permutation(self, n):
        return jax.random.permutation(self._next(), n)
kernel_name = 'adaLN_cond__memory_aug_recurrent_mem_tr__dense_activation_gelu__prompt'

def setup_inputs():
    _rng = _Rng(jax.random.key(int.from_bytes(__import__("os").urandom(4), "little")))
    _w = lambda a: (lambda t: t.astype(jnp.bfloat16) if jnp.issubdtype(t.dtype, jnp.floating) else t)(jnp.asarray(a))

    def _A_setup():
        B, S, Dm = (1, 2048, 1024)
        H, Dh = (32, 128)
        M, seg = (8, 32)
        seg = min(seg, S)
        S = S // seg * seg
        return {'x': _w((lambda *s: _rng.normal(s) * 0.05)(B, S, Dm)), 'mem0': _w((lambda *s: _rng.normal(s) * 0.05)(B, M, Dm)), 'Wq': _w((lambda *s: _rng.normal(s) * 0.05)(Dm, H, Dh) * Dm ** (-0.5)), 'Wk': _w((lambda *s: _rng.normal(s) * 0.05)(Dm, H, Dh) * Dm ** (-0.5)), 'Wv': _w((lambda *s: _rng.normal(s) * 0.05)(Dm, H, Dh) * Dm ** (-0.5)), 'Wo': _w((lambda *s: _rng.normal(s) * 0.05)(H, Dh, Dm) * (H * Dh) ** (-0.5)), 'seg_len': seg}
    _A_in = _A_setup()

    def _B_setup():
        B, S, D, F = (1, 2048, 1024, 3584)
        return {'x': _w((lambda *s: _rng.normal(s) * 0.05)(B, S, D)), 'w1': _w((lambda *s: _rng.normal(s) * 0.05)(D, F) * D ** (-0.5)), 'b1': _w((lambda *s: _rng.normal(s) * 0.05)(F) * 0.01), 'w2': _w((lambda *s: _rng.normal(s) * 0.05)(F, D) * F ** (-0.5)), 'b2': _w((lambda *s: _rng.normal(s) * 0.05)(D) * 0.01)}
    _B_in = _B_setup()
    return {'A_x': _A_in['x'], 'A_mem0': _A_in['mem0'], 'A_Wq': _A_in['Wq'], 'A_Wk': _A_in['Wk'], 'A_Wv': _A_in['Wv'], 'A_Wo': _A_in['Wo'], 'A_seg_len': _A_in['seg_len'], 'B_x': _B_in['x'], 'B_w1': _B_in['w1'], 'B_b1': _B_in['b1'], 'B_w2': _B_in['w2'], 'B_b2': _B_in['b2'], 'c': _w((lambda *s: _rng.normal(s) * 0.05)(1, 1024)), 'w_mod': _w((lambda *s: _rng.normal(s) * 0.05)(1024, 6 * 1024) * 1024 ** (-0.5))}

def reference(A_x, A_mem0, A_Wq, A_Wk, A_Wv, A_Wo, A_seg_len, B_x, B_w1, B_b1, B_w2, B_b2, c, w_mod):

    def _A_ref(x, mem0, Wq, Wk, Wv, Wo, seg_len):
        B, S, Dm = x.shape
        H, Dh = (Wq.shape[1], Wq.shape[2])
        M = mem0.shape[1]
        scale = Dh ** (-0.5)
        n_seg = S // seg_len
        L = M + seg_len
        idx = jnp.arange(L)
        mask = (idx[:, None] < M) | (idx[:, None] >= idx[None, :])
        mem = mem0
        outs = []
        for s in range(n_seg):
            xs = x[:, s * seg_len:(s + 1) * seg_len, :].copy()
            h = jnp.concatenate([mem, xs], axis=1)
            q = jnp.einsum('btd,dhe->bhte', h, Wq)
            k = jnp.einsum('btd,dhe->bhte', h, Wk)
            v = jnp.einsum('btd,dhe->bhte', h, Wv)
            scores = jnp.einsum('bhqe,bhke->bhqk', q, k) * scale
            scores = jnp.where(mask[None, None], scores, -1000000000.0)
            p = _softmax(scores, axis=-1)
            o = jnp.einsum('bhqk,bhke->bhqe', p, v)
            o = jnp.einsum('bhte,hed->btd', o, Wo)
            mem = o[:, :M, :].copy()
            outs.append(o[:, M:, :])
        return jnp.concatenate(outs, axis=1)

    def _B_ref(x, w1, b1, w2, b2):
        h = jnp.einsum('bsd,df->bsf', x, w1) + b1
        h = _gelu(h)
        return jnp.einsum('bsf,fd->bsd', h, w2) + b2
    x = A_x
    mod = (_silu(c) @ w_mod).reshape(c.shape[0], 6, 1, -1)
    sa, ca, ga, sb, cb, gb = (mod[:, 0].copy(), mod[:, 1].copy(), mod[:, 2].copy(), mod[:, 3].copy(), mod[:, 4].copy(), mod[:, 5].copy())
    h = _layernorm(x, axis=-1) * (1 + ca) + sa
    x = x + ga * _A_ref(h, A_mem0, A_Wq, A_Wk, A_Wv, A_Wo, A_seg_len)
    h = _layernorm(x, axis=-1) * (1 + cb) + sb
    x = x + gb * _B_ref(h, B_w1, B_b1, B_w2, B_b2)
    return x
```

```python
import functools

import jax
import jax.numpy as jnp
from jax import lax
import jax.experimental.pallas as pl
import jax.experimental.pallas.tpu as pltpu

F32 = jnp.float32
BF16 = jnp.bfloat16
U32 = jnp.uint32

S = 2048
D = 1024
H = 32
DH = 128
M = 8
SEG = 32
FF = 3584
NSEG = S // SEG
NP = H // 2
TPS = 24
T0 = S - NSEG * TPS
G0 = T0 // 8
RING = 72
ROFF = 8
EPS = 1e-5
FB = 256
FC = 512


def _dot(a, b):
    return jnp.dot(a, b, preferred_element_type=F32)


def _bf(x):
    return pltpu.bitcast(x, BF16)


def _u32(x):
    return pltpu.bitcast(x, U32)


def _ln_mod(x, scale1, shift):
    m = jnp.mean(x, axis=-1, keepdims=True)
    xc = x - m
    v = jnp.mean(xc * xc, axis=-1, keepdims=True)
    return xc * lax.rsqrt(v + EPS) * scale1 + shift


def _gelu(x):
    c = 0.7978845608028654
    return 0.5 * x * (1.0 + jnp.tanh(c * (x + 0.044715 * (x * x * x))))


def _interleave(a, b):
    n = a.shape[0] // 8
    parts = []
    for g in range(n):
        parts.append(a[8 * g:8 * g + 8])
        parts.append(b[8 * g:8 * g + 8])
    return _u32(jnp.concatenate(parts, axis=0).astype(BF16))


def _deinterleave(u):
    v = _bf(u).astype(F32)
    n = v.shape[0] // 16
    a = jnp.concatenate([v[16 * g:16 * g + 8] for g in range(n)], axis=0)
    b = jnp.concatenate([v[16 * g + 8:16 * g + 16] for g in range(n)], axis=0)
    return a, b


def _kernel(x_hbm, mem0_ref, wq_hbm, wk_hbm, wv_hbm, wo_hbm, w1_hbm, b1_ref, w2_hbm, b2_ref,
            c_ref, wmod_hbm, out_hbm,
            x_v, h_v, x1_v, wmod_v, mod_v, w_v, wo_v, w1_v, w2_v, qo_v, kv_v, fill_v, out_v,
            sem_w, sem_misc, sem_out):
    w32 = [r.bitcast(U32) for r in (wq_hbm, wk_hbm, wv_hbm)]
    wo32 = wo_hbm.bitcast(U32)

    def w_copies(p):
        return [pltpu.make_async_copy(w32[j].at[:, par, p, :], w_v.at[p * 6 + j * 2 + par], sem_w.at[p])
                for j in range(3) for par in range(2)]

    cp_mod0 = pltpu.make_async_copy(wmod_hbm.at[:, 0:2 * D], wmod_v.at[:, 0:2 * D], sem_misc.at[0])
    cp_x = pltpu.make_async_copy(x_hbm, x_v, sem_misc.at[1])
    cp_mod1 = pltpu.make_async_copy(wmod_hbm.at[:, 2 * D:6 * D], wmod_v.at[:, 2 * D:6 * D], sem_misc.at[2])
    cp_wo = [pltpu.make_async_copy(wo32.at[:, j * 128:(j + 1) * 128], wo_v.at[j], sem_misc.at[3])
             for j in range(8)]
    cp_w1 = pltpu.make_async_copy(w1_hbm, w1_v, sem_misc.at[4])
    cp_w2 = pltpu.make_async_copy(w2_hbm, w2_v, sem_misc.at[5])

    cp_mod0.start()
    cp_x.start()
    for p in range(2):
        for cp in w_copies(p):
            cp.start()

    ri = lax.broadcasted_iota(jnp.int32, (80, 80), 0)
    ci = lax.broadcasted_iota(jnp.int32, (80, 80), 1)
    same_head = ((ri >> 3) & 1) == ((ci >> 3) & 1)
    rpos = ((ri >> 4) << 3) + (ri & 7)
    cpos = ((ci >> 4) << 3) + (ci & 7)
    keep = (ri >= 64) | (ci >= 64) | (rpos >= cpos)
    fill_v[...] = jnp.where(same_head, jnp.where(keep, 0.0, -1e9), -jnp.inf).astype(F32)

    c = c_ref[...].astype(F32)
    sc = jnp.broadcast_to(c * jax.nn.sigmoid(c), (8, D)).astype(BF16)

    cp_mod0.wait()
    mod_v[:, 0:2 * D] = _dot(sc, wmod_v[:, 0:2 * D])
    cp_x.wait()

    def ln1_body(i, carry):
        r = pl.multiple_of(i * 64, 64)
        xb = x_v[pl.ds(r, 64), :].astype(F32)
        h_v[pl.ds(r, 64), :] = _ln_mod(xb, 1.0 + mod_v[0:1, D:2 * D], mod_v[0:1, 0:D]).astype(BF16)
        return carry

    lax.fori_loop(0, S // 64, ln1_body, 0)

    def p1_body(p, carry):
        for cp in w_copies(p):
            cp.wait()

        @pl.when(p + 2 < NP)
        def _():
            for cp in w_copies(p + 2):
                cp.start()

        @pl.when(p + 2 == NP)
        def _():
            for cp in cp_wo:
                cp.start()
            cp_mod1.start()
            cp_w1.start()
            cp_w2.start()

        hb = h_v[0:T0, :]
        for j in range(3):
            a = w_v[p * 6 + j * 2]
            b = w_v[p * 6 + j * 2 + 1]
            lo = (a & jnp.uint32(0xFFFF)) | (b << 16)
            hi = (a >> 16) | (b & jnp.uint32(0xFFFF0000))
            w_v[p * 6 + j * 2] = lo
            w_v[p * 6 + j * 2 + 1] = hi
            r = _interleave(_dot(hb, _bf(lo)), _dot(hb, _bf(hi)))
            if j == 0:
                qo_v[p, 0:8 * G0, :] = r
            else:
                kv_v[p, j - 1, 8 * ROFF:8 * (ROFF + G0), :] = r
        return carry

    lax.fori_loop(0, NP, p1_body, 0)

    for cp in cp_wo:
        cp.wait()
    cp_mod1.wait()
    mod_v[:, 2 * D:6 * D] = _dot(sc, wmod_v[:, 2 * D:6 * D])

    scale = DH ** -0.5

    def step(s, mem):
        t_in = pl.multiple_of(T0 + TPS * s, 8)
        lhs = jnp.concatenate([mem, h_v[pl.ds(t_in, TPS), :].astype(F32)], axis=0).astype(BF16)
        q_wr = pl.multiple_of(8 * (G0 + 3 * s), 8)
        kv_wr = pl.multiple_of(8 * lax.rem(3 * s, RING), 8)
        q_rd = pl.multiple_of(32 * s, 8)
        kv_rd = pl.multiple_of(8 * lax.rem(4 * s + ROFF, RING), 8)
        o_rd = pl.multiple_of(24 * s, 8)
        om = []
        for p in range(NP):
            stacks = []
            for j in range(3):
                r = _interleave(_dot(lhs, _bf(w_v[p * 6 + j * 2])), _dot(lhs, _bf(w_v[p * 6 + j * 2 + 1])))
                if j == 0:
                    qo_v[p, pl.ds(q_wr, 24), :] = r[8:32]
                    t = qo_v[p, pl.ds(q_rd, 32), :]
                else:
                    kv_v[p, j - 1, pl.ds(kv_wr, 24), :] = r[8:32]
                    t = kv_v[p, j - 1, pl.ds(kv_rd, 32), :]
                stacks.append(_bf(jnp.concatenate([t, r[0:8]], axis=0)))
            q, k, v = stacks
            sc_ = lax.dot_general(q, k, (((1,), (1,)), ((), ())), preferred_element_type=F32) * scale
            fill = fill_v[...]
            sc_ = jnp.where(fill == 0.0, sc_, fill)
            mx = jnp.max(sc_, axis=-1, keepdims=True)
            e = jnp.exp(sc_ - mx)
            l = jnp.sum(e, axis=-1, keepdims=True)
            o = _dot(e.astype(BF16), v) / l
            qo_v[p, pl.ds(q_rd, 32), :] = _u32(o[0:64].astype(BF16))
            oa, ob = _deinterleave(qo_v[p, pl.ds(o_rd, 24), :])
            om.append(jnp.concatenate([o[64:72], oa], axis=0).astype(BF16))
            om.append(jnp.concatenate([o[72:80], ob], axis=0).astype(BF16))
        lo = jnp.concatenate(om, axis=1)
        res = jnp.concatenate([_dot(lo, _bf(wo_v[j])) for j in range(8)], axis=1)
        x1_v[pl.ds(o_rd, TPS), :] = (x_v[pl.ds(o_rd, TPS), :].astype(F32)
                                     + mod_v[0:1, 2 * D:3 * D] * res[8:32])
        return res[0:8]

    lax.fori_loop(0, NSEG, step, mem0_ref[...].astype(F32))

    def wo_body(i, carry):
        r0 = pl.multiple_of(S - T0 + i * 128, 128)
        parts = []
        for p in range(NP):
            oa, ob = _deinterleave(qo_v[p, pl.ds(r0, 128), :])
            parts.append(oa.astype(BF16))
            parts.append(ob.astype(BF16))
        lo = jnp.concatenate(parts, axis=1)
        res = jnp.concatenate([_dot(lo, _bf(wo_v[j])) for j in range(8)], axis=1)
        x1_v[pl.ds(r0, 128), :] = x_v[pl.ds(r0, 128), :].astype(F32) + mod_v[0:1, 2 * D:3 * D] * res
        return carry

    lax.fori_loop(0, T0 // 128, wo_body, 0)

    cp_w1.wait()
    cp_w2.wait()

    def out_copy(i):
        r0 = pl.multiple_of(i * FB, FB)
        return pltpu.make_async_copy(out_v.at[pl.ds(r0, FB)], out_hbm.at[pl.ds(r0, FB)], sem_out.at[i])

    def ffn_body(i, carry):
        r0 = pl.multiple_of(i * FB, FB)
        x1 = x1_v[pl.ds(r0, FB), :]
        h2 = _ln_mod(x1, 1.0 + mod_v[0:1, 4 * D:5 * D], mod_v[0:1, 3 * D:4 * D]).astype(BF16)
        acc = None
        for f in range(FF // FC):
            a = _dot(h2, w1_v[:, f * FC:(f + 1) * FC]) + b1_ref[:, f * FC:(f + 1) * FC].astype(F32)
            y = _dot(_gelu(a).astype(BF16), w2_v[f * FC:(f + 1) * FC, :])
            acc = y if acc is None else acc + y
        acc = acc + b2_ref[...].astype(F32)
        out_v[pl.ds(r0, FB), :] = (x1_v[pl.ds(r0, FB), :] + mod_v[0:1, 5 * D:6 * D] * acc).astype(BF16)
        out_copy(i).start()
        return carry

    lax.fori_loop(0, S // FB, ffn_body, 0)
    for i in range(S // FB):
        out_copy(i).wait()


@functools.partial(jax.jit, static_argnames=("A_seg_len",))
def pallas_adaLN_cond__memory_aug_recurrent_mem_tr__dense_activation_gelu__prompt_kernel(
    A_x, A_mem0, A_Wq, A_Wk, A_Wv, A_Wo, A_seg_len, B_x, B_w1, B_b1, B_w2, B_b2, c, w_mod,
):
    assert A_seg_len == SEG and A_x.shape == (1, S, D)
    hbm = pl.BlockSpec(memory_space=pl.ANY)
    vmem = pl.BlockSpec(memory_space=pltpu.VMEM)
    out = pl.pallas_call(
        _kernel,
        out_shape=jax.ShapeDtypeStruct((S, D), BF16),
        in_specs=[hbm, vmem, hbm, hbm, hbm, hbm, hbm, vmem, hbm, vmem, vmem, hbm],
        out_specs=hbm,
        scratch_shapes=[
            pltpu.VMEM((S, D), BF16),
            pltpu.VMEM((S, D), BF16),
            pltpu.VMEM((S, D), F32),
            pltpu.VMEM((D, 6 * D), BF16),
            pltpu.VMEM((8, 6 * D), F32),
            pltpu.VMEM((6 * NP, D // 2, 128), U32),
            pltpu.VMEM((8, H * DH // 2, 128), U32),
            pltpu.VMEM((D, FF), BF16),
            pltpu.VMEM((FF, D), BF16),
            pltpu.VMEM((NP, S, 128), U32),
            pltpu.VMEM((NP, 2, 8 * RING, 128), U32),
            pltpu.VMEM((80, 80), F32),
            pltpu.VMEM((S, D), BF16),
            pltpu.SemaphoreType.DMA((NP,)),
            pltpu.SemaphoreType.DMA((6,)),
            pltpu.SemaphoreType.DMA((S // FB,)),
        ],
        compiler_params=pltpu.CompilerParams(vmem_limit_bytes=120 * 1024 * 1024),
    )(
        A_x.reshape(S, D), A_mem0.reshape(M, D),
        A_Wq.reshape(D // 2, 2, H, DH), A_Wk.reshape(D // 2, 2, H, DH), A_Wv.reshape(D // 2, 2, H, DH),
        A_Wo.reshape(H * DH, D), B_w1, B_b1.reshape(1, FF), B_w2, B_b2.reshape(1, D), c, w_mod,
    )
    return out.reshape(1, S, D)
```

```python
import functools

import jax
import jax.numpy as jnp
from jax import lax
import jax.experimental.pallas as pl
import jax.experimental.pallas.tpu as pltpu

F32 = jnp.float32
BF16 = jnp.bfloat16
U32 = jnp.uint32

S = 2048
D = 1024
H = 32
DH = 128
M = 8
SEG = 32
FF = 3584
NSEG = S // SEG
NP = H // 2
TPS = 24
T0 = S - NSEG * TPS
G0 = T0 // 8
RING = 72
ROFF = 8
EPS = 1e-5
FB = 256
FC = 512


def _dot(a, b):
    return jnp.dot(a, b, preferred_element_type=F32)


def _bf(x):
    return pltpu.bitcast(x, BF16)


def _u32(x):
    return pltpu.bitcast(x, U32)


def _ln_mod(x, scale1, shift):
    m = jnp.mean(x, axis=-1, keepdims=True)
    xc = x - m
    v = jnp.mean(xc * xc, axis=-1, keepdims=True)
    return xc * lax.rsqrt(v + EPS) * scale1 + shift


def _gelu(x):
    c = 0.7978845608028654
    return 0.5 * x * (1.0 + jnp.tanh(c * (x + 0.044715 * (x * x * x))))


def _interleave(a, b):
    n = a.shape[0] // 8
    parts = []
    for g in range(n):
        parts.append(a[8 * g:8 * g + 8])
        parts.append(b[8 * g:8 * g + 8])
    return _u32(jnp.concatenate(parts, axis=0).astype(BF16))


def _deinterleave(u):
    v = _bf(u).astype(F32)
    n = v.shape[0] // 16
    a = jnp.concatenate([v[16 * g:16 * g + 8] for g in range(n)], axis=0)
    b = jnp.concatenate([v[16 * g + 8:16 * g + 16] for g in range(n)], axis=0)
    return a, b


def _kernel(x_hbm, mem0_ref, wq_hbm, wk_hbm, wv_hbm, wo_hbm, w1_hbm, b1_ref, w2_hbm, b2_ref,
            c_ref, wmod_hbm, out_hbm,
            x_v, h_v, x1_v, wmod_v, mod_v, w_v, wo_v, w1_v, w2_v, qo_v, kv_v, fill_v, out_v,
            sem_w, sem_misc, sem_out):
    w32 = [r.bitcast(U32) for r in (wq_hbm, wk_hbm, wv_hbm)]
    wo32 = wo_hbm.bitcast(U32)

    def w_copies(p):
        return [pltpu.make_async_copy(w32[j].at[:, par, p, :], w_v.at[p * 6 + j * 2 + par], sem_w.at[p])
                for j in range(3) for par in range(2)]

    cp_mod0 = pltpu.make_async_copy(wmod_hbm.at[:, 0:2 * D], wmod_v.at[:, 0:2 * D], sem_misc.at[0])
    cp_x = pltpu.make_async_copy(x_hbm, x_v, sem_misc.at[1])
    cp_mod1 = pltpu.make_async_copy(wmod_hbm.at[:, 2 * D:6 * D], wmod_v.at[:, 2 * D:6 * D], sem_misc.at[2])
    cp_wo = [pltpu.make_async_copy(wo32.at[:, j * 128:(j + 1) * 128], wo_v.at[j], sem_misc.at[3])
             for j in range(8)]
    cp_w1 = pltpu.make_async_copy(w1_hbm, w1_v, sem_misc.at[4])
    cp_w2 = pltpu.make_async_copy(w2_hbm, w2_v, sem_misc.at[5])

    cp_mod0.start()
    cp_x.start()
    for p in range(2):
        for cp in w_copies(p):
            cp.start()

    ri = lax.broadcasted_iota(jnp.int32, (80, 80), 0)
    ci = lax.broadcasted_iota(jnp.int32, (80, 80), 1)
    same_head = ((ri >> 3) & 1) == ((ci >> 3) & 1)
    rpos = ((ri >> 4) << 3) + (ri & 7)
    cpos = ((ci >> 4) << 3) + (ci & 7)
    keep = (ri >= 64) | (ci >= 64) | (rpos >= cpos)
    fill_v[...] = jnp.where(same_head, jnp.where(keep, 0.0, -1e9), -jnp.inf).astype(F32)

    c = c_ref[...].astype(F32)
    sc = jnp.broadcast_to(c * jax.nn.sigmoid(c), (8, D)).astype(BF16)

    cp_mod0.wait()
    mod_v[:, 0:2 * D] = _dot(sc, wmod_v[:, 0:2 * D])
    cp_x.wait()

    def ln1_body(i, carry):
        r = pl.multiple_of(i * 64, 64)
        xb = x_v[pl.ds(r, 64), :].astype(F32)
        h_v[pl.ds(r, 64), :] = _ln_mod(xb, 1.0 + mod_v[0:1, D:2 * D], mod_v[0:1, 0:D]).astype(BF16)
        return carry

    lax.fori_loop(0, S // 64, ln1_body, 0)

    def p1_body(p, carry):
        for cp in w_copies(p):
            cp.wait()

        @pl.when(p + 2 < NP)
        def _():
            for cp in w_copies(p + 2):
                cp.start()

        @pl.when(p + 2 == NP)
        def _():
            for cp in cp_wo:
                cp.start()
            cp_mod1.start()
            cp_w1.start()
            cp_w2.start()

        hb = h_v[0:T0, :]
        for j in range(3):
            a = w_v[p * 6 + j * 2]
            b = w_v[p * 6 + j * 2 + 1]
            lo = (a & jnp.uint32(0xFFFF)) | (b << 16)
            hi = (a >> 16) | (b & jnp.uint32(0xFFFF0000))
            w_v[p * 6 + j * 2] = lo
            w_v[p * 6 + j * 2 + 1] = hi
            r = _interleave(_dot(hb, _bf(lo)), _dot(hb, _bf(hi)))
            if j == 0:
                qo_v[p, 0:8 * G0, :] = r
            else:
                kv_v[p, j - 1, 8 * ROFF:8 * (ROFF + G0), :] = r
        return carry

    lax.fori_loop(0, NP, p1_body, 0)

    for cp in cp_wo:
        cp.wait()
    cp_mod1.wait()
    mod_v[:, 2 * D:6 * D] = _dot(sc, wmod_v[:, 2 * D:6 * D])

    scale = DH ** -0.5

    def step(s, mem):
        t_in = pl.multiple_of(T0 + TPS * s, 8)
        lhs = jnp.concatenate([mem, h_v[pl.ds(t_in, TPS), :].astype(F32)], axis=0).astype(BF16)
        q_wr = pl.multiple_of(8 * (G0 + 3 * s), 8)
        kv_wr = pl.multiple_of(8 * lax.rem(3 * s, RING), 8)
        q_rd = pl.multiple_of(32 * s, 8)
        kv_rd = pl.multiple_of(8 * lax.rem(4 * s + ROFF, RING), 8)
        o_rd = pl.multiple_of(24 * s, 8)
        stk = {}
        prob = {}
        om = {}

        def proj(p):
            stacks = []
            for j in range(3):
                r = _interleave(_dot(lhs, _bf(w_v[p * 6 + j * 2])), _dot(lhs, _bf(w_v[p * 6 + j * 2 + 1])))
                if j == 0:
                    qo_v[p, pl.ds(q_wr, 24), :] = r[8:32]
                    t = qo_v[p, pl.ds(q_rd, 32), :]
                else:
                    kv_v[p, j - 1, pl.ds(kv_wr, 24), :] = r[8:32]
                    t = kv_v[p, j - 1, pl.ds(kv_rd, 32), :]
                stacks.append(_bf(jnp.concatenate([t, r[0:8]], axis=0)))
            stk[p] = stacks

        def qk(p):
            q, k, _ = stk[p]
            sc_ = lax.dot_general(q, k, (((1,), (1,)), ((), ())), preferred_element_type=F32) * scale
            fill = fill_v[...]
            sc_ = jnp.where(fill == 0.0, sc_, fill)
            mx = jnp.max(sc_, axis=-1, keepdims=True)
            e = jnp.exp(sc_ - mx)
            l = jnp.sum(e, axis=-1, keepdims=True)
            prob[p] = (e.astype(BF16), l)

        def pv(p):
            e, l = prob[p]
            o = _dot(e, stk[p][2]) / l
            qo_v[p, pl.ds(q_rd, 32), :] = _u32(o[0:64].astype(BF16))
            oa, ob = _deinterleave(qo_v[p, pl.ds(o_rd, 24), :])
            om[2 * p] = jnp.concatenate([o[64:72], oa], axis=0).astype(BF16)
            om[2 * p + 1] = jnp.concatenate([o[72:80], ob], axis=0).astype(BF16)

        def wo(j, h0, h1):
            lo = jnp.concatenate([om[h] for h in range(h0, h1)], axis=1)
            return _dot(lo, _bf(wo_v[j, h0 * 64:h1 * 64, :]))

        for p in range(NP):
            proj(p)
            if p >= 2:
                pv(p - 2)
            if p >= 1:
                qk(p - 1)
        HS = 26
        part = {}
        for j in (0, 1):
            part[j] = wo(j, 0, HS)
        pv(NP - 2)
        qk(NP - 1)
        for j in (2, 3):
            part[j] = wo(j, 0, HS)
        pv(NP - 1)
        for j in (4, 5, 6, 7):
            part[j] = wo(j, 0, HS)
        res = jnp.concatenate([wo(j, HS, H) + part[j] for j in range(8)], axis=1)
        x1_v[pl.ds(o_rd, TPS), :] = (x_v[pl.ds(o_rd, TPS), :].astype(F32)
                                     + mod_v[0:1, 2 * D:3 * D] * res[8:32])
        return res[0:8]

    lax.fori_loop(0, NSEG, step, mem0_ref[...].astype(F32))

    def wo_body(i, carry):
        r0 = pl.multiple_of(S - T0 + i * 128, 128)
        parts = []
        for p in range(NP):
            oa, ob = _deinterleave(qo_v[p, pl.ds(r0, 128), :])
            parts.append(oa.astype(BF16))
            parts.append(ob.astype(BF16))
        lo = jnp.concatenate(parts, axis=1)
        res = jnp.concatenate([_dot(lo, _bf(wo_v[j])) for j in range(8)], axis=1)
        x1_v[pl.ds(r0, 128), :] = x_v[pl.ds(r0, 128), :].astype(F32) + mod_v[0:1, 2 * D:3 * D] * res
        return carry

    lax.fori_loop(0, T0 // 128, wo_body, 0)

    cp_w1.wait()
    cp_w2.wait()

    def out_copy(i):
        r0 = pl.multiple_of(i * FB, FB)
        return pltpu.make_async_copy(out_v.at[pl.ds(r0, FB)], out_hbm.at[pl.ds(r0, FB)], sem_out.at[i])

    def ffn_body(i, carry):
        r0 = pl.multiple_of(i * FB, FB)
        x1 = x1_v[pl.ds(r0, FB), :]
        h2 = _ln_mod(x1, 1.0 + mod_v[0:1, 4 * D:5 * D], mod_v[0:1, 3 * D:4 * D]).astype(BF16)
        acc = None
        for f in range(FF // FC):
            a = _dot(h2, w1_v[:, f * FC:(f + 1) * FC]) + b1_ref[:, f * FC:(f + 1) * FC].astype(F32)
            y = _dot(_gelu(a).astype(BF16), w2_v[f * FC:(f + 1) * FC, :])
            acc = y if acc is None else acc + y
        acc = acc + b2_ref[...].astype(F32)
        out_v[pl.ds(r0, FB), :] = (x1_v[pl.ds(r0, FB), :] + mod_v[0:1, 5 * D:6 * D] * acc).astype(BF16)
        out_copy(i).start()
        return carry

    lax.fori_loop(0, S // FB, ffn_body, 0)
    for i in range(S // FB):
        out_copy(i).wait()


@functools.partial(jax.jit, static_argnames=("A_seg_len",))
def pallas_adaLN_cond__memory_aug_recurrent_mem_tr__dense_activation_gelu__prompt_kernel(
    A_x, A_mem0, A_Wq, A_Wk, A_Wv, A_Wo, A_seg_len, B_x, B_w1, B_b1, B_w2, B_b2, c, w_mod,
):
    assert A_seg_len == SEG and A_x.shape == (1, S, D)
    hbm = pl.BlockSpec(memory_space=pl.ANY)
    vmem = pl.BlockSpec(memory_space=pltpu.VMEM)
    out = pl.pallas_call(
        _kernel,
        out_shape=jax.ShapeDtypeStruct((S, D), BF16),
        in_specs=[hbm, vmem, hbm, hbm, hbm, hbm, hbm, vmem, hbm, vmem, vmem, hbm],
        out_specs=hbm,
        scratch_shapes=[
            pltpu.VMEM((S, D), BF16),
            pltpu.VMEM((S, D), BF16),
            pltpu.VMEM((S, D), F32),
            pltpu.VMEM((D, 6 * D), BF16),
            pltpu.VMEM((8, 6 * D), F32),
            pltpu.VMEM((6 * NP, D // 2, 128), U32),
            pltpu.VMEM((8, H * DH // 2, 128), U32),
            pltpu.VMEM((D, FF), BF16),
            pltpu.VMEM((FF, D), BF16),
            pltpu.VMEM((NP, S, 128), U32),
            pltpu.VMEM((NP, 2, 8 * RING, 128), U32),
            pltpu.VMEM((80, 80), F32),
            pltpu.VMEM((S, D), BF16),
            pltpu.SemaphoreType.DMA((NP,)),
            pltpu.SemaphoreType.DMA((6,)),
            pltpu.SemaphoreType.DMA((S // FB,)),
        ],
        compiler_params=pltpu.CompilerParams(vmem_limit_bytes=120 * 1024 * 1024),
    )(
        A_x.reshape(S, D), A_mem0.reshape(M, D),
        A_Wq.reshape(D // 2, 2, H, DH), A_Wk.reshape(D // 2, 2, H, DH), A_Wv.reshape(D // 2, 2, H, DH),
        A_Wo.reshape(H * DH, D), B_w1, B_b1.reshape(1, FF), B_w2, B_b2.reshape(1, D), c, w_mod,
    )
    return out.reshape(1, S, D)
```

```python
import functools

import jax
import jax.numpy as jnp
from jax import lax
import jax.experimental.pallas as pl
import jax.experimental.pallas.tpu as pltpu

F32 = jnp.float32
BF16 = jnp.bfloat16
U32 = jnp.uint32

S = 2048
D = 1024
H = 32
DH = 128
M = 8
SEG = 32
FF = 3584
NSEG = S // SEG
NP = H // 2
TPS = 24
T0 = S - NSEG * TPS
G0 = T0 // 8
RING = 72
ROFF = 8
EPS = 1e-5
FB = 256
FC = 512


def _dot(a, b):
    return jnp.dot(a, b, preferred_element_type=F32)


def _bf(x):
    return pltpu.bitcast(x, BF16)


def _u32(x):
    return pltpu.bitcast(x, U32)


def _ln_mod(x, scale1, shift):
    m = jnp.mean(x, axis=-1, keepdims=True)
    xc = x - m
    v = jnp.mean(xc * xc, axis=-1, keepdims=True)
    return xc * lax.rsqrt(v + EPS) * scale1 + shift


def _gelu(x):
    c = 0.7978845608028654
    return 0.5 * x * (1.0 + jnp.tanh(c * (x + 0.044715 * (x * x * x))))


def _interleave(a, b):
    n = a.shape[0] // 8
    parts = []
    for g in range(n):
        parts.append(a[8 * g:8 * g + 8])
        parts.append(b[8 * g:8 * g + 8])
    return _u32(jnp.concatenate(parts, axis=0).astype(BF16))


def _deinterleave(u):
    v = _bf(u).astype(F32)
    n = v.shape[0] // 16
    a = jnp.concatenate([v[16 * g:16 * g + 8] for g in range(n)], axis=0)
    b = jnp.concatenate([v[16 * g + 8:16 * g + 16] for g in range(n)], axis=0)
    return a, b


def _kernel(x_hbm, mem0_ref, wq_hbm, wk_hbm, wv_hbm, wo_hbm, w1_hbm, b1_ref, w2_hbm, b2_ref,
            c_ref, wmod_hbm, out_hbm,
            x_v, h_v, x1_v, wmod_v, mod_v, w_v, wo_v, w1_v, w2_v, qo_v, kv_v, fill_v, out_v,
            sem_w, sem_misc, sem_out):
    w32 = [r.bitcast(U32) for r in (wq_hbm, wk_hbm, wv_hbm)]
    wo32 = wo_hbm.bitcast(U32)

    def w_copies(p):
        return [pltpu.make_async_copy(w32[j].at[:, par, p, :], w_v.at[p * 6 + j * 2 + par], sem_w.at[p])
                for j in range(3) for par in range(2)]

    cp_mod0 = pltpu.make_async_copy(wmod_hbm.at[:, 0:2 * D], wmod_v.at[:, 0:2 * D], sem_misc.at[0])
    cp_x = pltpu.make_async_copy(x_hbm, x_v, sem_misc.at[1])
    cp_mod1 = pltpu.make_async_copy(wmod_hbm.at[:, 2 * D:6 * D], wmod_v.at[:, 2 * D:6 * D], sem_misc.at[2])
    cp_wo = [pltpu.make_async_copy(wo32.at[:, j * 128:(j + 1) * 128], wo_v.at[j], sem_misc.at[3])
             for j in range(8)]
    cp_w1 = pltpu.make_async_copy(w1_hbm, w1_v, sem_misc.at[4])
    cp_w2 = pltpu.make_async_copy(w2_hbm, w2_v, sem_misc.at[5])

    cp_mod0.start()
    cp_x.start()
    for p in range(2):
        for cp in w_copies(p):
            cp.start()

    ri = lax.broadcasted_iota(jnp.int32, (80, 80), 0)
    ci = lax.broadcasted_iota(jnp.int32, (80, 80), 1)
    same_head = ((ri >> 3) & 1) == ((ci >> 3) & 1)
    rpos = ((ri >> 4) << 3) + (ri & 7)
    cpos = ((ci >> 4) << 3) + (ci & 7)
    keep = (ri >= 64) | (ci >= 64) | (rpos >= cpos)
    fill_v[...] = jnp.where(same_head, jnp.where(keep, 0.0, -1e9), -jnp.inf).astype(F32)

    c = c_ref[...].astype(F32)
    sc = jnp.broadcast_to(c * jax.nn.sigmoid(c), (8, D)).astype(BF16)

    cp_mod0.wait()
    mod_v[:, 0:2 * D] = _dot(sc, wmod_v[:, 0:2 * D])
    cp_x.wait()

    def ln1_body(i, carry):
        r = pl.multiple_of(i * 64, 64)
        xb = x_v[pl.ds(r, 64), :].astype(F32)
        h_v[pl.ds(r, 64), :] = _ln_mod(xb, 1.0 + mod_v[0:1, D:2 * D], mod_v[0:1, 0:D]).astype(BF16)
        return carry

    lax.fori_loop(0, S // 64, ln1_body, 0)

    def p1_body(p, carry):
        for cp in w_copies(p):
            cp.wait()

        @pl.when(p + 2 < NP)
        def _():
            for cp in w_copies(p + 2):
                cp.start()

        @pl.when(p + 2 == NP)
        def _():
            for cp in cp_wo:
                cp.start()
            cp_mod1.start()
            cp_w1.start()
            cp_w2.start()

        hb = h_v[0:T0, :]
        for j in range(3):
            a = w_v[p * 6 + j * 2]
            b = w_v[p * 6 + j * 2 + 1]
            lo = (a & jnp.uint32(0xFFFF)) | (b << 16)
            hi = (a >> 16) | (b & jnp.uint32(0xFFFF0000))
            w_v[p * 6 + j * 2] = lo
            w_v[p * 6 + j * 2 + 1] = hi
            r = _interleave(_dot(hb, _bf(lo)), _dot(hb, _bf(hi)))
            if j == 0:
                qo_v[p, 0:8 * G0, :] = r
            else:
                kv_v[p, j - 1, 8 * ROFF:8 * (ROFF + G0), :] = r
        return carry

    lax.fori_loop(0, NP, p1_body, 0)

    for cp in cp_wo:
        cp.wait()
    cp_mod1.wait()
    mod_v[:, 2 * D:6 * D] = _dot(sc, wmod_v[:, 2 * D:6 * D])

    scale = DH ** -0.5

    def step(s, mem):
        t_in = pl.multiple_of(T0 + TPS * s, 8)
        lhs = jnp.concatenate([mem, h_v[pl.ds(t_in, TPS), :].astype(F32)], axis=0).astype(BF16)
        q_wr = pl.multiple_of(8 * (G0 + 3 * s), 8)
        kv_wr = pl.multiple_of(8 * lax.rem(3 * s, RING), 8)
        q_rd = pl.multiple_of(32 * s, 8)
        kv_rd = pl.multiple_of(8 * lax.rem(4 * s + ROFF, RING), 8)
        o_rd = pl.multiple_of(24 * s, 8)
        stk = {}
        prob = {}
        om = {}

        def proj(p):
            stacks = []
            for j in range(3):
                r = _interleave(_dot(lhs, _bf(w_v[p * 6 + j * 2])), _dot(lhs, _bf(w_v[p * 6 + j * 2 + 1])))
                if j == 0:
                    qo_v[p, pl.ds(q_wr, 24), :] = r[8:32]
                    t = qo_v[p, pl.ds(q_rd, 32), :]
                else:
                    kv_v[p, j - 1, pl.ds(kv_wr, 24), :] = r[8:32]
                    t = kv_v[p, j - 1, pl.ds(kv_rd, 32), :]
                stacks.append(_bf(jnp.concatenate([t, r[0:8]], axis=0)))
            stk[p] = stacks

        def qk(p):
            q, k, _ = stk[p]
            sc_ = lax.dot_general(q, k, (((1,), (1,)), ((), ())), preferred_element_type=F32) * scale
            fill = fill_v[...]
            sc_ = jnp.where(fill == 0.0, sc_, fill)
            mx = jnp.max(sc_, axis=-1, keepdims=True)
            e = jnp.exp(sc_ - mx)
            l = jnp.sum(e, axis=-1, keepdims=True)
            prob[p] = (e.astype(BF16), l)

        def pv(p):
            e, l = prob[p]
            o = _dot(e, stk[p][2]) / l
            qo_v[p, pl.ds(q_rd, 32), :] = _u32(o[0:64].astype(BF16))
            oa, ob = _deinterleave(qo_v[p, pl.ds(o_rd, 24), :])
            om[2 * p] = jnp.concatenate([o[64:72], oa], axis=0).astype(BF16)
            om[2 * p + 1] = jnp.concatenate([o[72:80], ob], axis=0).astype(BF16)

        def wo(j, h0, h1):
            lo = jnp.concatenate([om[h] for h in range(h0, h1)], axis=1)
            return _dot(lo, _bf(wo_v[j, h0 * 64:h1 * 64, :]))

        for p in range(0, NP, 2):
            proj(p)
            if p >= 4:
                pv(p - 4)
                pv(p - 3)
            if p >= 2:
                qk(p - 2)
                qk(p - 1)
            proj(p + 1)
        HS = 24
        part = {}
        part[0] = wo(0, 0, HS)
        pv(NP - 4)
        pv(NP - 3)
        qk(NP - 2)
        qk(NP - 1)
        for j in (1, 2, 3):
            part[j] = wo(j, 0, HS)
        pv(NP - 2)
        pv(NP - 1)
        for j in (4, 5, 6, 7):
            part[j] = wo(j, 0, HS)
        res = jnp.concatenate([wo(j, HS, H) + part[j] for j in range(8)], axis=1)
        x1_v[pl.ds(o_rd, TPS), :] = (x_v[pl.ds(o_rd, TPS), :].astype(F32)
                                     + mod_v[0:1, 2 * D:3 * D] * res[8:32])
        return res[0:8]

    lax.fori_loop(0, NSEG, step, mem0_ref[...].astype(F32))

    def wo_body(i, carry):
        r0 = pl.multiple_of(S - T0 + i * 128, 128)
        parts = []
        for p in range(NP):
            oa, ob = _deinterleave(qo_v[p, pl.ds(r0, 128), :])
            parts.append(oa.astype(BF16))
            parts.append(ob.astype(BF16))
        lo = jnp.concatenate(parts, axis=1)
        res = jnp.concatenate([_dot(lo, _bf(wo_v[j])) for j in range(8)], axis=1)
        x1_v[pl.ds(r0, 128), :] = x_v[pl.ds(r0, 128), :].astype(F32) + mod_v[0:1, 2 * D:3 * D] * res
        return carry

    lax.fori_loop(0, T0 // 128, wo_body, 0)

    cp_w1.wait()
    cp_w2.wait()

    def out_copy(i):
        r0 = pl.multiple_of(i * FB, FB)
        return pltpu.make_async_copy(out_v.at[pl.ds(r0, FB)], out_hbm.at[pl.ds(r0, FB)], sem_out.at[i])

    def ffn_body(i, carry):
        r0 = pl.multiple_of(i * FB, FB)
        x1 = x1_v[pl.ds(r0, FB), :]
        h2 = _ln_mod(x1, 1.0 + mod_v[0:1, 4 * D:5 * D], mod_v[0:1, 3 * D:4 * D]).astype(BF16)
        acc = None
        for f in range(FF // FC):
            a = _dot(h2, w1_v[:, f * FC:(f + 1) * FC]) + b1_ref[:, f * FC:(f + 1) * FC].astype(F32)
            y = _dot(_gelu(a).astype(BF16), w2_v[f * FC:(f + 1) * FC, :])
            acc = y if acc is None else acc + y
        acc = acc + b2_ref[...].astype(F32)
        out_v[pl.ds(r0, FB), :] = (x1_v[pl.ds(r0, FB), :] + mod_v[0:1, 5 * D:6 * D] * acc).astype(BF16)
        out_copy(i).start()
        return carry

    lax.fori_loop(0, S // FB, ffn_body, 0)
    for i in range(S // FB):
        out_copy(i).wait()


@functools.partial(jax.jit, static_argnames=("A_seg_len",))
def pallas_adaLN_cond__memory_aug_recurrent_mem_tr__dense_activation_gelu__prompt_kernel(
    A_x, A_mem0, A_Wq, A_Wk, A_Wv, A_Wo, A_seg_len, B_x, B_w1, B_b1, B_w2, B_b2, c, w_mod,
):
    assert A_seg_len == SEG and A_x.shape == (1, S, D)
    hbm = pl.BlockSpec(memory_space=pl.ANY)
    vmem = pl.BlockSpec(memory_space=pltpu.VMEM)
    out = pl.pallas_call(
        _kernel,
        out_shape=jax.ShapeDtypeStruct((S, D), BF16),
        in_specs=[hbm, vmem, hbm, hbm, hbm, hbm, hbm, vmem, hbm, vmem, vmem, hbm],
        out_specs=hbm,
        scratch_shapes=[
            pltpu.VMEM((S, D), BF16),
            pltpu.VMEM((S, D), BF16),
            pltpu.VMEM((S, D), F32),
            pltpu.VMEM((D, 6 * D), BF16),
            pltpu.VMEM((8, 6 * D), F32),
            pltpu.VMEM((6 * NP, D // 2, 128), U32),
            pltpu.VMEM((8, H * DH // 2, 128), U32),
            pltpu.VMEM((D, FF), BF16),
            pltpu.VMEM((FF, D), BF16),
            pltpu.VMEM((NP, S, 128), U32),
            pltpu.VMEM((NP, 2, 8 * RING, 128), U32),
            pltpu.VMEM((80, 80), F32),
            pltpu.VMEM((S, D), BF16),
            pltpu.SemaphoreType.DMA((NP,)),
            pltpu.SemaphoreType.DMA((6,)),
            pltpu.SemaphoreType.DMA((S // FB,)),
        ],
        compiler_params=pltpu.CompilerParams(vmem_limit_bytes=120 * 1024 * 1024),
    )(
        A_x.reshape(S, D), A_mem0.reshape(M, D),
        A_Wq.reshape(D // 2, 2, H, DH), A_Wk.reshape(D // 2, 2, H, DH), A_Wv.reshape(D // 2, 2, H, DH),
        A_Wo.reshape(H * DH, D), B_w1, B_b1.reshape(1, FF), B_w2, B_b2.reshape(1, D), c, w_mod,
    )
    return out.reshape(1, S, D)
```

```python
import functools

import jax
import jax.numpy as jnp
from jax import lax
import jax.experimental.pallas as pl
import jax.experimental.pallas.tpu as pltpu

F32 = jnp.float32
BF16 = jnp.bfloat16
U32 = jnp.uint32

S = 2048
D = 1024
H = 32
DH = 128
M = 8
SEG = 32
FF = 3584
NSEG = S // SEG
NP = H // 2
TPS = 24
T0 = S - NSEG * TPS
G0 = T0 // 8
RING = 72
ROFF = 8
EPS = 1e-5
FB = 256
FC = 512


def _dot(a, b):
    return jnp.dot(a, b, preferred_element_type=F32)


def _bf(x):
    return pltpu.bitcast(x, BF16)


def _u32(x):
    return pltpu.bitcast(x, U32)


def _ln_mod(x, scale1, shift):
    m = jnp.mean(x, axis=-1, keepdims=True)
    xc = x - m
    v = jnp.mean(xc * xc, axis=-1, keepdims=True)
    return xc * lax.rsqrt(v + EPS) * scale1 + shift


def _gelu(x):
    c = 0.7978845608028654
    return 0.5 * x * (1.0 + jnp.tanh(c * (x + 0.044715 * (x * x * x))))


def _interleave(a, b):
    n = a.shape[0] // 8
    parts = []
    for g in range(n):
        parts.append(a[8 * g:8 * g + 8])
        parts.append(b[8 * g:8 * g + 8])
    return _u32(jnp.concatenate(parts, axis=0).astype(BF16))


def _deinterleave(u):
    v = _bf(u).astype(F32)
    n = v.shape[0] // 16
    a = jnp.concatenate([v[16 * g:16 * g + 8] for g in range(n)], axis=0)
    b = jnp.concatenate([v[16 * g + 8:16 * g + 16] for g in range(n)], axis=0)
    return a, b


def _kernel(x_hbm, mem0_ref, wq_hbm, wk_hbm, wv_hbm, wo_hbm, w1_hbm, b1_ref, w2_hbm, b2_ref,
            c_ref, wmod_hbm, out_hbm,
            x_v, h_v, hn_v, x1_v, wmod_v, mod_v, sc_v, w_v, wo_v, w1_v, w2_v, qo_v, kv_v, fill_v, out_v,
            sem_w, sem_misc, sem_out):
    w32 = [r.bitcast(U32) for r in (wq_hbm, wk_hbm, wv_hbm)]
    wo32 = wo_hbm.bitcast(U32)

    def w_copies(p):
        return [pltpu.make_async_copy(w32[j].at[:, par, p, :], w_v.at[p * 6 + j * 2 + par], sem_w.at[p])
                for j in range(3) for par in range(2)]

    cp_mod0 = pltpu.make_async_copy(wmod_hbm.at[:, 0:2 * D], wmod_v.at[:, 0:2 * D], sem_misc.at[0])
    cp_x0 = pltpu.make_async_copy(x_hbm.at[0:T0], x_v.at[0:T0], sem_misc.at[1])
    cp_x1 = pltpu.make_async_copy(x_hbm.at[T0:S], x_v.at[T0:S], sem_misc.at[6])
    cp_mod1 = pltpu.make_async_copy(wmod_hbm.at[:, 2 * D:6 * D], wmod_v.at[:, 2 * D:6 * D], sem_misc.at[2])

    def wo_copy(j):
        c0 = j * 128 if isinstance(j, int) else pl.multiple_of(j * 128, 128)
        return pltpu.make_async_copy(wo32.at[:, pl.ds(c0, 128)], wo_v.at[j], sem_misc.at[3])

    cp_w1 = pltpu.make_async_copy(w1_hbm, w1_v, sem_misc.at[4])
    cp_w2 = pltpu.make_async_copy(w2_hbm, w2_v, sem_misc.at[5])

    cp_x0.start()
    cp_mod0.start()
    for cp in w_copies(0):
        cp.start()

    ri = lax.broadcasted_iota(jnp.int32, (80, 80), 0)
    ci = lax.broadcasted_iota(jnp.int32, (80, 80), 1)
    same_head = ((ri >> 3) & 1) == ((ci >> 3) & 1)
    rpos = ((ri >> 4) << 3) + (ri & 7)
    cpos = ((ci >> 4) << 3) + (ci & 7)
    keep = (ri >= 64) | (ci >= 64) | (rpos >= cpos)
    fill_v[...] = jnp.where(same_head, jnp.where(keep, 0.0, -1e9), -jnp.inf).astype(F32)

    c = c_ref[...].astype(F32)
    sc = jnp.broadcast_to(c * jax.nn.sigmoid(c), (8, D)).astype(BF16)

    sc_v[...] = sc
    cp_mod0.wait()
    for cp in w_copies(1):
        cp.start()
    mod_v[:, 0:2 * D] = _dot(sc, wmod_v[:, 0:2 * D])
    cp_x0.wait()

    def ln1(r, n):
        xb = x_v[pl.ds(r, n), :].astype(F32)
        return _ln_mod(xb, 1.0 + mod_v[0:1, D:2 * D], mod_v[0:1, 0:D])

    def ln1_body(i, carry):
        r = pl.multiple_of(i * 128, 128)
        h_v[pl.ds(r, 128), :] = ln1(r, 128).astype(BF16)
        return carry

    lax.fori_loop(0, T0 // 128, ln1_body, 0)

    def p1_body(p, carry):
        for cp in w_copies(p):
            cp.wait()

        @pl.when(p + 2 < NP)
        def _():
            for cp in w_copies(p + 2):
                cp.start()

        @pl.when(p == 2)
        def _():
            cp_x1.start()

        @pl.when(jnp.logical_and(p >= 4, p < 12))
        def _():
            wo_copy(p - 4).start()

        hb = h_v[...]
        for j in range(3):
            a = w_v[p * 6 + j * 2]
            b = w_v[p * 6 + j * 2 + 1]
            lo = (a & jnp.uint32(0xFFFF)) | (b << 16)
            hi = (a >> 16) | (b & jnp.uint32(0xFFFF0000))
            w_v[p * 6 + j * 2] = lo
            w_v[p * 6 + j * 2 + 1] = hi
            r = _interleave(_dot(hb, _bf(lo)), _dot(hb, _bf(hi)))
            if j == 0:
                qo_v[p, 0:8 * G0, :] = r
            else:
                kv_v[p, j - 1, 8 * ROFF:8 * (ROFF + G0), :] = r
        return carry

    lax.fori_loop(0, NP, p1_body, 0)

    cp_mod1.start()
    cp_w1.start()
    cp_w2.start()
    for j in range(8):
        wo_copy(j).wait()
    cp_x1.wait()
    hn_v[...] = ln1(T0, TPS)

    scale = DH ** -0.5

    def step(s, mem):
        lhs = jnp.concatenate([mem, hn_v[...]], axis=0).astype(BF16)
        t_nx = pl.multiple_of(jnp.minimum(T0 + TPS * (s + 1), S - TPS), 8)
        hn_v[...] = ln1(t_nx, TPS)
        q_wr = pl.multiple_of(8 * (G0 + 3 * s), 8)
        kv_wr = pl.multiple_of(8 * lax.rem(3 * s, RING), 8)
        q_rd = pl.multiple_of(32 * s, 8)
        kv_rd = pl.multiple_of(8 * lax.rem(4 * s + ROFF, RING), 8)
        o_rd = pl.multiple_of(24 * s, 8)
        stk = {}
        prob = {}
        om = {}

        def proj(p):
            stacks = []
            for j in range(3):
                r = _interleave(_dot(lhs, _bf(w_v[p * 6 + j * 2])), _dot(lhs, _bf(w_v[p * 6 + j * 2 + 1])))
                if j == 0:
                    qo_v[p, pl.ds(q_wr, 24), :] = r[8:32]
                    t = qo_v[p, pl.ds(q_rd, 32), :]
                else:
                    kv_v[p, j - 1, pl.ds(kv_wr, 24), :] = r[8:32]
                    t = kv_v[p, j - 1, pl.ds(kv_rd, 32), :]
                stacks.append(_bf(jnp.concatenate([t, r[0:8]], axis=0)))
            stk[p] = stacks

        def qk(p):
            q, k, _ = stk[p]
            sc_ = lax.dot_general(q, k, (((1,), (1,)), ((), ())), preferred_element_type=F32) * scale
            fill = fill_v[...]
            sc_ = jnp.where(fill == 0.0, sc_, fill)
            mx = jnp.max(sc_, axis=-1, keepdims=True)
            e = jnp.exp(sc_ - mx)
            l = jnp.sum(e, axis=-1, keepdims=True)
            prob[p] = (e.astype(BF16), l)

        def pv(p):
            e, l = prob[p]
            o = _dot(e, stk[p][2]) / l
            qo_v[p, pl.ds(q_rd, 32), :] = _u32(o[0:64].astype(BF16))
            oa, ob = _deinterleave(qo_v[p, pl.ds(o_rd, 24), :])
            om[2 * p] = jnp.concatenate([o[64:72], oa], axis=0).astype(BF16)
            om[2 * p + 1] = jnp.concatenate([o[72:80], ob], axis=0).astype(BF16)

        def wo(j, h0, h1):
            lo = jnp.concatenate([om[h] for h in range(h0, h1)], axis=1)
            return _dot(lo, _bf(wo_v[j, h0 * 64:h1 * 64, :]))

        for p in range(0, NP, 2):
            proj(p)
            if p >= 4:
                pv(p - 4)
                pv(p - 3)
            if p >= 2:
                qk(p - 2)
                qk(p - 1)
            proj(p + 1)
        HS = 24
        part = {}
        part[0] = wo(0, 0, HS)
        pv(NP - 4)
        pv(NP - 3)
        qk(NP - 2)
        qk(NP - 1)
        for j in (1, 2, 3):
            part[j] = wo(j, 0, HS)
        pv(NP - 2)
        pv(NP - 1)
        for j in (4, 5, 6, 7):
            part[j] = wo(j, 0, HS)
        res = jnp.concatenate([wo(j, HS, H) + part[j] for j in range(8)], axis=1)
        x1_v[pl.ds(o_rd, TPS), :] = res[8:32]
        return res[0:8]

    lax.fori_loop(0, NSEG, step, mem0_ref[...].astype(F32))

    cp_mod1.wait()

    def wo_body(i, carry):
        r0 = pl.multiple_of(S - T0 + i * 128, 128)
        parts = []
        for p in range(NP):
            oa, ob = _deinterleave(qo_v[p, pl.ds(r0, 128), :])
            parts.append(oa.astype(BF16))
            parts.append(ob.astype(BF16))
        lo = jnp.concatenate(parts, axis=1)
        for j in range(8):
            x1_v[pl.ds(r0, 128), j * 128:(j + 1) * 128] = _dot(lo, _bf(wo_v[j]))
            c0 = pl.multiple_of(2 * D + i * D + j * 128, 128)
            mod_v[:, pl.ds(c0, 128)] = _dot(sc_v[...], wmod_v[:, pl.ds(c0, 128)])
        return carry

    lax.fori_loop(0, T0 // 128, wo_body, 0)

    cp_w1.wait()
    cp_w2.wait()

    def out_copy(i):
        r0 = pl.multiple_of(i * FB, FB)
        return pltpu.make_async_copy(out_v.at[pl.ds(r0, FB)], out_hbm.at[pl.ds(r0, FB)], sem_out.at[i])

    def ffn_body(i, carry):
        r0 = pl.multiple_of(i * FB, FB)
        x1 = x_v[pl.ds(r0, FB), :].astype(F32) + mod_v[0:1, 2 * D:3 * D] * x1_v[pl.ds(r0, FB), :]
        x1_v[pl.ds(r0, FB), :] = x1
        h2 = _ln_mod(x1, 1.0 + mod_v[0:1, 4 * D:5 * D], mod_v[0:1, 3 * D:4 * D]).astype(BF16)
        acc = None
        for f in range(FF // FC):
            a = _dot(h2, w1_v[:, f * FC:(f + 1) * FC]) + b1_ref[:, f * FC:(f + 1) * FC].astype(F32)
            y = _dot(_gelu(a).astype(BF16), w2_v[f * FC:(f + 1) * FC, :])
            acc = y if acc is None else acc + y
        acc = acc + b2_ref[...].astype(F32)
        out_v[pl.ds(r0, FB), :] = (x1_v[pl.ds(r0, FB), :] + mod_v[0:1, 5 * D:6 * D] * acc).astype(BF16)
        out_copy(i).start()
        return carry

    lax.fori_loop(0, S // FB, ffn_body, 0)
    for i in range(S // FB):
        out_copy(i).wait()


@functools.partial(jax.jit, static_argnames=("A_seg_len",))
def pallas_adaLN_cond__memory_aug_recurrent_mem_tr__dense_activation_gelu__prompt_kernel(
    A_x, A_mem0, A_Wq, A_Wk, A_Wv, A_Wo, A_seg_len, B_x, B_w1, B_b1, B_w2, B_b2, c, w_mod,
):
    assert A_seg_len == SEG and A_x.shape == (1, S, D)
    hbm = pl.BlockSpec(memory_space=pl.ANY)
    vmem = pl.BlockSpec(memory_space=pltpu.VMEM)
    out = pl.pallas_call(
        _kernel,
        out_shape=jax.ShapeDtypeStruct((S, D), BF16),
        in_specs=[hbm, vmem, hbm, hbm, hbm, hbm, hbm, vmem, hbm, vmem, vmem, hbm],
        out_specs=hbm,
        scratch_shapes=[
            pltpu.VMEM((S, D), BF16),
            pltpu.VMEM((T0, D), BF16),
            pltpu.VMEM((TPS, D), F32),
            pltpu.VMEM((S, D), F32),
            pltpu.VMEM((D, 6 * D), BF16),
            pltpu.VMEM((8, 6 * D), F32),
            pltpu.VMEM((8, D), BF16),
            pltpu.VMEM((6 * NP, D // 2, 128), U32),
            pltpu.VMEM((8, H * DH // 2, 128), U32),
            pltpu.VMEM((D, FF), BF16),
            pltpu.VMEM((FF, D), BF16),
            pltpu.VMEM((NP, S, 128), U32),
            pltpu.VMEM((NP, 2, 8 * RING, 128), U32),
            pltpu.VMEM((80, 80), F32),
            pltpu.VMEM((S, D), BF16),
            pltpu.SemaphoreType.DMA((NP,)),
            pltpu.SemaphoreType.DMA((7,)),
            pltpu.SemaphoreType.DMA((S // FB,)),
        ],
        compiler_params=pltpu.CompilerParams(vmem_limit_bytes=120 * 1024 * 1024),
    )(
        A_x.reshape(S, D), A_mem0.reshape(M, D),
        A_Wq.reshape(D // 2, 2, H, DH), A_Wk.reshape(D // 2, 2, H, DH), A_Wv.reshape(D // 2, 2, H, DH),
        A_Wo.reshape(H * DH, D), B_w1, B_b1.reshape(1, FF), B_w2, B_b2.reshape(1, D), c, w_mod,
    )
    return out.reshape(1, S, D)
```

```python
import contextlib
import functools

import jax
import jax.numpy as jnp
from jax import lax
import jax.experimental.pallas as pl
import jax.experimental.pallas.tpu as pltpu

F32 = jnp.float32
BF16 = jnp.bfloat16
U32 = jnp.uint32

S = 2048
D = 1024
H = 32
DH = 128
M = 8
SEG = 32
FF = 3584
NSEG = S // SEG
NP = H // 2
TPS = 24
T0 = S - NSEG * TPS
G0 = T0 // 8
RING = 72
ROFF = 8
EPS = 1e-5
FB = 256
FC = 512


_SCOPES = False


def _scope(name):
    return jax.named_scope(name) if _SCOPES else contextlib.nullcontext()


def _dot(a, b):
    return jnp.dot(a, b, preferred_element_type=F32)


def _bf(x):
    return pltpu.bitcast(x, BF16)


def _u32(x):
    return pltpu.bitcast(x, U32)


def _ln_mod(x, scale1, shift):
    m = jnp.mean(x, axis=-1, keepdims=True)
    xc = x - m
    v = jnp.mean(xc * xc, axis=-1, keepdims=True)
    return xc * lax.rsqrt(v + EPS) * scale1 + shift


def _gelu(x):
    c = 0.7978845608028654
    return 0.5 * x * (1.0 + jnp.tanh(c * (x + 0.044715 * (x * x * x))))


def _interleave(a, b):
    n = a.shape[0] // 8
    parts = []
    for g in range(n):
        parts.append(a[8 * g:8 * g + 8])
        parts.append(b[8 * g:8 * g + 8])
    return _u32(jnp.concatenate(parts, axis=0).astype(BF16))


def _deinterleave(u):
    v = _bf(u).astype(F32)
    n = v.shape[0] // 16
    a = jnp.concatenate([v[16 * g:16 * g + 8] for g in range(n)], axis=0)
    b = jnp.concatenate([v[16 * g + 8:16 * g + 16] for g in range(n)], axis=0)
    return a, b


def _kernel(x_hbm, mem0_ref, wq_hbm, wk_hbm, wv_hbm, wo_hbm, w1_hbm, b1_ref, w2_hbm, b2_ref,
            c_ref, wmod_hbm, out_hbm,
            x_v, h_v, hn_v, h2_v, x1_v, wmod_v, mod_v, sc_v, w_v, wo_v, w1_v, w2_v, qo_v, kv_v, fill_v, out_v,
            sem_w, sem_misc, sem_out):
    w32 = [r.bitcast(U32) for r in (wq_hbm, wk_hbm, wv_hbm)]
    wo32 = wo_hbm.bitcast(U32)

    def w_copies(p):
        return [pltpu.make_async_copy(w32[j].at[:, par, p, :], w_v.at[p * 6 + j * 2 + par], sem_w.at[p])
                for j in range(3) for par in range(2)]

    cp_mod0 = pltpu.make_async_copy(wmod_hbm.at[:, 0:2 * D], wmod_v.at[:, 0:2 * D], sem_misc.at[0])
    cp_x0 = pltpu.make_async_copy(x_hbm.at[0:T0], x_v.at[0:T0], sem_misc.at[1])
    cp_x1 = pltpu.make_async_copy(x_hbm.at[T0:S], x_v.at[T0:S], sem_misc.at[6])
    cp_mod1 = pltpu.make_async_copy(wmod_hbm.at[:, 2 * D:6 * D], wmod_v.at[:, 2 * D:6 * D], sem_misc.at[2])

    def wo_copy(j):
        c0 = j * 128 if isinstance(j, int) else pl.multiple_of(j * 128, 128)
        return pltpu.make_async_copy(wo32.at[:, pl.ds(c0, 128)], wo_v.at[j], sem_misc.at[3])

    cp_w1 = pltpu.make_async_copy(w1_hbm, w1_v, sem_misc.at[4])
    cp_w2 = pltpu.make_async_copy(w2_hbm, w2_v, sem_misc.at[5])

    cp_x0.start()
    cp_mod0.start()
    for cp in w_copies(0):
        cp.start()

    ri = lax.broadcasted_iota(jnp.int32, (80, 80), 0)
    ci = lax.broadcasted_iota(jnp.int32, (80, 80), 1)
    same_head = ((ri >> 3) & 1) == ((ci >> 3) & 1)
    rpos = ((ri >> 4) << 3) + (ri & 7)
    cpos = ((ci >> 4) << 3) + (ci & 7)
    keep = (ri >= 64) | (ci >= 64) | (rpos >= cpos)
    fill_v[...] = jnp.where(same_head, jnp.where(keep, 0.0, -1e9), -jnp.inf).astype(F32)

    c = c_ref[...].astype(F32)
    sc = jnp.broadcast_to(c * jax.nn.sigmoid(c), (8, D)).astype(BF16)

    sc_v[...] = sc
    with _scope("wait_mod0"):
        cp_mod0.wait()
    for cp in w_copies(1):
        cp.start()
    mod_v[:, 0:2 * D] = _dot(sc, wmod_v[:, 0:2 * D])
    cp_x0.wait()

    def ln1(r, n):
        xb = x_v[pl.ds(r, n), :].astype(F32)
        return _ln_mod(xb, 1.0 + mod_v[0:1, D:2 * D], mod_v[0:1, 0:D])

    def ln1_body(i, carry):
        r = pl.multiple_of(i * 128, 128)
        h_v[pl.ds(r, 128), :] = ln1(r, 128).astype(BF16)
        return carry

    with _scope("ln1"):
        lax.fori_loop(0, T0 // 128, ln1_body, 0)

    def p1_body(p, carry):
        with _scope("wait_w"):
            for cp in w_copies(p):
                cp.wait()

        @pl.when(p + 2 < NP)
        def _():
            for cp in w_copies(p + 2):
                cp.start()

        @pl.when(p == 2)
        def _():
            cp_x1.start()

        @pl.when(jnp.logical_and(p >= 4, p < 12))
        def _():
            wo_copy(p - 4).start()

        hb = h_v[...]
        for j in range(3):
            a = w_v[p * 6 + j * 2]
            b = w_v[p * 6 + j * 2 + 1]
            lo = (a & jnp.uint32(0xFFFF)) | (b << 16)
            hi = (a >> 16) | (b & jnp.uint32(0xFFFF0000))
            w_v[p * 6 + j * 2] = lo
            w_v[p * 6 + j * 2 + 1] = hi
            r = _interleave(_dot(hb, _bf(lo)), _dot(hb, _bf(hi)))
            if j == 0:
                qo_v[p, 0:8 * G0, :] = r
            else:
                kv_v[p, j - 1, 8 * ROFF:8 * (ROFF + G0), :] = r
        return carry

    with _scope("phase1"):
        lax.fori_loop(0, NP, p1_body, 0)

    cp_mod1.start()
    cp_w1.start()
    cp_w2.start()
    with _scope("wait_wo"):
        for j in range(8):
            wo_copy(j).wait()
        cp_x1.wait()
    hn_v[...] = ln1(T0, TPS)

    scale = DH ** -0.5

    def step(s, mem):
        lhs = jnp.concatenate([mem, hn_v[...]], axis=0).astype(BF16)
        t_nx = pl.multiple_of(jnp.minimum(T0 + TPS * (s + 1), S - TPS), 8)
        hn_v[...] = ln1(t_nx, TPS)
        q_wr = pl.multiple_of(8 * (G0 + 3 * s), 8)
        kv_wr = pl.multiple_of(8 * lax.rem(3 * s, RING), 8)
        q_rd = pl.multiple_of(32 * s, 8)
        kv_rd = pl.multiple_of(8 * lax.rem(4 * s + ROFF, RING), 8)
        o_rd = pl.multiple_of(24 * s, 8)
        stk = {}
        prob = {}
        om = {}

        def proj(p):
            stacks = []
            for j in range(3):
                r = _interleave(_dot(lhs, _bf(w_v[p * 6 + j * 2])), _dot(lhs, _bf(w_v[p * 6 + j * 2 + 1])))
                if j == 0:
                    qo_v[p, pl.ds(q_wr, 24), :] = r[8:32]
                    t = qo_v[p, pl.ds(q_rd, 32), :]
                else:
                    kv_v[p, j - 1, pl.ds(kv_wr, 24), :] = r[8:32]
                    t = kv_v[p, j - 1, pl.ds(kv_rd, 32), :]
                stacks.append(_bf(jnp.concatenate([t, r[0:8]], axis=0)))
            stk[p] = stacks

        def qk(p):
            q, k, _ = stk[p]
            sc_ = lax.dot_general(q, k, (((1,), (1,)), ((), ())), preferred_element_type=F32) * scale
            fill = fill_v[...]
            sc_ = jnp.where(fill == 0.0, sc_, fill)
            mx = jnp.max(sc_, axis=-1, keepdims=True)
            e = jnp.exp(sc_ - mx)
            l = jnp.sum(e, axis=-1, keepdims=True)
            prob[p] = (e.astype(BF16), l)

        def pv(p):
            e, l = prob[p]
            o = _dot(e, stk[p][2]) / l
            qo_v[p, pl.ds(q_rd, 32), :] = _u32(o[0:64].astype(BF16))
            oa, ob = _deinterleave(qo_v[p, pl.ds(o_rd, 24), :])
            om[2 * p] = jnp.concatenate([o[64:72], oa], axis=0).astype(BF16)
            om[2 * p + 1] = jnp.concatenate([o[72:80], ob], axis=0).astype(BF16)

        def wo(j, h0, h1):
            lo = jnp.concatenate([om[h] for h in range(h0, h1)], axis=1)
            return _dot(lo, _bf(wo_v[j, h0 * 64:h1 * 64, :]))

        for p in range(0, NP, 2):
            proj(p)
            if p >= 4:
                pv(p - 4)
                pv(p - 3)
            if p >= 2:
                qk(p - 2)
                qk(p - 1)
            proj(p + 1)
        HS = 24
        part = {}
        part[0] = wo(0, 0, HS)
        pv(NP - 4)
        pv(NP - 3)
        qk(NP - 2)
        qk(NP - 1)
        for j in (1, 2, 3):
            part[j] = wo(j, 0, HS)
        pv(NP - 2)
        pv(NP - 1)
        for j in (4, 5, 6, 7):
            part[j] = wo(j, 0, HS)
        res = jnp.concatenate([wo(j, HS, H) + part[j] for j in range(8)], axis=1)
        x1_v[pl.ds(o_rd, TPS), :] = res[8:32]
        return res[0:8]

    with _scope("main"):
        lax.fori_loop(0, NSEG, step, mem0_ref[...].astype(F32))

    cp_mod1.wait()

    def wo_body(i, carry):
        r0 = pl.multiple_of(S - T0 + i * 128, 128)
        parts = []
        for p in range(NP):
            oa, ob = _deinterleave(qo_v[p, pl.ds(r0, 128), :])
            parts.append(oa.astype(BF16))
            parts.append(ob.astype(BF16))
        lo = jnp.concatenate(parts, axis=1)
        for j in range(8):
            x1_v[pl.ds(r0, 128), j * 128:(j + 1) * 128] = _dot(lo, _bf(wo_v[j]))
            c0 = pl.multiple_of(2 * D + i * D + j * 128, 128)
            mod_v[:, pl.ds(c0, 128)] = _dot(sc_v[...], wmod_v[:, pl.ds(c0, 128)])
        return carry

    with _scope("p3a"):
        lax.fori_loop(0, T0 // 128, wo_body, 0)

    cp_w1.wait()
    cp_w2.wait()

    def out_copy(i):
        r0 = pl.multiple_of(i * FB, FB)
        return pltpu.make_async_copy(out_v.at[pl.ds(r0, FB)], out_hbm.at[pl.ds(r0, FB)], sem_out.at[i])

    def resid1(r0, n):
        return x_v[pl.ds(r0, n), :].astype(F32) + mod_v[0:1, 2 * D:3 * D] * x1_v[pl.ds(r0, n), :]

    def ln2(slot, r0, k0, n):
        h2 = _ln_mod(resid1(r0 + k0, n), 1.0 + mod_v[0:1, 4 * D:5 * D], mod_v[0:1, 3 * D:4 * D])
        h2_v[slot, k0 // 2:(k0 + n) // 2, :] = _u32(h2.astype(BF16))

    ln2(0, 0, 0, FB)

    def ffn_body(i, carry):
        r0 = pl.multiple_of(i * FB, FB)
        rn = pl.multiple_of(jnp.minimum(r0 + FB, S - FB), FB)
        slot = lax.rem(i, 2)
        acc = None
        nf = FF // FC
        for f in range(nf):
            a = _dot(_bf(h2_v[slot]), w1_v[:, f * FC:(f + 1) * FC]) + b1_ref[:, f * FC:(f + 1) * FC].astype(F32)
            if 1 <= f <= 4:
                ln2(1 - slot, rn, (f - 1) * (FB // 4), FB // 4)
            y = _dot(_gelu(a).astype(BF16), w2_v[f * FC:(f + 1) * FC, :])
            acc = y if acc is None else y + acc
        acc = acc + b2_ref[...].astype(F32)
        out_v[pl.ds(r0, FB), :] = (resid1(r0, FB) + mod_v[0:1, 5 * D:6 * D] * acc).astype(BF16)
        out_copy(i).start()
        return carry

    with _scope("ffn"):
        lax.fori_loop(0, S // FB, ffn_body, 0)
    with _scope("wait_out"):
        for i in range(S // FB):
            out_copy(i).wait()


@functools.partial(jax.jit, static_argnames=("A_seg_len",))
def pallas_adaLN_cond__memory_aug_recurrent_mem_tr__dense_activation_gelu__prompt_kernel(
    A_x, A_mem0, A_Wq, A_Wk, A_Wv, A_Wo, A_seg_len, B_x, B_w1, B_b1, B_w2, B_b2, c, w_mod,
):
    assert A_seg_len == SEG and A_x.shape == (1, S, D)
    hbm = pl.BlockSpec(memory_space=pl.ANY)
    vmem = pl.BlockSpec(memory_space=pltpu.VMEM)
    out = pl.pallas_call(
        _kernel,
        out_shape=jax.ShapeDtypeStruct((S, D), BF16),
        in_specs=[hbm, vmem, hbm, hbm, hbm, hbm, hbm, vmem, hbm, vmem, vmem, hbm],
        out_specs=hbm,
        scratch_shapes=[
            pltpu.VMEM((S, D), BF16),
            pltpu.VMEM((T0, D), BF16),
            pltpu.VMEM((TPS, D), F32),
            pltpu.VMEM((2, FB // 2, D), U32),
            pltpu.VMEM((S, D), F32),
            pltpu.VMEM((D, 6 * D), BF16),
            pltpu.VMEM((8, 6 * D), F32),
            pltpu.VMEM((8, D), BF16),
            pltpu.VMEM((6 * NP, D // 2, 128), U32),
            pltpu.VMEM((8, H * DH // 2, 128), U32),
            pltpu.VMEM((D, FF), BF16),
            pltpu.VMEM((FF, D), BF16),
            pltpu.VMEM((NP, S, 128), U32),
            pltpu.VMEM((NP, 2, 8 * RING, 128), U32),
            pltpu.VMEM((80, 80), F32),
            pltpu.VMEM((S, D), BF16),
            pltpu.SemaphoreType.DMA((NP,)),
            pltpu.SemaphoreType.DMA((7,)),
            pltpu.SemaphoreType.DMA((S // FB,)),
        ],
        compiler_params=pltpu.CompilerParams(vmem_limit_bytes=120 * 1024 * 1024, disable_bounds_checks=True),
    )(
        A_x.reshape(S, D), A_mem0.reshape(M, D),
        A_Wq.reshape(D // 2, 2, H, DH), A_Wk.reshape(D // 2, 2, H, DH), A_Wv.reshape(D // 2, 2, H, DH),
        A_Wo.reshape(H * DH, D), B_w1, B_b1.reshape(1, FF), B_w2, B_b2.reshape(1, D), c, w_mod,
    )
    return out.reshape(1, S, D)
```

```python
import contextlib
import functools

import jax
import jax.numpy as jnp
from jax import lax
import jax.experimental.pallas as pl
import jax.experimental.pallas.tpu as pltpu

F32 = jnp.float32
BF16 = jnp.bfloat16
U32 = jnp.uint32

S = 2048
D = 1024
H = 32
DH = 128
M = 8
SEG = 32
FF = 3584
NSEG = S // SEG
NP = H // 2
TPS = 24
T0 = S - NSEG * TPS
G0 = T0 // 8
RING = 72
ROFF = 8
EPS = 1e-5
PSTORE = True
LOG2E = 1.4426950408889634
UNROLL = 2
FB = 256
FC = 512


def _make_sched(g):
    out = []

    def rng(a, b):
        return tuple(range(max(a, 0), max(b, 0)))

    for p in range(NP):
        out.append(("proj", p))
        if p % g == 0 and p >= g:
            out.append(("attn", rng(p - 2 * g, p - g), rng(p - g, p)))
    h1 = 2 * (NP - 2 * g)
    h2 = 2 * (NP - g)
    if g == 4:
        out += [("wo", j, 0, h1) for j in (0, 1)]
        out.append(("attn", rng(NP - 2 * g, NP - g), rng(NP - g, NP)))
        out += [("wo", j, 0, h1) for j in (2, 3, 4, 5)]
        out.append(("attn", rng(NP - g, NP), ()))
        out += [("wo", j, 0, h1) for j in (6, 7)]
        out += [("wo", j, h1, h2) for j in range(8)]
        out += [("wo", j, h2, H) for j in range(8)]
    else:
        out += [("wo", 0, 0, h1)]
        out.append(("attn", rng(NP - 2 * g, NP - g), rng(NP - g, NP)))
        out += [("wo", j, 0, h1) for j in (1, 2, 3)]
        out.append(("attn", rng(NP - g, NP), ()))
        out += [("wo", j, 0, h1) for j in (4, 5, 6, 7)]
        out += [("wo", j, h1, H) for j in range(8)]
    return out


SCHED = _make_sched(2)
_SCOPES = False


def _scope(name):
    return jax.named_scope(name) if _SCOPES else contextlib.nullcontext()


def _dot(a, b):
    return jnp.dot(a, b, preferred_element_type=F32)


def _bf(x):
    return pltpu.bitcast(x, BF16)


def _u32(x):
    return pltpu.bitcast(x, U32)


def _ln_mod(x, scale1, shift):
    m = jnp.mean(x, axis=-1, keepdims=True)
    xc = x - m
    v = jnp.mean(xc * xc, axis=-1, keepdims=True)
    return xc * lax.rsqrt(v + EPS) * scale1 + shift


def _gelu(x):
    c = 0.7978845608028654
    return 0.5 * x * (1.0 + jnp.tanh(c * (x + 0.044715 * (x * x * x))))


def _interleave(a, b):
    n = a.shape[0] // 8
    parts = []
    for g in range(n):
        parts.append(a[8 * g:8 * g + 8])
        parts.append(b[8 * g:8 * g + 8])
    return jnp.concatenate(parts, axis=0)


def _deinterleave(v):
    n = v.shape[0] // 16
    a = jnp.concatenate([v[16 * g:16 * g + 8] for g in range(n)], axis=0)
    b = jnp.concatenate([v[16 * g + 8:16 * g + 16] for g in range(n)], axis=0)
    return a, b


def _kernel(x_hbm, mem0_ref, wq_hbm, wk_hbm, wv_hbm, wo_hbm, w1_hbm, b1_ref, w2_hbm, b2_ref,
            c_ref, wmod_hbm, out_hbm,
            x_v, h_v, hn_v, h2_v, x1_v, wmod_v, mod_v, sc_v, w_v, wo_v, w1_v, w2_v, qo_v, kv_v, mr_v, lo_v, pr_v, fill_v, out_v,
            sem_w, sem_misc, sem_out):
    w32 = [r.bitcast(U32) for r in (wq_hbm, wk_hbm, wv_hbm)]
    wo32 = wo_hbm.bitcast(U32)

    def w_copies(p):
        return [pltpu.make_async_copy(w32[j].at[:, par, p, :], w_v.at[p * 6 + j * 2 + par], sem_w.at[p])
                for j in range(3) for par in range(2)]

    cp_mod0 = pltpu.make_async_copy(wmod_hbm.at[:, 0:2 * D], wmod_v.at[:, 0:2 * D], sem_misc.at[0])
    cp_x0 = pltpu.make_async_copy(x_hbm.at[0:T0], x_v.at[0:T0], sem_misc.at[1])
    cp_x1 = pltpu.make_async_copy(x_hbm.at[T0:S], x_v.at[T0:S], sem_misc.at[6])
    cp_mod1 = pltpu.make_async_copy(wmod_hbm.at[:, 2 * D:6 * D], wmod_v.at[:, 2 * D:6 * D], sem_misc.at[2])

    def wo_copy(j):
        c0 = j * 128 if isinstance(j, int) else pl.multiple_of(j * 128, 128)
        return pltpu.make_async_copy(wo32.at[:, pl.ds(c0, 128)], wo_v.at[j], sem_misc.at[3])

    cp_w1 = pltpu.make_async_copy(w1_hbm, w1_v, sem_misc.at[4])
    cp_w2 = pltpu.make_async_copy(w2_hbm, w2_v, sem_misc.at[5])

    cp_x0.start()
    cp_mod0.start()
    for cp in w_copies(0):
        cp.start()

    scale = DH ** -0.5
    ri = lax.broadcasted_iota(jnp.int32, (80, 128), 0)
    ci = lax.broadcasted_iota(jnp.int32, (80, 128), 1)
    same_head = (((ri >> 3) & 1) == ((ci >> 3) & 1)) & (ci < 80)
    rpos = ((ri >> 4) << 3) + (ri & 7)
    cpos = ((ci >> 4) << 3) + (ci & 7)
    keep = (ri >= 64) | (ci >= 64) | (rpos >= cpos)
    fill_v[...] = jnp.where(same_head, jnp.where(keep, 0.0, -1e9 / scale), -jnp.inf).astype(F32)

    c = c_ref[...].astype(F32)
    sc = jnp.broadcast_to(c * jax.nn.sigmoid(c), (8, D)).astype(BF16)

    sc_v[...] = sc
    with _scope("wait_mod0"):
        cp_mod0.wait()
    for cp in w_copies(1):
        cp.start()
    mod_v[:, 0:2 * D] = _dot(sc, wmod_v[:, 0:2 * D])
    cp_x0.wait()

    def ln1(r, n):
        xb = x_v[pl.ds(r, n), :].astype(F32)
        return _ln_mod(xb, 1.0 + mod_v[0:1, D:2 * D], mod_v[0:1, 0:D])

    def ln1_body(i, carry):
        r = pl.multiple_of(i * 128, 128)
        h_v[pl.ds(r, 128), :] = ln1(r, 128).astype(BF16)
        return carry

    with _scope("ln1"):
        lax.fori_loop(0, T0 // 128, ln1_body, 0)

    def p1_body(p, carry):
        with _scope("wait_w"):
            for cp in w_copies(p):
                cp.wait()

        @pl.when(p + 2 < NP)
        def _():
            for cp in w_copies(p + 2):
                cp.start()

        @pl.when(p == 2)
        def _():
            cp_x1.start()

        @pl.when(jnp.logical_and(p >= 4, p < 12))
        def _():
            wo_copy(p - 4).start()

        hb = h_v[...]
        for j in range(3):
            a = w_v[p * 6 + j * 2]
            b = w_v[p * 6 + j * 2 + 1]
            lo = (a & jnp.uint32(0xFFFF)) | (b << 16)
            hi = (a >> 16) | (b & jnp.uint32(0xFFFF0000))
            w_v[p * 6 + j * 2] = lo
            w_v[p * 6 + j * 2 + 1] = hi
            r = _interleave(_dot(hb, _bf(lo)), _dot(hb, _bf(hi))).astype(BF16)
            if j == 0:
                qo_v[p, 0:16 * G0, :] = r
            else:
                kv_v[p, j - 1, 16 * ROFF:16 * (ROFF + G0), :] = r
        return carry

    with _scope("phase1"):
        lax.fori_loop(0, NP, p1_body, 0)

    with _scope("wait_wo"):
        for j in range(8):
            wo_copy(j).wait()
        cp_x1.wait()
    hn_v[...] = ln1(T0, TPS)

    def step(s, mem):
        lhs = jnp.concatenate([mem, hn_v[...]], axis=0).astype(BF16)
        t_nx = pl.multiple_of(jnp.minimum(T0 + TPS * (s + 1), S - TPS), 8)
        hn_v[...] = ln1(t_nx, TPS)
        q_wr = pl.multiple_of(16 * (G0 + 3 * s), 16)
        kv_wr = pl.multiple_of(16 * lax.rem(3 * s, RING), 16)
        q_rd = pl.multiple_of(64 * s, 16)
        kv_rd = pl.multiple_of(16 * lax.rem(4 * s + ROFF, RING), 16)
        o_rd = pl.multiple_of(48 * s, 16)
        prob = {}
        pending = []

        def flush():
            for p, j, r in pending:
                if j == 0:
                    qo_v[p, pl.ds(q_wr, 48), :] = r.astype(BF16)
                else:
                    kv_v[p, j - 1, pl.ds(kv_wr, 48), :] = r.astype(BF16)
            pending.clear()

        def proj(p):
            flush()
            if p == 0:
                half = [_dot(lhs[:, 0:D // 2], _bf(w_v[c, 0:D // 4, :])) for c in range(6)]
                cols = [_dot(lhs[:, D // 2:D], _bf(w_v[c, D // 4:D // 2, :])) + half[c] for c in range(6)]
            for j in range(3):
                if p == 0:
                    r = _interleave(cols[j * 2], cols[j * 2 + 1])
                else:
                    r = _interleave(_dot(lhs, _bf(w_v[p * 6 + j * 2])), _dot(lhs, _bf(w_v[p * 6 + j * 2 + 1])))
                pending.append((p, j, r[16:64]))
                mr_v[p * 3 + j] = r[0:16].astype(BF16)

        def stack(p, j):
            t = qo_v[p, pl.ds(q_rd, 64), :] if j == 0 else kv_v[p, j - 1, pl.ds(kv_rd, 64), :]
            return jnp.concatenate([t, mr_v[p * 3 + j]], axis=0)

        def attn(pvs, qks):
            if any(p in pvs or p in qks for p, _, _ in pending):
                flush()
            vs = [stack(p, 2) for p in pvs]
            qs = [stack(p, 0) for p in qks]
            ks = [stack(p, 1) for p in qks]
            os_ = [_dot(pr_v[p, :, 0:80] if PSTORE else prob[p][:, 0:80].astype(BF16), v) for p, v in zip(pvs, vs)]
            ss = [lax.dot_general(q, k, (((1,), (1,)), ((), ())), preferred_element_type=F32)
                  for q, k in zip(qs, ks)]
            flush()
            for p, o in zip(pvs, os_):
                qo_v[p, pl.ds(q_rd, 64), :] = o[0:64].astype(BF16)
                oa, ob = _deinterleave(qo_v[p, pl.ds(o_rd, 48), :].astype(F32))
                lo_v[2 * p] = jnp.concatenate([o[64:72], oa], axis=0).astype(BF16)
                lo_v[2 * p + 1] = jnp.concatenate([o[72:80], ob], axis=0).astype(BF16)
            for p, sc_ in zip(qks, ss):
                fill = fill_v[...]
                sc_ = jnp.concatenate([sc_, jnp.zeros((80, 48), F32)], axis=1)
                sc_ = jnp.where(fill == 0.0, sc_, fill)
                mx = jnp.max(sc_, axis=-1, keepdims=True)
                e = jnp.exp2((sc_ - mx) * (scale * LOG2E))
                l = jnp.sum(e, axis=-1, keepdims=True)
                r = pl.reciprocal(l, approx=True)
                prob[p] = e * (r * (2.0 - l * r))
                if PSTORE:
                    pr_v[p] = prob[p].astype(BF16)

        part = {}

        def wo(j, h0, h1):
            lo = jnp.concatenate([lo_v[h] for h in range(h0, h1)], axis=1)
            r = _dot(lo, _bf(wo_v[j, h0 * 64:h1 * 64, :]))
            part[j] = r + part[j] if j in part else r

        for op in SCHED:
            if op[0] == "proj":
                proj(op[1])
            elif op[0] == "attn":
                attn(op[1], op[2])
            else:
                wo(*op[1:])
        res = jnp.concatenate([part[j] for j in range(8)], axis=1)
        x1_v[pl.ds(pl.multiple_of(TPS * s, 8), TPS), :] = res[8:32]
        return res[0:8]

    with _scope("main"):
        def steps(i, mem):
            @pl.when(i == 1)
            def _():
                cp_mod1.start()
                cp_w1.start()
                cp_w2.start()

            with _scope("iter"):
                for u in range(UNROLL):
                    mem = step(i * UNROLL + u, mem)
            return mem

        lax.fori_loop(0, NSEG // UNROLL, steps, mem0_ref[...].astype(F32))

    cp_mod1.wait()

    def wo_body(i, carry):
        r0 = pl.multiple_of(S - T0 + i * 128, 128)
        parts = []
        for p in range(NP):
            oa, ob = _deinterleave(qo_v[p, pl.ds(2 * r0, 256), :].astype(F32))
            parts.append(oa)
            parts.append(ob)
        lo = jnp.concatenate(parts, axis=1).astype(BF16)
        for j in range(8):
            x1_v[pl.ds(r0, 128), j * 128:(j + 1) * 128] = _dot(lo, _bf(wo_v[j]))
            c0 = pl.multiple_of(2 * D + i * D + j * 128, 128)
            mod_v[:, pl.ds(c0, 128)] = _dot(sc_v[...], wmod_v[:, pl.ds(c0, 128)])
        return carry

    with _scope("p3a"):
        lax.fori_loop(0, T0 // 128, wo_body, 0)

    cp_w1.wait()
    cp_w2.wait()

    def out_copy(i):
        r0 = pl.multiple_of(i * FB, FB)
        return pltpu.make_async_copy(out_v.at[pl.ds(r0, FB)], out_hbm.at[pl.ds(r0, FB)], sem_out.at[i])

    def resid1(r0, n):
        return x_v[pl.ds(r0, n), :].astype(F32) + mod_v[0:1, 2 * D:3 * D] * x1_v[pl.ds(r0, n), :]

    def ln2(slot, r0, k0, n):
        h2 = _ln_mod(resid1(r0 + k0, n), 1.0 + mod_v[0:1, 4 * D:5 * D], mod_v[0:1, 3 * D:4 * D])
        h2_v[slot, k0 // 2:(k0 + n) // 2, :] = _u32(h2.astype(BF16))

    ln2(0, 0, 0, FB)

    def ffn_body(i, carry):
        r0 = pl.multiple_of(i * FB, FB)
        rn = pl.multiple_of(jnp.minimum(r0 + FB, S - FB), FB)
        slot = lax.rem(i, 2)
        acc = None
        nf = FF // FC
        for f in range(nf):
            a = _dot(_bf(h2_v[slot]), w1_v[:, f * FC:(f + 1) * FC]) + b1_ref[:, f * FC:(f + 1) * FC].astype(F32)
            if 1 <= f <= 4:
                ln2(1 - slot, rn, (f - 1) * (FB // 4), FB // 4)
            y = _dot(_gelu(a).astype(BF16), w2_v[f * FC:(f + 1) * FC, :])
            acc = y if acc is None else y + acc
        acc = acc + b2_ref[...].astype(F32)
        out_v[pl.ds(r0, FB), :] = (resid1(r0, FB) + mod_v[0:1, 5 * D:6 * D] * acc).astype(BF16)
        out_copy(i).start()
        return carry

    with _scope("ffn"):
        lax.fori_loop(0, S // FB, ffn_body, 0)
    with _scope("wait_out"):
        for i in range(S // FB):
            out_copy(i).wait()


@functools.partial(jax.jit, static_argnames=("A_seg_len",))
def pallas_adaLN_cond__memory_aug_recurrent_mem_tr__dense_activation_gelu__prompt_kernel(
    A_x, A_mem0, A_Wq, A_Wk, A_Wv, A_Wo, A_seg_len, B_x, B_w1, B_b1, B_w2, B_b2, c, w_mod,
):
    assert A_seg_len == SEG and A_x.shape == (1, S, D)
    hbm = pl.BlockSpec(memory_space=pl.ANY)
    vmem = pl.BlockSpec(memory_space=pltpu.VMEM)
    out = pl.pallas_call(
        _kernel,
        out_shape=jax.ShapeDtypeStruct((S, D), BF16),
        in_specs=[hbm, vmem, hbm, hbm, hbm, hbm, hbm, vmem, hbm, vmem, vmem, hbm],
        out_specs=hbm,
        scratch_shapes=[
            pltpu.VMEM((S, D), BF16),
            pltpu.VMEM((T0, D), BF16),
            pltpu.VMEM((TPS, D), F32),
            pltpu.VMEM((2, FB // 2, D), U32),
            pltpu.VMEM((S, D), F32),
            pltpu.VMEM((D, 6 * D), BF16),
            pltpu.VMEM((8, 6 * D), F32),
            pltpu.VMEM((8, D), BF16),
            pltpu.VMEM((6 * NP, D // 2, 128), U32),
            pltpu.VMEM((8, H * DH // 2, 128), U32),
            pltpu.VMEM((D, FF), BF16),
            pltpu.VMEM((FF, D), BF16),
            pltpu.VMEM((NP, 2 * S, 128), BF16),
            pltpu.VMEM((NP, 2, 16 * RING, 128), BF16),
            pltpu.VMEM((3 * NP, 16, 128), BF16),
            pltpu.VMEM((H, 32, 128), BF16),
            pltpu.VMEM((NP, 80, 128), BF16),
            pltpu.VMEM((80, 128), F32),
            pltpu.VMEM((S, D), BF16),
            pltpu.SemaphoreType.DMA((NP,)),
            pltpu.SemaphoreType.DMA((7,)),
            pltpu.SemaphoreType.DMA((S // FB,)),
        ],
        compiler_params=pltpu.CompilerParams(vmem_limit_bytes=120 * 1024 * 1024, disable_bounds_checks=True),
    )(
        A_x.reshape(S, D), A_mem0.reshape(M, D),
        A_Wq.reshape(D // 2, 2, H, DH), A_Wk.reshape(D // 2, 2, H, DH), A_Wv.reshape(D // 2, 2, H, DH),
        A_Wo.reshape(H * DH, D), B_w1, B_b1.reshape(1, FF), B_w2, B_b2.reshape(1, D), c, w_mod,
    )
    return out.reshape(1, S, D)
```

```python
import contextlib
import functools

import jax
import jax.numpy as jnp
from jax import lax
import jax.experimental.pallas as pl
import jax.experimental.pallas.tpu as pltpu

F32 = jnp.float32
BF16 = jnp.bfloat16
U32 = jnp.uint32

S = 2048
D = 1024
H = 32
DH = 128
M = 8
SEG = 32
FF = 3584
NSEG = S // SEG
NP = H // 2
TPS = 24
T0 = S - NSEG * TPS
G0 = T0 // 8
RING = 72
ROFF = 8
EPS = 1e-5
LNP = (48, 48, 48, 48, 32, 32)
PSTORE = True
LOG2E = 1.4426950408889634
UNROLL = 2
FB = 256
FC = 512


def _make_sched(g):
    out = []

    def rng(a, b):
        return tuple(range(max(a, 0), max(b, 0)))

    for p in range(NP):
        out.append(("proj", p))
        if p % g == 0 and p >= g:
            out.append(("attn", rng(p - 2 * g, p - g), rng(p - g, p)))
    h1 = 2 * (NP - 2 * g)
    h2 = 2 * (NP - g)
    if g == 4:
        out += [("wo", j, 0, h1) for j in (0, 1)]
        out.append(("attn", rng(NP - 2 * g, NP - g), rng(NP - g, NP)))
        out += [("wo", j, 0, h1) for j in (2, 3, 4, 5)]
        out.append(("attn", rng(NP - g, NP), ()))
        out += [("wo", j, 0, h1) for j in (6, 7)]
        out += [("wo", j, h1, h2) for j in range(8)]
        out += [("wo", j, h2, H) for j in range(8)]
    else:
        out += [("wo", 0, 0, h1)]
        out.append(("attn", rng(NP - 2 * g, NP - g), rng(NP - g, NP)))
        out += [("wo", j, 0, h1) for j in (1, 2, 3)]
        out.append(("attn", rng(NP - g, NP), ()))
        out += [("wo", j, 0, h1) for j in (4, 5, 6, 7)]
        out += [("wo", j, h1, H) for j in range(8)]
    return out


SCHED = _make_sched(2)
_SCOPES = False


def _scope(name):
    return jax.named_scope(name) if _SCOPES else contextlib.nullcontext()


def _dot(a, b):
    return jnp.dot(a, b, preferred_element_type=F32)


def _bf(x):
    return pltpu.bitcast(x, BF16)


def _u32(x):
    return pltpu.bitcast(x, U32)


def _ln_mod(x, scale1, shift):
    m = jnp.mean(x, axis=-1, keepdims=True)
    xc = x - m
    v = jnp.mean(xc * xc, axis=-1, keepdims=True)
    return xc * lax.rsqrt(v + EPS) * scale1 + shift


def _gelu(x):
    c = 0.7978845608028654
    return 0.5 * x * (1.0 + jnp.tanh(c * (x + 0.044715 * (x * x * x))))


def _interleave(a, b):
    n = a.shape[0] // 8
    parts = []
    for g in range(n):
        parts.append(a[8 * g:8 * g + 8])
        parts.append(b[8 * g:8 * g + 8])
    return jnp.concatenate(parts, axis=0)


def _deinterleave(v):
    n = v.shape[0] // 16
    a = jnp.concatenate([v[16 * g:16 * g + 8] for g in range(n)], axis=0)
    b = jnp.concatenate([v[16 * g + 8:16 * g + 16] for g in range(n)], axis=0)
    return a, b


def _kernel(x_hbm, mem0_ref, wq_hbm, wk_hbm, wv_hbm, wo_hbm, w1_hbm, b1_ref, w2_hbm, b2_ref,
            c_ref, wmod_hbm, out_hbm,
            x_v, h_v, hn_v, h2_v, x1_v, wmod_v, mod_v, sc_v, w_v, wo_v, w1_v, w2_v, qo_v, kv_v, mr_v, lo_v, pr_v, fill_v, out_v, bias_v,
            sem_w, sem_misc, sem_out):
    w32 = [r.bitcast(U32) for r in (wq_hbm, wk_hbm, wv_hbm)]
    wo32 = wo_hbm.bitcast(U32)

    def w_copies(p):
        return [pltpu.make_async_copy(w32[j].at[:, par, p, :], w_v.at[p * 6 + j * 2 + par], sem_w.at[p])
                for j in range(3) for par in range(2)]

    cp_mod0 = pltpu.make_async_copy(wmod_hbm.at[:, 0:2 * D], wmod_v.at[:, 0:2 * D], sem_misc.at[0])
    cp_x0 = pltpu.make_async_copy(x_hbm.at[0:T0], x_v.at[0:T0], sem_misc.at[1])
    cp_x1 = pltpu.make_async_copy(x_hbm.at[T0:S], x_v.at[T0:S], sem_misc.at[6])
    cp_mod1 = pltpu.make_async_copy(wmod_hbm.at[:, 2 * D:6 * D], wmod_v.at[:, 2 * D:6 * D], sem_misc.at[2])

    def wo_copy(j):
        c0 = j * 128 if isinstance(j, int) else pl.multiple_of(j * 128, 128)
        return pltpu.make_async_copy(wo32.at[:, pl.ds(c0, 128)], wo_v.at[j], sem_misc.at[3])

    cp_w1 = pltpu.make_async_copy(w1_hbm, w1_v, sem_misc.at[4])
    cp_w2 = pltpu.make_async_copy(w2_hbm, w2_v, sem_misc.at[5])

    cp_x0.start()
    cp_mod0.start()
    for cp in w_copies(0):
        cp.start()

    scale = DH ** -0.5
    ri = lax.broadcasted_iota(jnp.int32, (80, 128), 0)
    ci = lax.broadcasted_iota(jnp.int32, (80, 128), 1)
    same_head = (((ri >> 3) & 1) == ((ci >> 3) & 1)) & (ci < 80)
    rpos = ((ri >> 4) << 3) + (ri & 7)
    cpos = ((ci >> 4) << 3) + (ci & 7)
    keep = (ri >= 64) | (ci >= 64) | (rpos >= cpos)
    fill_v[...] = jnp.where(same_head, jnp.where(keep, 0.0, -1e9 / scale), -jnp.inf).astype(F32)

    c = c_ref[...].astype(F32)
    sc = jnp.broadcast_to(c * jax.nn.sigmoid(c), (8, D)).astype(BF16)

    sc_v[...] = sc
    bias_v[:, 0:FF] = b1_ref[...].astype(F32).reshape(1, FF)
    bias_v[:, FF:FF + D] = b2_ref[...].astype(F32).reshape(1, D)
    with _scope("wait_mod0"):
        cp_mod0.wait()
    for cp in w_copies(1):
        cp.start()
    mod_v[:, 0:2 * D] = _dot(sc, wmod_v[:, 0:2 * D])
    cp_x0.wait()

    def ln1(r, n):
        xb = x_v[pl.ds(r, n), :].astype(F32)
        return _ln_mod(xb, 1.0 + mod_v[0:1, D:2 * D], mod_v[0:1, 0:D])

    def ln1_body(i, carry):
        r = pl.multiple_of(i * 128, 128)
        h_v[pl.ds(r, 128), :] = ln1(r, 128).astype(BF16)
        return carry

    with _scope("ln1"):
        lax.fori_loop(0, T0 // 128, ln1_body, 0)

    def p1_body(p, carry):
        with _scope("wait_w"):
            for cp in w_copies(p):
                cp.wait()

        @pl.when(p + 2 < NP)
        def _():
            for cp in w_copies(p + 2):
                cp.start()

        @pl.when(p == 2)
        def _():
            cp_x1.start()

        @pl.when(jnp.logical_and(p >= 4, p < 12))
        def _():
            wo_copy(p - 4).start()

        hb = h_v[...]
        for j in range(3):
            a = w_v[p * 6 + j * 2]
            b = w_v[p * 6 + j * 2 + 1]
            lo = (a & jnp.uint32(0xFFFF)) | (b << 16)
            hi = (a >> 16) | (b & jnp.uint32(0xFFFF0000))
            w_v[p * 6 + j * 2] = lo
            w_v[p * 6 + j * 2 + 1] = hi
            r = _interleave(_dot(hb, _bf(lo)), _dot(hb, _bf(hi))).astype(BF16)
            if j == 0:
                qo_v[p, 0:16 * G0, :] = r
            else:
                kv_v[p, j - 1, 16 * ROFF:16 * (ROFF + G0), :] = r
        return carry

    with _scope("phase1"):
        lax.fori_loop(0, NP, p1_body, 0)

    with _scope("wait_wo"):
        for j in range(8):
            wo_copy(j).wait()
        cp_x1.wait()
    hn_v[...] = ln1(T0, TPS)

    def step(s, mem):
        lhs = jnp.concatenate([mem, hn_v[...]], axis=0).astype(BF16)
        t_nx = pl.multiple_of(jnp.minimum(T0 + TPS * (s + 1), S - TPS), 8)
        hn_v[...] = ln1(t_nx, TPS)
        q_wr = pl.multiple_of(16 * (G0 + 3 * s), 16)
        kv_wr = pl.multiple_of(16 * lax.rem(3 * s, RING), 16)
        q_rd = pl.multiple_of(64 * s, 16)
        kv_rd = pl.multiple_of(16 * lax.rem(4 * s + ROFF, RING), 16)
        o_rd = pl.multiple_of(48 * s, 16)
        prob = {}
        pending = []

        def flush():
            for p, j, r in pending:
                if j == 0:
                    qo_v[p, pl.ds(q_wr, 48), :] = r.astype(BF16)
                else:
                    kv_v[p, j - 1, pl.ds(kv_wr, 48), :] = r.astype(BF16)
            pending.clear()

        def proj(p):
            flush()
            if p == 0:
                half = [_dot(lhs[:, 0:D // 2], _bf(w_v[c, 0:D // 4, :])) for c in range(6)]
                cols = [_dot(lhs[:, D // 2:D], _bf(w_v[c, D // 4:D // 2, :])) + half[c] for c in range(6)]
            for j in range(3):
                if p == 0:
                    r = _interleave(cols[j * 2], cols[j * 2 + 1])
                else:
                    r = _interleave(_dot(lhs, _bf(w_v[p * 6 + j * 2])), _dot(lhs, _bf(w_v[p * 6 + j * 2 + 1])))
                pending.append((p, j, r[16:64]))
                mr_v[p * 3 + j] = r[0:16].astype(BF16)

        def stack(p, j):
            t = qo_v[p, pl.ds(q_rd, 64), :] if j == 0 else kv_v[p, j - 1, pl.ds(kv_rd, 64), :]
            return jnp.concatenate([t, mr_v[p * 3 + j]], axis=0)

        def attn(pvs, qks):
            if any(p in pvs or p in qks for p, _, _ in pending):
                flush()
            vs = [stack(p, 2) for p in pvs]
            qs = [stack(p, 0) for p in qks]
            ks = [stack(p, 1) for p in qks]
            os_ = [_dot(pr_v[p, :, 0:80] if PSTORE else prob[p][:, 0:80].astype(BF16), v) for p, v in zip(pvs, vs)]
            ss = [lax.dot_general(q, k, (((1,), (1,)), ((), ())), preferred_element_type=F32)
                  for q, k in zip(qs, ks)]
            flush()
            for p, o in zip(pvs, os_):
                qo_v[p, pl.ds(q_rd, 64), :] = o[0:64].astype(BF16)
                oa, ob = _deinterleave(qo_v[p, pl.ds(o_rd, 48), :].astype(F32))
                lo_v[2 * p] = jnp.concatenate([o[64:72], oa], axis=0).astype(BF16)
                lo_v[2 * p + 1] = jnp.concatenate([o[72:80], ob], axis=0).astype(BF16)
            for p, sc_ in zip(qks, ss):
                fill = fill_v[...]
                sc_ = jnp.concatenate([sc_, jnp.zeros((80, 48), F32)], axis=1)
                sc_ = jnp.where(fill == 0.0, sc_, fill)
                mx = jnp.max(sc_, axis=-1, keepdims=True)
                e = jnp.exp2((sc_ - mx) * (scale * LOG2E))
                l = jnp.sum(e, axis=-1, keepdims=True)
                r = pl.reciprocal(l, approx=True)
                prob[p] = e * (r * (2.0 - l * r))
                if PSTORE:
                    pr_v[p] = prob[p].astype(BF16)

        part = {}

        def wo(j, h0, h1):
            lo = jnp.concatenate([lo_v[h] for h in range(h0, h1)], axis=1)
            r = _dot(lo, _bf(wo_v[j, h0 * 64:h1 * 64, :]))
            part[j] = r + part[j] if j in part else r

        for op in SCHED:
            if op[0] == "proj":
                proj(op[1])
            elif op[0] == "attn":
                attn(op[1], op[2])
            else:
                wo(*op[1:])
        res = jnp.concatenate([part[j] for j in range(8)], axis=1)
        x1_v[pl.ds(pl.multiple_of(TPS * s, 8), TPS), :] = res[8:32]
        return res[0:8]

    with _scope("main"):
        def steps(i, mem):
            @pl.when(i == 1)
            def _():
                cp_mod1.start()
                cp_w1.start()
                cp_w2.start()

            with _scope("iter"):
                for u in range(UNROLL):
                    mem = step(i * UNROLL + u, mem)
            return mem

        lax.fori_loop(0, NSEG // UNROLL, steps, mem0_ref[...].astype(F32))

    cp_mod1.wait()

    def wo_body(i, carry):
        r0 = pl.multiple_of(S - T0 + i * 128, 128)
        parts = []
        for p in range(NP):
            oa, ob = _deinterleave(qo_v[p, pl.ds(2 * r0, 256), :].astype(F32))
            parts.append(oa)
            parts.append(ob)
        lo = jnp.concatenate(parts, axis=1).astype(BF16)
        for j in range(8):
            x1_v[pl.ds(r0, 128), j * 128:(j + 1) * 128] = _dot(lo, _bf(wo_v[j]))
            c0 = pl.multiple_of(2 * D + i * D + j * 128, 128)
            mod_v[:, pl.ds(c0, 128)] = _dot(sc_v[...], wmod_v[:, pl.ds(c0, 128)])
        return carry

    with _scope("p3a"):
        lax.fori_loop(0, T0 // 128, wo_body, 0)

    cp_w1.wait()
    cp_w2.wait()

    def out_copy(i):
        r0 = pl.multiple_of(i * FB, FB)
        return pltpu.make_async_copy(out_v.at[pl.ds(r0, FB)], out_hbm.at[pl.ds(r0, FB)], sem_out.at[i])

    def resid1(r0, n):
        return x_v[pl.ds(r0, n), :].astype(F32) + mod_v[0:1, 2 * D:3 * D] * x1_v[pl.ds(r0, n), :]

    def ln2(slot, r0, k0, n):
        h2 = _ln_mod(resid1(r0 + k0, n), 1.0 + mod_v[0:1, 4 * D:5 * D], mod_v[0:1, 3 * D:4 * D])
        h2_v[slot, k0 // 2:(k0 + n) // 2, :] = _u32(h2.astype(BF16))

    ln2(0, 0, 0, FB)

    def ffn_body(i, carry):
        r0 = pl.multiple_of(i * FB, FB)
        rn = pl.multiple_of(jnp.minimum(r0 + FB, S - FB), FB)
        slot = lax.rem(i, 2)
        acc = None
        nf = FF // FC
        for f in range(nf):
            a = _dot(_bf(h2_v[slot]), w1_v[:, f * FC:(f + 1) * FC]) + bias_v[0:1, f * FC:(f + 1) * FC]
            if f < len(LNP):
                ln2(1 - slot, rn, sum(LNP[:f]), LNP[f])
            y = _dot(_gelu(a).astype(BF16), w2_v[f * FC:(f + 1) * FC, :])
            acc = y if acc is None else y + acc
        acc = acc + bias_v[0:1, FF:FF + D]
        out_v[pl.ds(r0, FB), :] = (resid1(r0, FB) + mod_v[0:1, 5 * D:6 * D] * acc).astype(BF16)
        out_copy(i).start()
        return carry

    with _scope("ffn"):
        lax.fori_loop(0, S // FB, ffn_body, 0)
    with _scope("wait_out"):
        for i in range(S // FB):
            out_copy(i).wait()


@functools.partial(jax.jit, static_argnames=("A_seg_len",))
def pallas_adaLN_cond__memory_aug_recurrent_mem_tr__dense_activation_gelu__prompt_kernel(
    A_x, A_mem0, A_Wq, A_Wk, A_Wv, A_Wo, A_seg_len, B_x, B_w1, B_b1, B_w2, B_b2, c, w_mod,
):
    assert A_seg_len == SEG and A_x.shape == (1, S, D)
    hbm = pl.BlockSpec(memory_space=pl.ANY)
    vmem = pl.BlockSpec(memory_space=pltpu.VMEM)
    out = pl.pallas_call(
        _kernel,
        out_shape=jax.ShapeDtypeStruct((S, D), BF16),
        in_specs=[hbm, vmem, hbm, hbm, hbm, hbm, hbm, vmem, hbm, vmem, vmem, hbm],
        out_specs=hbm,
        scratch_shapes=[
            pltpu.VMEM((S, D), BF16),
            pltpu.VMEM((T0, D), BF16),
            pltpu.VMEM((TPS, D), F32),
            pltpu.VMEM((2, FB // 2, D), U32),
            pltpu.VMEM((S, D), F32),
            pltpu.VMEM((D, 6 * D), BF16),
            pltpu.VMEM((8, 6 * D), F32),
            pltpu.VMEM((8, D), BF16),
            pltpu.VMEM((6 * NP, D // 2, 128), U32),
            pltpu.VMEM((8, H * DH // 2, 128), U32),
            pltpu.VMEM((D, FF), BF16),
            pltpu.VMEM((FF, D), BF16),
            pltpu.VMEM((NP, 2 * S, 128), BF16),
            pltpu.VMEM((NP, 2, 16 * RING, 128), BF16),
            pltpu.VMEM((3 * NP, 16, 128), BF16),
            pltpu.VMEM((H, 32, 128), BF16),
            pltpu.VMEM((NP, 80, 128), BF16),
            pltpu.VMEM((80, 128), F32),
            pltpu.VMEM((S, D), BF16),
            pltpu.VMEM((1, FF + D), F32),
            pltpu.SemaphoreType.DMA((NP,)),
            pltpu.SemaphoreType.DMA((7,)),
            pltpu.SemaphoreType.DMA((S // FB,)),
        ],
        compiler_params=pltpu.CompilerParams(vmem_limit_bytes=120 * 1024 * 1024, disable_bounds_checks=True),
    )(
        A_x.reshape(S, D), A_mem0.reshape(M, D),
        A_Wq.reshape(D // 2, 2, H, DH), A_Wk.reshape(D // 2, 2, H, DH), A_Wv.reshape(D // 2, 2, H, DH),
        A_Wo.reshape(H * DH, D), B_w1, B_b1, B_w2, B_b2, c, w_mod,
    )
    return out.reshape(1, S, D)
```

```python
import contextlib
import functools

import jax
import jax.numpy as jnp
from jax import lax
import jax.experimental.pallas as pl
import jax.experimental.pallas.tpu as pltpu

F32 = jnp.float32
BF16 = jnp.bfloat16
U32 = jnp.uint32

S = 2048
D = 1024
H = 32
DH = 128
M = 8
SEG = 32
FF = 3584
NSEG = S // SEG
NP = H // 2
TPS = 24
T0 = S - NSEG * TPS
G0 = T0 // 8
RING = 72
ROFF = 8
EPS = 1e-5
P1U = 1
PA = 4
LNP = (48, 48, 48, 48, 32, 32)
PSTORE = True
LOG2E = 1.4426950408889634
UNROLL = 2
FB = 256
FC = 512
SEM_W, SEM_A, SEM_M, SEM_MISC, SEM_OUT = 0, 16, 24, 32, 40
SEM_N = SEM_OUT + S // FB


def _make_sched(g):
    out = []

    def rng(a, b):
        return tuple(range(max(a, 0), max(b, 0)))

    for p in range(NP):
        out.append(("proj", p))
        if p % g == 0 and p >= g:
            out.append(("attn", rng(p - 2 * g, p - g), rng(p - g, p)))
    h1 = 2 * (NP - 2 * g)
    h2 = 2 * (NP - g)
    if g == 4:
        out += [("wo", j, 0, h1) for j in (0, 1)]
        out.append(("attn", rng(NP - 2 * g, NP - g), rng(NP - g, NP)))
        out += [("wo", j, 0, h1) for j in (2, 3, 4, 5)]
        out.append(("attn", rng(NP - g, NP), ()))
        out += [("wo", j, 0, h1) for j in (6, 7)]
        out += [("wo", j, h1, h2) for j in range(8)]
        out += [("wo", j, h2, H) for j in range(8)]
    else:
        out += [("wo", 0, 0, h1)]
        out.append(("attn", rng(NP - 2 * g, NP - g), rng(NP - g, NP)))
        out += [("wo", j, 0, h1) for j in (1, 2, 3)]
        out.append(("attn", rng(NP - g, NP), ()))
        out += [("wo", j, 0, h1) for j in (4, 5, 6, 7)]
        out += [("wo", j, h1, H) for j in range(8)]
    return out


SCHED = _make_sched(2)
_SCOPES = False


def _scope(name):
    return jax.named_scope(name) if _SCOPES else contextlib.nullcontext()


def _dot(a, b):
    return jnp.dot(a, b, preferred_element_type=F32)


def _bf(x):
    return pltpu.bitcast(x, BF16)


def _u32(x):
    return pltpu.bitcast(x, U32)


def _ln(x):
    m = jnp.mean(x, axis=-1, keepdims=True)
    xc = x - m
    v = jnp.mean(xc * xc, axis=-1, keepdims=True)
    return xc * lax.rsqrt(v + EPS)


def _gelu(x):
    c = 0.7978845608028654
    return 0.5 * x * (1.0 + jnp.tanh(c * (x + 0.044715 * (x * x * x))))


def _interleave(a, b):
    n = a.shape[0] // 8
    parts = []
    for g in range(n):
        parts.append(a[8 * g:8 * g + 8])
        parts.append(b[8 * g:8 * g + 8])
    return jnp.concatenate(parts, axis=0)


def _deinterleave(v):
    n = v.shape[0] // 16
    a = jnp.concatenate([v[16 * g:16 * g + 8] for g in range(n)], axis=0)
    b = jnp.concatenate([v[16 * g + 8:16 * g + 16] for g in range(n)], axis=0)
    return a, b


def _kernel(x_hbm, mem0_ref, wq_hbm, wk_hbm, wv_hbm, wo_hbm, w1_hbm, b1_ref, w2_hbm, b2_ref,
            c_ref, wmod_hbm, out_hbm,
            x_v, h_v, hn_v, h2_v, x1_v, wmod_v, mod_v, sc_v, w_v, wo_v, w1_v, w2_v, qo_v, kv_v, mr_v, lo_v, pr_v, fill_v, out_v, bias_v, n_v,
            sems):
    w32 = [r.bitcast(U32) for r in (wq_hbm, wk_hbm, wv_hbm)]
    wo32 = wo_hbm.bitcast(U32)

    def w_copies(p):
        return [pltpu.make_async_copy(w32[j].at[:, par, p, :], w_v.at[p * 6 + j * 2 + par], sems.at[SEM_W + p])
                for j in range(3) for par in range(2)]

    def _mult(i, m):
        return i * m if isinstance(i, int) else pl.multiple_of(i * m, m)

    def wa_copies(k):
        r = pl.ds(_mult(k, 64), 64)
        return [pltpu.make_async_copy(w32[j].at[r, par, p, :], w_v.at[p * 6 + j * 2 + par, r], sems.at[SEM_A + k])
                for p in range(PA) for j in range(3) for par in range(2)]

    def m_copies(k):
        cols = [pl.ds(_mult(k + 8 * t, 128), 128) for t in range(2)]
        return [pltpu.make_async_copy(wmod_hbm.at[:, cs], wmod_v.at[:, cs], sems.at[SEM_M + k]) for cs in cols]

    def start(cps):
        for cp in cps:
            cp.start()

    def wait(cps):
        for cp in cps:
            cp.wait()

    cp_x0 = pltpu.make_async_copy(x_hbm.at[0:T0], x_v.at[0:T0], sems.at[SEM_MISC + 1])
    cp_x1 = pltpu.make_async_copy(x_hbm.at[T0:S], x_v.at[T0:S], sems.at[SEM_MISC + 6])
    cp_mod1 = pltpu.make_async_copy(wmod_hbm.at[:, 2 * D:6 * D], wmod_v.at[:, 2 * D:6 * D], sems.at[SEM_MISC + 2])

    def wo_copy(j):
        return pltpu.make_async_copy(wo32.at[:, pl.ds(_mult(j, 128), 128)], wo_v.at[j], sems.at[SEM_MISC + 3])

    cp_w1 = pltpu.make_async_copy(w1_hbm, w1_v, sems.at[SEM_MISC + 4])
    cp_w2 = pltpu.make_async_copy(w2_hbm, w2_v, sems.at[SEM_MISC + 5])

    cp_x0.start()
    start(m_copies(0))
    for k in range(2):
        start(m_copies(k + 1))
        start(wa_copies(k))

    scale = DH ** -0.5
    ri = lax.broadcasted_iota(jnp.int32, (80, 128), 0)
    ci = lax.broadcasted_iota(jnp.int32, (80, 128), 1)
    same_head = (((ri >> 3) & 1) == ((ci >> 3) & 1)) & (ci < 80)
    rpos = ((ri >> 4) << 3) + (ri & 7)
    cpos = ((ci >> 4) << 3) + (ci & 7)
    keep = (ri >= 64) | (ci >= 64) | (rpos >= cpos)
    fill_v[...] = jnp.where(same_head, jnp.where(keep, 0.0, -1e9 / scale), -jnp.inf).astype(F32)

    c = c_ref[...].astype(F32)
    sc = jnp.broadcast_to(c * jax.nn.sigmoid(c), (8, D)).astype(BF16)

    sc_v[...] = sc
    bias_v[:, 0:FF] = b1_ref[...].astype(F32).reshape(1, FF)
    bias_v[:, FF:FF + D] = b2_ref[...].astype(F32).reshape(1, D)

    def zero_body(i, carry):
        x1_v[pl.ds(pl.multiple_of(i * 64, 64), 64), :] = jnp.zeros((64, D), F32)
        return carry

    lax.fori_loop(0, PA * 6, zero_body, 0)

    def relayout(c, rows):
        a = w_v[c, rows, :]
        b = w_v[c + 1, rows, :]
        lo = (a & jnp.uint32(0xFFFF)) | (b << 16)
        hi = (a >> 16) | (b & jnp.uint32(0xFFFF0000))
        w_v[c, rows, :] = lo
        w_v[c + 1, rows, :] = hi
        return _bf(lo), _bf(hi)

    def store_lead(p, j, a, b):
        r = _interleave(a, b).astype(BF16)
        if j == 0:
            qo_v[p, 0:16 * G0, :] = r
        else:
            kv_v[p, j - 1, 16 * ROFF:16 * (ROFF + G0), :] = r

    def mod_tile(ct):
        cs = pl.ds(_mult(ct, 128), 128)
        m = _dot(sc_v[...], wmod_v[:, cs])
        mod_v[:, cs] = m
        return m[0:1]

    with _scope("wait_x0"):
        cp_x0.wait()

    def ln1_body(i, carry):
        r = pl.multiple_of(i * 128, 128)
        n = _ln(x_v[pl.ds(r, 128), :].astype(F32))
        for k in range(8):
            n_v[k, pl.ds(r, 128), :] = n[:, k * 128:(k + 1) * 128]
        return carry

    with _scope("ln1"):
        lax.fori_loop(0, T0 // 128, ln1_body, 0)
    start(m_copies(3))
    start(wa_copies(2))
    with _scope("wait_m0"):
        wait(m_copies(0))
    h_v[0] = (n_v[0] * (1.0 + mod_tile(8)) + mod_tile(0)).astype(BF16)

    def sa_body(k, carry):
        with _scope("wait_a"):
            wait(wa_copies(k))

            @pl.when(k < 7)
            def _():
                wait(m_copies(k + 1))

        kn = jnp.minimum(k + 1, 7)
        rows = pl.ds(pl.multiple_of(k * 64, 64), 64)
        hk = h_v[k]
        for p in range(PA):
            for j in range(3):
                c = p * 6 + j * 2
                res = []
                for t, w in enumerate(relayout(c, rows)):
                    acc = x1_v.at[(c + t) // 8 * T0:((c + t) // 8 + 1) * T0,
                                  (c + t) % 8 * 128:((c + t) % 8 + 1) * 128]
                    r = _dot(hk, w) + acc[...]
                    acc[...] = r
                    res.append(r)
                store_lead(p, j, *res)
            if p == 0:
                sh = mod_tile(kn)
            if p == 1:
                s1 = 1.0 + mod_tile(kn + 8)
        h_v[kn] = (n_v[kn] * s1 + sh).astype(BF16)

        @pl.when(k + 4 < 8)
        def _():
            start(m_copies(k + 4))

        @pl.when(k + 3 < 8)
        def _():
            start(wa_copies(k + 3))

        @pl.when(k >= 4)
        def _():
            start(w_copies(PA + k - 4))

        return carry

    with _scope("stageA"):
        lax.fori_loop(0, 8, sa_body, 0)

    def ln1(r, n):
        xb = x_v[pl.ds(r, n), :].astype(F32)
        return _ln(xb) * (1.0 + mod_v[0:1, D:2 * D]) + mod_v[0:1, 0:D]

    def p1_body(i, carry):
        p0 = PA + P1U * i
        with _scope("wait_w"):
            for u in range(P1U):
                wait(w_copies(p0 + u))

        hb = jnp.concatenate([h_v[k] for k in range(8)], axis=1)
        for u in range(P1U):
            p = p0 + u
            for j in range(3):
                lo, hi = relayout(p * 6 + j * 2, slice(None))
                store_lead(p, j, _dot(hb, lo), _dot(hb, hi))

        @pl.when(p0 + 4 < NP)
        def _():
            for u in range(P1U):
                start(w_copies(p0 + 4 + u))
                wo_copy(P1U * i + u).start()

        @pl.when(p0 + 4 == NP)
        def _():
            cp_x1.start()

        return carry

    with _scope("phase1"):
        lax.fori_loop(0, (NP - PA) // P1U, p1_body, 0)

    with _scope("wait_wo"):
        for j in range(8):
            wo_copy(j).wait()
        cp_x1.wait()
    hn_v[...] = ln1(T0, TPS)

    def step(s, mem):
        lhs = jnp.concatenate([mem, hn_v[...]], axis=0).astype(BF16)
        t_nx = pl.multiple_of(jnp.minimum(T0 + TPS * (s + 1), S - TPS), 8)
        hn_v[...] = ln1(t_nx, TPS)
        q_wr = pl.multiple_of(16 * (G0 + 3 * s), 16)
        kv_wr = pl.multiple_of(16 * lax.rem(3 * s, RING), 16)
        q_rd = pl.multiple_of(64 * s, 16)
        kv_rd = pl.multiple_of(16 * lax.rem(4 * s + ROFF, RING), 16)
        o_rd = pl.multiple_of(48 * s, 16)
        prob = {}
        pending = []

        def flush():
            for p, j, r in pending:
                if j == 0:
                    qo_v[p, pl.ds(q_wr, 48), :] = r.astype(BF16)
                else:
                    kv_v[p, j - 1, pl.ds(kv_wr, 48), :] = r.astype(BF16)
            pending.clear()

        def proj(p):
            flush()
            if p == 0:
                half = [_dot(lhs[:, 0:D // 2], _bf(w_v[c, 0:D // 4, :])) for c in range(6)]
                cols = [_dot(lhs[:, D // 2:D], _bf(w_v[c, D // 4:D // 2, :])) + half[c] for c in range(6)]
            for j in range(3):
                if p == 0:
                    r = _interleave(cols[j * 2], cols[j * 2 + 1])
                else:
                    r = _interleave(_dot(lhs, _bf(w_v[p * 6 + j * 2])), _dot(lhs, _bf(w_v[p * 6 + j * 2 + 1])))
                pending.append((p, j, r[16:64]))
                mr_v[p * 3 + j] = r[0:16].astype(BF16)

        def stack(p, j):
            t = qo_v[p, pl.ds(q_rd, 64), :] if j == 0 else kv_v[p, j - 1, pl.ds(kv_rd, 64), :]
            return jnp.concatenate([t, mr_v[p * 3 + j]], axis=0)

        def attn(pvs, qks):
            if any(p in pvs or p in qks for p, _, _ in pending):
                flush()
            vs = [stack(p, 2) for p in pvs]
            qs = [stack(p, 0) for p in qks]
            ks = [stack(p, 1) for p in qks]
            os_ = [_dot(pr_v[p, :, 0:80] if PSTORE else prob[p][:, 0:80].astype(BF16), v) for p, v in zip(pvs, vs)]
            ss = [lax.dot_general(q, k, (((1,), (1,)), ((), ())), preferred_element_type=F32)
                  for q, k in zip(qs, ks)]
            flush()
            for p, o in zip(pvs, os_):
                qo_v[p, pl.ds(q_rd, 64), :] = o[0:64].astype(BF16)
                oa, ob = _deinterleave(qo_v[p, pl.ds(o_rd, 48), :].astype(F32))
                lo_v[2 * p] = jnp.concatenate([o[64:72], oa], axis=0).astype(BF16)
                lo_v[2 * p + 1] = jnp.concatenate([o[72:80], ob], axis=0).astype(BF16)
            for p, sc_ in zip(qks, ss):
                fill = fill_v[...]
                sc_ = jnp.concatenate([sc_, jnp.zeros((80, 48), F32)], axis=1)
                sc_ = jnp.where(fill == 0.0, sc_, fill)
                mx = jnp.max(sc_, axis=-1, keepdims=True)
                e = jnp.exp2((sc_ - mx) * (scale * LOG2E))
                l = jnp.sum(e, axis=-1, keepdims=True)
                r = pl.reciprocal(l, approx=True)
                prob[p] = e * (r * (2.0 - l * r))
                if PSTORE:
                    pr_v[p] = prob[p].astype(BF16)

        part = {}

        def wo(j, h0, h1):
            lo = jnp.concatenate([lo_v[h] for h in range(h0, h1)], axis=1)
            r = _dot(lo, _bf(wo_v[j, h0 * 64:h1 * 64, :]))
            part[j] = r + part[j] if j in part else r

        for op in SCHED:
            if op[0] == "proj":
                proj(op[1])
            elif op[0] == "attn":
                attn(op[1], op[2])
            else:
                wo(*op[1:])
        res = jnp.concatenate([part[j] for j in range(8)], axis=1)
        x1_v[pl.ds(pl.multiple_of(TPS * s, 8), TPS), :] = res[8:32]
        return res[0:8]

    with _scope("main"):
        def steps(i, mem):
            @pl.when(i == 1)
            def _():
                cp_mod1.start()
                cp_w1.start()
                cp_w2.start()

            with _scope("iter"):
                for u in range(UNROLL):
                    mem = step(i * UNROLL + u, mem)
            return mem

        lax.fori_loop(0, NSEG // UNROLL, steps, mem0_ref[...].astype(F32))

    cp_mod1.wait()

    def wo_body(i, carry):
        r0 = pl.multiple_of(S - T0 + i * 128, 128)
        parts = []
        for p in range(NP):
            oa, ob = _deinterleave(qo_v[p, pl.ds(2 * r0, 256), :].astype(F32))
            parts.append(oa)
            parts.append(ob)
        lo = jnp.concatenate(parts, axis=1).astype(BF16)
        for j in range(8):
            x1_v[pl.ds(r0, 128), j * 128:(j + 1) * 128] = _dot(lo, _bf(wo_v[j]))
            mod_tile(16 + i * 8 + j)
        return carry

    with _scope("p3a"):
        lax.fori_loop(0, T0 // 128, wo_body, 0)

    cp_w1.wait()
    cp_w2.wait()

    def out_copy(i):
        r0 = pl.multiple_of(i * FB, FB)
        return pltpu.make_async_copy(out_v.at[pl.ds(r0, FB)], out_hbm.at[pl.ds(r0, FB)], sems.at[SEM_OUT + i])

    def resid1(r0, n):
        return x_v[pl.ds(r0, n), :].astype(F32) + mod_v[0:1, 2 * D:3 * D] * x1_v[pl.ds(r0, n), :]

    def ln2(slot, r0, k0, n):
        h2 = _ln(resid1(r0 + k0, n)) * (1.0 + mod_v[0:1, 4 * D:5 * D]) + mod_v[0:1, 3 * D:4 * D]
        h2_v[slot, k0 // 2:(k0 + n) // 2, :] = _u32(h2.astype(BF16))

    ln2(0, 0, 0, FB)

    def ffn_body(i, carry):
        r0 = pl.multiple_of(i * FB, FB)
        rn = pl.multiple_of(jnp.minimum(r0 + FB, S - FB), FB)
        slot = lax.rem(i, 2)
        acc = None
        nf = FF // FC
        for f in range(nf):
            a = _dot(_bf(h2_v[slot]), w1_v[:, f * FC:(f + 1) * FC]) + bias_v[0:1, f * FC:(f + 1) * FC]
            if f < len(LNP):
                ln2(1 - slot, rn, sum(LNP[:f]), LNP[f])
            y = _dot(_gelu(a).astype(BF16), w2_v[f * FC:(f + 1) * FC, :])
            acc = y if acc is None else y + acc
        acc = acc + bias_v[0:1, FF:FF + D]
        out_v[pl.ds(r0, FB), :] = (resid1(r0, FB) + mod_v[0:1, 5 * D:6 * D] * acc).astype(BF16)
        out_copy(i).start()
        return carry

    with _scope("ffn"):
        lax.fori_loop(0, S // FB, ffn_body, 0)
    with _scope("wait_out"):
        for i in range(S // FB):
            out_copy(i).wait()


@functools.partial(jax.jit, static_argnames=("A_seg_len",))
def pallas_adaLN_cond__memory_aug_recurrent_mem_tr__dense_activation_gelu__prompt_kernel(
    A_x, A_mem0, A_Wq, A_Wk, A_Wv, A_Wo, A_seg_len, B_x, B_w1, B_b1, B_w2, B_b2, c, w_mod,
):
    assert A_seg_len == SEG and A_x.shape == (1, S, D)
    hbm = pl.BlockSpec(memory_space=pl.ANY)
    vmem = pl.BlockSpec(memory_space=pltpu.VMEM)
    out = pl.pallas_call(
        _kernel,
        out_shape=jax.ShapeDtypeStruct((S, D), BF16),
        in_specs=[hbm, vmem, hbm, hbm, hbm, hbm, hbm, vmem, hbm, vmem, vmem, hbm],
        out_specs=hbm,
        scratch_shapes=[
            pltpu.VMEM((S, D), BF16),
            pltpu.VMEM((8, T0, 128), BF16),
            pltpu.VMEM((TPS, D), F32),
            pltpu.VMEM((2, FB // 2, D), U32),
            pltpu.VMEM((S, D), F32),
            pltpu.VMEM((D, 6 * D), BF16),
            pltpu.VMEM((8, 6 * D), F32),
            pltpu.VMEM((8, D), BF16),
            pltpu.VMEM((6 * NP, D // 2, 128), U32),
            pltpu.VMEM((8, H * DH // 2, 128), U32),
            pltpu.VMEM((D, FF), BF16),
            pltpu.VMEM((FF, D), BF16),
            pltpu.VMEM((NP, 2 * S, 128), BF16),
            pltpu.VMEM((NP, 2, 16 * RING, 128), BF16),
            pltpu.VMEM((3 * NP, 16, 128), BF16),
            pltpu.VMEM((H, 32, 128), BF16),
            pltpu.VMEM((NP, 80, 128), BF16),
            pltpu.VMEM((80, 128), F32),
            pltpu.VMEM((S, D), BF16),
            pltpu.VMEM((1, FF + D), F32),
            pltpu.VMEM((8, T0, 128), F32),
            pltpu.SemaphoreType.DMA((SEM_N,)),
        ],
        compiler_params=pltpu.CompilerParams(vmem_limit_bytes=120 * 1024 * 1024, disable_bounds_checks=True),
    )(
        A_x.reshape(S, D), A_mem0.reshape(M, D),
        A_Wq.reshape(D // 2, 2, H, DH), A_Wk.reshape(D // 2, 2, H, DH), A_Wv.reshape(D // 2, 2, H, DH),
        A_Wo.reshape(H * DH, D), B_w1, B_b1, B_w2, B_b2, c, w_mod,
    )
    return out.reshape(1, S, D)
```

```python
import contextlib
import functools

import jax
import jax.numpy as jnp
from jax import lax
import jax.experimental.pallas as pl
import jax.experimental.pallas.tpu as pltpu

F32 = jnp.float32
BF16 = jnp.bfloat16
U32 = jnp.uint32

S = 2048
D = 1024
H = 32
DH = 128
M = 8
SEG = 32
FF = 3584
NSEG = S // SEG
NP = H // 2
TPS = 24
T0 = S - NSEG * TPS
G0 = T0 // 8
RING = 72
ROFF = 8
EPS = 1e-5
P1U = 1
PA = 4
LNP = (48, 48, 48, 48, 32, 32)
PSTORE = True
LOG2E = 1.4426950408889634
UNROLL = 2
FB = 256
FC = 512
SEM_W, SEM_A, SEM_M, SEM_MISC, SEM_OUT = 0, 16, 24, 32, 40
SEM_N = SEM_OUT + S // FB


def _make_sched(g):
    out = []

    def rng(a, b):
        return tuple(range(max(a, 0), max(b, 0)))

    for p in range(NP):
        out.append(("proj", p))
        if p % g == 0 and p >= g:
            out.append(("attn", rng(p - 2 * g, p - g), rng(p - g, p)))
    h1 = 2 * (NP - 2 * g)
    h2 = 2 * (NP - g)
    if g == 4:
        out += [("wo", j, 0, h1) for j in (0, 1)]
        out.append(("attn", rng(NP - 2 * g, NP - g), rng(NP - g, NP)))
        out += [("wo", j, 0, h1) for j in (2, 3, 4, 5)]
        out.append(("attn", rng(NP - g, NP), ()))
        out += [("wo", j, 0, h1) for j in (6, 7)]
        out += [("wo", j, h1, h2) for j in range(8)]
        out += [("wo", j, h2, H) for j in range(8)]
    else:
        out += [("wo", 0, 0, h1)]
        out.append(("attn", rng(NP - 2 * g, NP - g), rng(NP - g, NP)))
        out += [("wo", j, 0, h1) for j in (1, 2, 3)]
        out.append(("attn", rng(NP - g, NP), ()))
        out += [("wo", j, 0, h1) for j in (4, 5, 6, 7)]
        out += [("wo", j, h1, H) for j in range(8)]
    return out


SCHED = _make_sched(2)
_SCOPES = False


def _scope(name):
    return jax.named_scope(name) if _SCOPES else contextlib.nullcontext()


def _dot(a, b):
    return jnp.dot(a, b, preferred_element_type=F32)


def _bf(x):
    return pltpu.bitcast(x, BF16)


def _u32(x):
    return pltpu.bitcast(x, U32)


def _ln(x):
    m = jnp.mean(x, axis=-1, keepdims=True)
    xc = x - m
    v = jnp.mean(xc * xc, axis=-1, keepdims=True)
    return xc * lax.rsqrt(v + EPS)


def _gelu(x):
    c = 0.7978845608028654
    return 0.5 * x * (1.0 + jnp.tanh(c * (x + 0.044715 * (x * x * x))))


def _interleave(a, b):
    n = a.shape[0] // 8
    parts = []
    for g in range(n):
        parts.append(a[8 * g:8 * g + 8])
        parts.append(b[8 * g:8 * g + 8])
    return jnp.concatenate(parts, axis=0)


def _deinterleave(v):
    n = v.shape[0] // 16
    a = jnp.concatenate([v[16 * g:16 * g + 8] for g in range(n)], axis=0)
    b = jnp.concatenate([v[16 * g + 8:16 * g + 16] for g in range(n)], axis=0)
    return a, b


def _kernel(x_hbm, mem0_ref, wq_hbm, wk_hbm, wv_hbm, wo_hbm, w1_hbm, b1_ref, w2_hbm, b2_ref,
            c_ref, wmod_hbm, out_hbm,
            x_v, h_v, hn_v, h2_v, x1_v, wmod_v, mod_v, sc_v, w_v, wo_v, w1_v, w2_v, qo_v, kv_v, mr_v, lo_v, pr_v, fill_v, out_v, bias_v, n_v,
            sems):
    w32 = [r.bitcast(U32) for r in (wq_hbm, wk_hbm, wv_hbm)]
    wo32 = wo_hbm.bitcast(U32)

    def w_copies(p):
        return [pltpu.make_async_copy(w32[j].at[:, par, p, :], w_v.at[p * 6 + j * 2 + par], sems.at[SEM_W + p])
                for j in range(3) for par in range(2)]

    def _mult(i, m):
        return i * m if isinstance(i, int) else pl.multiple_of(i * m, m)

    def wa_copies(k, pair=None):
        r = pl.ds(_mult(k, 64), 64)
        return [pltpu.make_async_copy(w32[j].at[r, par, p, :], w_v.at[p * 6 + j * 2 + par, r], sems.at[SEM_A + k])
                for p in (range(PA) if pair is None else (pair,)) for j in range(3) for par in range(2)]

    def m_copies(k):
        cols = [pl.ds(_mult(k + 8 * t, 128), 128) for t in range(2)]
        return [pltpu.make_async_copy(wmod_hbm.at[:, cs], wmod_v.at[:, cs], sems.at[SEM_M + k]) for cs in cols]

    def start(cps):
        for cp in cps:
            cp.start()

    def wait(cps):
        for cp in cps:
            cp.wait()

    cp_x0 = pltpu.make_async_copy(x_hbm.at[0:T0], x_v.at[0:T0], sems.at[SEM_MISC + 1])
    cp_x1 = pltpu.make_async_copy(x_hbm.at[T0:S], x_v.at[T0:S], sems.at[SEM_MISC + 6])
    cp_mod1 = pltpu.make_async_copy(wmod_hbm.at[:, 2 * D:6 * D], wmod_v.at[:, 2 * D:6 * D], sems.at[SEM_MISC + 2])

    def wo_copy(j):
        return pltpu.make_async_copy(wo32.at[:, pl.ds(_mult(j, 128), 128)], wo_v.at[j], sems.at[SEM_MISC + 3])

    cp_w1 = pltpu.make_async_copy(w1_hbm, w1_v, sems.at[SEM_MISC + 4])
    cp_w2 = pltpu.make_async_copy(w2_hbm, w2_v, sems.at[SEM_MISC + 5])

    cp_x0.start()
    start(m_copies(0))
    for k in range(2):
        start(m_copies(k + 1))
        start(wa_copies(k))

    scale = DH ** -0.5
    ri = lax.broadcasted_iota(jnp.int32, (80, 128), 0)
    ci = lax.broadcasted_iota(jnp.int32, (80, 128), 1)
    same_head = (((ri >> 3) & 1) == ((ci >> 3) & 1)) & (ci < 80)
    rpos = ((ri >> 4) << 3) + (ri & 7)
    cpos = ((ci >> 4) << 3) + (ci & 7)
    keep = (ri >= 64) | (ci >= 64) | (rpos >= cpos)
    fill_v[...] = jnp.where(same_head, jnp.where(keep, 0.0, -1e9 / scale), -jnp.inf).astype(F32)

    c = c_ref[...].astype(F32)
    sc = jnp.broadcast_to(c * jax.nn.sigmoid(c), (8, D)).astype(BF16)

    sc_v[...] = sc
    bias_v[:, 0:FF] = b1_ref[...].astype(F32).reshape(1, FF)
    bias_v[:, FF:FF + D] = b2_ref[...].astype(F32).reshape(1, D)

    def zero_body(i, carry):
        x1_v[pl.ds(pl.multiple_of(i * 64, 64), 64), :] = jnp.zeros((64, D), F32)
        return carry

    lax.fori_loop(0, PA * 6, zero_body, 0)

    def relayout(c, rows):
        a = w_v[c, rows, :]
        b = w_v[c + 1, rows, :]
        lo = (a & jnp.uint32(0xFFFF)) | (b << 16)
        hi = (a >> 16) | (b & jnp.uint32(0xFFFF0000))
        w_v[c, rows, :] = lo
        w_v[c + 1, rows, :] = hi
        return _bf(lo), _bf(hi)

    def store_lead(p, j, a, b):
        r = _interleave(a, b).astype(BF16)
        if j == 0:
            qo_v[p, 0:16 * G0, :] = r
        else:
            kv_v[p, j - 1, 16 * ROFF:16 * (ROFF + G0), :] = r

    def mod_tile(ct):
        cs = pl.ds(_mult(ct, 128), 128)
        m = _dot(sc_v[...], wmod_v[:, cs])
        mod_v[:, cs] = m
        return m[0:1]

    with _scope("wait_x0"):
        cp_x0.wait()

    def ln1_body(i, carry):
        r = pl.multiple_of(i * 128, 128)
        n = _ln(x_v[pl.ds(r, 128), :].astype(F32))
        for k in range(8):
            n_v[k, pl.ds(r, 128), :] = n[:, k * 128:(k + 1) * 128]
        return carry

    with _scope("ln1"):
        lax.fori_loop(0, T0 // 128, ln1_body, 0)
    start(m_copies(3))
    start(wa_copies(2))
    with _scope("wait_m0"):
        wait(m_copies(0))
    h_v[0] = (n_v[0] * (1.0 + mod_tile(8)) + mod_tile(0)).astype(BF16)

    def sa_body(k, carry):
        with _scope("wait_a"):
            wait(wa_copies(k))

            @pl.when(k < 7)
            def _():
                wait(m_copies(k + 1))

        kn = jnp.minimum(k + 1, 7)
        rows = pl.ds(pl.multiple_of(k * 64, 64), 64)
        hk = h_v[k]
        for p in range(PA):
            for j in range(3):
                c = p * 6 + j * 2
                res = []
                for t, w in enumerate(relayout(c, rows)):
                    acc = x1_v.at[(c + t) // 8 * T0:((c + t) // 8 + 1) * T0,
                                  (c + t) % 8 * 128:((c + t) % 8 + 1) * 128]
                    r = _dot(hk, w) + acc[...]
                    acc[...] = r
                    res.append(r)
                store_lead(p, j, *res)
                if c == 2:
                    sh = mod_tile(kn)
                if c == 6:
                    s1 = 1.0 + mod_tile(kn + 8)

                    @pl.when(k + 4 < 8)
                    def _():
                        start(m_copies(k + 4))

            @pl.when(k + 3 < 8)
            def _():
                start(wa_copies(k + 3, p))

        h_v[kn] = (n_v[kn] * s1 + sh).astype(BF16)


        @pl.when(k >= 4)
        def _():
            start(w_copies(PA + k - 4))

        return carry

    with _scope("stageA"):
        lax.fori_loop(0, 8, sa_body, 0)

    def ln1(r, n):
        xb = x_v[pl.ds(r, n), :].astype(F32)
        return _ln(xb) * (1.0 + mod_v[0:1, D:2 * D]) + mod_v[0:1, 0:D]

    def p1_body(i, carry):
        p0 = PA + P1U * i
        with _scope("wait_w"):
            for u in range(P1U):
                wait(w_copies(p0 + u))

        hb = jnp.concatenate([h_v[k] for k in range(8)], axis=1)
        for u in range(P1U):
            p = p0 + u
            for j in range(3):
                lo, hi = relayout(p * 6 + j * 2, slice(None))
                store_lead(p, j, _dot(hb, lo), _dot(hb, hi))

        @pl.when(p0 + 4 < NP)
        def _():
            for u in range(P1U):
                start(w_copies(p0 + 4 + u))
                wo_copy(P1U * i + u).start()

        @pl.when(p0 + 4 == NP)
        def _():
            cp_x1.start()

        return carry

    with _scope("phase1"):
        lax.fori_loop(0, (NP - PA) // P1U, p1_body, 0)

    with _scope("wait_wo"):
        for j in range(8):
            wo_copy(j).wait()
        cp_x1.wait()
    hn_v[...] = ln1(T0, TPS)

    def step(s, mem):
        lhs = jnp.concatenate([mem, hn_v[...]], axis=0).astype(BF16)
        t_nx = pl.multiple_of(jnp.minimum(T0 + TPS * (s + 1), S - TPS), 8)
        hn_v[...] = ln1(t_nx, TPS)
        q_wr = pl.multiple_of(16 * (G0 + 3 * s), 16)
        kv_wr = pl.multiple_of(16 * lax.rem(3 * s, RING), 16)
        q_rd = pl.multiple_of(64 * s, 16)
        kv_rd = pl.multiple_of(16 * lax.rem(4 * s + ROFF, RING), 16)
        o_rd = pl.multiple_of(48 * s, 16)
        prob = {}
        pending = []

        def flush():
            for p, j, r in pending:
                if j == 0:
                    qo_v[p, pl.ds(q_wr, 48), :] = r.astype(BF16)
                else:
                    kv_v[p, j - 1, pl.ds(kv_wr, 48), :] = r.astype(BF16)
            pending.clear()

        def proj(p):
            flush()
            if p == 0:
                half = [_dot(lhs[:, 0:D // 2], _bf(w_v[c, 0:D // 4, :])) for c in range(6)]
                cols = [_dot(lhs[:, D // 2:D], _bf(w_v[c, D // 4:D // 2, :])) + half[c] for c in range(6)]
            for j in range(3):
                if p == 0:
                    r = _interleave(cols[j * 2], cols[j * 2 + 1])
                else:
                    r = _interleave(_dot(lhs, _bf(w_v[p * 6 + j * 2])), _dot(lhs, _bf(w_v[p * 6 + j * 2 + 1])))
                pending.append((p, j, r[16:64]))
                mr_v[p * 3 + j] = r[0:16].astype(BF16)

        def stack(p, j):
            t = qo_v[p, pl.ds(q_rd, 64), :] if j == 0 else kv_v[p, j - 1, pl.ds(kv_rd, 64), :]
            return jnp.concatenate([t, mr_v[p * 3 + j]], axis=0)

        def attn(pvs, qks):
            if any(p in pvs or p in qks for p, _, _ in pending):
                flush()
            vs = [stack(p, 2) for p in pvs]
            qs = [stack(p, 0) for p in qks]
            ks = [stack(p, 1) for p in qks]
            os_ = [_dot(pr_v[p, :, 0:80] if PSTORE else prob[p][:, 0:80].astype(BF16), v) for p, v in zip(pvs, vs)]
            ss = [lax.dot_general(q, k, (((1,), (1,)), ((), ())), preferred_element_type=F32)
                  for q, k in zip(qs, ks)]
            flush()
            for p, o in zip(pvs, os_):
                qo_v[p, pl.ds(q_rd, 64), :] = o[0:64].astype(BF16)
                oa, ob = _deinterleave(qo_v[p, pl.ds(o_rd, 48), :].astype(F32))
                lo_v[2 * p] = jnp.concatenate([o[64:72], oa], axis=0).astype(BF16)
                lo_v[2 * p + 1] = jnp.concatenate([o[72:80], ob], axis=0).astype(BF16)
            for p, sc_ in zip(qks, ss):
                fill = fill_v[...]
                sc_ = jnp.concatenate([sc_, jnp.zeros((80, 48), F32)], axis=1)
                sc_ = jnp.where(fill == 0.0, sc_, fill)
                mx = jnp.max(sc_, axis=-1, keepdims=True)
                e = jnp.exp2((sc_ - mx) * (scale * LOG2E))
                l = jnp.sum(e, axis=-1, keepdims=True)
                r = pl.reciprocal(l, approx=True)
                prob[p] = e * (r * (2.0 - l * r))
                if PSTORE:
                    pr_v[p] = prob[p].astype(BF16)

        part = {}

        def wo(j, h0, h1):
            lo = jnp.concatenate([lo_v[h] for h in range(h0, h1)], axis=1)
            r = _dot(lo, _bf(wo_v[j, h0 * 64:h1 * 64, :]))
            part[j] = r + part[j] if j in part else r

        for op in SCHED:
            if op[0] == "proj":
                proj(op[1])
            elif op[0] == "attn":
                attn(op[1], op[2])
            else:
                wo(*op[1:])
        res = jnp.concatenate([part[j] for j in range(8)], axis=1)
        x1_v[pl.ds(pl.multiple_of(TPS * s, 8), TPS), :] = res[8:32]
        return res[0:8]

    with _scope("main"):
        def steps(i, mem):
            @pl.when(i == 1)
            def _():
                cp_mod1.start()
                cp_w1.start()
                cp_w2.start()

            with _scope("iter"):
                for u in range(UNROLL):
                    mem = step(i * UNROLL + u, mem)
            return mem

        lax.fori_loop(0, NSEG // UNROLL, steps, mem0_ref[...].astype(F32))

    cp_mod1.wait()

    def wo_body(i, carry):
        r0 = pl.multiple_of(S - T0 + i * 128, 128)
        parts = []
        for p in range(NP):
            oa, ob = _deinterleave(qo_v[p, pl.ds(2 * r0, 256), :].astype(F32))
            parts.append(oa)
            parts.append(ob)
        lo = jnp.concatenate(parts, axis=1).astype(BF16)
        for j in range(8):
            x1_v[pl.ds(r0, 128), j * 128:(j + 1) * 128] = _dot(lo, _bf(wo_v[j]))
            mod_tile(16 + i * 8 + j)
        return carry

    with _scope("p3a"):
        lax.fori_loop(0, T0 // 128, wo_body, 0)

    cp_w1.wait()
    cp_w2.wait()

    def out_copy(i):
        r0 = pl.multiple_of(i * FB, FB)
        return pltpu.make_async_copy(out_v.at[pl.ds(r0, FB)], out_hbm.at[pl.ds(r0, FB)], sems.at[SEM_OUT + i])

    def resid1(r0, n):
        return x_v[pl.ds(r0, n), :].astype(F32) + mod_v[0:1, 2 * D:3 * D] * x1_v[pl.ds(r0, n), :]

    def ln2(slot, r0, k0, n):
        h2 = _ln(resid1(r0 + k0, n)) * (1.0 + mod_v[0:1, 4 * D:5 * D]) + mod_v[0:1, 3 * D:4 * D]
        h2_v[slot, k0 // 2:(k0 + n) // 2, :] = _u32(h2.astype(BF16))

    ln2(0, 0, 0, FB)

    def ffn_body(i, carry):
        r0 = pl.multiple_of(i * FB, FB)
        rn = pl.multiple_of(jnp.minimum(r0 + FB, S - FB), FB)
        slot = lax.rem(i, 2)
        acc = None
        nf = FF // FC
        for f in range(nf):
            a = _dot(_bf(h2_v[slot]), w1_v[:, f * FC:(f + 1) * FC]) + bias_v[0:1, f * FC:(f + 1) * FC]
            if f < len(LNP):
                ln2(1 - slot, rn, sum(LNP[:f]), LNP[f])
            y = _dot(_gelu(a).astype(BF16), w2_v[f * FC:(f + 1) * FC, :])
            acc = y if acc is None else y + acc
        acc = acc + bias_v[0:1, FF:FF + D]
        out_v[pl.ds(r0, FB), :] = (resid1(r0, FB) + mod_v[0:1, 5 * D:6 * D] * acc).astype(BF16)
        out_copy(i).start()
        return carry

    with _scope("ffn"):
        lax.fori_loop(0, S // FB, ffn_body, 0)
    with _scope("wait_out"):
        for i in range(S // FB):
            out_copy(i).wait()


@functools.partial(jax.jit, static_argnames=("A_seg_len",))
def pallas_adaLN_cond__memory_aug_recurrent_mem_tr__dense_activation_gelu__prompt_kernel(
    A_x, A_mem0, A_Wq, A_Wk, A_Wv, A_Wo, A_seg_len, B_x, B_w1, B_b1, B_w2, B_b2, c, w_mod,
):
    assert A_seg_len == SEG and A_x.shape == (1, S, D)
    hbm = pl.BlockSpec(memory_space=pl.ANY)
    vmem = pl.BlockSpec(memory_space=pltpu.VMEM)
    out = pl.pallas_call(
        _kernel,
        out_shape=jax.ShapeDtypeStruct((S, D), BF16),
        in_specs=[hbm, vmem, hbm, hbm, hbm, hbm, hbm, vmem, hbm, vmem, vmem, hbm],
        out_specs=hbm,
        scratch_shapes=[
            pltpu.VMEM((S, D), BF16),
            pltpu.VMEM((8, T0, 128), BF16),
            pltpu.VMEM((TPS, D), F32),
            pltpu.VMEM((2, FB // 2, D), U32),
            pltpu.VMEM((S, D), F32),
            pltpu.VMEM((D, 6 * D), BF16),
            pltpu.VMEM((8, 6 * D), F32),
            pltpu.VMEM((8, D), BF16),
            pltpu.VMEM((6 * NP, D // 2, 128), U32),
            pltpu.VMEM((8, H * DH // 2, 128), U32),
            pltpu.VMEM((D, FF), BF16),
            pltpu.VMEM((FF, D), BF16),
            pltpu.VMEM((NP, 2 * S, 128), BF16),
            pltpu.VMEM((NP, 2, 16 * RING, 128), BF16),
            pltpu.VMEM((3 * NP, 16, 128), BF16),
            pltpu.VMEM((H, 32, 128), BF16),
            pltpu.VMEM((NP, 80, 128), BF16),
            pltpu.VMEM((80, 128), F32),
            pltpu.VMEM((S, D), BF16),
            pltpu.VMEM((1, FF + D), F32),
            pltpu.VMEM((8, T0, 128), F32),
            pltpu.SemaphoreType.DMA((SEM_N,)),
        ],
        compiler_params=pltpu.CompilerParams(vmem_limit_bytes=120 * 1024 * 1024, disable_bounds_checks=True),
    )(
        A_x.reshape(S, D), A_mem0.reshape(M, D),
        A_Wq.reshape(D // 2, 2, H, DH), A_Wk.reshape(D // 2, 2, H, DH), A_Wv.reshape(D // 2, 2, H, DH),
        A_Wo.reshape(H * DH, D), B_w1, B_b1, B_w2, B_b2, c, w_mod,
    )
    return out.reshape(1, S, D)
```

```python
import contextlib
import functools

import jax
import jax.numpy as jnp
from jax import lax
import jax.experimental.pallas as pl
import jax.experimental.pallas.tpu as pltpu

F32 = jnp.float32
BF16 = jnp.bfloat16
U32 = jnp.uint32

S = 2048
D = 1024
H = 32
DH = 128
M = 8
SEG = 32
FF = 3584
NSEG = S // SEG
NP = H // 2
TPS = 24
T0 = S - NSEG * TPS
G0 = T0 // 8
RING = 72
ROFF = 8
EPS = 1e-5
P1U = 1
PA = 4
LNP = (48, 48, 48, 48, 32, 32)
PSTORE = True
LOG2E = 1.4426950408889634
UNROLL = 2
FB = 256
OC = 256
FC = 512
SEM_W, SEM_A, SEM_M, SEM_MISC, SEM_OUT = 0, 16, 24, 32, 40
SEM_N = SEM_OUT + S // FB


def _make_sched(g):
    out = []

    def rng(a, b):
        return tuple(range(max(a, 0), max(b, 0)))

    for p in range(NP):
        out.append(("proj", p))
        if p % g == 0 and p >= g:
            out.append(("attn", rng(p - 2 * g, p - g), rng(p - g, p)))
    h1 = 2 * (NP - 2 * g)
    h2 = 2 * (NP - g)
    if g == 4:
        out += [("wo", j, 0, h1) for j in (0, 1)]
        out.append(("attn", rng(NP - 2 * g, NP - g), rng(NP - g, NP)))
        out += [("wo", j, 0, h1) for j in (2, 3, 4, 5)]
        out.append(("attn", rng(NP - g, NP), ()))
        out += [("wo", j, 0, h1) for j in (6, 7)]
        out += [("wo", j, h1, h2) for j in range(8)]
        out += [("wo", j, h2, H) for j in range(8)]
    else:
        out += [("wo", 0, 0, h1)]
        out.append(("attn", rng(NP - 2 * g, NP - g), rng(NP - g, NP)))
        out += [("wo", j, 0, h1) for j in (1, 2, 3)]
        out.append(("attn", rng(NP - g, NP), ()))
        out += [("wo", j, 0, h1) for j in (4, 5, 6, 7)]
        out += [("wo", j, h1, H) for j in range(8)]
    return out


SCHED = _make_sched(2)
_SCOPES = False


def _scope(name):
    return jax.named_scope(name) if _SCOPES else contextlib.nullcontext()


def _dot(a, b):
    return jnp.dot(a, b, preferred_element_type=F32)


def _bf(x):
    return pltpu.bitcast(x, BF16)


def _u32(x):
    return pltpu.bitcast(x, U32)


def _ln(x):
    m = jnp.mean(x, axis=-1, keepdims=True)
    xc = x - m
    v = jnp.mean(xc * xc, axis=-1, keepdims=True)
    return xc * lax.rsqrt(v + EPS)


def _gelu(x):
    c = 0.7978845608028654
    return 0.5 * x * (1.0 + jnp.tanh(c * (x + 0.044715 * (x * x * x))))


def _interleave(a, b):
    n = a.shape[0] // 8
    parts = []
    for g in range(n):
        parts.append(a[8 * g:8 * g + 8])
        parts.append(b[8 * g:8 * g + 8])
    return jnp.concatenate(parts, axis=0)


def _deinterleave(v):
    n = v.shape[0] // 16
    a = jnp.concatenate([v[16 * g:16 * g + 8] for g in range(n)], axis=0)
    b = jnp.concatenate([v[16 * g + 8:16 * g + 16] for g in range(n)], axis=0)
    return a, b


def _kernel(x_hbm, mem0_hbm, wq_hbm, wk_hbm, wv_hbm, wo_hbm, w1_hbm, b1_hbm, w2_hbm, b2_hbm,
            c_hbm, wmod_hbm, out_hbm,
            x_v, h_v, hn_v, h2_v, x1_v, wmod_v, mod_v, sc_v, w_v, wo_v, w1_v, w2_v, qo_v, kv_v, mr_v, lo_v, pr_v, fill_v, out_v, bias_v, n_v,
            mem0_ref, b1_ref, b2_ref, c_ref,
            sems):
    w32 = [r.bitcast(U32) for r in (wq_hbm, wk_hbm, wv_hbm)]
    wo32 = wo_hbm.bitcast(U32)

    def w_copies(p):
        return [pltpu.make_async_copy(w32[j].at[:, par, p, :], w_v.at[p * 6 + j * 2 + par], sems.at[SEM_W + p])
                for j in range(3) for par in range(2)]

    def _mult(i, m):
        return i * m if isinstance(i, int) else pl.multiple_of(i * m, m)

    def wa_copies(k, pair=None):
        r = pl.ds(_mult(k, 64), 64)
        return [pltpu.make_async_copy(w32[j].at[r, par, p, :], w_v.at[p * 6 + j * 2 + par, r], sems.at[SEM_A + k])
                for p in (range(PA) if pair is None else (pair,)) for j in range(3) for par in range(2)]

    def m_copies(k):
        cols = [pl.ds(_mult(k + 8 * t, 128), 128) for t in range(2)]
        return [pltpu.make_async_copy(wmod_hbm.at[:, cs], wmod_v.at[:, cs], sems.at[SEM_M + k]) for cs in cols]

    def start(cps):
        for cp in cps:
            cp.start()

    def wait(cps):
        for cp in cps:
            cp.wait()

    cp_x0 = pltpu.make_async_copy(x_hbm.at[0:T0], x_v.at[0:T0], sems.at[SEM_MISC + 1])
    cp_x1 = pltpu.make_async_copy(x_hbm.at[T0:S], x_v.at[T0:S], sems.at[SEM_MISC + 6])
    cp_mod1 = pltpu.make_async_copy(wmod_hbm.at[:, 2 * D:6 * D], wmod_v.at[:, 2 * D:6 * D], sems.at[SEM_MISC + 2])

    def wo_copy(j):
        return pltpu.make_async_copy(wo32.at[:, pl.ds(_mult(j, 128), 128)], wo_v.at[j], sems.at[SEM_MISC + 3])

    cp_w1 = pltpu.make_async_copy(w1_hbm, w1_v, sems.at[SEM_MISC + 4])
    cp_w2 = pltpu.make_async_copy(w2_hbm, w2_v, sems.at[SEM_MISC + 5])

    cp_small = [pltpu.make_async_copy(src, dst, sems.at[SEM_MISC])
                for src, dst in ((c_hbm, c_ref), (mem0_hbm, mem0_ref), (b1_hbm, b1_ref), (b2_hbm, b2_ref))]

    start(cp_small)
    cp_x0.start()
    start(m_copies(0))
    for k in range(2):
        start(m_copies(k + 1))
        start(wa_copies(k))

    scale = DH ** -0.5
    ri = lax.broadcasted_iota(jnp.int32, (80, 128), 0)
    ci = lax.broadcasted_iota(jnp.int32, (80, 128), 1)
    same_head = (((ri >> 3) & 1) == ((ci >> 3) & 1)) & (ci < 80)
    rpos = ((ri >> 4) << 3) + (ri & 7)
    cpos = ((ci >> 4) << 3) + (ci & 7)
    keep = (ri >= 64) | (ci >= 64) | (rpos >= cpos)
    fill_v[...] = jnp.where(same_head, jnp.where(keep, 0.0, -1e9 / scale), -jnp.inf).astype(F32)

    wait(cp_small)
    c = c_ref[...].astype(F32)
    sc = jnp.broadcast_to(c * jax.nn.sigmoid(c), (8, D)).astype(BF16)

    sc_v[...] = sc
    bias_v[:, 0:FF] = b1_ref[...].astype(F32).reshape(1, FF)
    bias_v[:, FF:FF + D] = b2_ref[...].astype(F32).reshape(1, D)

    def zero_body(i, carry):
        x1_v[pl.ds(pl.multiple_of(i * 64, 64), 64), :] = jnp.zeros((64, D), F32)
        return carry

    lax.fori_loop(0, PA * 6, zero_body, 0)

    def relayout(c, rows):
        a = w_v[c, rows, :]
        b = w_v[c + 1, rows, :]
        lo = (a & jnp.uint32(0xFFFF)) | (b << 16)
        hi = (a >> 16) | (b & jnp.uint32(0xFFFF0000))
        w_v[c, rows, :] = lo
        w_v[c + 1, rows, :] = hi
        return _bf(lo), _bf(hi)

    def store_lead(p, j, a, b):
        r = _interleave(a, b).astype(BF16)
        if j == 0:
            qo_v[p, 0:16 * G0, :] = r
        else:
            kv_v[p, j - 1, 16 * ROFF:16 * (ROFF + G0), :] = r

    def mod_tile(ct):
        cs = pl.ds(_mult(ct, 128), 128)
        m = _dot(sc_v[...], wmod_v[:, cs])
        mod_v[:, cs] = m
        return m[0:1]

    with _scope("wait_x0"):
        cp_x0.wait()

    def ln1_body(i, carry):
        r = pl.multiple_of(i * 128, 128)
        n = _ln(x_v[pl.ds(r, 128), :].astype(F32))
        for k in range(8):
            n_v[k, pl.ds(r, 128), :] = n[:, k * 128:(k + 1) * 128]
        return carry

    with _scope("ln1"):
        lax.fori_loop(0, T0 // 128, ln1_body, 0)
    start(m_copies(3))
    start(wa_copies(2))
    with _scope("wait_m0"):
        wait(m_copies(0))
    h_v[0] = (n_v[0] * (1.0 + mod_tile(8)) + mod_tile(0)).astype(BF16)

    def sa_body(k, carry):
        with _scope("wait_a"):
            wait(wa_copies(k))

            @pl.when(k < 7)
            def _():
                wait(m_copies(k + 1))

        kn = jnp.minimum(k + 1, 7)
        rows = pl.ds(pl.multiple_of(k * 64, 64), 64)
        hk = h_v[k]
        for p in range(PA):
            for j in range(3):
                c = p * 6 + j * 2
                res = []
                for t, w in enumerate(relayout(c, rows)):
                    acc = x1_v.at[(c + t) // 8 * T0:((c + t) // 8 + 1) * T0,
                                  (c + t) % 8 * 128:((c + t) % 8 + 1) * 128]
                    r = _dot(hk, w) + acc[...]
                    acc[...] = r
                    res.append(r)
                store_lead(p, j, *res)
                if c == 2:
                    sh = mod_tile(kn)
                if c == 6:
                    s1 = 1.0 + mod_tile(kn + 8)

                    @pl.when(k + 4 < 8)
                    def _():
                        start(m_copies(k + 4))

            @pl.when(k + 3 < 8)
            def _():
                start(wa_copies(k + 3, p))

        h_v[kn] = (n_v[kn] * s1 + sh).astype(BF16)


        @pl.when(k >= 4)
        def _():
            start(w_copies(PA + k - 4))

        return carry

    with _scope("stageA"):
        lax.fori_loop(0, 8, sa_body, 0)

    def ln1(r, n):
        xb = x_v[pl.ds(r, n), :].astype(F32)
        return _ln(xb) * (1.0 + mod_v[0:1, D:2 * D]) + mod_v[0:1, 0:D]

    def p1_body(i, carry):
        p0 = PA + P1U * i
        with _scope("wait_w"):
            for u in range(P1U):
                wait(w_copies(p0 + u))

        hb = jnp.concatenate([h_v[k] for k in range(8)], axis=1)
        for u in range(P1U):
            p = p0 + u
            for j in range(3):
                lo, hi = relayout(p * 6 + j * 2, slice(None))
                store_lead(p, j, _dot(hb, lo), _dot(hb, hi))

        @pl.when(p0 + 4 < NP)
        def _():
            for u in range(P1U):
                start(w_copies(p0 + 4 + u))
                wo_copy(P1U * i + u).start()

        @pl.when(p0 + 4 == NP)
        def _():
            cp_x1.start()

        return carry

    with _scope("phase1"):
        lax.fori_loop(0, (NP - PA) // P1U, p1_body, 0)

    with _scope("wait_wo"):
        for j in range(8):
            wo_copy(j).wait()
        cp_x1.wait()
    hn_v[...] = ln1(T0, TPS)

    def step(s, mem):
        lhs = jnp.concatenate([mem, hn_v[...]], axis=0).astype(BF16)
        t_nx = pl.multiple_of(jnp.minimum(T0 + TPS * (s + 1), S - TPS), 8)
        hn_v[...] = ln1(t_nx, TPS)
        q_wr = pl.multiple_of(16 * (G0 + 3 * s), 16)
        kv_wr = pl.multiple_of(16 * lax.rem(3 * s, RING), 16)
        q_rd = pl.multiple_of(64 * s, 16)
        kv_rd = pl.multiple_of(16 * lax.rem(4 * s + ROFF, RING), 16)
        o_rd = pl.multiple_of(48 * s, 16)
        prob = {}
        pending = []

        def flush():
            for p, j, r in pending:
                if j == 0:
                    qo_v[p, pl.ds(q_wr, 48), :] = r.astype(BF16)
                else:
                    kv_v[p, j - 1, pl.ds(kv_wr, 48), :] = r.astype(BF16)
            pending.clear()

        def proj(p):
            flush()
            if p == 0:
                half = [_dot(lhs[:, 0:D // 2], _bf(w_v[c, 0:D // 4, :])) for c in range(6)]
                cols = [_dot(lhs[:, D // 2:D], _bf(w_v[c, D // 4:D // 2, :])) + half[c] for c in range(6)]
            for j in range(3):
                if p == 0:
                    r = _interleave(cols[j * 2], cols[j * 2 + 1])
                else:
                    r = _interleave(_dot(lhs, _bf(w_v[p * 6 + j * 2])), _dot(lhs, _bf(w_v[p * 6 + j * 2 + 1])))
                pending.append((p, j, r[16:64]))
                mr_v[p * 3 + j] = r[0:16].astype(BF16)

        def stack(p, j):
            t = qo_v[p, pl.ds(q_rd, 64), :] if j == 0 else kv_v[p, j - 1, pl.ds(kv_rd, 64), :]
            return jnp.concatenate([t, mr_v[p * 3 + j]], axis=0)

        def attn(pvs, qks):
            if any(p in pvs or p in qks for p, _, _ in pending):
                flush()
            vs = [stack(p, 2) for p in pvs]
            qs = [stack(p, 0) for p in qks]
            ks = [stack(p, 1) for p in qks]
            os_ = [_dot(pr_v[p, :, 0:80] if PSTORE else prob[p][:, 0:80].astype(BF16), v) for p, v in zip(pvs, vs)]
            ss = [lax.dot_general(q, k, (((1,), (1,)), ((), ())), preferred_element_type=F32)
                  for q, k in zip(qs, ks)]
            flush()
            for p, o in zip(pvs, os_):
                qo_v[p, pl.ds(q_rd, 64), :] = o[0:64].astype(BF16)
                oa, ob = _deinterleave(qo_v[p, pl.ds(o_rd, 48), :].astype(F32))
                lo_v[2 * p] = jnp.concatenate([o[64:72], oa], axis=0).astype(BF16)
                lo_v[2 * p + 1] = jnp.concatenate([o[72:80], ob], axis=0).astype(BF16)
            for p, sc_ in zip(qks, ss):
                fill = fill_v[...]
                sc_ = jnp.concatenate([sc_, jnp.zeros((80, 48), F32)], axis=1)
                sc_ = jnp.where(fill == 0.0, sc_, fill)
                mx = jnp.max(sc_, axis=-1, keepdims=True)
                e = jnp.exp2((sc_ - mx) * (scale * LOG2E))
                l = jnp.sum(e, axis=-1, keepdims=True)
                r = pl.reciprocal(l, approx=True)
                prob[p] = e * (r * (2.0 - l * r))
                if PSTORE:
                    pr_v[p] = prob[p].astype(BF16)

        part = {}

        def wo(j, h0, h1):
            lo = jnp.concatenate([lo_v[h] for h in range(h0, h1)], axis=1)
            r = _dot(lo, _bf(wo_v[j, h0 * 64:h1 * 64, :]))
            part[j] = r + part[j] if j in part else r

        for op in SCHED:
            if op[0] == "proj":
                proj(op[1])
            elif op[0] == "attn":
                attn(op[1], op[2])
            else:
                wo(*op[1:])
        res = jnp.concatenate([part[j] for j in range(8)], axis=1)
        x1_v[pl.ds(pl.multiple_of(TPS * s, 8), TPS), :] = res[8:32]
        return res[0:8]

    with _scope("main"):
        def steps(i, mem):
            @pl.when(i == 1)
            def _():
                cp_mod1.start()
                cp_w1.start()
                cp_w2.start()

            with _scope("iter"):
                for u in range(UNROLL):
                    mem = step(i * UNROLL + u, mem)
            return mem

        lax.fori_loop(0, NSEG // UNROLL, steps, mem0_ref[...].astype(F32))

    cp_mod1.wait()

    def wo_body(i, carry):
        r0 = pl.multiple_of(S - T0 + i * 128, 128)
        parts = []
        for p in range(NP):
            oa, ob = _deinterleave(qo_v[p, pl.ds(2 * r0, 256), :].astype(F32))
            parts.append(oa)
            parts.append(ob)
        lo = jnp.concatenate(parts, axis=1).astype(BF16)
        for j in range(8):
            x1_v[pl.ds(r0, 128), j * 128:(j + 1) * 128] = _dot(lo, _bf(wo_v[j]))
            mod_tile(16 + i * 8 + j)
        return carry

    with _scope("p3a"):
        lax.fori_loop(0, T0 // 128, wo_body, 0)

    cp_w1.wait()
    cp_w2.wait()

    def out_copy(i, q):
        rows = pl.ds(_mult(i, FB), FB)
        cols = pl.ds(q * OC, OC)
        return pltpu.make_async_copy(out_v.at[rows, cols], out_hbm.at[rows, cols], sems.at[SEM_OUT + i])

    def resid1(r0, n, c0=0, nc=D):
        return (x_v[pl.ds(r0, n), c0:c0 + nc].astype(F32)
                + mod_v[0:1, 2 * D + c0:2 * D + c0 + nc] * x1_v[pl.ds(r0, n), c0:c0 + nc])

    def ln2(slot, r0, k0, n):
        h2 = _ln(resid1(r0 + k0, n)) * (1.0 + mod_v[0:1, 4 * D:5 * D]) + mod_v[0:1, 3 * D:4 * D]
        h2_v[slot, k0 // 2:(k0 + n) // 2, :] = _u32(h2.astype(BF16))

    ln2(0, 0, 0, FB)

    def ffn_body(i, carry):
        r0 = pl.multiple_of(i * FB, FB)
        rn = pl.multiple_of(jnp.minimum(r0 + FB, S - FB), FB)
        slot = lax.rem(i, 2)
        acc = None
        nf = FF // FC
        for f in range(nf):
            a = _dot(_bf(h2_v[slot]), w1_v[:, f * FC:(f + 1) * FC]) + bias_v[0:1, f * FC:(f + 1) * FC]
            if f < len(LNP):
                ln2(1 - slot, rn, sum(LNP[:f]), LNP[f])
            y = _dot(_gelu(a).astype(BF16), w2_v[f * FC:(f + 1) * FC, :])
            acc = y if acc is None else y + acc
        y = (acc + bias_v[0:1, FF:FF + D]) * mod_v[0:1, 5 * D:6 * D]
        for q in range(D // OC):
            c0 = q * OC
            out_v[pl.ds(r0, FB), c0:c0 + OC] = (resid1(r0, FB, c0, OC) + y[:, c0:c0 + OC]).astype(BF16)
            out_copy(i, q).start()
        return carry

    with _scope("ffn"):
        lax.fori_loop(0, S // FB, ffn_body, 0)
    with _scope("wait_out"):
        for i in range(S // FB):
            for q in range(D // OC):
                out_copy(i, q).wait()


@functools.partial(jax.jit, static_argnames=("A_seg_len",))
def pallas_adaLN_cond__memory_aug_recurrent_mem_tr__dense_activation_gelu__prompt_kernel(
    A_x, A_mem0, A_Wq, A_Wk, A_Wv, A_Wo, A_seg_len, B_x, B_w1, B_b1, B_w2, B_b2, c, w_mod,
):
    assert A_seg_len == SEG and A_x.shape == (1, S, D)
    hbm = pl.BlockSpec(memory_space=pl.ANY)
    out = pl.pallas_call(
        _kernel,
        out_shape=jax.ShapeDtypeStruct((S, D), BF16),
        in_specs=[hbm] * 12,
        out_specs=hbm,
        scratch_shapes=[
            pltpu.VMEM((S, D), BF16),
            pltpu.VMEM((8, T0, 128), BF16),
            pltpu.VMEM((TPS, D), F32),
            pltpu.VMEM((2, FB // 2, D), U32),
            pltpu.VMEM((S, D), F32),
            pltpu.VMEM((D, 6 * D), BF16),
            pltpu.VMEM((8, 6 * D), F32),
            pltpu.VMEM((8, D), BF16),
            pltpu.VMEM((6 * NP, D // 2, 128), U32),
            pltpu.VMEM((8, H * DH // 2, 128), U32),
            pltpu.VMEM((D, FF), BF16),
            pltpu.VMEM((FF, D), BF16),
            pltpu.VMEM((NP, 2 * S, 128), BF16),
            pltpu.VMEM((NP, 2, 16 * RING, 128), BF16),
            pltpu.VMEM((3 * NP, 16, 128), BF16),
            pltpu.VMEM((H, 32, 128), BF16),
            pltpu.VMEM((NP, 80, 128), BF16),
            pltpu.VMEM((80, 128), F32),
            pltpu.VMEM((S, D), BF16),
            pltpu.VMEM((1, FF + D), F32),
            pltpu.VMEM((8, T0, 128), F32),
            pltpu.VMEM((M, D), BF16),
            pltpu.VMEM((FF,), BF16),
            pltpu.VMEM((D,), BF16),
            pltpu.VMEM((1, D), BF16),
            pltpu.SemaphoreType.DMA((SEM_N,)),
        ],
        compiler_params=pltpu.CompilerParams(vmem_limit_bytes=120 * 1024 * 1024, disable_bounds_checks=True,
                                             disable_semaphore_checks=True),
    )(
        A_x.reshape(S, D), A_mem0.reshape(M, D),
        A_Wq.reshape(D // 2, 2, H, DH), A_Wk.reshape(D // 2, 2, H, DH), A_Wv.reshape(D // 2, 2, H, DH),
        A_Wo.reshape(H * DH, D), B_w1, B_b1, B_w2, B_b2, c, w_mod,
    )
    return out.reshape(1, S, D)
```

```python
import contextlib

import jax
import jax.numpy as jnp
from jax import lax
import jax.experimental.pallas as pl
import jax.experimental.pallas.tpu as pltpu

F32 = jnp.float32
BF16 = jnp.bfloat16
U32 = jnp.uint32

S = 2048
D = 1024
H = 32
DH = 128
M = 8
SEG = 32
FF = 3584
NSEG = S // SEG
NP = H // 2
TPS = 24
T0 = S - NSEG * TPS
EPS = 1e-5
P1U = 2
PA = 4
LNP = (64, 64, 32, 32, 32, 32)
MODPOS = (5, 0, 24)
LOG2E = 1.4426950408889634
UNROLL = 2
FB = 256
OC = 256
FC = 512
SEM_W, SEM_A, SEM_M, SEM_MISC, SEM_OUT = 0, 16, 24, 32, 40
SEM_N = SEM_OUT + S // FB


def _make_sched(g):
    out = []

    def rng(a, b):
        return tuple(range(max(a, 0), max(b, 0)))

    for p in range(NP):
        out.append(("proj", p))
        if p % g == 0 and p >= g:
            out.append(("attn", rng(p - 2 * g, p - g), rng(p - g, p)))
    h1 = 2 * (NP - 2 * g)
    h2 = 2 * (NP - g)
    if g == 4:
        out += [("wo", j, 0, h1) for j in (0, 1)]
        out.append(("attn", rng(NP - 2 * g, NP - g), rng(NP - g, NP)))
        out += [("wo", j, 0, h1) for j in (2, 3, 4, 5)]
        out.append(("attn", rng(NP - g, NP), ()))
        out += [("wo", j, 0, h1) for j in (6, 7)]
        out += [("wo", j, h1, h2) for j in range(8)]
        out += [("wo", j, h2, H) for j in range(8)]
    else:
        out += [("wo", 0, 0, h1)]
        out.append(("attn", rng(NP - 2 * g, NP - g), rng(NP - g, NP)))
        out += [("wo", j, 0, h1) for j in (1, 2, 3)]
        out.append(("attn", rng(NP - g, NP), ()))
        out += [("wo", j, 0, h1) for j in (4, 5, 6, 7)]
        out += [("wo", j, h1, H) for j in range(8)]
    return out


SCHED = _make_sched(2)
_SCOPES = False


def _scope(name):
    return jax.named_scope(name) if _SCOPES else contextlib.nullcontext()


def _dot(a, b):
    return jnp.dot(a, b, preferred_element_type=F32)


def _bf(x):
    return pltpu.bitcast(x, BF16)


def _u32(x):
    return pltpu.bitcast(x, U32)


def _ln(x):
    m = jnp.mean(x, axis=-1, keepdims=True)
    xc = x - m
    v = jnp.mean(xc * xc, axis=-1, keepdims=True)
    return xc * lax.rsqrt(v + EPS)


def _gelu(x):
    c = 0.7978845608028654
    return 0.5 * x * (1.0 + jnp.tanh(c * (x + 0.044715 * (x * x * x))))


def _interleave(a, b):
    n = a.shape[0] // 8
    parts = []
    for g in range(n):
        parts.append(a[8 * g:8 * g + 8])
        parts.append(b[8 * g:8 * g + 8])
    return jnp.concatenate(parts, axis=0)


def _deinterleave(v):
    n = v.shape[0] // 16
    a = jnp.concatenate([v[16 * g:16 * g + 8] for g in range(n)], axis=0)
    b = jnp.concatenate([v[16 * g + 8:16 * g + 16] for g in range(n)], axis=0)
    return a, b


def _kernel(x_hbm, mem0_hbm, wq_hbm, wk_hbm, wv_hbm, wo_hbm, w1_hbm, b1_hbm, w2_hbm, b2_hbm,
            c_hbm, wmod_hbm, out_hbm,
            x_v, h_v, hn_v, h2_v, x1_v, wmod_v, mod_v, sc_v, w_v, wo_v, w1_v, w2_v, lead_v, fr_v, lo_v, pr_v, fill_v, out_v, bias_v, n_v,
            mem0_ref, b1_ref, b2_ref, c_ref,
            sems):
    w32 = [r.bitcast(U32) for r in (wq_hbm, wk_hbm, wv_hbm)]
    wo32 = wo_hbm.bitcast(U32)

    def w_copies(p):
        return [pltpu.make_async_copy(w32[j].at[:, par, p, :], w_v.at[p * 6 + j * 2 + par], sems.at[SEM_W + p])
                for j in range(3) for par in range(2)]

    def _mult(i, m):
        return i * m if isinstance(i, int) else pl.multiple_of(i * m, m)

    def wa_copies(k, pair=None):
        r = pl.ds(_mult(k, 64), 64)
        return [pltpu.make_async_copy(w32[j].at[r, par, p, :], w_v.at[p * 6 + j * 2 + par, r], sems.at[SEM_A + k])
                for p in (range(PA) if pair is None else (pair,)) for j in range(3) for par in range(2)]

    def m_copies(k):
        cols = [pl.ds(_mult(k + 8 * t, 128), 128) for t in range(2)]
        return [pltpu.make_async_copy(wmod_hbm.at[:, cs], wmod_v.at[:, cs], sems.at[SEM_M + k]) for cs in cols]

    def start(cps):
        for cp in cps:
            cp.start()

    def wait(cps):
        for cp in cps:
            cp.wait()

    cp_x0 = pltpu.make_async_copy(x_hbm.at[:, 0:8, :], x_v.at[:, 0:8, :], sems.at[SEM_MISC + 1])
    cp_x1 = pltpu.make_async_copy(x_hbm.at[:, 8:SEG, :], x_v.at[:, 8:SEG, :], sems.at[SEM_MISC + 6])

    def mod1_copy(t):
        cs = pl.ds(_mult(2 + t, D), D)
        return pltpu.make_async_copy(wmod_hbm.at[:, cs], wmod_v.at[:, cs], sems.at[SEM_M + t])

    def wo_copy(j):
        return pltpu.make_async_copy(wo32.at[:, pl.ds(_mult(j, 128), 128)], wo_v.at[j], sems.at[SEM_MISC + 3])

    cp_w1 = pltpu.make_async_copy(w1_hbm, w1_v, sems.at[SEM_MISC + 4])
    cp_w2 = pltpu.make_async_copy(w2_hbm, w2_v, sems.at[SEM_MISC + 5])

    cp_small = [pltpu.make_async_copy(src, dst, sems.at[SEM_MISC])
                for src, dst in ((c_hbm, c_ref), (mem0_hbm, mem0_ref), (b1_hbm, b1_ref), (b2_hbm, b2_ref))]

    start(cp_small)
    cp_x0.start()
    start(m_copies(0))
    for k in range(2):
        start(m_copies(k + 1))
        start(wa_copies(k))

    scale = DH ** -0.5
    ri = lax.broadcasted_iota(jnp.int32, (80, 128), 0)
    ci = lax.broadcasted_iota(jnp.int32, (80, 128), 1)
    same_head = (((ri >> 3) & 1) == ((ci >> 3) & 1)) & (ci < 80)
    rpos = (((ri >> 4) & 3) << 3) + (ri & 7)
    cpos = (((ci >> 4) & 3) << 3) + (ci & 7)
    keep = (ri < 16) | (ci < 16) | (rpos >= cpos)
    fill_v[...] = jnp.where(same_head, jnp.where(keep, 0.0, -1e9 / scale), -jnp.inf).astype(F32)

    wait(cp_small)
    c = c_ref[...].astype(F32)
    sc = jnp.broadcast_to(c * jax.nn.sigmoid(c), (8, D)).astype(BF16)

    sc_v[...] = sc
    bias_v[:, 0:FF] = b1_ref[...].astype(F32).reshape(1, FF)
    bias_v[:, FF:FF + D] = b2_ref[...].astype(F32).reshape(1, D)

    def zero_body(i, carry):
        x1_v[pl.ds(pl.multiple_of(i * 64, 64), 64), :] = jnp.zeros((64, D), F32)
        return carry

    lax.fori_loop(0, PA * 6, zero_body, 0)

    def relayout(c, rows):
        a = w_v[c, rows, :]
        b = w_v[c + 1, rows, :]
        lo = (a & jnp.uint32(0xFFFF)) | (b << 16)
        hi = (a >> 16) | (b & jnp.uint32(0xFFFF0000))
        w_v[c, rows, :] = lo
        w_v[c + 1, rows, :] = hi
        return _bf(lo), _bf(hi)

    def store_lead(p, j, a, b):
        lead_v[p * 3 + j] = _interleave(a, b).astype(BF16)

    def mod_tile(ct):
        cs = pl.ds(_mult(ct, 128), 128)
        m = _dot(sc_v[...], wmod_v[:, cs])
        mod_v[:, cs] = m
        return m[0:1]

    with _scope("wait_x0"):
        cp_x0.wait()

    def ln1_body(i, carry):
        r = pl.multiple_of(i * 128, 128)
        n = _ln(x_v[pl.ds(i * 16, 16), 0:8, :].astype(F32).reshape(128, D))
        for k in range(8):
            n_v[k, pl.ds(r, 128), :] = n[:, k * 128:(k + 1) * 128]
        return carry

    with _scope("ln1"):
        lax.fori_loop(0, T0 // 128, ln1_body, 0)
    start(m_copies(3))
    start(wa_copies(2))
    with _scope("wait_m0"):
        wait(m_copies(0))
    h_v[0] = (n_v[0] * (1.0 + mod_tile(8)) + mod_tile(0)).astype(BF16)

    def sa_body(k, carry):
        with _scope("wait_a"):
            wait(wa_copies(k))

            @pl.when(k < 7)
            def _():
                wait(m_copies(k + 1))

        kn = jnp.minimum(k + 1, 7)
        rows = pl.ds(pl.multiple_of(k * 64, 64), 64)
        hk = h_v[k]
        for p in range(PA):
            for j in range(3):
                c = p * 6 + j * 2
                res = []
                for t, w in enumerate(relayout(c, rows)):
                    acc = x1_v.at[(c + t) // 8 * T0:((c + t) // 8 + 1) * T0,
                                  (c + t) % 8 * 128:((c + t) % 8 + 1) * 128]
                    r = _dot(hk, w) + acc[...]
                    acc[...] = r
                    res.append(r)
                store_lead(p, j, *res)
                if c == 2:
                    sh = mod_tile(kn)
                if c == 6:
                    s1 = 1.0 + mod_tile(kn + 8)

                    @pl.when(k + 4 < 8)
                    def _():
                        start(m_copies(k + 4))

            @pl.when(k + 3 < 8)
            def _():
                start(wa_copies(k + 3, p))

        h_v[kn] = (n_v[kn] * s1 + sh).astype(BF16)


        @pl.when(k >= 4)
        def _():
            start(w_copies(PA + k - 4))

        return carry

    with _scope("stageA"):
        lax.fori_loop(0, 8, sa_body, 0)

    def ln1(seg):
        xb = x_v[seg, 8:SEG, :].astype(F32)
        return _ln(xb) * (1.0 + mod_v[0:1, D:2 * D]) + mod_v[0:1, 0:D]

    def p1_body(i, carry):
        p0 = PA + P1U * i
        with _scope("wait_w"):
            for u in range(P1U):
                wait(w_copies(p0 + u))

        hb = jnp.concatenate([h_v[k] for k in range(8)], axis=1)
        for u in range(P1U):
            p = p0 + u
            for j in range(3):
                lo, hi = relayout(p * 6 + j * 2, slice(None))
                store_lead(p, j, _dot(hb, lo), _dot(hb, hi))

        @pl.when(p0 + 4 < NP)
        def _():
            for u in range(P1U):
                start(w_copies(p0 + 4 + u))
                wo_copy(P1U * i + u).start()

        @pl.when(p0 + 4 == NP)
        def _():
            cp_x1.start()
            mod1_copy(0).start()

        return carry

    with _scope("phase1"):
        lax.fori_loop(0, (NP - PA) // P1U, p1_body, 0)

    with _scope("wait_wo"):
        for j in range(8):
            wo_copy(j).wait()
        cp_x1.wait()
        mod1_copy(0).wait()
    hn_v[...] = ln1(0)

    def step(s, odd, mem):
        lhs = jnp.concatenate([mem, hn_v[...]], axis=0).astype(BF16)
        hn_v[...] = ln1(jnp.minimum(s + 1, NSEG - 1))
        ld_rd = pl.multiple_of(16 * s, 16)
        mo = 48 if odd else 32

        def proj(p):
            if p == 0:
                half = [_dot(lhs[:, 0:D // 2], _bf(w_v[c, 0:D // 4, :])) for c in range(6)]
                cols = [_dot(lhs[:, D // 2:D], _bf(w_v[c, D // 4:D // 2, :])) + half[c] for c in range(6)]
            for j in range(3):
                if p == 0:
                    r = _interleave(cols[j * 2], cols[j * 2 + 1])
                else:
                    r = _interleave(_dot(lhs, _bf(w_v[p * 6 + j * 2])), _dot(lhs, _bf(w_v[p * 6 + j * 2 + 1])))
                fr_v[p * 3 + j] = r.astype(BF16)

        def stack(p, j):
            return jnp.concatenate([fr_v[p * 3 + j], lead_v[p * 3 + j, pl.ds(ld_rd, 16), :]], axis=0)

        def attn(pvs, qks):
            os_ = [_dot(pr_v[p, :, 0:80], stack(p, 2)) for p in pvs]
            ss = [lax.dot_general(stack(p, 0), stack(p, 1), (((1,), (1,)), ((), ())),
                                  preferred_element_type=F32) for p in qks]
            for p, o in zip(pvs, os_):
                for t, oh in enumerate(_deinterleave(o)):
                    h = 2 * p + t
                    if odd:
                        lo_v[1, h, 0:8, :] = oh[0:8].astype(BF16)
                        lo_v[1, h, 16:48, :] = oh[8:40].astype(BF16)
                    else:
                        lo_v[0, h, 0:32, :] = oh[0:32].astype(BF16)
                        lo_v[1, h, 8:16, :] = oh[32:40].astype(BF16)
            for p, sc_ in zip(qks, ss):
                fill = fill_v[...]
                sc_ = jnp.concatenate([sc_, jnp.zeros((80, 48), F32)], axis=1)
                sc_ = jnp.where(fill == 0.0, sc_, fill)
                mx = jnp.max(sc_, axis=-1, keepdims=True)
                e = jnp.exp2((sc_ - mx) * (scale * LOG2E))
                l = jnp.sum(e, axis=-1, keepdims=True)
                r = pl.reciprocal(l, approx=True)
                pr_v[p] = (e * (r * (2.0 - l * r))).astype(BF16)

        part = {}

        def wo(j, h0, h1):
            lo = jnp.concatenate([lo_v[int(odd), h, 0:mo, :] for h in range(h0, h1)], axis=1)
            r = _dot(lo, _bf(wo_v[j, h0 * 64:h1 * 64, :]))
            part[j] = r + part[j] if j in part else r

        for op in SCHED:
            if op[0] == "proj":
                proj(op[1])
            elif op[0] == "attn":
                attn(op[1], op[2])
            else:
                wo(*op[1:])
                if odd and op[1:] == MODPOS:
                    mod_tile(16 + s // 2)
        res = jnp.concatenate([part[j] for j in range(8)], axis=1)
        t0 = pl.multiple_of(SEG * s, SEG)
        if odd:
            x1_v[pl.ds(t0 - SEG, 8), :] = res[8:16]
            x1_v[pl.ds(t0, SEG), :] = jnp.concatenate([res[40:48], res[16:40]], axis=0)
        else:
            x1_v[pl.ds(t0 + 8, TPS), :] = res[8:32]
        return res[0:8]

    with _scope("main"):
        def steps(i, mem):
            @pl.when(i == 1)
            def _():
                for t in range(1, 4):
                    mod1_copy(t).start()
                cp_w1.start()
                cp_w2.start()

            with _scope("iter"):
                for u in range(UNROLL):
                    mem = step(i * UNROLL + u, u % 2 == 1, mem)

            @pl.when(jnp.logical_and(lax.rem(i, 8) == 7, i < 24))
            def _():
                mod1_copy(i // 8 + 1).wait()

            return mem

        lax.fori_loop(0, NSEG // UNROLL, steps, mem0_ref[...].astype(F32))

    cp_w1.wait()
    cp_w2.wait()

    def out_copy(i, q):
        rows = pl.ds(_mult(i, FB), FB)
        cols = pl.ds(q * OC, OC)
        return pltpu.make_async_copy(out_v.at[rows, cols], out_hbm.at[rows, cols], sems.at[SEM_OUT + i])

    def resid1(r0, n, c0=0, nc=D):
        xb = x_v[pl.ds(r0 // SEG, n // SEG), :, c0:c0 + nc].astype(F32).reshape(n, nc)
        return (xb
                + mod_v[0:1, 2 * D + c0:2 * D + c0 + nc] * x1_v[pl.ds(r0, n), c0:c0 + nc])

    def ln2(slot, r0, k0, n):
        h2 = _ln(resid1(r0 + k0, n)) * (1.0 + mod_v[0:1, 4 * D:5 * D]) + mod_v[0:1, 3 * D:4 * D]
        h2_v[slot, k0 // 2:(k0 + n) // 2, :] = _u32(h2.astype(BF16))

    ln2(0, 0, 0, FB)

    def ffn_body(i, carry):
        r0 = pl.multiple_of(i * FB, FB)
        rn = pl.multiple_of(jnp.minimum(r0 + FB, S - FB), FB)
        slot = lax.rem(i, 2)
        acc = None
        nf = FF // FC
        for f in range(nf):
            a = _dot(_bf(h2_v[slot]), w1_v[:, f * FC:(f + 1) * FC]) + bias_v[0:1, f * FC:(f + 1) * FC]
            if f < len(LNP):
                ln2(1 - slot, rn, sum(LNP[:f]), LNP[f])
            y = _dot(_gelu(a).astype(BF16), w2_v[f * FC:(f + 1) * FC, :])
            acc = y if acc is None else y + acc
        y = (acc + bias_v[0:1, FF:FF + D]) * mod_v[0:1, 5 * D:6 * D]
        for q in range(D // OC):
            c0 = q * OC
            out_v[pl.ds(r0, FB), c0:c0 + OC] = (resid1(r0, FB, c0, OC) + y[:, c0:c0 + OC]).astype(BF16)
            out_copy(i, q).start()
        return carry

    with _scope("ffn"):
        lax.fori_loop(0, S // FB, ffn_body, 0)
    with _scope("wait_out"):
        for i in range(S // FB):
            for q in range(D // OC):
                out_copy(i, q).wait()


@jax.jit
def pallas_adaLN_cond__memory_aug_recurrent_mem_tr__dense_activation_gelu__prompt_kernel(
    A_x, A_mem0, A_Wq, A_Wk, A_Wv, A_Wo, A_seg_len, B_x, B_w1, B_b1, B_w2, B_b2, c, w_mod,
):
    del A_seg_len, B_x
    assert A_x.shape == (1, S, D)
    hbm = pl.BlockSpec(memory_space=pl.ANY)
    out = pl.pallas_call(
        _kernel,
        out_shape=jax.ShapeDtypeStruct((S, D), BF16),
        in_specs=[hbm] * 12,
        out_specs=hbm,
        scratch_shapes=[
            pltpu.VMEM((NSEG, SEG, D), BF16),
            pltpu.VMEM((8, T0, 128), BF16),
            pltpu.VMEM((TPS, D), F32),
            pltpu.VMEM((2, FB // 2, D), U32),
            pltpu.VMEM((S, D), F32),
            pltpu.VMEM((D, 6 * D), BF16),
            pltpu.VMEM((8, 6 * D), F32),
            pltpu.VMEM((8, D), BF16),
            pltpu.VMEM((6 * NP, D // 2, 128), U32),
            pltpu.VMEM((8, H * DH // 2, 128), U32),
            pltpu.VMEM((D, FF), BF16),
            pltpu.VMEM((FF, D), BF16),
            pltpu.VMEM((3 * NP, 2 * T0, 128), BF16),
            pltpu.VMEM((3 * NP, 64, 128), BF16),
            pltpu.VMEM((2, H, 48, 128), BF16),
            pltpu.VMEM((NP, 80, 128), BF16),
            pltpu.VMEM((80, 128), F32),
            pltpu.VMEM((S, D), BF16),
            pltpu.VMEM((1, FF + D), F32),
            pltpu.VMEM((8, T0, 128), F32),
            pltpu.VMEM((M, D), BF16),
            pltpu.VMEM((FF,), BF16),
            pltpu.VMEM((D,), BF16),
            pltpu.VMEM((1, D), BF16),
            pltpu.SemaphoreType.DMA((SEM_N,)),
        ],
        compiler_params=pltpu.CompilerParams(vmem_limit_bytes=120 * 1024 * 1024, disable_bounds_checks=True,
                                             disable_semaphore_checks=True),
    )(
        A_x.reshape(NSEG, SEG, D), A_mem0.reshape(M, D),
        A_Wq.reshape(D // 2, 2, H, DH), A_Wk.reshape(D // 2, 2, H, DH), A_Wv.reshape(D // 2, 2, H, DH),
        A_Wo.reshape(H * DH, D), B_w1, B_b1, B_w2, B_b2, c, w_mod,
    )
    return out.reshape(1, S, D)
```

```python
import contextlib

import jax
import jax.numpy as jnp
from jax import lax
import jax.experimental.pallas as pl
import jax.experimental.pallas.tpu as pltpu

F32 = jnp.float32
BF16 = jnp.bfloat16
U32 = jnp.uint32

S = 2048
D = 1024
H = 32
DH = 128
M = 8
SEG = 32
FF = 3584
NSEG = S // SEG
NP = H // 2
TPS = 24
T0 = S - NSEG * TPS
EPS = 1e-5
P1U = 2
PA = 4
LNP = (64, 64, 32, 32, 32, 32)
MODPOS = ((5, 0, 24), (6, 0, 24))
LOG2E = 1.4426950408889634
UNROLL = 2
FB = 256
OC = 256
FC = 512
SEM_W, SEM_A, SEM_M, SEM_MISC, SEM_OUT = 0, 16, 24, 32, 40
SEM_N = SEM_OUT + S // FB


def _make_sched(g):
    out = []

    def rng(a, b):
        return tuple(range(max(a, 0), max(b, 0)))

    for p in range(NP):
        out.append(("proj", p))
        if p % g == 0 and p >= g:
            out.append(("attn", rng(p - 2 * g, p - g), rng(p - g, p)))
    h1 = 2 * (NP - 2 * g)
    h2 = 2 * (NP - g)
    if g == 4:
        out += [("wo", j, 0, h1) for j in (0, 1)]
        out.append(("attn", rng(NP - 2 * g, NP - g), rng(NP - g, NP)))
        out += [("wo", j, 0, h1) for j in (2, 3, 4, 5)]
        out.append(("attn", rng(NP - g, NP), ()))
        out += [("wo", j, 0, h1) for j in (6, 7)]
        out += [("wo", j, h1, h2) for j in range(8)]
        out += [("wo", j, h2, H) for j in range(8)]
    else:
        out += [("wo", 0, 0, h1)]
        out.append(("attn", rng(NP - 2 * g, NP - g), rng(NP - g, NP)))
        out += [("wo", j, 0, h1) for j in (1, 2, 3)]
        out.append(("attn", rng(NP - g, NP), ()))
        out += [("wo", j, 0, h1) for j in (4, 5, 6, 7)]
        out += [("wo", j, h1, H) for j in range(8)]
    return out


SCHED = _make_sched(2)
_SCOPES = False


def _scope(name):
    return jax.named_scope(name) if _SCOPES else contextlib.nullcontext()


def _dot(a, b):
    return jnp.dot(a, b, preferred_element_type=F32)


def _bf(x):
    return pltpu.bitcast(x, BF16)


def _u32(x):
    return pltpu.bitcast(x, U32)


def _ln(x):
    m = jnp.mean(x, axis=-1, keepdims=True)
    xc = x - m
    v = jnp.mean(xc * xc, axis=-1, keepdims=True)
    return xc * lax.rsqrt(v + EPS)


def _gelu(x):
    c = 0.7978845608028654
    return 0.5 * x * (1.0 + jnp.tanh(c * (x + 0.044715 * (x * x * x))))


def _interleave(a, b):
    n = a.shape[0] // 8
    parts = []
    for g in range(n):
        parts.append(a[8 * g:8 * g + 8])
        parts.append(b[8 * g:8 * g + 8])
    return jnp.concatenate(parts, axis=0)


def _deinterleave(v):
    n = v.shape[0] // 16
    a = jnp.concatenate([v[16 * g:16 * g + 8] for g in range(n)], axis=0)
    b = jnp.concatenate([v[16 * g + 8:16 * g + 16] for g in range(n)], axis=0)
    return a, b


def _kernel(x_hbm, mem0_hbm, wq_hbm, wk_hbm, wv_hbm, wo_hbm, w1_hbm, b1_hbm, w2_hbm, b2_hbm,
            c_hbm, wmod_hbm, out_hbm,
            x_v, h_v, hn_v, h2_v, x1_v, wmod_v, mod_v, sc_v, w_v, wo_v, w1_v, w2_v, lead_v, fr_v, lo_v, pr_v, fill_v, out_v, bias_v, n_v,
            mem0_ref, b1_ref, b2_ref, c_ref,
            sems):
    w32 = [r.bitcast(U32) for r in (wq_hbm, wk_hbm, wv_hbm)]
    wo32 = wo_hbm.bitcast(U32)

    def w_copies(p):
        return [pltpu.make_async_copy(w32[j].at[:, par, p, :], w_v.at[p * 6 + j * 2 + par], sems.at[SEM_W + p])
                for j in range(3) for par in range(2)]

    def _mult(i, m):
        return i * m if isinstance(i, int) else pl.multiple_of(i * m, m)

    def wa_copies(k, pair=None):
        r = pl.ds(_mult(k, 64), 64)
        return [pltpu.make_async_copy(w32[j].at[r, par, p, :], w_v.at[p * 6 + j * 2 + par, r], sems.at[SEM_A + k])
                for p in (range(PA) if pair is None else (pair,)) for j in range(3) for par in range(2)]

    def m_copies(k):
        cols = [pl.ds(_mult(k + 8 * t, 128), 128) for t in range(2)]
        return [pltpu.make_async_copy(wmod_hbm.at[:, cs], wmod_v.at[:, cs], sems.at[SEM_M + k]) for cs in cols]

    def start(cps):
        for cp in cps:
            cp.start()

    def wait(cps):
        for cp in cps:
            cp.wait()

    cp_x0 = pltpu.make_async_copy(x_hbm.at[:, 0:8, :], x_v.at[:, 0:8, :], sems.at[SEM_MISC + 1])
    cp_x1 = pltpu.make_async_copy(x_hbm.at[1:NSEG, 8:SEG, :], x_v.at[1:NSEG, 8:SEG, :], sems.at[SEM_MISC + 6])

    def mod1_copy(t):
        cs = pl.ds(_mult(2 + t, D), D)
        return pltpu.make_async_copy(wmod_hbm.at[:, cs], wmod_v.at[:, cs], sems.at[SEM_M + t])

    def wo_copy(j):
        return pltpu.make_async_copy(wo32.at[:, pl.ds(_mult(j, 128), 128)], wo_v.at[j], sems.at[SEM_MISC + 3])

    cp_w1 = pltpu.make_async_copy(w1_hbm, w1_v, sems.at[SEM_MISC + 4])
    cp_w2 = pltpu.make_async_copy(w2_hbm, w2_v, sems.at[SEM_MISC + 5])

    cp_small = [pltpu.make_async_copy(src, dst, sems.at[SEM_MISC])
                for src, dst in ((c_hbm, c_ref), (mem0_hbm, mem0_ref), (b1_hbm, b1_ref), (b2_hbm, b2_ref),
                                 (x_hbm.at[0, 8:SEG, :], x_v.at[0, 8:SEG, :]))]

    start(cp_small)
    cp_x0.start()
    start(m_copies(0))
    for k in range(2):
        start(m_copies(k + 1))
        start(wa_copies(k))

    scale = DH ** -0.5
    ri = lax.broadcasted_iota(jnp.int32, (80, 128), 0)
    ci = lax.broadcasted_iota(jnp.int32, (80, 128), 1)
    same_head = (((ri >> 3) & 1) == ((ci >> 3) & 1)) & (ci < 80)
    rpos = (((ri >> 4) & 3) << 3) + (ri & 7)
    cpos = (((ci >> 4) & 3) << 3) + (ci & 7)
    keep = (ri < 16) | (ci < 16) | (rpos >= cpos)
    fill_v[...] = jnp.where(same_head, jnp.where(keep, 0.0, -1e9 / scale), -jnp.inf).astype(F32)

    wait(cp_small)
    c = c_ref[...].astype(F32)
    sc = jnp.broadcast_to(c * jax.nn.sigmoid(c), (8, D)).astype(BF16)

    sc_v[...] = sc
    bias_v[:, 0:FF] = b1_ref[...].astype(F32).reshape(1, FF)
    bias_v[:, FF:FF + D] = b2_ref[...].astype(F32).reshape(1, D)

    def zero_body(i, carry):
        x1_v[pl.ds(pl.multiple_of(i * 64, 64), 64), :] = jnp.zeros((64, D), F32)
        return carry

    lax.fori_loop(0, PA * 6, zero_body, 0)

    def relayout(c, rows):
        a = w_v[c, rows, :]
        b = w_v[c + 1, rows, :]
        lo = (a & jnp.uint32(0xFFFF)) | (b << 16)
        hi = (a >> 16) | (b & jnp.uint32(0xFFFF0000))
        w_v[c, rows, :] = lo
        w_v[c + 1, rows, :] = hi
        return _bf(lo), _bf(hi)

    def store_lead(p, j, a, b):
        lead_v[p * 3 + j] = _interleave(a, b).astype(BF16)

    def mod_tile(ct):
        cs = pl.ds(_mult(ct, 128), 128)
        m = _dot(sc_v[...], wmod_v[:, cs])
        mod_v[:, cs] = m
        return m[0:1]

    with _scope("wait_x0"):
        cp_x0.wait()

    def ln1_body(i, carry):
        r = pl.multiple_of(i * 128, 128)
        n = _ln(x_v[pl.ds(i * 16, 16), 0:8, :].astype(F32).reshape(128, D))
        for k in range(8):
            n_v[k, pl.ds(r, 128), :] = n[:, k * 128:(k + 1) * 128]
        return carry

    with _scope("ln1"):
        lax.fori_loop(0, T0 // 128, ln1_body, 0)
    start(m_copies(3))
    start(wa_copies(2))
    with _scope("wait_m0"):
        wait(m_copies(0))
    h_v[0] = (n_v[0] * (1.0 + mod_tile(8)) + mod_tile(0)).astype(BF16)

    def sa_body(k, carry):
        with _scope("wait_a"):
            wait(wa_copies(k))

            @pl.when(k < 7)
            def _():
                wait(m_copies(k + 1))

        kn = jnp.minimum(k + 1, 7)
        rows = pl.ds(pl.multiple_of(k * 64, 64), 64)
        hk = h_v[k]
        for p in range(PA):
            for j in range(3):
                c = p * 6 + j * 2
                res = []
                for t, w in enumerate(relayout(c, rows)):
                    acc = x1_v.at[(c + t) // 8 * T0:((c + t) // 8 + 1) * T0,
                                  (c + t) % 8 * 128:((c + t) % 8 + 1) * 128]
                    r = _dot(hk, w) + acc[...]
                    acc[...] = r
                    res.append(r)
                store_lead(p, j, *res)
                if c == 2:
                    sh = mod_tile(kn)
                if c == 6:
                    s1 = 1.0 + mod_tile(kn + 8)

                    @pl.when(k + 4 < 8)
                    def _():
                        start(m_copies(k + 4))

            @pl.when(k + 3 < 8)
            def _():
                start(wa_copies(k + 3, p))

        h_v[kn] = (n_v[kn] * s1 + sh).astype(BF16)


        @pl.when(k >= 4)
        def _():
            start(w_copies(PA + k - 4))

        return carry

    with _scope("stageA"):
        lax.fori_loop(0, 8, sa_body, 0)

    def ln1(seg):
        xb = x_v[seg, 8:SEG, :].astype(F32)
        return _ln(xb) * (1.0 + mod_v[0:1, D:2 * D]) + mod_v[0:1, 0:D]

    def p1_body(i, carry):
        p0 = PA + P1U * i
        with _scope("wait_w"):
            for u in range(P1U):
                wait(w_copies(p0 + u))

        hb = jnp.concatenate([h_v[k] for k in range(8)], axis=1)
        for u in range(P1U):
            p = p0 + u
            for j in range(3):
                lo, hi = relayout(p * 6 + j * 2, slice(None))
                store_lead(p, j, _dot(hb, lo), _dot(hb, hi))
        hn_v[...] = ln1(0)

        @pl.when(p0 + 4 < NP)
        def _():
            for u in range(P1U):
                start(w_copies(p0 + 4 + u))
                wo_copy(P1U * i + u).start()

        @pl.when(p0 + 4 == NP)
        def _():
            cp_x1.start()
            mod1_copy(0).start()

        return carry

    with _scope("phase1"):
        lax.fori_loop(0, (NP - PA) // P1U, p1_body, 0)

    with _scope("wait_wo"):
        for j in range(8):
            wo_copy(j).wait()
        cp_x1.wait()
        mod1_copy(0).wait()

    def step(s, odd, mem):
        lhs = jnp.concatenate([mem, hn_v[...]], axis=0).astype(BF16)
        hn_v[...] = ln1(jnp.minimum(s + 1, NSEG - 1))
        ld_rd = pl.multiple_of(16 * s, 16)
        mo = 48 if odd else 32

        def proj(p):
            if p == 0:
                half = [_dot(lhs[:, 0:D // 2], _bf(w_v[c, 0:D // 4, :])) for c in range(6)]
                cols = [_dot(lhs[:, D // 2:D], _bf(w_v[c, D // 4:D // 2, :])) + half[c] for c in range(6)]
            for j in range(3):
                if p == 0:
                    r = _interleave(cols[j * 2], cols[j * 2 + 1])
                else:
                    r = _interleave(_dot(lhs, _bf(w_v[p * 6 + j * 2])), _dot(lhs, _bf(w_v[p * 6 + j * 2 + 1])))
                fr_v[p * 3 + j] = r.astype(BF16)

        def stack(p, j):
            return jnp.concatenate([fr_v[p * 3 + j], lead_v[p * 3 + j, pl.ds(ld_rd, 16), :]], axis=0)

        def attn(pvs, qks):
            os_ = [_dot(pr_v[p, :, 0:80], stack(p, 2)) for p in pvs]
            ss = [lax.dot_general(stack(p, 0), stack(p, 1), (((1,), (1,)), ((), ())),
                                  preferred_element_type=F32) for p in qks]
            for p, o in zip(pvs, os_):
                for t, oh in enumerate(_deinterleave(o)):
                    h = 2 * p + t
                    if odd:
                        lo_v[1, h, 0:8, :] = oh[0:8].astype(BF16)
                        lo_v[1, h, 16:48, :] = oh[8:40].astype(BF16)
                    else:
                        lo_v[0, h, 0:32, :] = oh[0:32].astype(BF16)
                        lo_v[1, h, 8:16, :] = oh[32:40].astype(BF16)
            for p, sc_ in zip(qks, ss):
                fill = fill_v[...]
                sc_ = jnp.concatenate([sc_, jnp.zeros((80, 48), F32)], axis=1)
                sc_ = jnp.where(fill == 0.0, sc_, fill)
                mx = jnp.max(sc_, axis=-1, keepdims=True)
                e = jnp.exp2((sc_ - mx) * (scale * LOG2E))
                l = jnp.sum(e, axis=-1, keepdims=True)
                r = pl.reciprocal(l, approx=True)
                pr_v[p] = (e * (r * (2.0 - l * r))).astype(BF16)

        part = {}

        def wo(j, h0, h1):
            lo = jnp.concatenate([lo_v[int(odd), h, 0:mo, :] for h in range(h0, h1)], axis=1)
            r = _dot(lo, _bf(wo_v[j, h0 * 64:h1 * 64, :]))
            part[j] = r + part[j] if j in part else r

        for op in SCHED:
            if op[0] == "proj":
                proj(op[1])
            elif op[0] == "attn":
                attn(op[1], op[2])
            else:
                wo(*op[1:])
                if odd and op[1:] in MODPOS:
                    cs = pl.ds(pl.multiple_of((16 + s // 2) * 128, 128), 128)
                    k0 = MODPOS.index(op[1:]) * (D // 2)
                    m = _dot(sc_v[:, k0:k0 + D // 2], wmod_v[k0:k0 + D // 2, cs])
                    if k0 == 0:
                        mhalf = m
                    else:
                        mod_v[:, cs] = m + mhalf
        res = jnp.concatenate([part[j] for j in range(8)], axis=1)
        t0 = pl.multiple_of(SEG * s, SEG)
        if odd:
            x1_v[pl.ds(t0 - SEG, 8), :] = res[8:16]
            x1_v[pl.ds(t0, SEG), :] = jnp.concatenate([res[40:48], res[16:40]], axis=0)
        else:
            x1_v[pl.ds(t0 + 8, TPS), :] = res[8:32]
        return res[0:8]

    with _scope("main"):
        def steps(i, mem):
            @pl.when(i == 1)
            def _():
                for t in range(1, 4):
                    mod1_copy(t).start()
                cp_w1.start()
                cp_w2.start()

            with _scope("iter"):
                for u in range(UNROLL):
                    mem = step(i * UNROLL + u, u % 2 == 1, mem)

            @pl.when(jnp.logical_and(lax.rem(i, 8) == 7, i < 24))
            def _():
                mod1_copy(i // 8 + 1).wait()

            return mem

        lax.fori_loop(0, NSEG // UNROLL, steps, mem0_ref[...].astype(F32))

    cp_w1.wait()
    cp_w2.wait()

    def out_copy(i, q):
        rows = pl.ds(_mult(i, FB), FB)
        cols = pl.ds(q * OC, OC)
        return pltpu.make_async_copy(out_v.at[rows, cols], out_hbm.at[rows, cols], sems.at[SEM_OUT + i])

    def resid1(r0, n, c0=0, nc=D):
        xb = x_v[pl.ds(r0 // SEG, n // SEG), :, c0:c0 + nc].astype(F32).reshape(n, nc)
        return (xb
                + mod_v[0:1, 2 * D + c0:2 * D + c0 + nc] * x1_v[pl.ds(r0, n), c0:c0 + nc])

    def ln2(slot, r0, k0, n):
        h2 = _ln(resid1(r0 + k0, n)) * (1.0 + mod_v[0:1, 4 * D:5 * D]) + mod_v[0:1, 3 * D:4 * D]
        h2_v[slot, k0 // 2:(k0 + n) // 2, :] = _u32(h2.astype(BF16))

    ln2(0, 0, 0, FB)

    def ffn_body(i, carry):
        r0 = pl.multiple_of(i * FB, FB)
        rn = pl.multiple_of(jnp.minimum(r0 + FB, S - FB), FB)
        slot = lax.rem(i, 2)
        acc = None
        nf = FF // FC
        for f in range(nf):
            a = _dot(_bf(h2_v[slot]), w1_v[:, f * FC:(f + 1) * FC]) + bias_v[0:1, f * FC:(f + 1) * FC]
            if f < len(LNP) and LNP[f]:
                ln2(1 - slot, rn, sum(LNP[:f]), LNP[f])
            y = _dot(_gelu(a).astype(BF16), w2_v[f * FC:(f + 1) * FC, :])
            acc = y if acc is None else y + acc
        y = (acc + bias_v[0:1, FF:FF + D]) * mod_v[0:1, 5 * D:6 * D]
        for q in range(D // OC):
            c0 = q * OC
            out_v[pl.ds(r0, FB), c0:c0 + OC] = (resid1(r0, FB, c0, OC) + y[:, c0:c0 + OC]).astype(BF16)
            out_copy(i, q).start()
        return carry

    with _scope("ffn"):
        lax.fori_loop(0, S // FB, ffn_body, 0)
    with _scope("wait_out"):
        for i in range(S // FB):
            for q in range(D // OC):
                out_copy(i, q).wait()


@jax.jit
def pallas_adaLN_cond__memory_aug_recurrent_mem_tr__dense_activation_gelu__prompt_kernel(
    A_x, A_mem0, A_Wq, A_Wk, A_Wv, A_Wo, A_seg_len, B_x, B_w1, B_b1, B_w2, B_b2, c, w_mod,
):
    del A_seg_len, B_x
    assert A_x.shape == (1, S, D)
    hbm = pl.BlockSpec(memory_space=pl.ANY)
    out = pl.pallas_call(
        _kernel,
        out_shape=jax.ShapeDtypeStruct((S, D), BF16),
        in_specs=[hbm] * 12,
        out_specs=hbm,
        scratch_shapes=[
            pltpu.VMEM((NSEG, SEG, D), BF16),
            pltpu.VMEM((8, T0, 128), BF16),
            pltpu.VMEM((TPS, D), F32),
            pltpu.VMEM((2, FB // 2, D), U32),
            pltpu.VMEM((S, D), F32),
            pltpu.VMEM((D, 6 * D), BF16),
            pltpu.VMEM((8, 6 * D), F32),
            pltpu.VMEM((8, D), BF16),
            pltpu.VMEM((6 * NP, D // 2, 128), U32),
            pltpu.VMEM((8, H * DH // 2, 128), U32),
            pltpu.VMEM((D, FF), BF16),
            pltpu.VMEM((FF, D), BF16),
            pltpu.VMEM((3 * NP, 2 * T0, 128), BF16),
            pltpu.VMEM((3 * NP, 64, 128), BF16),
            pltpu.VMEM((2, H, 48, 128), BF16),
            pltpu.VMEM((NP, 80, 128), BF16),
            pltpu.VMEM((80, 128), F32),
            pltpu.VMEM((S, D), BF16),
            pltpu.VMEM((1, FF + D), F32),
            pltpu.VMEM((8, T0, 128), F32),
            pltpu.VMEM((M, D), BF16),
            pltpu.VMEM((FF,), BF16),
            pltpu.VMEM((D,), BF16),
            pltpu.VMEM((1, D), BF16),
            pltpu.SemaphoreType.DMA((SEM_N,)),
        ],
        compiler_params=pltpu.CompilerParams(vmem_limit_bytes=120 * 1024 * 1024, disable_bounds_checks=True,
                                             disable_semaphore_checks=True),
    )(
        A_x.reshape(NSEG, SEG, D), A_mem0.reshape(M, D),
        A_Wq.reshape(D // 2, 2, H, DH), A_Wk.reshape(D // 2, 2, H, DH), A_Wv.reshape(D // 2, 2, H, DH),
        A_Wo.reshape(H * DH, D), B_w1, B_b1, B_w2, B_b2, c, w_mod,
    )
    return out.reshape(1, S, D)
```

```python
import contextlib

import jax
import jax.numpy as jnp
from jax import lax
import jax.experimental.pallas as pl
import jax.experimental.pallas.tpu as pltpu

F32 = jnp.float32
BF16 = jnp.bfloat16
U32 = jnp.uint32

S = 2048
D = 1024
H = 32
DH = 128
M = 8
SEG = 32
FF = 3584
NSEG = S // SEG
NP = H // 2
TPS = 24
T0 = S - NSEG * TPS
EPS = 1e-5
P1U = 2
PA = 4
LNP = (32, 32, 32, 32)
MODPOS = ((5, 0, 24), (6, 0, 24))
LOG2E = 1.4426950408889634
UNROLL = 2
FB = 256
OC = 128
FC = 256
FH = FF // 2
DH2 = D // 2
TSUM = (0, 2, 3, 5, 6)
SEM_W, SEM_A, SEM_M, SEM_MISC, SEM_OUT = 0, 16, 24, 32, 40
SEM_N = SEM_OUT + S // FB


def _make_sched(g):
    out = []

    def rng(a, b):
        return tuple(range(max(a, 0), max(b, 0)))

    for p in range(NP):
        out.append(("proj", p))
        if p % g == 0 and p >= g:
            out.append(("attn", rng(p - 2 * g, p - g), rng(p - g, p)))
    h1 = 2 * (NP - 2 * g)
    h2 = 2 * (NP - g)
    if g == 4:
        out += [("wo", j, 0, h1) for j in (0, 1)]
        out.append(("attn", rng(NP - 2 * g, NP - g), rng(NP - g, NP)))
        out += [("wo", j, 0, h1) for j in (2, 3, 4, 5)]
        out.append(("attn", rng(NP - g, NP), ()))
        out += [("wo", j, 0, h1) for j in (6, 7)]
        out += [("wo", j, h1, h2) for j in range(8)]
        out += [("wo", j, h2, H) for j in range(8)]
    else:
        out += [("wo", 0, 0, h1)]
        out.append(("attn", rng(NP - 2 * g, NP - g), rng(NP - g, NP)))
        out += [("wo", j, 0, h1) for j in (1, 2, 3)]
        out.append(("attn", rng(NP - g, NP), ()))
        out += [("wo", j, 0, h1) for j in (4, 5, 6, 7)]
        out += [("wo", j, h1, H) for j in range(8)]
    return out


SCHED = _make_sched(2)
_SCOPES = False


def _scope(name):
    return jax.named_scope(name) if _SCOPES else contextlib.nullcontext()


def _dot(a, b):
    return jnp.dot(a, b, preferred_element_type=F32)


def _bf(x):
    return pltpu.bitcast(x, BF16)


def _u32(x):
    return pltpu.bitcast(x, U32)


def _ln(x):
    m = jnp.mean(x, axis=-1, keepdims=True)
    xc = x - m
    v = jnp.mean(xc * xc, axis=-1, keepdims=True)
    return xc * lax.rsqrt(v + EPS)


def _gelu(x):
    c = 0.7978845608028654
    return 0.5 * x * (1.0 + jnp.tanh(c * (x + 0.044715 * (x * x * x))))


def _strassen_lhs(a11, a12, a21, a22):
    return [a11 + a22, a21 + a22, a11, a22, a11 + a12, a21 - a11, a12 - a22]


def _strassen_rhs(b11, b12, b21, b22):
    return [b11 + b22, b11, b12 - b22, b21 - b11, b22, b11 + b12, b21 + b22]


def _strassen_out(m):
    return (m[0] + m[3] - m[4] + m[6], m[2] + m[4], m[1] + m[3], m[0] - m[1] + m[2] + m[5])


def _interleave(a, b):
    n = a.shape[0] // 8
    parts = []
    for g in range(n):
        parts.append(a[8 * g:8 * g + 8])
        parts.append(b[8 * g:8 * g + 8])
    return jnp.concatenate(parts, axis=0)


def _deinterleave(v):
    n = v.shape[0] // 16
    a = jnp.concatenate([v[16 * g:16 * g + 8] for g in range(n)], axis=0)
    b = jnp.concatenate([v[16 * g + 8:16 * g + 16] for g in range(n)], axis=0)
    return a, b


def _kernel(x_hbm, mem0_hbm, wq_hbm, wk_hbm, wv_hbm, wo_hbm, w1_hbm, b1_hbm, w2_hbm, b2_hbm,
            c_hbm, wmod_hbm, out_hbm,
            x_v, h_v, hn_v, h2_v, x1_v, wmod_v, mod_v, sc_v, w_v, wo_v, w1_v, w2_v, lead_v, fr_v, lo_v, pr_v, fill_v, out_v, bias_v, n_v,
            mem0_ref, b1_ref, b2_ref, c_ref, t1_v, t2_v,
            sems):
    w32 = [r.bitcast(U32) for r in (wq_hbm, wk_hbm, wv_hbm)]
    wo32 = wo_hbm.bitcast(U32)

    def w_copies(p):
        return [pltpu.make_async_copy(w32[j].at[:, par, p, :], w_v.at[p * 6 + j * 2 + par], sems.at[SEM_W + p])
                for j in range(3) for par in range(2)]

    def _mult(i, m):
        return i * m if isinstance(i, int) else pl.multiple_of(i * m, m)

    def wa_copies(k, pair=None):
        r = pl.ds(_mult(k, 64), 64)
        return [pltpu.make_async_copy(w32[j].at[r, par, p, :], w_v.at[p * 6 + j * 2 + par, r], sems.at[SEM_A + k])
                for p in (range(PA) if pair is None else (pair,)) for j in range(3) for par in range(2)]

    def m_copies(k):
        cols = [pl.ds(_mult(k + 8 * t, 128), 128) for t in range(2)]
        return [pltpu.make_async_copy(wmod_hbm.at[:, cs], wmod_v.at[:, cs], sems.at[SEM_M + k]) for cs in cols]

    def start(cps):
        for cp in cps:
            cp.start()

    def wait(cps):
        for cp in cps:
            cp.wait()

    cp_x0 = pltpu.make_async_copy(x_hbm.at[:, 0:8, :], x_v.at[:, 0:8, :], sems.at[SEM_MISC + 1])
    cp_x1 = pltpu.make_async_copy(x_hbm.at[1:NSEG, 8:SEG, :], x_v.at[1:NSEG, 8:SEG, :], sems.at[SEM_MISC + 6])

    def mod1_copy(t):
        cs = pl.ds(_mult(2 + t, D), D)
        return pltpu.make_async_copy(wmod_hbm.at[:, cs], wmod_v.at[:, cs], sems.at[SEM_M + t])

    def wo_copy(j):
        return pltpu.make_async_copy(wo32.at[:, pl.ds(_mult(j, 128), 128)], wo_v.at[j], sems.at[SEM_MISC + 3])

    cp_w1 = pltpu.make_async_copy(w1_hbm, w1_v, sems.at[SEM_MISC + 4])
    cp_w2 = pltpu.make_async_copy(w2_hbm, w2_v, sems.at[SEM_MISC + 5])

    cp_small = [pltpu.make_async_copy(src, dst, sems.at[SEM_MISC])
                for src, dst in ((c_hbm, c_ref), (mem0_hbm, mem0_ref), (b1_hbm, b1_ref), (b2_hbm, b2_ref),
                                 (x_hbm.at[0, 8:SEG, :], x_v.at[0, 8:SEG, :]))]

    start(cp_small)
    cp_x0.start()
    start(m_copies(0))
    for k in range(2):
        start(m_copies(k + 1))
        start(wa_copies(k))

    scale = DH ** -0.5
    ri = lax.broadcasted_iota(jnp.int32, (80, 128), 0)
    ci = lax.broadcasted_iota(jnp.int32, (80, 128), 1)
    same_head = (((ri >> 3) & 1) == ((ci >> 3) & 1)) & (ci < 80)
    rpos = (((ri >> 4) & 3) << 3) + (ri & 7)
    cpos = (((ci >> 4) & 3) << 3) + (ci & 7)
    keep = (ri < 16) | (ci < 16) | (rpos >= cpos)
    fill_v[...] = jnp.where(same_head, jnp.where(keep, 0.0, -1e9 / scale), -jnp.inf).astype(F32)

    wait(cp_small)
    c = c_ref[...].astype(F32)
    sc = jnp.broadcast_to(c * jax.nn.sigmoid(c), (8, D)).astype(BF16)

    sc_v[...] = sc
    bias_v[:, 0:FF] = b1_ref[...].astype(F32).reshape(1, FF)
    bias_v[:, FF:FF + D] = b2_ref[...].astype(F32).reshape(1, D)

    def zero_body(i, carry):
        x1_v[pl.ds(pl.multiple_of(i * 64, 64), 64), :] = jnp.zeros((64, D), F32)
        return carry

    lax.fori_loop(0, PA * 6, zero_body, 0)

    def relayout(c, rows):
        a = w_v[c, rows, :]
        b = w_v[c + 1, rows, :]
        lo = (a & jnp.uint32(0xFFFF)) | (b << 16)
        hi = (a >> 16) | (b & jnp.uint32(0xFFFF0000))
        w_v[c, rows, :] = lo
        w_v[c + 1, rows, :] = hi
        return _bf(lo), _bf(hi)

    def store_lead(p, j, a, b):
        lead_v[p * 3 + j] = _interleave(a, b).astype(BF16)

    def mod_tile(ct):
        cs = pl.ds(_mult(ct, 128), 128)
        m = _dot(sc_v[...], wmod_v[:, cs])
        mod_v[:, cs] = m
        return m[0:1]

    with _scope("wait_x0"):
        cp_x0.wait()

    def ln1_body(i, carry):
        r = pl.multiple_of(i * 128, 128)
        n = _ln(x_v[pl.ds(i * 16, 16), 0:8, :].astype(F32).reshape(128, D))
        for k in range(8):
            n_v[k, pl.ds(r, 128), :] = n[:, k * 128:(k + 1) * 128]
        return carry

    with _scope("ln1"):
        lax.fori_loop(0, T0 // 128, ln1_body, 0)
    start(m_copies(3))
    start(wa_copies(2))
    with _scope("wait_m0"):
        wait(m_copies(0))
    h_v[0] = (n_v[0] * (1.0 + mod_tile(8)) + mod_tile(0)).astype(BF16)

    def sa_body(k, carry):
        with _scope("wait_a"):
            wait(wa_copies(k))

            @pl.when(k < 7)
            def _():
                wait(m_copies(k + 1))

        kn = jnp.minimum(k + 1, 7)
        rows = pl.ds(pl.multiple_of(k * 64, 64), 64)
        hk = h_v[k]
        for p in range(PA):
            for j in range(3):
                c = p * 6 + j * 2
                res = []
                for t, w in enumerate(relayout(c, rows)):
                    acc = x1_v.at[(c + t) // 8 * T0:((c + t) // 8 + 1) * T0,
                                  (c + t) % 8 * 128:((c + t) % 8 + 1) * 128]
                    r = _dot(hk, w) + acc[...]
                    acc[...] = r
                    res.append(r)
                store_lead(p, j, *res)
                if c == 2:
                    sh = mod_tile(kn)
                if c == 6:
                    s1 = 1.0 + mod_tile(kn + 8)

                    @pl.when(k + 4 < 8)
                    def _():
                        start(m_copies(k + 4))

            @pl.when(k + 3 < 8)
            def _():
                start(wa_copies(k + 3, p))

        h_v[kn] = (n_v[kn] * s1 + sh).astype(BF16)


        @pl.when(k >= 4)
        def _():
            start(w_copies(PA + k - 4))

        return carry

    with _scope("stageA"):
        lax.fori_loop(0, 8, sa_body, 0)

    def ln1(seg):
        xb = x_v[seg, 8:SEG, :].astype(F32)
        return _ln(xb) * (1.0 + mod_v[0:1, D:2 * D]) + mod_v[0:1, 0:D]

    def p1_body(i, carry):
        p0 = PA + P1U * i
        with _scope("wait_w"):
            for u in range(P1U):
                wait(w_copies(p0 + u))

        hb = jnp.concatenate([h_v[k] for k in range(8)], axis=1)
        for u in range(P1U):
            p = p0 + u
            for j in range(3):
                lo, hi = relayout(p * 6 + j * 2, slice(None))
                store_lead(p, j, _dot(hb, lo), _dot(hb, hi))
        hn_v[...] = ln1(0)

        @pl.when(p0 + 4 < NP)
        def _():
            for u in range(P1U):
                start(w_copies(p0 + 4 + u))
                wo_copy(P1U * i + u).start()

        @pl.when(p0 + 4 == NP)
        def _():
            cp_x1.start()
            mod1_copy(0).start()

        return carry

    with _scope("phase1"):
        lax.fori_loop(0, (NP - PA) // P1U, p1_body, 0)

    with _scope("wait_wo"):
        for j in range(8):
            wo_copy(j).wait()
        cp_x1.wait()
        mod1_copy(0).wait()

    def step(s, odd, mem):
        lhs = jnp.concatenate([mem, hn_v[...]], axis=0).astype(BF16)
        hn_v[...] = ln1(jnp.minimum(s + 1, NSEG - 1))
        ld_rd = pl.multiple_of(16 * s, 16)
        mo = 48 if odd else 32

        def proj(p):
            if p == 0:
                half = [_dot(lhs[:, 0:D // 2], _bf(w_v[c, 0:D // 4, :])) for c in range(6)]
                cols = [_dot(lhs[:, D // 2:D], _bf(w_v[c, D // 4:D // 2, :])) + half[c] for c in range(6)]
            for j in range(3):
                if p == 0:
                    r = _interleave(cols[j * 2], cols[j * 2 + 1])
                else:
                    r = _interleave(_dot(lhs, _bf(w_v[p * 6 + j * 2])), _dot(lhs, _bf(w_v[p * 6 + j * 2 + 1])))
                fr_v[p * 3 + j] = r.astype(BF16)

        def stack(p, j):
            return jnp.concatenate([fr_v[p * 3 + j], lead_v[p * 3 + j, pl.ds(ld_rd, 16), :]], axis=0)

        def attn(pvs, qks):
            os_ = [_dot(pr_v[p, :, 0:80], stack(p, 2)) for p in pvs]
            ss = [lax.dot_general(stack(p, 0), stack(p, 1), (((1,), (1,)), ((), ())),
                                  preferred_element_type=F32) for p in qks]
            for p, o in zip(pvs, os_):
                for t, oh in enumerate(_deinterleave(o)):
                    h = 2 * p + t
                    if odd:
                        lo_v[1, h, 0:8, :] = oh[0:8].astype(BF16)
                        lo_v[1, h, 16:48, :] = oh[8:40].astype(BF16)
                    else:
                        lo_v[0, h, 0:32, :] = oh[0:32].astype(BF16)
                        lo_v[1, h, 8:16, :] = oh[32:40].astype(BF16)
            for p, sc_ in zip(qks, ss):
                fill = fill_v[...]
                sc_ = jnp.concatenate([sc_, jnp.zeros((80, 48), F32)], axis=1)
                sc_ = jnp.where(fill == 0.0, sc_, fill)
                mx = jnp.max(sc_, axis=-1, keepdims=True)
                e = jnp.exp2((sc_ - mx) * (scale * LOG2E))
                l = jnp.sum(e, axis=-1, keepdims=True)
                r = pl.reciprocal(l, approx=True)
                pr_v[p] = (e * (r * (2.0 - l * r))).astype(BF16)

        part = {}

        def wo(j, h0, h1):
            lo = jnp.concatenate([lo_v[int(odd), h, 0:mo, :] for h in range(h0, h1)], axis=1)
            r = _dot(lo, _bf(wo_v[j, h0 * 64:h1 * 64, :]))
            part[j] = r + part[j] if j in part else r

        for op in SCHED:
            if op[0] == "proj":
                proj(op[1])
            elif op[0] == "attn":
                attn(op[1], op[2])
            else:
                wo(*op[1:])
                if odd and op[1:] in MODPOS:
                    cs = pl.ds(pl.multiple_of((16 + s // 2) * 128, 128), 128)
                    k0 = MODPOS.index(op[1:]) * (D // 2)
                    m = _dot(sc_v[:, k0:k0 + D // 2], wmod_v[k0:k0 + D // 2, cs])
                    if k0 == 0:
                        mhalf = m
                    else:
                        mod_v[:, cs] = m + mhalf
        res = jnp.concatenate([part[j] for j in range(8)], axis=1)
        t0 = pl.multiple_of(SEG * s, SEG)
        if odd:
            x1_v[pl.ds(t0 - SEG, 8), :] = res[8:16]
            x1_v[pl.ds(t0, SEG), :] = jnp.concatenate([res[40:48], res[16:40]], axis=0)
        else:
            x1_v[pl.ds(t0 + 8, TPS), :] = res[8:32]
        return res[0:8]

    with _scope("main"):
        def steps(i, mem):
            @pl.when(i == 1)
            def _():
                for t in range(1, 4):
                    mod1_copy(t).start()
                cp_w1.start()
                cp_w2.start()

            with _scope("iter"):
                for u in range(UNROLL):
                    mem = step(i * UNROLL + u, u % 2 == 1, mem)

            @pl.when(jnp.logical_and(lax.rem(i, 8) == 7, i < 24))
            def _():
                mod1_copy(i // 8 + 1).wait()

            return mem

        lax.fori_loop(0, NSEG // UNROLL, steps, mem0_ref[...].astype(F32))

    cp_w1.wait()
    cp_w2.wait()

    def prep_w1(r0, n):
        rows, rows2 = pl.ds(r0, n), pl.ds(D // 2 + r0, n)
        t = _strassen_rhs(w1_v[rows, 0:FH].astype(F32), w1_v[rows, FH:FF].astype(F32),
                          w1_v[rows2, 0:FH].astype(F32), w1_v[rows2, FH:FF].astype(F32))
        for k, i in enumerate(TSUM):
            t1_v[k, rows, :] = t[i].astype(BF16)

    def prep_w2(r0, n):
        rows, rows2 = pl.ds(r0, n), pl.ds(FH + r0, n)
        t = _strassen_rhs(w2_v[rows, 0:DH2].astype(F32), w2_v[rows, DH2:D].astype(F32),
                          w2_v[rows2, 0:DH2].astype(F32), w2_v[rows2, DH2:D].astype(F32))
        for k, i in enumerate(TSUM):
            t2_v[k, rows, :] = t[i].astype(BF16)

    def prep_body(i, carry):
        prep_w1(pl.multiple_of(i * 16, 16), 16)
        prep_w2(pl.multiple_of(i * 56, 8), 56)
        return carry

    with _scope("prep"):
        lax.fori_loop(0, 32, prep_body, 0)

    def rhs1(i, c0, n):
        if i == 1:
            return w1_v[0:DH2, c0:c0 + n]
        if i == 4:
            return w1_v[DH2:D, FH + c0:FH + c0 + n]
        return t1_v[TSUM.index(i), :, c0:c0 + n]

    def rhs2(i, k0, nk, c0, n):
        if i == 1:
            return w2_v[k0:k0 + nk, c0:c0 + n]
        if i == 4:
            return w2_v[FH + k0:FH + k0 + nk, DH2 + c0:DH2 + c0 + n]
        return t2_v[TSUM.index(i), k0:k0 + nk, c0:c0 + n]

    def out_copy(i, q):
        rows = pl.ds(_mult(i, FB), FB)
        return [pltpu.make_async_copy(out_v.at[rows, cols], out_hbm.at[rows, cols], sems.at[SEM_OUT + i])
                for cols in (pl.ds(q * OC, OC), pl.ds(DH2 + q * OC, OC))]

    HB = FB // 2

    def resid1(r0, n, c0=0, nc=D):
        xb = x_v[pl.ds(r0 // SEG, n // SEG), :, c0:c0 + nc].astype(F32).reshape(n, nc)
        return xb + mod_v[0:1, 2 * D + c0:2 * D + c0 + nc] * x1_v[pl.ds(r0, n), c0:c0 + nc]

    def ln2(slot, r0, k0, n):
        top, bot = [_ln(resid1(r0 + t * HB + k0, n)) * (1.0 + mod_v[0:1, 4 * D:5 * D]) + mod_v[0:1, 3 * D:4 * D]
                    for t in range(2)]
        ss = _strassen_lhs(top[:, 0:DH2], top[:, DH2:D], bot[:, 0:DH2], bot[:, DH2:D])
        for i in range(7):
            h2_v[slot, i, k0 // 2:(k0 + n) // 2, :] = _u32(ss[i].astype(BF16))

    ln2(0, 0, 0, HB)

    def ffn_body(i, carry):
        r0 = pl.multiple_of(i * FB, FB)
        rn = pl.multiple_of(jnp.minimum(r0 + FB, S - FB), FB)
        slot = lax.rem(i, 2)
        nf = FH // FC
        acc = {}

        def up(f):
            gs = []
            for t in range(FC // 128):
                c0 = f * FC + t * 128
                c = _strassen_out([_dot(_bf(h2_v[slot, k]), rhs1(k, c0, 128)) for k in range(7)])
                b1a, b1b = bias_v[0:1, c0:c0 + 128], bias_v[0:1, FH + c0:FH + c0 + 128]
                gs.append(_strassen_lhs(_gelu(c[0] + b1a), _gelu(c[1] + b1b), _gelu(c[2] + b1a), _gelu(c[3] + b1b)))
            return [jnp.concatenate([g[k] for g in gs], axis=1).astype(BF16) for k in range(7)]

        def down(f, g):
            for q in range(DH2 // OC):
                for k in range(7):
                    y = _dot(g[k], rhs2(k, f * FC, FC, q * OC, OC))
                    acc[k, q] = y + acc[k, q] if f else y
                if f == nf - 1:
                    c = _strassen_out([acc[k, q] for k in range(7)])
                    for t in range(4):
                        rr, c0 = r0 + (t // 2) * HB, (t % 2) * DH2 + q * OC
                        y = (c[t] + bias_v[0:1, FF + c0:FF + c0 + OC]) * mod_v[0:1, 5 * D + c0:5 * D + c0 + OC]
                        out_v[pl.ds(rr, HB), c0:c0 + OC] = (resid1(rr, HB, c0, OC) + y).astype(BF16)
                    start(out_copy(i, q))

        g = up(0)
        for f in range(nf):
            gn = up(f + 1) if f + 1 < nf else None
            if f < len(LNP) and LNP[f]:
                ln2(1 - slot, rn, sum(LNP[:f]), LNP[f])
            down(f, g)
            g = gn
        return carry

    with _scope("ffn"):
        lax.fori_loop(0, S // FB, ffn_body, 0)
    with _scope("wait_out"):
        for i in range(S // FB):
            for q in range(DH2 // OC):
                wait(out_copy(i, q))


@jax.jit
def pallas_adaLN_cond__memory_aug_recurrent_mem_tr__dense_activation_gelu__prompt_kernel(
    A_x, A_mem0, A_Wq, A_Wk, A_Wv, A_Wo, A_seg_len, B_x, B_w1, B_b1, B_w2, B_b2, c, w_mod,
):
    del A_seg_len, B_x
    assert A_x.shape == (1, S, D)
    hbm = pl.BlockSpec(memory_space=pl.ANY)
    out = pl.pallas_call(
        _kernel,
        out_shape=jax.ShapeDtypeStruct((S, D), BF16),
        in_specs=[hbm] * 12,
        out_specs=hbm,
        scratch_shapes=[
            pltpu.VMEM((NSEG, SEG, D), BF16),
            pltpu.VMEM((8, T0, 128), BF16),
            pltpu.VMEM((TPS, D), F32),
            pltpu.VMEM((2, 7, FB // 4, D // 2), U32),
            pltpu.VMEM((S, D), F32),
            pltpu.VMEM((D, 6 * D), BF16),
            pltpu.VMEM((8, 6 * D), F32),
            pltpu.VMEM((8, D), BF16),
            pltpu.VMEM((6 * NP, D // 2, 128), U32),
            pltpu.VMEM((8, H * DH // 2, 128), U32),
            pltpu.VMEM((D, FF), BF16),
            pltpu.VMEM((FF, D), BF16),
            pltpu.VMEM((3 * NP, 2 * T0, 128), BF16),
            pltpu.VMEM((3 * NP, 64, 128), BF16),
            pltpu.VMEM((2, H, 48, 128), BF16),
            pltpu.VMEM((NP, 80, 128), BF16),
            pltpu.VMEM((80, 128), F32),
            pltpu.VMEM((S, D), BF16),
            pltpu.VMEM((1, FF + D), F32),
            pltpu.VMEM((8, T0, 128), F32),
            pltpu.VMEM((M, D), BF16),
            pltpu.VMEM((FF,), BF16),
            pltpu.VMEM((D,), BF16),
            pltpu.VMEM((1, D), BF16),
            pltpu.VMEM((5, D // 2, FF // 2), BF16),
            pltpu.VMEM((5, FF // 2, D // 2), BF16),
            pltpu.SemaphoreType.DMA((SEM_N,)),
        ],
        compiler_params=pltpu.CompilerParams(vmem_limit_bytes=120 * 1024 * 1024, disable_bounds_checks=True,
                                             disable_semaphore_checks=True),
    )(
        A_x.reshape(NSEG, SEG, D), A_mem0.reshape(M, D),
        A_Wq.reshape(D // 2, 2, H, DH), A_Wk.reshape(D // 2, 2, H, DH), A_Wv.reshape(D // 2, 2, H, DH),
        A_Wo.reshape(H * DH, D), B_w1, B_b1, B_w2, B_b2, c, w_mod,
    )
    return out.reshape(1, S, D)
```

```python
import contextlib

import jax
import jax.numpy as jnp
from jax import lax
import jax.experimental.pallas as pl
import jax.experimental.pallas.tpu as pltpu

F32 = jnp.float32
BF16 = jnp.bfloat16
U32 = jnp.uint32

S = 2048
D = 1024
H = 32
DH = 128
M = 8
SEG = 32
FF = 3584
NSEG = S // SEG
NP = H // 2
TPS = 24
T0 = S - NSEG * TPS
EPS = 1e-5
P1U = 2
PA = 4
LNP = (16,) * 8
MODPOS = ((5, 0, 24), (6, 0, 24))
LOG2E = 1.4426950408889634
UNROLL = 2
FB = 256
OC = 128
FC = 256
FH = FF // 2
DH2 = D // 2
TSUM = (0, 2, 3, 5, 6)
SEM_W, SEM_A, SEM_M, SEM_MISC, SEM_OUT = 0, 16, 24, 32, 40
SEM_N = SEM_OUT + S // FB


def _make_sched(g):
    out = []

    def rng(a, b):
        return tuple(range(max(a, 0), max(b, 0)))

    for p in range(NP):
        out.append(("proj", p))
        if p % g == 0 and p >= g:
            out.append(("attn", rng(p - 2 * g, p - g), rng(p - g, p)))
    h1 = 2 * (NP - 2 * g)
    h2 = 2 * (NP - g)
    if g == 4:
        out += [("wo", j, 0, h1) for j in (0, 1)]
        out.append(("attn", rng(NP - 2 * g, NP - g), rng(NP - g, NP)))
        out += [("wo", j, 0, h1) for j in (2, 3, 4, 5)]
        out.append(("attn", rng(NP - g, NP), ()))
        out += [("wo", j, 0, h1) for j in (6, 7)]
        out += [("wo", j, h1, h2) for j in range(8)]
        out += [("wo", j, h2, H) for j in range(8)]
    else:
        out += [("wo", 0, 0, h1)]
        out.append(("attn", rng(NP - 2 * g, NP - g), rng(NP - g, NP)))
        out += [("wo", j, 0, h1) for j in (1, 2, 3)]
        out.append(("attn", rng(NP - g, NP), ()))
        out += [("wo", j, 0, h1) for j in (4, 5, 6, 7)]
        out += [("wo", j, h1, H) for j in range(8)]
    return out


SCHED = _make_sched(2)
_SCOPES = False


def _scope(name):
    return jax.named_scope(name) if _SCOPES else contextlib.nullcontext()


def _dot(a, b):
    return jnp.dot(a, b, preferred_element_type=F32)


def _bf(x):
    return pltpu.bitcast(x, BF16)


def _u32(x):
    return pltpu.bitcast(x, U32)


def _ld(ref, idx, r0, n):
    r = r0 // 2 if isinstance(r0, int) else pl.multiple_of(r0 // 2, 8)
    return _bf(ref.bitcast(U32)[(*idx, pl.ds(r, n // 2), slice(None))])


def _ln(x):
    m = jnp.mean(x, axis=-1, keepdims=True)
    xc = x - m
    v = jnp.mean(xc * xc, axis=-1, keepdims=True)
    return xc * lax.rsqrt(v + EPS)


def _gelu(x):
    c = 0.7978845608028654
    return 0.5 * x * (1.0 + jnp.tanh(c * (x + 0.044715 * (x * x * x))))


def _strassen_lhs(a11, a12, a21, a22):
    return [a11 + a22, a21 + a22, a11, a22, a11 + a12, a21 - a11, a12 - a22]


def _strassen_rhs(b11, b12, b21, b22):
    return [b11 + b22, b11, b12 - b22, b21 - b11, b22, b11 + b12, b21 + b22]


def _strassen_out(m):
    return (m[0] + m[3] - m[4] + m[6], m[2] + m[4], m[1] + m[3], m[0] - m[1] + m[2] + m[5])


def _interleave(a, b):
    n = a.shape[0] // 8
    parts = []
    for g in range(n):
        parts.append(a[8 * g:8 * g + 8])
        parts.append(b[8 * g:8 * g + 8])
    return jnp.concatenate(parts, axis=0)


def _deinterleave(v):
    n = v.shape[0] // 16
    a = jnp.concatenate([v[16 * g:16 * g + 8] for g in range(n)], axis=0)
    b = jnp.concatenate([v[16 * g + 8:16 * g + 16] for g in range(n)], axis=0)
    return a, b


def _kernel(x_hbm, mem0_hbm, wq_hbm, wk_hbm, wv_hbm, wo_hbm, w1_hbm, b1_hbm, w2_hbm, b2_hbm,
            c_hbm, wmod_hbm, out_hbm,
            x_v, h_v, hn_v, h2_v, x1_v, wmod_v, mod_v, sc_v, w_v, wo_v, w1_v, w2_v, lead_v, fr_v, lo_v, pr_v, fill_v, out_v, bias_v, n_v,
            mem0_ref, b1_ref, b2_ref, c_ref, t1_v, t2_v,
            sems):
    w32 = [r.bitcast(U32) for r in (wq_hbm, wk_hbm, wv_hbm)]
    wo32 = wo_hbm.bitcast(U32)

    def w_copies(p):
        return [pltpu.make_async_copy(w32[j].at[:, par, p, :], w_v.at[p * 6 + j * 2 + par], sems.at[SEM_W + p])
                for j in range(3) for par in range(2)]

    def _mult(i, m):
        return i * m if isinstance(i, int) else pl.multiple_of(i * m, m)

    def wa_copies(k, pair=None):
        r = pl.ds(_mult(k, 64), 64)
        return [pltpu.make_async_copy(w32[j].at[r, par, p, :], w_v.at[p * 6 + j * 2 + par, r], sems.at[SEM_A + k])
                for p in (range(PA) if pair is None else (pair,)) for j in range(3) for par in range(2)]

    def m_copies(k):
        cols = [pl.ds(_mult(k + 8 * t, 128), 128) for t in range(2)]
        return [pltpu.make_async_copy(wmod_hbm.at[:, cs], wmod_v.at[:, cs], sems.at[SEM_M + k]) for cs in cols]

    def start(cps):
        for cp in cps:
            cp.start()

    def wait(cps):
        for cp in cps:
            cp.wait()

    cp_x0 = pltpu.make_async_copy(x_hbm.at[:, 0:8, :], x_v.at[:, 0:8, :], sems.at[SEM_MISC + 1])
    cp_x1 = pltpu.make_async_copy(x_hbm.at[1:NSEG, 8:SEG, :], x_v.at[1:NSEG, 8:SEG, :], sems.at[SEM_MISC + 6])

    def mod1_copy(t):
        cs = pl.ds(_mult(2 + t, D), D)
        return pltpu.make_async_copy(wmod_hbm.at[:, cs], wmod_v.at[:, cs], sems.at[SEM_M + t])

    def wo_copy(j):
        return pltpu.make_async_copy(wo32.at[:, pl.ds(_mult(j, 128), 128)], wo_v.at[j], sems.at[SEM_MISC + 3])

    cp_w1 = [pltpu.make_async_copy(w1_hbm.at[:, j * 128:(j + 1) * 128], w1_v.at[j], sems.at[SEM_MISC + 4])
             for j in range(FF // 128)]
    cp_w2 = [pltpu.make_async_copy(w2_hbm.at[:, j * 128:(j + 1) * 128], w2_v.at[j], sems.at[SEM_MISC + 5])
             for j in range(D // 128)]

    cp_small = [pltpu.make_async_copy(src, dst, sems.at[SEM_MISC])
                for src, dst in ((c_hbm, c_ref), (mem0_hbm, mem0_ref), (b1_hbm, b1_ref), (b2_hbm, b2_ref),
                                 (x_hbm.at[0, 8:SEG, :], x_v.at[0, 8:SEG, :]))]

    start(cp_small)
    cp_x0.start()
    start(m_copies(0))
    for k in range(2):
        start(m_copies(k + 1))
        start(wa_copies(k))

    scale = DH ** -0.5
    ri = lax.broadcasted_iota(jnp.int32, (80, 128), 0)
    ci = lax.broadcasted_iota(jnp.int32, (80, 128), 1)
    same_head = (((ri >> 3) & 1) == ((ci >> 3) & 1)) & (ci < 80)
    rpos = (((ri >> 4) & 3) << 3) + (ri & 7)
    cpos = (((ci >> 4) & 3) << 3) + (ci & 7)
    keep = (ri < 16) | (ci < 16) | (rpos >= cpos)
    fill_v[...] = jnp.where(same_head, jnp.where(keep, 0.0, -1e9 / scale), -jnp.inf).astype(F32)

    wait(cp_small)
    c = c_ref[...].astype(F32)
    sc = jnp.broadcast_to(c * jax.nn.sigmoid(c), (8, D)).astype(BF16)

    sc_v[...] = sc
    bias_v[:, 0:FF] = b1_ref[...].astype(F32).reshape(1, FF)
    bias_v[:, FF:FF + D] = b2_ref[...].astype(F32).reshape(1, D)

    def zero_body(i, carry):
        x1_v[pl.ds(pl.multiple_of(i * 64, 64), 64), :] = jnp.zeros((64, D), F32)
        return carry

    lax.fori_loop(0, PA * 6, zero_body, 0)

    def relayout(c, rows):
        a = w_v[c, rows, :]
        b = w_v[c + 1, rows, :]
        lo = (a & jnp.uint32(0xFFFF)) | (b << 16)
        hi = (a >> 16) | (b & jnp.uint32(0xFFFF0000))
        w_v[c, rows, :] = lo
        w_v[c + 1, rows, :] = hi
        return _bf(lo), _bf(hi)

    def store_lead(p, j, a, b):
        lead_v[p * 3 + j] = _interleave(a, b).astype(BF16)

    def mod_tile(ct):
        cs = pl.ds(_mult(ct, 128), 128)
        m = _dot(sc_v[...], wmod_v[:, cs])
        mod_v[:, cs] = m
        return m[0:1]

    with _scope("wait_x0"):
        cp_x0.wait()

    def ln1_body(i, carry):
        r = pl.multiple_of(i * 128, 128)
        n = _ln(x_v[pl.ds(i * 16, 16), 0:8, :].astype(F32).reshape(128, D))
        for k in range(8):
            n_v[k, pl.ds(r, 128), :] = n[:, k * 128:(k + 1) * 128]
        return carry

    with _scope("ln1"):
        lax.fori_loop(0, T0 // 128, ln1_body, 0)
    start(m_copies(3))
    start(wa_copies(2))
    with _scope("wait_m0"):
        wait(m_copies(0))
    h_v[0] = (n_v[0] * (1.0 + mod_tile(8)) + mod_tile(0)).astype(BF16)

    def sa_body(k, carry):
        with _scope("wait_a"):
            wait(wa_copies(k))

            @pl.when(k < 7)
            def _():
                wait(m_copies(k + 1))

        kn = jnp.minimum(k + 1, 7)
        rows = pl.ds(pl.multiple_of(k * 64, 64), 64)
        hk = h_v[k]
        for p in range(PA):
            for j in range(3):
                c = p * 6 + j * 2
                res = []
                for t, w in enumerate(relayout(c, rows)):
                    acc = x1_v.at[(c + t) // 8 * T0:((c + t) // 8 + 1) * T0,
                                  (c + t) % 8 * 128:((c + t) % 8 + 1) * 128]
                    r = _dot(hk, w) + acc[...]
                    acc[...] = r
                    res.append(r)
                store_lead(p, j, *res)
                if c == 2:
                    sh = mod_tile(kn)
                if c == 6:
                    s1 = 1.0 + mod_tile(kn + 8)

                    @pl.when(k + 4 < 8)
                    def _():
                        start(m_copies(k + 4))

            @pl.when(k + 3 < 8)
            def _():
                start(wa_copies(k + 3, p))

        h_v[kn] = (n_v[kn] * s1 + sh).astype(BF16)


        @pl.when(k >= 4)
        def _():
            start(w_copies(PA + k - 4))

        return carry

    with _scope("stageA"):
        lax.fori_loop(0, 8, sa_body, 0)

    def ln1(seg):
        xb = x_v[seg, 8:SEG, :].astype(F32)
        return _ln(xb) * (1.0 + mod_v[0:1, D:2 * D]) + mod_v[0:1, 0:D]

    def p1_body(i, carry):
        p0 = PA + P1U * i
        with _scope("wait_w"):
            for u in range(P1U):
                wait(w_copies(p0 + u))

        hb = jnp.concatenate([h_v[k] for k in range(8)], axis=1)
        for u in range(P1U):
            p = p0 + u
            for j in range(3):
                lo, hi = relayout(p * 6 + j * 2, slice(None))
                store_lead(p, j, _dot(hb, lo), _dot(hb, hi))
        hn_v[...] = ln1(0)

        @pl.when(p0 + 4 < NP)
        def _():
            for u in range(P1U):
                start(w_copies(p0 + 4 + u))
                wo_copy(P1U * i + u).start()

        @pl.when(p0 + 4 == NP)
        def _():
            cp_x1.start()
            mod1_copy(0).start()

        return carry

    with _scope("phase1"):
        lax.fori_loop(0, (NP - PA) // P1U, p1_body, 0)

    with _scope("wait_wo"):
        for j in range(8):
            wo_copy(j).wait()
        cp_x1.wait()
        mod1_copy(0).wait()

    def step(s, odd, mem):
        lhs = jnp.concatenate([mem, hn_v[...]], axis=0).astype(BF16)
        hn_v[...] = ln1(jnp.minimum(s + 1, NSEG - 1))
        ld_rd = pl.multiple_of(16 * s, 16)
        mo = 48 if odd else 32

        def proj(p):
            if p == 0:
                half = [_dot(lhs[:, 0:D // 2], _bf(w_v[c, 0:D // 4, :])) for c in range(6)]
                cols = [_dot(lhs[:, D // 2:D], _bf(w_v[c, D // 4:D // 2, :])) + half[c] for c in range(6)]
            for j in range(3):
                if p == 0:
                    r = _interleave(cols[j * 2], cols[j * 2 + 1])
                else:
                    r = _interleave(_dot(lhs, _bf(w_v[p * 6 + j * 2])), _dot(lhs, _bf(w_v[p * 6 + j * 2 + 1])))
                fr_v[p * 3 + j] = r.astype(BF16)

        def stack(p, j):
            return jnp.concatenate([fr_v[p * 3 + j], lead_v[p * 3 + j, pl.ds(ld_rd, 16), :]], axis=0)

        def attn(pvs, qks):
            os_ = [_dot(pr_v[p, :, 0:80], stack(p, 2)) for p in pvs]
            ss = [lax.dot_general(stack(p, 0), stack(p, 1), (((1,), (1,)), ((), ())),
                                  preferred_element_type=F32) for p in qks]
            for p, o in zip(pvs, os_):
                for t, oh in enumerate(_deinterleave(o)):
                    h = 2 * p + t
                    if odd:
                        lo_v[1, h, 0:8, :] = oh[0:8].astype(BF16)
                        lo_v[1, h, 16:48, :] = oh[8:40].astype(BF16)
                    else:
                        lo_v[0, h, 0:32, :] = oh[0:32].astype(BF16)
                        lo_v[1, h, 8:16, :] = oh[32:40].astype(BF16)
            for p, sc_ in zip(qks, ss):
                fill = fill_v[...]
                sc_ = jnp.concatenate([sc_, jnp.zeros((80, 48), F32)], axis=1)
                sc_ = jnp.where(fill == 0.0, sc_, fill)
                mx = jnp.max(sc_, axis=-1, keepdims=True)
                e = jnp.exp2((sc_ - mx) * (scale * LOG2E))
                l = jnp.sum(e, axis=-1, keepdims=True)
                r = pl.reciprocal(l, approx=True)
                pr_v[p] = (e * (r * (2.0 - l * r))).astype(BF16)

        part = {}

        def wo(j, h0, h1):
            lo = jnp.concatenate([lo_v[int(odd), h, 0:mo, :] for h in range(h0, h1)], axis=1)
            r = _dot(lo, _bf(wo_v[j, h0 * 64:h1 * 64, :]))
            part[j] = r + part[j] if j in part else r

        for op in SCHED:
            if op[0] == "proj":
                proj(op[1])
            elif op[0] == "attn":
                attn(op[1], op[2])
            else:
                wo(*op[1:])
                if odd and op[1:] in MODPOS:
                    cs = pl.ds(pl.multiple_of((16 + s // 2) * 128, 128), 128)
                    k0 = MODPOS.index(op[1:]) * (D // 2)
                    m = _dot(sc_v[:, k0:k0 + D // 2], wmod_v[k0:k0 + D // 2, cs])
                    if k0 == 0:
                        mhalf = m
                    else:
                        mod_v[:, cs] = m + mhalf
        res = jnp.concatenate([part[j] for j in range(8)], axis=1)
        t0 = pl.multiple_of(SEG * s, SEG)
        if odd:
            x1_v[pl.ds(t0 - SEG, 8), :] = res[8:16]
            x1_v[pl.ds(t0, SEG), :] = jnp.concatenate([res[40:48], res[16:40]], axis=0)
        else:
            x1_v[pl.ds(t0 + 8, TPS), :] = res[8:32]
        return res[0:8]

    with _scope("main"):
        def steps(i, mem):
            @pl.when(i == 1)
            def _():
                for t in range(1, 4):
                    mod1_copy(t).start()
                start(cp_w1)
                start(cp_w2)

            with _scope("iter"):
                for u in range(UNROLL):
                    mem = step(i * UNROLL + u, u % 2 == 1, mem)

            @pl.when(jnp.logical_and(lax.rem(i, 8) == 7, i < 24))
            def _():
                mod1_copy(i // 8 + 1).wait()

            return mem

        lax.fori_loop(0, NSEG // UNROLL, steps, mem0_ref[...].astype(F32))

    wait(cp_w1)
    wait(cp_w2)

    def prep(w, t_v, kh, nh, j, r0, n):
        t = _strassen_rhs(*[_ld(w, (j + b * nh,), a * kh + r0, n).astype(F32) for a in range(2) for b in range(2)])
        for k, i in enumerate(TSUM):
            t_v[k, j, pl.ds(r0, n), :] = t[i].astype(BF16)

    def prep_body(i, carry):
        for j in range(FH // 128):
            prep(w1_v, t1_v, DH2, FH // 128, j, pl.multiple_of(i * 16, 16), 16)
        prep(w2_v, t2_v, FH, DH2 // 128, lax.rem(i, 4), pl.multiple_of((i // 4) * 224, 16), 224)
        return carry

    with _scope("prep"):
        lax.fori_loop(0, 32, prep_body, 0)

    def rhs(w, t_v, kh, nh, i, j, k0, nk):
        if i == 1:
            return _ld(w, (j,), k0, nk)
        if i == 4:
            return _ld(w, (j + nh,), kh + k0, nk)
        return _ld(t_v, (TSUM.index(i), j), k0, nk)

    def out_copy(i, q):
        rows = pl.ds(_mult(i, FB), FB)
        return [pltpu.make_async_copy(out_v.at[rows, cols], out_hbm.at[rows, cols], sems.at[SEM_OUT + i])
                for cols in (pl.ds(q * OC, OC), pl.ds(DH2 + q * OC, OC))]

    HB = FB // 2

    def resid1(r0, k0, n, c0=0, nc=D):
        if n >= SEG:
            xb = x_v[pl.ds((r0 + k0) // SEG, n // SEG), :, c0:c0 + nc].astype(F32).reshape(n, nc)
        else:
            xb = x_v[r0 // SEG + k0 // SEG, k0 % SEG:k0 % SEG + n, c0:c0 + nc].astype(F32)
        return xb + mod_v[0:1, 2 * D + c0:2 * D + c0 + nc] * x1_v[pl.ds(r0 + k0, n), c0:c0 + nc]

    def ln2(slot, r0, k0, n):
        top, bot = [_ln(resid1(r0, t * HB + k0, n)) * (1.0 + mod_v[0:1, 4 * D:5 * D]) + mod_v[0:1, 3 * D:4 * D]
                    for t in range(2)]
        ss = _strassen_lhs(top[:, 0:DH2], top[:, DH2:D], bot[:, 0:DH2], bot[:, DH2:D])
        for i in range(7):
            for j in range(DH2 // 128):
                h2_v[slot, i, j, k0:k0 + n, :] = ss[i][:, j * 128:(j + 1) * 128].astype(BF16)

    ln2(0, 0, 0, HB)

    def ffn_body(i, carry):
        r0 = pl.multiple_of(i * FB, FB)
        rn = pl.multiple_of(jnp.minimum(r0 + FB, S - FB), FB)
        slot = lax.rem(i, 2)
        nf = FH // FC
        nt = FC // 128
        nq = DH2 // OC
        acc = {}
        gs = {}

        def up(f, t):
            c0 = f * FC + t * 128
            c = _strassen_out([
                _dot(jnp.concatenate([_ld(h2_v, (slot, k, j), 0, HB) for j in range(DH2 // 128)], axis=1),
                     rhs(w1_v, t1_v, DH2, FH // 128, k, c0 // 128, 0, DH2)) for k in range(7)])
            b1a, b1b = bias_v[0:1, c0:c0 + 128], bias_v[0:1, FH + c0:FH + c0 + 128]
            gs[f, t] = _strassen_lhs(_gelu(c[0] + b1a), _gelu(c[1] + b1b), _gelu(c[2] + b1a), _gelu(c[3] + b1b))
            if t == nt - 1:
                gs[f] = [jnp.concatenate([gs[f, u][k] for u in range(nt)], axis=1).astype(BF16) for k in range(7)]

        def down(f, q):
            for k in range(7):
                y = _dot(gs[f][k], rhs(w2_v, t2_v, FH, DH2 // 128, k, q, f * FC, FC))
                acc[k, q] = y + acc[k, q] if f else y
            if f == nf - 1:
                c = _strassen_out([acc[k, q] for k in range(7)])
                for t in range(4):
                    k0, c0 = (t // 2) * HB, (t % 2) * DH2 + q * OC
                    y = (c[t] + bias_v[0:1, FF + c0:FF + c0 + OC]) * mod_v[0:1, 5 * D + c0:5 * D + c0 + OC]
                    out_v[pl.ds(r0 + k0, HB), c0:c0 + OC] = (resid1(r0, k0, HB, c0, OC) + y).astype(BF16)
                start(out_copy(i, q))

        for t in range(nt):
            up(0, t)
        w = 0
        for f in range(nf):
            for t in range(nt):
                if f + 1 < nf:
                    up(f + 1, t)
                if w < len(LNP) and LNP[w]:
                    ln2(1 - slot, rn, sum(LNP[:w]), LNP[w])
                w += 1
                for q in range(t * nq // nt, (t + 1) * nq // nt):
                    down(f, q)
        return carry

    with _scope("ffn"):
        lax.fori_loop(0, S // FB, ffn_body, 0)
    with _scope("wait_out"):
        for i in range(S // FB):
            for q in range(DH2 // OC):
                wait(out_copy(i, q))


@jax.jit
def pallas_adaLN_cond__memory_aug_recurrent_mem_tr__dense_activation_gelu__prompt_kernel(
    A_x, A_mem0, A_Wq, A_Wk, A_Wv, A_Wo, A_seg_len, B_x, B_w1, B_b1, B_w2, B_b2, c, w_mod,
):
    del A_seg_len, B_x
    assert A_x.shape == (1, S, D)
    hbm = pl.BlockSpec(memory_space=pl.ANY)
    out = pl.pallas_call(
        _kernel,
        out_shape=jax.ShapeDtypeStruct((S, D), BF16),
        in_specs=[hbm] * 12,
        out_specs=hbm,
        scratch_shapes=[
            pltpu.VMEM((NSEG, SEG, D), BF16),
            pltpu.VMEM((8, T0, 128), BF16),
            pltpu.VMEM((TPS, D), F32),
            pltpu.VMEM((2, 7, 4, FB // 2, 128), BF16),
            pltpu.VMEM((S, D), F32),
            pltpu.VMEM((D, 6 * D), BF16),
            pltpu.VMEM((8, 6 * D), F32),
            pltpu.VMEM((8, D), BF16),
            pltpu.VMEM((6 * NP, D // 2, 128), U32),
            pltpu.VMEM((8, H * DH // 2, 128), U32),
            pltpu.VMEM((FF // 128, D, 128), BF16),
            pltpu.VMEM((D // 128, FF, 128), BF16),
            pltpu.VMEM((3 * NP, 2 * T0, 128), BF16),
            pltpu.VMEM((3 * NP, 64, 128), BF16),
            pltpu.VMEM((2, H, 48, 128), BF16),
            pltpu.VMEM((NP, 80, 128), BF16),
            pltpu.VMEM((80, 128), F32),
            pltpu.VMEM((S, D), BF16),
            pltpu.VMEM((1, FF + D), F32),
            pltpu.VMEM((8, T0, 128), F32),
            pltpu.VMEM((M, D), BF16),
            pltpu.VMEM((FF,), BF16),
            pltpu.VMEM((D,), BF16),
            pltpu.VMEM((1, D), BF16),
            pltpu.VMEM((5, FH // 128, DH2, 128), BF16),
            pltpu.VMEM((5, DH2 // 128, FH, 128), BF16),
            pltpu.SemaphoreType.DMA((SEM_N,)),
        ],
        compiler_params=pltpu.CompilerParams(vmem_limit_bytes=120 * 1024 * 1024, disable_bounds_checks=True,
                                             disable_semaphore_checks=True),
    )(
        A_x.reshape(NSEG, SEG, D), A_mem0.reshape(M, D),
        A_Wq.reshape(D // 2, 2, H, DH), A_Wk.reshape(D // 2, 2, H, DH), A_Wv.reshape(D // 2, 2, H, DH),
        A_Wo.reshape(H * DH, D), B_w1, B_b1, B_w2, B_b2, c, w_mod,
    )
    return out.reshape(1, S, D)
```

```python
import contextlib

import jax
import jax.numpy as jnp
from jax import lax
import jax.experimental.pallas as pl
import jax.experimental.pallas.tpu as pltpu

F32 = jnp.float32
BF16 = jnp.bfloat16
U32 = jnp.uint32

S = 2048
D = 1024
H = 32
DH = 128
M = 8
SEG = 32
FF = 3584
NSEG = S // SEG
NP = H // 2
TPS = 24
T0 = S - NSEG * TPS
EPS = 1e-5
P1U = 2
PA = 4
LNP = (16,) * 8
MODPOS = ((5, 0, 24), (6, 0, 24))
LOG2E = 1.4426950408889634
FB = 256
OC = 128
FC = 256
FH = FF // 2
DH2 = D // 2
T1_ROW = 3 * NP * 2 * T0
T2_ROW = T1_ROW + 5 * (FH // 128) * DH2
LT_ROWS = T2_ROW + 5 * (DH2 // 128) * FH
TSUM = (0, 2, 3, 5, 6)
SEM_W, SEM_A, SEM_M, SEM_MISC, SEM_OUT = 0, 16, 24, 32, 40
SEM_N = SEM_OUT + S // FB


def _make_sched(g):
    out = []

    def rng(a, b):
        return tuple(range(max(a, 0), max(b, 0)))

    for p in range(NP):
        out.append(("proj", p))
        if p % g == 0 and p >= g:
            out.append(("attn", rng(p - 2 * g, p - g), rng(p - g, p)))
    h1 = 2 * (NP - 2 * g)
    h2 = 2 * (NP - g)
    if g == 4:
        out += [("wo", j, 0, h1) for j in (0, 1)]
        out.append(("attn", rng(NP - 2 * g, NP - g), rng(NP - g, NP)))
        out += [("wo", j, 0, h1) for j in (2, 3, 4, 5)]
        out.append(("attn", rng(NP - g, NP), ()))
        out += [("wo", j, 0, h1) for j in (6, 7)]
        out += [("wo", j, h1, h2) for j in range(8)]
        out += [("wo", j, h2, H) for j in range(8)]
    else:
        out += [("wo", 0, 0, h1)]
        out.append(("attn", rng(NP - 2 * g, NP - g), rng(NP - g, NP)))
        out += [("wo", j, 0, h1) for j in (1, 2, 3)]
        out.append(("attn", rng(NP - g, NP), ()))
        out += [("wo", j, 0, h1) for j in (4, 5, 6, 7)]
        out += [("wo", j, h1, H) for j in range(8)]
    return out


SCHED = _make_sched(2)
_SCOPES = False


def _scope(name):
    return jax.named_scope(name) if _SCOPES else contextlib.nullcontext()


def _dot(a, b):
    return jnp.dot(a, b, preferred_element_type=F32)


def _bf(x):
    return pltpu.bitcast(x, BF16)


def _u32(x):
    return pltpu.bitcast(x, U32)


def _ld(ref, idx, r0, n):
    return _bf(ref.bitcast(U32)[(*idx, pl.ds(r0 // 2, n // 2), slice(None))])


def _ln(x):
    m = jnp.mean(x, axis=-1, keepdims=True)
    xc = x - m
    v = jnp.mean(xc * xc, axis=-1, keepdims=True)
    return xc * lax.rsqrt(v + EPS)


def _gelu(x):
    c = 0.7978845608028654
    return 0.5 * x * (1.0 + jnp.tanh(c * (x + 0.044715 * (x * x * x))))


def _strassen_lhs(a11, a12, a21, a22):
    return [a11 + a22, a21 + a22, a11, a22, a11 + a12, a21 - a11, a12 - a22]


def _strassen_rhs(b11, b12, b21, b22):
    return [b11 + b22, b11, b12 - b22, b21 - b11, b22, b11 + b12, b21 + b22]


def _strassen_out(m):
    return (m[0] + m[3] - m[4] + m[6], m[2] + m[4], m[1] + m[3], m[0] - m[1] + m[2] + m[5])


def _interleave(a, b):
    n = a.shape[0] // 8
    parts = []
    for g in range(n):
        parts.append(a[8 * g:8 * g + 8])
        parts.append(b[8 * g:8 * g + 8])
    return jnp.concatenate(parts, axis=0)


def _deinterleave(v):
    n = v.shape[0] // 16
    a = jnp.concatenate([v[16 * g:16 * g + 8] for g in range(n)], axis=0)
    b = jnp.concatenate([v[16 * g + 8:16 * g + 16] for g in range(n)], axis=0)
    return a, b


def _kernel(x_hbm, mem0_hbm, wq_hbm, wk_hbm, wv_hbm, wo_hbm, w1_hbm, b1_hbm, w2_hbm, b2_hbm,
            c_hbm, wmod_hbm, out_hbm,
            x_v, h_v, hn_v, h2_v, x1_v, wmod_v, mod_v, sc_v, w_v, wo_v, w1_v, w2_v, lt_v, fr_v, lo_v, pr_v, fill_v, out_v, bias_v, n_v,
            mem0_ref, b1_ref, b2_ref, c_ref,
            sems):
    w32 = [r.bitcast(U32) for r in (wq_hbm, wk_hbm, wv_hbm)]
    wo32 = wo_hbm.bitcast(U32)

    def w_copies(p):
        return [pltpu.make_async_copy(w32[j].at[:, par, p, :], w_v.at[p * 6 + j * 2 + par], sems.at[SEM_W + p])
                for j in range(3) for par in range(2)]

    def _mult(i, m):
        return i * m if isinstance(i, int) else pl.multiple_of(i * m, m)

    def wa_copies(k, pair=None):
        r = pl.ds(_mult(k, 64), 64)
        return [pltpu.make_async_copy(w32[j].at[r, par, p, :], w_v.at[p * 6 + j * 2 + par, r], sems.at[SEM_A + k])
                for p in (range(PA) if pair is None else (pair,)) for j in range(3) for par in range(2)]

    def m_copies(k):
        cols = [pl.ds(_mult(k + 8 * t, 128), 128) for t in range(2)]
        return [pltpu.make_async_copy(wmod_hbm.at[:, cs], wmod_v.at[:, cs], sems.at[SEM_M + k]) for cs in cols]

    def start(cps):
        for cp in cps:
            cp.start()

    def wait(cps):
        for cp in cps:
            cp.wait()

    cp_x0 = pltpu.make_async_copy(x_hbm.at[:, 0:8, :], x_v.at[:, 0:8, :], sems.at[SEM_MISC + 1])
    cp_x1 = pltpu.make_async_copy(x_hbm.at[1:NSEG, 8:SEG, :], x_v.at[1:NSEG, 8:SEG, :], sems.at[SEM_MISC + 6])

    def wo_copy(j):
        return pltpu.make_async_copy(wo32.at[:, pl.ds(_mult(j, 128), 128)], wo_v.at[j], sems.at[SEM_MISC + 3])

    def ffn_copies(first):
        sem = sems.at[SEM_MISC + (4 if first else 5)]
        cs = pl.ds(2 * D, D) if first else pl.ds(3 * D, 3 * D)
        cps = [pltpu.make_async_copy(wmod_hbm.at[:, cs], wmod_v.at[:, cs], sem)]
        for src, dst, nt in ((w1_hbm, w1_v, FF // 128), (w2_hbm, w2_v, D // 128)):
            cps += [pltpu.make_async_copy(src.at[:, j * 128:(j + 1) * 128], dst.at[j], sem)
                    for j in range(nt) if (j % (nt // 2) == 0) == first]
        return cps

    cp_small = [pltpu.make_async_copy(src, dst, sems.at[SEM_MISC])
                for src, dst in ((c_hbm, c_ref), (mem0_hbm, mem0_ref), (b1_hbm, b1_ref), (b2_hbm, b2_ref),
                                 (x_hbm.at[0, 8:SEG, :], x_v.at[0, 8:SEG, :]))]

    start(cp_small)
    cp_x0.start()
    start(m_copies(0))
    for k in range(2):
        start(m_copies(k + 1))
        start(wa_copies(k))

    scale = DH ** -0.5
    ri = lax.broadcasted_iota(jnp.int32, (80, 128), 0)
    ci = lax.broadcasted_iota(jnp.int32, (80, 128), 1)
    same_head = (((ri >> 3) & 1) == ((ci >> 3) & 1)) & (ci < 80)
    rpos = (((ri >> 4) & 3) << 3) + (ri & 7)
    cpos = (((ci >> 4) & 3) << 3) + (ci & 7)
    keep = (ri < 16) | (ci < 16) | (rpos >= cpos)
    fill_v[...] = jnp.where(same_head, jnp.where(keep, 0.0, -1e9 / scale), -jnp.inf).astype(F32)

    wait(cp_small)
    c = c_ref[...].astype(F32)
    sc = jnp.broadcast_to(c * jax.nn.sigmoid(c), (8, D)).astype(BF16)

    sc_v[...] = sc
    bias_v[:, 0:FF] = b1_ref[...].astype(F32).reshape(1, FF)
    bias_v[:, FF:FF + D] = b2_ref[...].astype(F32).reshape(1, D)

    def zero_body(i, carry):
        x1_v[pl.ds(pl.multiple_of(i * 64, 64), 64), :] = jnp.zeros((64, D), F32)
        return carry

    lax.fori_loop(0, PA * 6, zero_body, 0)

    def relayout(c, rows):
        a = w_v[c, rows, :]
        b = w_v[c + 1, rows, :]
        lo = (a & jnp.uint32(0xFFFF)) | (b << 16)
        hi = (a >> 16) | (b & jnp.uint32(0xFFFF0000))
        w_v[c, rows, :] = lo
        w_v[c + 1, rows, :] = hi
        return _bf(lo), _bf(hi)

    def store_lead(p, j, a, b):
        lt_v[pl.ds(_mult(p * 3 + j, 2 * T0), 2 * T0), :] = _interleave(a, b).astype(BF16)

    def mod_tile(ct):
        cs = pl.ds(_mult(ct, 128), 128)
        m = _dot(sc_v[...], wmod_v[:, cs])
        mod_v[:, cs] = m
        return m[0:1]

    with _scope("wait_x0"):
        cp_x0.wait()

    def ln1_body(i, carry):
        r = pl.multiple_of(i * 128, 128)
        n = _ln(x_v[pl.ds(i * 16, 16), 0:8, :].astype(F32).reshape(128, D))
        for k in range(8):
            n_v[k, pl.ds(r, 128), :] = n[:, k * 128:(k + 1) * 128]
        return carry

    with _scope("ln1"):
        lax.fori_loop(0, T0 // 128, ln1_body, 0)
    start(m_copies(3))
    start(wa_copies(2))
    with _scope("wait_m0"):
        wait(m_copies(0))
    h_v[0] = (n_v[0] * (1.0 + mod_tile(8)) + mod_tile(0)).astype(BF16)

    def sa_body(k, carry):
        with _scope("wait_a"):
            wait(wa_copies(k))

            @pl.when(k < 7)
            def _():
                wait(m_copies(k + 1))

        kn = jnp.minimum(k + 1, 7)
        rows = pl.ds(pl.multiple_of(k * 64, 64), 64)
        hk = _ld(h_v, (k,), 0, T0)
        for p in range(PA):
            for j in range(3):
                c = p * 6 + j * 2
                res = []
                for t, w in enumerate(relayout(c, rows)):
                    acc = x1_v.at[(c + t) // 8 * T0:((c + t) // 8 + 1) * T0,
                                  (c + t) % 8 * 128:((c + t) % 8 + 1) * 128]
                    r = _dot(hk, w) + acc[...]
                    acc[...] = r
                    res.append(r)
                store_lead(p, j, *res)
                if c == 2:
                    sh = mod_tile(kn)
                if c == 6:
                    s1 = 1.0 + mod_tile(kn + 8)

                    @pl.when(k + 4 < 8)
                    def _():
                        start(m_copies(k + 4))

            @pl.when(k + 3 < 8)
            def _():
                start(wa_copies(k + 3, p))

        h_v[kn] = (n_v[kn] * s1 + sh).astype(BF16)


        @pl.when(k >= 4)
        def _():
            start(w_copies(PA + k - 4))

        return carry

    with _scope("stageA"):
        lax.fori_loop(0, 8, sa_body, 0)

    def ln1(seg):
        xb = x_v[seg, 8:SEG, :].astype(F32)
        return _ln(xb) * (1.0 + mod_v[0:1, D:2 * D]) + mod_v[0:1, 0:D]

    def p1_body(i, carry):
        p0 = PA + P1U * i
        with _scope("wait_w"):
            for u in range(P1U):
                wait(w_copies(p0 + u))

        hb = jnp.concatenate([_ld(h_v, (k,), 0, T0) for k in range(8)], axis=1)
        for u in range(P1U):
            p = p0 + u
            for j in range(3):
                lo, hi = relayout(p * 6 + j * 2, slice(None))
                store_lead(p, j, _dot(hb, lo), _dot(hb, hi))
        hn_v[...] = ln1(0)

        @pl.when(p0 + 4 < NP)
        def _():
            for u in range(P1U):
                start(w_copies(p0 + 4 + u))
                wo_copy(P1U * i + u).start()

        @pl.when(p0 + 8 == NP)
        def _():
            cp_x1.start()

        @pl.when(p0 + 6 == NP)
        def _():
            start(ffn_copies(True))

        return carry

    with _scope("phase1"):
        lax.fori_loop(0, (NP - PA) // P1U, p1_body, 0)

    with _scope("wait_wo"):
        for j in range(8):
            wo_copy(j).wait()
        cp_x1.wait()
        wait(ffn_copies(True))
    start(ffn_copies(False))

    def prep_views(w, t_row, kh, nh, j, r0):
        src = w.at[pl.ds(j, nh + 1), pl.ds(pl.multiple_of(r0, 256), kh + 256), :]
        dst = lt_v.at[pl.ds(pl.multiple_of(t_row + j * kh + r0, 256), 4 * nh * kh + 256), :]
        return src, dst, kh, nh

    def prep(views, r0, n):
        src, dst, kh, nh = views
        t = _strassen_rhs(*[_ld(src, (b * nh,), a * kh + r0, n).astype(F32) for a in range(2) for b in range(2)])
        for k, i in enumerate(TSUM):
            dst[k * nh * kh + r0:k * nh * kh + r0 + n, :] = t[i].astype(BF16)

    def step(it, odd, mem):
        s = 2 * it + int(odd)
        lead = lt_v.at[pl.ds(pl.multiple_of(16 * s, 16), T1_ROW), :]
        lhs = jnp.concatenate([mem, hn_v[...]], axis=0).astype(BF16)
        hn_v[...] = ln1(jnp.minimum(s + 1, NSEG - 1))
        mo = 48 if odd else 32

        def proj(p):
            if p == 0:
                half = [_dot(lhs[:, 0:D // 2], _bf(w_v[c, 0:D // 4, :])) for c in range(6)]
                cols = [_dot(lhs[:, D // 2:D], _bf(w_v[c, D // 4:D // 2, :])) + half[c] for c in range(6)]
            for j in range(3):
                if p == 0:
                    r = _interleave(cols[j * 2], cols[j * 2 + 1])
                else:
                    r = _interleave(_dot(lhs, _bf(w_v[p * 6 + j * 2])), _dot(lhs, _bf(w_v[p * 6 + j * 2 + 1])))
                fr_v[p * 3 + j] = r.astype(BF16)

        def stack(p, j):
            return jnp.concatenate([fr_v[p * 3 + j],
                                    _ld(lead, (), (p * 3 + j) * 2 * T0, 16)], axis=0)

        def attn(pvs, qks):
            os_ = [_dot(pr_v[p, :, 0:80], stack(p, 2)) for p in pvs]
            ss = [lax.dot_general(stack(p, 0), stack(p, 1), (((1,), (1,)), ((), ())),
                                  preferred_element_type=F32) for p in qks]
            for p, o in zip(pvs, os_):
                for t, oh in enumerate(_deinterleave(o)):
                    h = 2 * p + t
                    if odd:
                        lo_v[1, h, 0:8, :] = oh[0:8].astype(BF16)
                        lo_v[1, h, 16:48, :] = oh[8:40].astype(BF16)
                    else:
                        lo_v[0, h, 0:32, :] = oh[0:32].astype(BF16)
                        lo_v[1, h, 8:16, :] = oh[32:40].astype(BF16)
            for p, sc_ in zip(qks, ss):
                fill = fill_v[...]
                sc_ = jnp.concatenate([sc_, jnp.zeros((80, 48), F32)], axis=1)
                sc_ = jnp.where(fill == 0.0, sc_, fill)
                mx = jnp.max(sc_, axis=-1, keepdims=True)
                e = jnp.exp2((sc_ - mx) * (scale * LOG2E))
                l = jnp.sum(e, axis=-1, keepdims=True)
                r = pl.reciprocal(l, approx=True)
                pr_v[p] = (e * (r * (2.0 - l * r))).astype(BF16)

        part = {}

        def wo(j, h0, h1):
            lo = jnp.concatenate([lo_v[int(odd), h, 0:mo, :] for h in range(h0, h1)], axis=1)
            r = _dot(lo, _bf(wo_v[j, h0 * 64:h1 * 64, :]))
            part[j] = r + part[j] if j in part else r

        pc = jnp.maximum(it - 4, 0)
        if odd:
            views = prep_views(w2_v, T2_ROW, FH, DH2 // 128, lax.div(pc, 7), lax.rem(pc, 7) * 256)
        else:
            views = prep_views(w1_v, T1_ROW, DH2, FH // 128, pc >> 1, (pc & 1) * 256)
        npiece = 0
        for op in SCHED:
            if op[0] == "proj":
                proj(op[1])
            elif op[0] == "attn":
                attn(op[1], op[2])
                if npiece < 8:
                    prep(views, npiece * 32, 32)
                    npiece += 1
            else:
                wo(*op[1:])
                if odd and op[1:] in MODPOS:
                    cs = pl.ds(pl.multiple_of((16 + it) * 128, 128), 128)
                    k0 = MODPOS.index(op[1:]) * (D // 2)
                    m = _dot(sc_v[:, k0:k0 + D // 2], wmod_v[k0:k0 + D // 2, cs])
                    if k0 == 0:
                        mhalf = m
                    else:
                        mod_v[:, cs] = m + mhalf
        res = jnp.concatenate([part[j] for j in range(8)], axis=1)
        t0 = pl.multiple_of(SEG * s, SEG)
        if odd:
            x1_v[pl.ds(t0 - SEG, 8), :] = res[8:16]
            x1_v[pl.ds(t0, SEG), :] = jnp.concatenate([res[40:48], res[16:40]], axis=0)
        else:
            x1_v[pl.ds(t0 + 8, TPS), :] = res[8:32]
        return res[0:8]

    with _scope("main"):
        def steps(i, mem):
            with _scope("iter"):
                mem = step(i, True, step(i, False, mem))

            @pl.when(i == 4)
            def _():
                wait(ffn_copies(False))

            return mem

        lax.fori_loop(0, NSEG // 2, steps, mem0_ref[...].astype(F32))

    def rhs(w, t_row, kh, nh, i, j, k0, nk):
        if i == 1:
            return _ld(w, (j,), k0, nk)
        if i == 4:
            return _ld(w, (j + nh,), kh + k0, nk)
        return _ld(lt_v, (), t_row + (TSUM.index(i) * nh + j) * kh + k0, nk)

    def out_copy(i, q):
        rows = pl.ds(_mult(i, FB), FB)
        return [pltpu.make_async_copy(out_v.at[rows, cols], out_hbm.at[rows, cols], sems.at[SEM_OUT + i])
                for cols in (pl.ds(q * OC, OC), pl.ds(DH2 + q * OC, OC))]

    HB = FB // 2

    def resid1(r0, k0, n, c0=0, nc=D):
        if n >= SEG:
            xb = x_v[pl.ds((r0 >> 5) + k0 // SEG, n // SEG), :, c0:c0 + nc].astype(F32).reshape(n, nc)
        else:
            xb = x_v[(r0 >> 5) + k0 // SEG, k0 % SEG:k0 % SEG + n, c0:c0 + nc].astype(F32)
        return xb + mod_v[0:1, 2 * D + c0:2 * D + c0 + nc] * x1_v[pl.ds(r0 + k0, n), c0:c0 + nc]

    def ln2(slot, r0, k0, n):
        top, bot = [_ln(resid1(r0, t * HB + k0, n)) * (1.0 + mod_v[0:1, 4 * D:5 * D]) + mod_v[0:1, 3 * D:4 * D]
                    for t in range(2)]
        ss = _strassen_lhs(top[:, 0:DH2], top[:, DH2:D], bot[:, 0:DH2], bot[:, DH2:D])
        for i in range(7):
            for j in range(DH2 // 128):
                h2_v[slot, i, j, k0:k0 + n, :] = ss[i][:, j * 128:(j + 1) * 128].astype(BF16)

    ln2(0, 0, 0, HB)

    def ffn_body(i, carry):
        r0 = pl.multiple_of(i * FB, FB)
        rn = pl.multiple_of(jnp.minimum(r0 + FB, S - FB), FB)
        slot = lax.rem(i, 2)
        nf = FH // FC
        nt = FC // 128
        nq = DH2 // OC
        acc = {}
        gs = {}

        def up(f, t):
            c0 = f * FC + t * 128
            c = _strassen_out([
                _dot(jnp.concatenate([_ld(h2_v, (slot, k, j), 0, HB) for j in range(DH2 // 128)], axis=1),
                     rhs(w1_v, T1_ROW, DH2, FH // 128, k, c0 // 128, 0, DH2)) for k in range(7)])
            b1a, b1b = bias_v[0:1, c0:c0 + 128], bias_v[0:1, FH + c0:FH + c0 + 128]
            gs[f, t] = _strassen_lhs(_gelu(c[0] + b1a), _gelu(c[1] + b1b), _gelu(c[2] + b1a), _gelu(c[3] + b1b))
            if t == nt - 1:
                gs[f] = [jnp.concatenate([gs[f, u][k] for u in range(nt)], axis=1).astype(BF16) for k in range(7)]

        def down(f, q):
            for k in range(7):
                y = _dot(gs[f][k], rhs(w2_v, T2_ROW, FH, DH2 // 128, k, q, f * FC, FC))
                acc[k, q] = y + acc[k, q] if f else y
            if f == nf - 1:
                c = _strassen_out([acc[k, q] for k in range(7)])
                for t in range(4):
                    k0, c0 = (t // 2) * HB, (t % 2) * DH2 + q * OC
                    y = (c[t] + bias_v[0:1, FF + c0:FF + c0 + OC]) * mod_v[0:1, 5 * D + c0:5 * D + c0 + OC]
                    out_v[pl.ds(r0 + k0, HB), c0:c0 + OC] = (resid1(r0, k0, HB, c0, OC) + y).astype(BF16)
                start(out_copy(i, q))

        for t in range(nt):
            up(0, t)
        w = 0
        for f in range(nf):
            for t in range(nt):
                if f + 1 < nf:
                    up(f + 1, t)
                if w < len(LNP) and LNP[w]:
                    ln2(1 - slot, rn, sum(LNP[:w]), LNP[w])
                w += 1
                for q in range(t * nq // nt, (t + 1) * nq // nt):
                    down(f, q)
        return carry

    with _scope("ffn"):
        lax.fori_loop(0, S // FB, ffn_body, 0)
    with _scope("wait_out"):
        for i in range(S // FB):
            for q in range(DH2 // OC):
                wait(out_copy(i, q))


@jax.jit
def pallas_adaLN_cond__memory_aug_recurrent_mem_tr__dense_activation_gelu__prompt_kernel(
    A_x, A_mem0, A_Wq, A_Wk, A_Wv, A_Wo, A_seg_len, B_x, B_w1, B_b1, B_w2, B_b2, c, w_mod,
):
    del A_seg_len, B_x
    assert A_x.shape == (1, S, D)
    hbm = pl.BlockSpec(memory_space=pl.ANY)
    out = pl.pallas_call(
        _kernel,
        out_shape=jax.ShapeDtypeStruct((S, D), BF16),
        in_specs=[hbm] * 12,
        out_specs=hbm,
        scratch_shapes=[
            pltpu.VMEM((NSEG, SEG, D), BF16),
            pltpu.VMEM((8, T0, 128), BF16),
            pltpu.VMEM((TPS, D), F32),
            pltpu.VMEM((2, 7, 4, FB // 2, 128), BF16),
            pltpu.VMEM((S, D), F32),
            pltpu.VMEM((D, 6 * D), BF16),
            pltpu.VMEM((8, 6 * D), F32),
            pltpu.VMEM((8, D), BF16),
            pltpu.VMEM((6 * NP, D // 2, 128), U32),
            pltpu.VMEM((8, H * DH // 2, 128), U32),
            pltpu.VMEM((FF // 128, D, 128), BF16),
            pltpu.VMEM((D // 128, FF, 128), BF16),
            pltpu.VMEM((LT_ROWS, 128), BF16),
            pltpu.VMEM((3 * NP, 64, 128), BF16),
            pltpu.VMEM((2, H, 48, 128), BF16),
            pltpu.VMEM((NP, 80, 128), BF16),
            pltpu.VMEM((80, 128), F32),
            pltpu.VMEM((S, D), BF16),
            pltpu.VMEM((1, FF + D), F32),
            pltpu.VMEM((8, T0, 128), F32),
            pltpu.VMEM((M, D), BF16),
            pltpu.VMEM((FF,), BF16),
            pltpu.VMEM((D,), BF16),
            pltpu.VMEM((1, D), BF16),
            pltpu.SemaphoreType.DMA((SEM_N,)),
        ],
        compiler_params=pltpu.CompilerParams(vmem_limit_bytes=120 * 1024 * 1024, disable_bounds_checks=True,
                                             disable_semaphore_checks=True),
    )(
        A_x.reshape(NSEG, SEG, D), A_mem0.reshape(M, D),
        A_Wq.reshape(D // 2, 2, H, DH), A_Wk.reshape(D // 2, 2, H, DH), A_Wv.reshape(D // 2, 2, H, DH),
        A_Wo.reshape(H * DH, D), B_w1, B_b1, B_w2, B_b2, c, w_mod,
    )
    return out.reshape(1, S, D)
```

```python
import contextlib

import jax
import jax.numpy as jnp
from jax import lax
import jax.experimental.pallas as pl
import jax.experimental.pallas.tpu as pltpu

F32 = jnp.float32
BF16 = jnp.bfloat16
U32 = jnp.uint32

S = 2048
D = 1024
H = 32
DH = 128
M = 8
SEG = 32
FF = 3584
NSEG = S // SEG
NP = H // 2
TPS = 24
T0 = S - NSEG * TPS
EPS = 1e-5
NEARLY = 4
PA = 4
LNP = (16,) * 8
MODPOS = ((5, 0, 24), (6, 0, 24))
LOG2E = 1.4426950408889634
FB = 256
OC = 128
FC = 256
FH = FF // 2
DH2 = D // 2
T1_ROW = 3 * NP * 2 * T0
T2_ROW = T1_ROW + 5 * (FH // 128) * DH2
LT_ROWS = T2_ROW + 5 * (DH2 // 128) * FH
SSUM = (0, 1, 4, 5, 6)
TSUM = (0, 2, 3, 5, 6)
SEM_W, SEM_A, SEM_M, SEM_MISC, SEM_OUT = 0, 16, 24, 32, 40
SEM_N = SEM_OUT + S // FB


def _make_sched(g):
    out = []

    def rng(a, b):
        return tuple(range(max(a, 0), max(b, 0)))

    for p in range(NP):
        out.append(("proj", p))
        if p % g == 0 and p >= g:
            out.append(("attn", rng(p - 2 * g, p - g), rng(p - g, p)))
    h1 = 2 * (NP - 2 * g)
    h2 = 2 * (NP - g)
    if g == 4:
        out += [("wo", j, 0, h1) for j in (0, 1)]
        out.append(("attn", rng(NP - 2 * g, NP - g), rng(NP - g, NP)))
        out += [("wo", j, 0, h1) for j in (2, 3, 4, 5)]
        out.append(("attn", rng(NP - g, NP), ()))
        out += [("wo", j, 0, h1) for j in (6, 7)]
        out += [("wo", j, h1, h2) for j in range(8)]
        out += [("wo", j, h2, H) for j in range(8)]
    else:
        out += [("wo", 0, 0, h1)]
        out.append(("attn", rng(NP - 2 * g, NP - g), rng(NP - g, NP)))
        out += [("wo", j, 0, h1) for j in (1, 2, 3)]
        out.append(("attn", rng(NP - g, NP), ()))
        out += [("wo", j, 0, h1) for j in (4, 5, 6, 7)]
        out += [("wo", j, h1, H) for j in range(8)]
    return out


SCHED = _make_sched(2)
_SCOPES = False


def _scope(name):
    return jax.named_scope(name) if _SCOPES else contextlib.nullcontext()


def _dot(a, b):
    return jnp.dot(a, b, preferred_element_type=F32)


def _bf(x):
    return pltpu.bitcast(x, BF16)


def _u32(x):
    return pltpu.bitcast(x, U32)


def _ld(ref, idx, r0, n):
    return _bf(ref.bitcast(U32)[(*idx, pl.ds(r0 // 2, n // 2), slice(None))])


def _ln(x):
    m = jnp.mean(x, axis=-1, keepdims=True)
    xc = x - m
    v = jnp.mean(xc * xc, axis=-1, keepdims=True)
    return xc * lax.rsqrt(v + EPS)


def _gelu(x):
    c = 0.7978845608028654
    return 0.5 * x * (1.0 + jnp.tanh(c * (x + 0.044715 * (x * x * x))))


def _strassen_lhs(a11, a12, a21, a22):
    return [a11 + a22, a21 + a22, a11, a22, a11 + a12, a21 - a11, a12 - a22]


def _strassen_rhs(b11, b12, b21, b22):
    return [b11 + b22, b11, b12 - b22, b21 - b11, b22, b11 + b12, b21 + b22]


def _strassen_out(m):
    return (m[0] + m[3] - m[4] + m[6], m[2] + m[4], m[1] + m[3], m[0] - m[1] + m[2] + m[5])


def _interleave(a, b):
    n = a.shape[0] // 8
    parts = []
    for g in range(n):
        parts.append(a[8 * g:8 * g + 8])
        parts.append(b[8 * g:8 * g + 8])
    return jnp.concatenate(parts, axis=0)


def _deinterleave(v):
    n = v.shape[0] // 16
    a = jnp.concatenate([v[16 * g:16 * g + 8] for g in range(n)], axis=0)
    b = jnp.concatenate([v[16 * g + 8:16 * g + 16] for g in range(n)], axis=0)
    return a, b


def _kernel(x_hbm, mem0_hbm, wq_hbm, wk_hbm, wv_hbm, wo_hbm, w1_hbm, b1_hbm, w2_hbm, b2_hbm,
            c_hbm, wmod_hbm, out_hbm,
            x_v, h_v, hn_v, h2_v, x1_v, wmod_v, mod_v, sc_v, w_v, wo_v, w1_v, w2_v, lt_v, fr_v, lo_v, pr_v, fill_v, out_v, bias_v, n_v,
            mem0_ref, b1_ref, b2_ref, c_ref, hs_v,
            sems):
    w32 = [r.bitcast(U32) for r in (wq_hbm, wk_hbm, wv_hbm)]
    wo32 = wo_hbm.bitcast(U32)

    def w_copies(p):
        return [pltpu.make_async_copy(w32[j].at[:, par, p, :], w_v.at[p * 6 + j * 2 + par], sems.at[SEM_W + p])
                for j in range(3) for par in range(2)]

    def _mult(i, m):
        return i * m if isinstance(i, int) else pl.multiple_of(i * m, m)

    def wa_copies(k, pair=None):
        r = pl.ds(_mult(k, 64), 64)
        return [pltpu.make_async_copy(w32[j].at[r, par, p, :], w_v.at[p * 6 + j * 2 + par, r], sems.at[SEM_A + k])
                for p in (range(PA) if pair is None else (pair,)) for j in range(3) for par in range(2)]

    def m_copies(k):
        cols = [pl.ds(_mult(k + 8 * t, 128), 128) for t in range(2)]
        return [pltpu.make_async_copy(wmod_hbm.at[:, cs], wmod_v.at[:, cs], sems.at[SEM_M + k]) for cs in cols]

    def start(cps):
        for cp in cps:
            cp.start()

    def wait(cps):
        for cp in cps:
            cp.wait()

    cp_x0 = pltpu.make_async_copy(x_hbm.at[:, 0:8, :], x_v.at[:, 0:8, :], sems.at[SEM_MISC + 1])

    def wo_copy(j):
        return pltpu.make_async_copy(wo32.at[:, pl.ds(_mult(j, 128), 128)], wo_v.at[j], sems.at[SEM_MISC + 3])

    def late_copies(first):
        sem = sems.at[SEM_MISC + (4 if first else 5)]
        cs = pl.ds(2 * D, NEARLY * 128) if first else pl.ds(2 * D + NEARLY * 128, 4 * D - NEARLY * 128)
        sg = slice(1, 2 * NEARLY + 1) if first else slice(2 * NEARLY + 1, NSEG)
        cps = [(x_hbm.at[sg, 8:SEG, :], x_v.at[sg, 8:SEG, :]), (wmod_hbm.at[:, cs], wmod_v.at[:, cs])]
        for src, dst, nt, kh in ((w1_hbm, w1_v, FF // 128, DH2), (w2_hbm, w2_v, D // 128, FH)):
            for j in range(nt):
                cols = slice(j * 128, (j + 1) * 128)
                if j % (nt // 2):
                    rows = [] if first else [slice(None)]
                else:
                    rows = [slice(a * kh, a * kh + 256) if first else slice(a * kh + 256, (a + 1) * kh)
                            for a in range(2)]
                cps += [(src.at[r, cols], dst.at[j, r]) for r in rows]
        return [pltpu.make_async_copy(src, dst, sem) for src, dst in cps]

    cp_small = [pltpu.make_async_copy(src, dst, sems.at[SEM_MISC])
                for src, dst in ((c_hbm, c_ref), (mem0_hbm, mem0_ref), (b1_hbm, b1_ref), (b2_hbm, b2_ref),
                                 (x_hbm.at[0, 8:SEG, :], x_v.at[0, 8:SEG, :]))]

    start(cp_small)
    cp_x0.start()
    start(m_copies(0))
    for k in range(2):
        start(m_copies(k + 1))
        start(wa_copies(k))

    scale = DH ** -0.5
    ri = lax.broadcasted_iota(jnp.int32, (80, 128), 0)
    ci = lax.broadcasted_iota(jnp.int32, (80, 128), 1)
    same_head = (((ri >> 3) & 1) == ((ci >> 3) & 1)) & (ci < 80)
    rpos = (((ri >> 4) & 3) << 3) + (ri & 7)
    cpos = (((ci >> 4) & 3) << 3) + (ci & 7)
    keep = (ri < 16) | (ci < 16) | (rpos >= cpos)
    fill_v[...] = jnp.where(same_head, jnp.where(keep, 0.0, -1e9 / scale), -jnp.inf).astype(F32)

    wait(cp_small)
    c = c_ref[...].astype(F32)
    sc = jnp.broadcast_to(c * jax.nn.sigmoid(c), (8, D)).astype(BF16)

    sc_v[...] = sc
    bias_v[:, 0:FF] = b1_ref[...].astype(F32).reshape(1, FF)
    bias_v[:, FF:FF + D] = b2_ref[...].astype(F32).reshape(1, D)

    def zero_body(i, carry):
        x1_v[pl.ds(pl.multiple_of(i * 64, 64), 64), :] = jnp.zeros((64, D), F32)
        return carry

    lax.fori_loop(0, PA * 6, zero_body, 0)

    def relayout(c, rows):
        a = w_v[c, rows, :]
        b = w_v[c + 1, rows, :]
        lo = (a & jnp.uint32(0xFFFF)) | (b << 16)
        hi = (a >> 16) | (b & jnp.uint32(0xFFFF0000))
        w_v[c, rows, :] = lo
        w_v[c + 1, rows, :] = hi
        return _bf(lo), _bf(hi)

    def store_lead(p, j, a, b):
        lt_v[pl.ds(_mult(p * 3 + j, 2 * T0), 2 * T0), :] = _interleave(a, b).astype(BF16)

    def mod_tile(ct):
        cs = pl.ds(_mult(ct, 128), 128)
        m = _dot(sc_v[...], wmod_v[:, cs])
        mod_v[:, cs] = m
        return m[0:1]

    with _scope("wait_x0"):
        cp_x0.wait()

    def ln1_body(i, carry):
        r = pl.multiple_of(i * 128, 128)
        n = _ln(x_v[pl.ds(i * 16, 16), 0:8, :].astype(F32).reshape(128, D))
        for k in range(8):
            n_v[k, pl.ds(r, 128), :] = n[:, k * 128:(k + 1) * 128]
        return carry

    with _scope("ln1"):
        lax.fori_loop(0, T0 // 128, ln1_body, 0)
    start(m_copies(3))
    start(wa_copies(2))
    with _scope("wait_m0"):
        wait(m_copies(0))
    h_v[0] = (n_v[0] * (1.0 + mod_tile(8)) + mod_tile(0)).astype(BF16)

    def sa_body(k, carry):
        with _scope("wait_a"):
            wait(wa_copies(k))

            @pl.when(k < 7)
            def _():
                wait(m_copies(k + 1))

        kn = jnp.minimum(k + 1, 7)
        rows = pl.ds(pl.multiple_of(k * 64, 64), 64)
        hk = _ld(h_v, (k,), 0, T0)
        for p in range(PA):
            for j in range(3):
                c = p * 6 + j * 2
                res = []
                for t, w in enumerate(relayout(c, rows)):
                    acc = x1_v.at[(c + t) // 8 * T0:((c + t) // 8 + 1) * T0,
                                  (c + t) % 8 * 128:((c + t) % 8 + 1) * 128]
                    r = _dot(hk, w) + acc[...]
                    acc[...] = r
                    res.append(r)
                store_lead(p, j, *res)
                if c == 2:
                    sh = mod_tile(kn)
                if c == 6:
                    s1 = 1.0 + mod_tile(kn + 8)

                    @pl.when(k + 4 < 8)
                    def _():
                        start(m_copies(k + 4))

            @pl.when(k + 3 < 8)
            def _():
                start(wa_copies(k + 3, p))

        h_v[kn] = (n_v[kn] * s1 + sh).astype(BF16)


        @pl.when(k >= 4)
        def _():
            start(w_copies(PA + k - 4))

        return carry

    with _scope("stageA"):
        lax.fori_loop(0, 8, sa_body, 0)

    def ln1(seg):
        xb = x_v[seg, 8:SEG, :].astype(F32)
        return _ln(xb) * (1.0 + mod_v[0:1, D:2 * D]) + mod_v[0:1, 0:D]

    TH = T0 // 2
    for t in range(4):
        ha, hb = h_v[t].astype(F32), h_v[t + 4].astype(F32)
        ss = _strassen_lhs(ha[0:TH], hb[0:TH], ha[TH:T0], hb[TH:T0])
        for k, i in enumerate(SSUM):
            hs_v[k, t] = ss[i].astype(BF16)

    def lhs1(i):
        if i == 2:
            tiles = [_ld(h_v, (t,), 0, TH) for t in range(4)]
        elif i == 3:
            tiles = [_ld(h_v, (t + 4,), TH, TH) for t in range(4)]
        else:
            tiles = [_ld(hs_v, (SSUM.index(i), t), 0, TH) for t in range(4)]
        return jnp.concatenate(tiles, axis=1)

    def p1_body(i, carry):
        p0 = PA + 2 * i
        with _scope("wait_w"):
            wait(w_copies(p0) + w_copies(p0 + 1))

        for u in range(6):
            p, j = p0 + u // 3, u % 3
            lo, hi = relayout(p * 6 + j * 2, slice(None))
            b = [lo[0:DH2], hi[0:DH2], lo[DH2:D], hi[DH2:D]]
            t = _strassen_rhs(*[x.astype(F32) for x in b])
            t = [b[0] if k == 1 else b[3] if k == 4 else t[k].astype(BF16) for k in range(7)]
            c = _strassen_out([_dot(lhs1(k), t[k]) for k in range(7)])
            store_lead(p, j, jnp.concatenate([c[0], c[2]], axis=0), jnp.concatenate([c[1], c[3]], axis=0))

            if u < 4:
                @pl.when(i < 2)
                def _():
                    start(w_copies(PA + 4 + 4 * i + u))
            elif u == 4:
                @pl.when(jnp.logical_and(i >= 1, i < 3))
                def _():
                    start([wo_copy(4 * (i - 1) + q) for q in range(4)])
            else:
                @pl.when(i == 2)
                def _():
                    start(late_copies(True))

        hn_v[...] = ln1(0)
        return carry

    with _scope("phase1"):
        lax.fori_loop(0, (NP - PA) // 2, p1_body, 0)

    with _scope("wait_wo"):
        wait([wo_copy(j) for j in range(8)])
        wait(late_copies(True))
    start(late_copies(False))

    def prep_views(w, t_row, kh, nh, j, r0):
        src = w.at[pl.ds(j, nh + 1), pl.ds(pl.multiple_of(r0, 256), kh + 256), :]
        dst = lt_v.at[pl.ds(pl.multiple_of(t_row + j * kh + r0, 256), 4 * nh * kh + 256), :]
        return src, dst, kh, nh

    def prep(views, r0, n):
        src, dst, kh, nh = views
        t = _strassen_rhs(*[_ld(src, (b * nh,), a * kh + r0, n).astype(F32) for a in range(2) for b in range(2)])
        for k, i in enumerate(TSUM):
            dst[k * nh * kh + r0:k * nh * kh + r0 + n, :] = t[i].astype(BF16)

    def step(it, odd, mem):
        s = 2 * it + int(odd)
        lead = lt_v.at[pl.ds(pl.multiple_of(16 * s, 16), T1_ROW), :]
        lhs = jnp.concatenate([mem, hn_v[...]], axis=0).astype(BF16)
        hn_v[...] = ln1(jnp.minimum(s + 1, NSEG - 1))
        mo = 48 if odd else 32

        def proj(p):
            if p == 0:
                half = [_dot(lhs[:, 0:D // 2], _bf(w_v[c, 0:D // 4, :])) for c in range(6)]
                cols = [_dot(lhs[:, D // 2:D], _bf(w_v[c, D // 4:D // 2, :])) + half[c] for c in range(6)]
            for j in range(3):
                if p == 0:
                    r = _interleave(cols[j * 2], cols[j * 2 + 1])
                else:
                    r = _interleave(_dot(lhs, _bf(w_v[p * 6 + j * 2])), _dot(lhs, _bf(w_v[p * 6 + j * 2 + 1])))
                fr_v[p * 3 + j] = r.astype(BF16)

        def stack(p, j):
            return jnp.concatenate([fr_v[p * 3 + j],
                                    _ld(lead, (), (p * 3 + j) * 2 * T0, 16)], axis=0)

        def attn(pvs, qks):
            os_ = [_dot(pr_v[p, :, 0:80], stack(p, 2)) for p in pvs]
            ss = [lax.dot_general(stack(p, 0), stack(p, 1), (((1,), (1,)), ((), ())),
                                  preferred_element_type=F32) for p in qks]
            for p, o in zip(pvs, os_):
                for t, oh in enumerate(_deinterleave(o)):
                    h = 2 * p + t
                    if odd:
                        lo_v[1, h, 0:8, :] = oh[0:8].astype(BF16)
                        lo_v[1, h, 16:48, :] = oh[8:40].astype(BF16)
                    else:
                        lo_v[0, h, 0:32, :] = oh[0:32].astype(BF16)
                        lo_v[1, h, 8:16, :] = oh[32:40].astype(BF16)
            for p, sc_ in zip(qks, ss):
                fill = fill_v[...]
                sc_ = jnp.concatenate([sc_, jnp.zeros((80, 48), F32)], axis=1)
                sc_ = jnp.where(fill == 0.0, sc_, fill)
                mx = jnp.max(sc_, axis=-1, keepdims=True)
                e = jnp.exp2((sc_ - mx) * (scale * LOG2E))
                l = jnp.sum(e, axis=-1, keepdims=True)
                r = pl.reciprocal(l, approx=True)
                pr_v[p] = (e * (r * (2.0 - l * r))).astype(BF16)

        part = {}

        def wo(j, h0, h1):
            lo = jnp.concatenate([lo_v[int(odd), h, 0:mo, :] for h in range(h0, h1)], axis=1)
            r = _dot(lo, _bf(wo_v[j, h0 * 64:h1 * 64, :]))
            part[j] = r + part[j] if j in part else r

        pc = jnp.maximum(it - 4, 0)
        if odd:
            views = prep_views(w2_v, T2_ROW, FH, DH2 // 128, lax.div(pc, 7), lax.rem(pc, 7) * 256)
        else:
            views = prep_views(w1_v, T1_ROW, DH2, FH // 128, pc >> 1, (pc & 1) * 256)
        npiece = 0
        for op in SCHED:
            if op[0] == "proj":
                proj(op[1])
            elif op[0] == "attn":
                attn(op[1], op[2])
                if npiece < 8:
                    prep(views, npiece * 32, 32)
                    npiece += 1
            else:
                wo(*op[1:])
                if odd and op[1:] in MODPOS:
                    cs = pl.ds(pl.multiple_of((16 + it) * 128, 128), 128)
                    k0 = MODPOS.index(op[1:]) * (D // 2)
                    m = _dot(sc_v[:, k0:k0 + D // 2], wmod_v[k0:k0 + D // 2, cs])
                    if k0 == 0:
                        mhalf = m
                    else:
                        mod_v[:, cs] = m + mhalf
        res = jnp.concatenate([part[j] for j in range(8)], axis=1)
        t0 = pl.multiple_of(SEG * s, SEG)
        if odd:
            x1_v[pl.ds(t0 - SEG, 8), :] = res[8:16]
            x1_v[pl.ds(t0, SEG), :] = jnp.concatenate([res[40:48], res[16:40]], axis=0)
        else:
            x1_v[pl.ds(t0 + 8, TPS), :] = res[8:32]
        return res[0:8]

    with _scope("main"):
        def steps(i, mem):
            with _scope("iter"):
                mem = step(i, True, step(i, False, mem))

            @pl.when(i == NEARLY - 1)
            def _():
                wait(late_copies(False))

            return mem

        lax.fori_loop(0, NSEG // 2, steps, mem0_ref[...].astype(F32))

    def rhs(w, t_row, kh, nh, i, j, k0, nk):
        if i == 1:
            return _ld(w, (j,), k0, nk)
        if i == 4:
            return _ld(w, (j + nh,), kh + k0, nk)
        return _ld(lt_v, (), t_row + (TSUM.index(i) * nh + j) * kh + k0, nk)

    def out_copy(i, q):
        rows = pl.ds(_mult(i, FB), FB)
        return [pltpu.make_async_copy(out_v.at[rows, cols], out_hbm.at[rows, cols], sems.at[SEM_OUT + i])
                for cols in (pl.ds(q * OC, OC), pl.ds(DH2 + q * OC, OC))]

    HB = FB // 2

    def resid1(r0, k0, n, c0=0, nc=D):
        if n >= SEG:
            xb = x_v[pl.ds((r0 >> 5) + k0 // SEG, n // SEG), :, c0:c0 + nc].astype(F32).reshape(n, nc)
        else:
            xb = x_v[(r0 >> 5) + k0 // SEG, k0 % SEG:k0 % SEG + n, c0:c0 + nc].astype(F32)
        return xb + mod_v[0:1, 2 * D + c0:2 * D + c0 + nc] * x1_v[pl.ds(r0 + k0, n), c0:c0 + nc]

    def ln2(slot, r0, k0, n):
        top, bot = [_ln(resid1(r0, t * HB + k0, n)) * (1.0 + mod_v[0:1, 4 * D:5 * D]) + mod_v[0:1, 3 * D:4 * D]
                    for t in range(2)]
        ss = _strassen_lhs(top[:, 0:DH2], top[:, DH2:D], bot[:, 0:DH2], bot[:, DH2:D])
        for i in range(7):
            for j in range(DH2 // 128):
                h2_v[slot, i, j, k0:k0 + n, :] = ss[i][:, j * 128:(j + 1) * 128].astype(BF16)

    ln2(0, 0, 0, HB)

    def ffn_body(i, carry):
        r0 = pl.multiple_of(i * FB, FB)
        rn = pl.multiple_of(jnp.minimum(r0 + FB, S - FB), FB)
        slot = lax.rem(i, 2)
        nf = FH // FC
        nt = FC // 128
        nq = DH2 // OC
        acc = {}
        gs = {}

        def up(f, t):
            c0 = f * FC + t * 128
            c = _strassen_out([
                _dot(jnp.concatenate([_ld(h2_v, (slot, k, j), 0, HB) for j in range(DH2 // 128)], axis=1),
                     rhs(w1_v, T1_ROW, DH2, FH // 128, k, c0 // 128, 0, DH2)) for k in range(7)])
            b1a, b1b = bias_v[0:1, c0:c0 + 128], bias_v[0:1, FH + c0:FH + c0 + 128]
            gs[f, t] = _strassen_lhs(_gelu(c[0] + b1a), _gelu(c[1] + b1b), _gelu(c[2] + b1a), _gelu(c[3] + b1b))
            if t == nt - 1:
                gs[f] = [jnp.concatenate([gs[f, u][k] for u in range(nt)], axis=1).astype(BF16) for k in range(7)]

        def down(f, q):
            for k in range(7):
                y = _dot(gs[f][k], rhs(w2_v, T2_ROW, FH, DH2 // 128, k, q, f * FC, FC))
                acc[k, q] = y + acc[k, q] if f else y
            if f == nf - 1:
                c = _strassen_out([acc[k, q] for k in range(7)])
                for t in range(4):
                    k0, c0 = (t // 2) * HB, (t % 2) * DH2 + q * OC
                    y = (c[t] + bias_v[0:1, FF + c0:FF + c0 + OC]) * mod_v[0:1, 5 * D + c0:5 * D + c0 + OC]
                    out_v[pl.ds(r0 + k0, HB), c0:c0 + OC] = (resid1(r0, k0, HB, c0, OC) + y).astype(BF16)
                start(out_copy(i, q))

        for t in range(nt):
            up(0, t)
        w = 0
        for f in range(nf):
            for t in range(nt):
                if f + 1 < nf:
                    up(f + 1, t)
                if w < len(LNP) and LNP[w]:
                    ln2(1 - slot, rn, sum(LNP[:w]), LNP[w])
                w += 1
                for q in range(t * nq // nt, (t + 1) * nq // nt):
                    down(f, q)
        return carry

    with _scope("ffn"):
        lax.fori_loop(0, S // FB, ffn_body, 0)
    with _scope("wait_out"):
        for i in range(S // FB):
            for q in range(DH2 // OC):
                wait(out_copy(i, q))


@jax.jit
def pallas_adaLN_cond__memory_aug_recurrent_mem_tr__dense_activation_gelu__prompt_kernel(
    A_x, A_mem0, A_Wq, A_Wk, A_Wv, A_Wo, A_seg_len, B_x, B_w1, B_b1, B_w2, B_b2, c, w_mod,
):
    del A_seg_len, B_x
    assert A_x.shape == (1, S, D)
    hbm = pl.BlockSpec(memory_space=pl.ANY)
    out = pl.pallas_call(
        _kernel,
        out_shape=jax.ShapeDtypeStruct((S, D), BF16),
        in_specs=[hbm] * 12,
        out_specs=hbm,
        scratch_shapes=[
            pltpu.VMEM((NSEG, SEG, D), BF16),
            pltpu.VMEM((8, T0, 128), BF16),
            pltpu.VMEM((TPS, D), F32),
            pltpu.VMEM((2, 7, 4, FB // 2, 128), BF16),
            pltpu.VMEM((S, D), F32),
            pltpu.VMEM((D, 6 * D), BF16),
            pltpu.VMEM((8, 6 * D), F32),
            pltpu.VMEM((8, D), BF16),
            pltpu.VMEM((6 * NP, D // 2, 128), U32),
            pltpu.VMEM((8, H * DH // 2, 128), U32),
            pltpu.VMEM((FF // 128, D, 128), BF16),
            pltpu.VMEM((D // 128, FF, 128), BF16),
            pltpu.VMEM((LT_ROWS, 128), BF16),
            pltpu.VMEM((3 * NP, 64, 128), BF16),
            pltpu.VMEM((2, H, 48, 128), BF16),
            pltpu.VMEM((NP, 80, 128), BF16),
            pltpu.VMEM((80, 128), F32),
            pltpu.VMEM((S, D), BF16),
            pltpu.VMEM((1, FF + D), F32),
            pltpu.VMEM((8, T0, 128), F32),
            pltpu.VMEM((M, D), BF16),
            pltpu.VMEM((FF,), BF16),
            pltpu.VMEM((D,), BF16),
            pltpu.VMEM((1, D), BF16),
            pltpu.VMEM((5, 4, T0 // 2, 128), BF16),
            pltpu.SemaphoreType.DMA((SEM_N,)),
        ],
        compiler_params=pltpu.CompilerParams(vmem_limit_bytes=120 * 1024 * 1024, disable_bounds_checks=True,
                                             disable_semaphore_checks=True),
    )(
        A_x.reshape(NSEG, SEG, D), A_mem0.reshape(M, D),
        A_Wq.reshape(D // 2, 2, H, DH), A_Wk.reshape(D // 2, 2, H, DH), A_Wv.reshape(D // 2, 2, H, DH),
        A_Wo.reshape(H * DH, D), B_w1, B_b1, B_w2, B_b2, c, w_mod,
    )
    return out.reshape(1, S, D)
```

```python
import contextlib

import jax
import jax.numpy as jnp
from jax import lax
import jax.experimental.pallas as pl
import jax.experimental.pallas.tpu as pltpu

F32 = jnp.float32
BF16 = jnp.bfloat16
U32 = jnp.uint32

S = 2048
D = 1024
H = 32
DH = 128
M = 8
SEG = 32
FF = 3584
NSEG = S // SEG
NP = H // 2
TPS = 24
T0 = S - NSEG * TPS
EPS = 1e-5
P1ORD = (1, 4, 3, 2, 0, 6, 5)
UPORD = (1, 4, 3, 2, 0, 6, 5)
DNORD = (1, 4, 3, 2, 0, 6, 5)
NEARLY = 4
PA = 4
LNP = (16,) * 8
MODPOS = ((5, 0, 24), (6, 0, 24))
LOG2E = 1.4426950408889634
FB = 256
OC = 128
FC = 256
FH = FF // 2
DH2 = D // 2
T1_ROW = 3 * NP * 2 * T0
T2_ROW = T1_ROW + 5 * (FH // 128) * DH2
LT_ROWS = T2_ROW + 5 * (DH2 // 128) * FH
SSUM = (0, 1, 4, 5, 6)
TSUM = (0, 2, 3, 5, 6)
SEM_W, SEM_A, SEM_M, SEM_MISC, SEM_OUT = 0, 16, 24, 32, 40
SEM_N = SEM_OUT + S // FB


def _make_sched(g):
    out = []

    def rng(a, b):
        return tuple(range(max(a, 0), max(b, 0)))

    for p in range(NP):
        out.append(("proj", p))
        if p % g == 0 and p >= g:
            out.append(("attn", rng(p - 2 * g, p - g), rng(p - g, p)))
    h1 = 2 * (NP - 2 * g)
    h2 = 2 * (NP - g)
    if g == 4:
        out += [("wo", j, 0, h1) for j in (0, 1)]
        out.append(("attn", rng(NP - 2 * g, NP - g), rng(NP - g, NP)))
        out += [("wo", j, 0, h1) for j in (2, 3, 4, 5)]
        out.append(("attn", rng(NP - g, NP), ()))
        out += [("wo", j, 0, h1) for j in (6, 7)]
        out += [("wo", j, h1, h2) for j in range(8)]
        out += [("wo", j, h2, H) for j in range(8)]
    else:
        out += [("wo", 0, 0, h1)]
        out.append(("attn", rng(NP - 2 * g, NP - g), rng(NP - g, NP)))
        out += [("wo", j, 0, h1) for j in (1, 2, 3)]
        out.append(("attn", rng(NP - g, NP), ()))
        out += [("wo", j, 0, h1) for j in (4, 5, 6, 7)]
        out += [("wo", j, h1, H) for j in range(8)]
    return out


SCHED = _make_sched(2)
_SCOPES = False


def _scope(name):
    return jax.named_scope(name) if _SCOPES else contextlib.nullcontext()


def _dot(a, b):
    return jnp.dot(a, b, preferred_element_type=F32)


def _bf(x):
    return pltpu.bitcast(x, BF16)


def _u32(x):
    return pltpu.bitcast(x, U32)


def _ld(ref, idx, r0, n):
    return _bf(ref.bitcast(U32)[(*idx, pl.ds(r0 // 2, n // 2), slice(None))])


def _ln(x):
    m = jnp.mean(x, axis=-1, keepdims=True)
    xc = x - m
    v = jnp.mean(xc * xc, axis=-1, keepdims=True)
    return xc * lax.rsqrt(v + EPS)


def _gelu(x):
    c = 0.7978845608028654
    return 0.5 * x * (1.0 + jnp.tanh(c * (x + 0.044715 * (x * x * x))))


def _strassen_lhs(a11, a12, a21, a22):
    return [a11 + a22, a21 + a22, a11, a22, a11 + a12, a21 - a11, a12 - a22]


def _strassen_rhs(b11, b12, b21, b22):
    return [b11 + b22, b11, b12 - b22, b21 - b11, b22, b11 + b12, b21 + b22]


def _strassen_out(m):
    return (m[0] + m[3] - m[4] + m[6], m[2] + m[4], m[1] + m[3], m[0] - m[1] + m[2] + m[5])


def _interleave(a, b):
    n = a.shape[0] // 8
    parts = []
    for g in range(n):
        parts.append(a[8 * g:8 * g + 8])
        parts.append(b[8 * g:8 * g + 8])
    return jnp.concatenate(parts, axis=0)


def _deinterleave(v):
    n = v.shape[0] // 16
    a = jnp.concatenate([v[16 * g:16 * g + 8] for g in range(n)], axis=0)
    b = jnp.concatenate([v[16 * g + 8:16 * g + 16] for g in range(n)], axis=0)
    return a, b


def _kernel(x_hbm, mem0_hbm, wq_hbm, wk_hbm, wv_hbm, wo_hbm, w1_hbm, b1_hbm, w2_hbm, b2_hbm,
            c_hbm, wmod_hbm, out_hbm,
            x_v, h_v, hn_v, h2_v, x1_v, wmod_v, mod_v, sc_v, w_v, wo_v, w1_v, w2_v, lt_v, fr_v, lo_v, pr_v, fill_v, out_v, bias_v, n_v,
            mem0_ref, b1_ref, b2_ref, c_ref, hs_v,
            sems):
    w32 = [r.bitcast(U32) for r in (wq_hbm, wk_hbm, wv_hbm)]
    wo32 = wo_hbm.bitcast(U32)

    def w_copies(p):
        return [pltpu.make_async_copy(w32[j].at[:, par, p, :], w_v.at[p * 6 + j * 2 + par], sems.at[SEM_W + p])
                for j in range(3) for par in range(2)]

    def _mult(i, m):
        return i * m if isinstance(i, int) else pl.multiple_of(i * m, m)

    def wa_copies(k, pair=None):
        r = pl.ds(_mult(k, 64), 64)
        return [pltpu.make_async_copy(w32[j].at[r, par, p, :], w_v.at[p * 6 + j * 2 + par, r], sems.at[SEM_A + k])
                for p in (range(PA) if pair is None else (pair,)) for j in range(3) for par in range(2)]

    def m_copies(k):
        cols = [pl.ds(_mult(k + 8 * t, 128), 128) for t in range(2)]
        return [pltpu.make_async_copy(wmod_hbm.at[:, cs], wmod_v.at[:, cs], sems.at[SEM_M + k]) for cs in cols]

    def start(cps):
        for cp in cps:
            cp.start()

    def wait(cps):
        for cp in cps:
            cp.wait()

    cp_x0 = pltpu.make_async_copy(x_hbm.at[:, 0:8, :], x_v.at[:, 0:8, :], sems.at[SEM_MISC + 1])

    def wo_copy(j):
        return pltpu.make_async_copy(wo32.at[:, pl.ds(_mult(j, 128), 128)], wo_v.at[j], sems.at[SEM_MISC + 3])

    def late_copies(first):
        sem = sems.at[SEM_MISC + (4 if first else 5)]
        cs = pl.ds(2 * D, NEARLY * 128) if first else pl.ds(2 * D + NEARLY * 128, 4 * D - NEARLY * 128)
        sg = slice(1, 2 * NEARLY + 1) if first else slice(2 * NEARLY + 1, NSEG)
        cps = [(x_hbm.at[sg, 8:SEG, :], x_v.at[sg, 8:SEG, :]), (wmod_hbm.at[:, cs], wmod_v.at[:, cs])]
        for src, dst, nt, kh in ((w1_hbm, w1_v, FF // 128, DH2), (w2_hbm, w2_v, D // 128, FH)):
            for j in range(nt):
                cols = slice(j * 128, (j + 1) * 128)
                if j % (nt // 2):
                    rows = [] if first else [slice(None)]
                else:
                    rows = [slice(a * kh, a * kh + 256) if first else slice(a * kh + 256, (a + 1) * kh)
                            for a in range(2)]
                cps += [(src.at[r, cols], dst.at[j, r]) for r in rows]
        return [pltpu.make_async_copy(src, dst, sem) for src, dst in cps]

    cp_small = [pltpu.make_async_copy(src, dst, sems.at[SEM_MISC])
                for src, dst in ((c_hbm, c_ref), (mem0_hbm, mem0_ref), (b1_hbm, b1_ref), (b2_hbm, b2_ref),
                                 (x_hbm.at[0, 8:SEG, :], x_v.at[0, 8:SEG, :]))]

    start(cp_small)
    cp_x0.start()
    start(m_copies(0))
    for k in range(2):
        start(m_copies(k + 1))
        start(wa_copies(k))

    scale = DH ** -0.5
    ri = lax.broadcasted_iota(jnp.int32, (80, 128), 0)
    ci = lax.broadcasted_iota(jnp.int32, (80, 128), 1)
    same_head = (((ri >> 3) & 1) == ((ci >> 3) & 1)) & (ci < 80)
    rpos = (((ri >> 4) & 3) << 3) + (ri & 7)
    cpos = (((ci >> 4) & 3) << 3) + (ci & 7)
    keep = (ri < 16) | (ci < 16) | (rpos >= cpos)
    fill_v[...] = jnp.where(same_head, jnp.where(keep, 0.0, -1e9 / scale), -jnp.inf).astype(F32)

    wait(cp_small)
    c = c_ref[...].astype(F32)
    sc = jnp.broadcast_to(c * jax.nn.sigmoid(c), (8, D)).astype(BF16)

    sc_v[...] = sc
    bias_v[:, 0:FF] = b1_ref[...].astype(F32).reshape(1, FF)
    bias_v[:, FF:FF + D] = b2_ref[...].astype(F32).reshape(1, D)

    def zero_body(i, carry):
        x1_v[pl.ds(pl.multiple_of(i * 64, 64), 64), :] = jnp.zeros((64, D), F32)
        return carry

    lax.fori_loop(0, PA * 6, zero_body, 0)

    def relayout(c, rows):
        a = w_v[c, rows, :]
        b = w_v[c + 1, rows, :]
        lo = (a & jnp.uint32(0xFFFF)) | (b << 16)
        hi = (a >> 16) | (b & jnp.uint32(0xFFFF0000))
        w_v[c, rows, :] = lo
        w_v[c + 1, rows, :] = hi
        return _bf(lo), _bf(hi)

    def store_lead(p, j, a, b):
        lt_v[pl.ds(_mult(p * 3 + j, 2 * T0), 2 * T0), :] = _interleave(a, b).astype(BF16)

    def mod_tile(ct):
        cs = pl.ds(_mult(ct, 128), 128)
        m = _dot(sc_v[...], wmod_v[:, cs])
        mod_v[:, cs] = m
        return m[0:1]

    with _scope("wait_x0"):
        cp_x0.wait()

    def ln1_body(i, carry):
        r = pl.multiple_of(i * 128, 128)
        n = _ln(x_v[pl.ds(i * 16, 16), 0:8, :].astype(F32).reshape(128, D))
        for k in range(8):
            n_v[k, pl.ds(r, 128), :] = n[:, k * 128:(k + 1) * 128]
        return carry

    with _scope("ln1"):
        lax.fori_loop(0, T0 // 128, ln1_body, 0)
    start(m_copies(3))
    start(wa_copies(2))
    with _scope("wait_m0"):
        wait(m_copies(0))
    h_v[0] = (n_v[0] * (1.0 + mod_tile(8)) + mod_tile(0)).astype(BF16)

    def sa_body(k, carry):
        with _scope("wait_a"):
            wait(wa_copies(k))

            @pl.when(k < 7)
            def _():
                wait(m_copies(k + 1))

        kn = jnp.minimum(k + 1, 7)
        rows = pl.ds(pl.multiple_of(k * 64, 64), 64)
        hk = _ld(h_v, (k,), 0, T0)
        for p in range(PA):
            for j in range(3):
                c = p * 6 + j * 2
                res = []
                for t, w in enumerate(relayout(c, rows)):
                    acc = x1_v.at[(c + t) // 8 * T0:((c + t) // 8 + 1) * T0,
                                  (c + t) % 8 * 128:((c + t) % 8 + 1) * 128]
                    r = _dot(hk, w) + acc[...]
                    acc[...] = r
                    res.append(r)
                store_lead(p, j, *res)
                if c == 2:
                    sh = mod_tile(kn)
                if c == 6:
                    s1 = 1.0 + mod_tile(kn + 8)

                    @pl.when(k + 4 < 8)
                    def _():
                        start(m_copies(k + 4))

            @pl.when(k + 3 < 8)
            def _():
                start(wa_copies(k + 3, p))

        h_v[kn] = (n_v[kn] * s1 + sh).astype(BF16)


        @pl.when(k >= 4)
        def _():
            start(w_copies(PA + k - 4))

        return carry

    with _scope("stageA"):
        lax.fori_loop(0, 8, sa_body, 0)

    def ln1(seg):
        xb = x_v[seg, 8:SEG, :].astype(F32)
        return _ln(xb) * (1.0 + mod_v[0:1, D:2 * D]) + mod_v[0:1, 0:D]

    TH = T0 // 2
    for t in range(4):
        ha, hb = h_v[t].astype(F32), h_v[t + 4].astype(F32)
        ss = _strassen_lhs(ha[0:TH], hb[0:TH], ha[TH:T0], hb[TH:T0])
        for k, i in enumerate(SSUM):
            hs_v[k, t] = ss[i].astype(BF16)

    def lhs1(i):
        if i == 2:
            tiles = [_ld(h_v, (t,), 0, TH) for t in range(4)]
        elif i == 3:
            tiles = [_ld(h_v, (t + 4,), TH, TH) for t in range(4)]
        else:
            tiles = [_ld(hs_v, (SSUM.index(i), t), 0, TH) for t in range(4)]
        return jnp.concatenate(tiles, axis=1)

    def p1_body(i, carry):
        p0 = PA + 2 * i
        with _scope("wait_w"):
            wait(w_copies(p0) + w_copies(p0 + 1))

        for u in range(6):
            p, j = p0 + u // 3, u % 3
            lo, hi = relayout(p * 6 + j * 2, slice(None))
            b = [lo[0:DH2], hi[0:DH2], lo[DH2:D], hi[DH2:D]]
            t = _strassen_rhs(*[x.astype(F32) for x in b])
            t = [b[0] if k == 1 else b[3] if k == 4 else t[k].astype(BF16) for k in range(7)]
            m = {k: _dot(lhs1(k), t[k]) for k in P1ORD}
            c = _strassen_out(m)
            store_lead(p, j, jnp.concatenate([c[0], c[2]], axis=0), jnp.concatenate([c[1], c[3]], axis=0))

            if u < 4:
                @pl.when(i < 2)
                def _():
                    start(w_copies(PA + 4 + 4 * i + u))
            elif u == 4:
                @pl.when(jnp.logical_and(i >= 1, i < 3))
                def _():
                    start([wo_copy(4 * (i - 1) + q) for q in range(4)])
            else:
                @pl.when(i == 2)
                def _():
                    start(late_copies(True))

        hn_v[...] = ln1(0)
        return carry

    with _scope("phase1"):
        lax.fori_loop(0, (NP - PA) // 2, p1_body, 0)

    with _scope("wait_wo"):
        wait([wo_copy(j) for j in range(8)])
        wait(late_copies(True))
    start(late_copies(False))

    def prep_views(w, t_row, kh, nh, j, r0):
        src = w.at[pl.ds(j, nh + 1), pl.ds(pl.multiple_of(r0, 256), kh + 256), :]
        dst = lt_v.at[pl.ds(pl.multiple_of(t_row + j * kh + r0, 256), 4 * nh * kh + 256), :]
        return src, dst, kh, nh

    def prep(views, r0, n):
        src, dst, kh, nh = views
        t = _strassen_rhs(*[_ld(src, (b * nh,), a * kh + r0, n).astype(F32) for a in range(2) for b in range(2)])
        for k, i in enumerate(TSUM):
            dst[k * nh * kh + r0:k * nh * kh + r0 + n, :] = t[i].astype(BF16)

    def step(it, odd, mem):
        s = 2 * it + int(odd)
        lead = lt_v.at[pl.ds(pl.multiple_of(16 * s, 16), T1_ROW), :]
        lhs = jnp.concatenate([mem, hn_v[...]], axis=0).astype(BF16)
        hn_v[...] = ln1(jnp.minimum(s + 1, NSEG - 1))
        mo = 48 if odd else 32

        def proj(p):
            if p == 0:
                half = [_dot(lhs[:, 0:D // 2], _bf(w_v[c, 0:D // 4, :])) for c in range(6)]
                cols = [_dot(lhs[:, D // 2:D], _bf(w_v[c, D // 4:D // 2, :])) + half[c] for c in range(6)]
            for j in range(3):
                if p == 0:
                    r = _interleave(cols[j * 2], cols[j * 2 + 1])
                else:
                    r = _interleave(_dot(lhs, _bf(w_v[p * 6 + j * 2])), _dot(lhs, _bf(w_v[p * 6 + j * 2 + 1])))
                fr_v[p * 3 + j] = r.astype(BF16)

        def stack(p, j):
            return jnp.concatenate([fr_v[p * 3 + j],
                                    _ld(lead, (), (p * 3 + j) * 2 * T0, 16)], axis=0)

        def attn(pvs, qks):
            os_ = [_dot(pr_v[p, :, 0:80], stack(p, 2)) for p in pvs]
            ss = [lax.dot_general(stack(p, 0), stack(p, 1), (((1,), (1,)), ((), ())),
                                  preferred_element_type=F32) for p in qks]
            for p, o in zip(pvs, os_):
                for t, oh in enumerate(_deinterleave(o)):
                    h = 2 * p + t
                    if odd:
                        lo_v[1, h, 0:8, :] = oh[0:8].astype(BF16)
                        lo_v[1, h, 16:48, :] = oh[8:40].astype(BF16)
                    else:
                        lo_v[0, h, 0:32, :] = oh[0:32].astype(BF16)
                        lo_v[1, h, 8:16, :] = oh[32:40].astype(BF16)
            for p, sc_ in zip(qks, ss):
                fill = fill_v[...]
                sc_ = jnp.concatenate([sc_, jnp.zeros((80, 48), F32)], axis=1)
                sc_ = jnp.where(fill == 0.0, sc_, fill)
                mx = jnp.max(sc_, axis=-1, keepdims=True)
                e = jnp.exp2((sc_ - mx) * (scale * LOG2E))
                l = jnp.sum(e, axis=-1, keepdims=True)
                r = pl.reciprocal(l, approx=True)
                pr_v[p] = (e * (r * (2.0 - l * r))).astype(BF16)

        part = {}

        def wo(j, h0, h1):
            lo = jnp.concatenate([lo_v[int(odd), h, 0:mo, :] for h in range(h0, h1)], axis=1)
            r = _dot(lo, _bf(wo_v[j, h0 * 64:h1 * 64, :]))
            part[j] = r + part[j] if j in part else r

        pc = jnp.maximum(it - 4, 0)
        if odd:
            views = prep_views(w2_v, T2_ROW, FH, DH2 // 128, lax.div(pc, 7), lax.rem(pc, 7) * 256)
        else:
            views = prep_views(w1_v, T1_ROW, DH2, FH // 128, pc >> 1, (pc & 1) * 256)
        npiece = 0
        for op in SCHED:
            if op[0] == "proj":
                proj(op[1])
            elif op[0] == "attn":
                attn(op[1], op[2])
                if npiece < 8:
                    prep(views, npiece * 32, 32)
                    npiece += 1
            else:
                wo(*op[1:])
                if odd and op[1:] in MODPOS:
                    cs = pl.ds(pl.multiple_of((16 + it) * 128, 128), 128)
                    k0 = MODPOS.index(op[1:]) * (D // 2)
                    m = _dot(sc_v[:, k0:k0 + D // 2], wmod_v[k0:k0 + D // 2, cs])
                    if k0 == 0:
                        mhalf = m
                    else:
                        mod_v[:, cs] = m + mhalf
        res = jnp.concatenate([part[j] for j in range(8)], axis=1)
        t0 = pl.multiple_of(SEG * s, SEG)
        if odd:
            x1_v[pl.ds(t0 - SEG, 8), :] = res[8:16]
            x1_v[pl.ds(t0, SEG), :] = jnp.concatenate([res[40:48], res[16:40]], axis=0)
        else:
            x1_v[pl.ds(t0 + 8, TPS), :] = res[8:32]
        return res[0:8]

    with _scope("main"):
        def steps(i, mem):
            with _scope("iter"):
                mem = step(i, True, step(i, False, mem))

            @pl.when(i == NEARLY - 1)
            def _():
                wait(late_copies(False))

            return mem

        lax.fori_loop(0, NSEG // 2, steps, mem0_ref[...].astype(F32))

    def rhs(w, t_row, kh, nh, i, j, k0, nk):
        if i == 1:
            return _ld(w, (j,), k0, nk)
        if i == 4:
            return _ld(w, (j + nh,), kh + k0, nk)
        return _ld(lt_v, (), t_row + (TSUM.index(i) * nh + j) * kh + k0, nk)

    def out_copy(i, q):
        rows = pl.ds(_mult(i, FB), FB)
        return [pltpu.make_async_copy(out_v.at[rows, cols], out_hbm.at[rows, cols], sems.at[SEM_OUT + i])
                for cols in (pl.ds(q * OC, OC), pl.ds(DH2 + q * OC, OC))]

    HB = FB // 2

    def resid1(r0, k0, n, c0=0, nc=D):
        if n >= SEG:
            xb = x_v[pl.ds((r0 >> 5) + k0 // SEG, n // SEG), :, c0:c0 + nc].astype(F32).reshape(n, nc)
        else:
            xb = x_v[(r0 >> 5) + k0 // SEG, k0 % SEG:k0 % SEG + n, c0:c0 + nc].astype(F32)
        return xb + mod_v[0:1, 2 * D + c0:2 * D + c0 + nc] * x1_v[pl.ds(r0 + k0, n), c0:c0 + nc]

    def ln2(slot, r0, k0, n):
        top, bot = [_ln(resid1(r0, t * HB + k0, n)) * (1.0 + mod_v[0:1, 4 * D:5 * D]) + mod_v[0:1, 3 * D:4 * D]
                    for t in range(2)]
        ss = _strassen_lhs(top[:, 0:DH2], top[:, DH2:D], bot[:, 0:DH2], bot[:, DH2:D])
        for i in range(7):
            for j in range(DH2 // 128):
                h2_v[slot, i, j, k0:k0 + n, :] = ss[i][:, j * 128:(j + 1) * 128].astype(BF16)

    ln2(0, 0, 0, HB)

    def ffn_body(i, carry):
        r0 = pl.multiple_of(i * FB, FB)
        rn = pl.multiple_of(jnp.minimum(r0 + FB, S - FB), FB)
        slot = lax.rem(i, 2)
        nf = FH // FC
        nt = FC // 128
        nq = DH2 // OC
        acc = {}
        gs = {}

        def up(f, t):
            c0 = f * FC + t * 128
            c = _strassen_out({
                k: _dot(jnp.concatenate([_ld(h2_v, (slot, k, j), 0, HB) for j in range(DH2 // 128)], axis=1),
                        rhs(w1_v, T1_ROW, DH2, FH // 128, k, c0 // 128, 0, DH2)) for k in UPORD})
            b1a, b1b = bias_v[0:1, c0:c0 + 128], bias_v[0:1, FH + c0:FH + c0 + 128]
            gs[f, t] = _strassen_lhs(_gelu(c[0] + b1a), _gelu(c[1] + b1b), _gelu(c[2] + b1a), _gelu(c[3] + b1b))
            if t == nt - 1:
                gs[f] = [jnp.concatenate([gs[f, u][k] for u in range(nt)], axis=1).astype(BF16) for k in range(7)]

        def down(f, q):
            for k in DNORD:
                y = _dot(gs[f][k], rhs(w2_v, T2_ROW, FH, DH2 // 128, k, q, f * FC, FC))
                acc[k, q] = y + acc[k, q] if f else y
            if f == nf - 1:
                c = _strassen_out([acc[k, q] for k in range(7)])
                for t in range(4):
                    k0, c0 = (t // 2) * HB, (t % 2) * DH2 + q * OC
                    y = (c[t] + bias_v[0:1, FF + c0:FF + c0 + OC]) * mod_v[0:1, 5 * D + c0:5 * D + c0 + OC]
                    out_v[pl.ds(r0 + k0, HB), c0:c0 + OC] = (resid1(r0, k0, HB, c0, OC) + y).astype(BF16)
                start(out_copy(i, q))

        for t in range(nt):
            up(0, t)
        w = 0
        for f in range(nf):
            for t in range(nt):
                if f + 1 < nf:
                    up(f + 1, t)
                if w < len(LNP) and LNP[w]:
                    ln2(1 - slot, rn, sum(LNP[:w]), LNP[w])
                w += 1
                for q in range(t * nq // nt, (t + 1) * nq // nt):
                    down(f, q)
        return carry

    with _scope("ffn"):
        lax.fori_loop(0, S // FB, ffn_body, 0)
    with _scope("wait_out"):
        for i in range(S // FB):
            for q in range(DH2 // OC):
                wait(out_copy(i, q))


@jax.jit
def pallas_adaLN_cond__memory_aug_recurrent_mem_tr__dense_activation_gelu__prompt_kernel(
    A_x, A_mem0, A_Wq, A_Wk, A_Wv, A_Wo, A_seg_len, B_x, B_w1, B_b1, B_w2, B_b2, c, w_mod,
):
    del A_seg_len, B_x
    assert A_x.shape == (1, S, D)
    hbm = pl.BlockSpec(memory_space=pl.ANY)
    out = pl.pallas_call(
        _kernel,
        out_shape=jax.ShapeDtypeStruct((S, D), BF16),
        in_specs=[hbm] * 12,
        out_specs=hbm,
        scratch_shapes=[
            pltpu.VMEM((NSEG, SEG, D), BF16),
            pltpu.VMEM((8, T0, 128), BF16),
            pltpu.VMEM((TPS, D), F32),
            pltpu.VMEM((2, 7, 4, FB // 2, 128), BF16),
            pltpu.VMEM((S, D), F32),
            pltpu.VMEM((D, 6 * D), BF16),
            pltpu.VMEM((8, 6 * D), F32),
            pltpu.VMEM((8, D), BF16),
            pltpu.VMEM((6 * NP, D // 2, 128), U32),
            pltpu.VMEM((8, H * DH // 2, 128), U32),
            pltpu.VMEM((FF // 128, D, 128), BF16),
            pltpu.VMEM((D // 128, FF, 128), BF16),
            pltpu.VMEM((LT_ROWS, 128), BF16),
            pltpu.VMEM((3 * NP, 64, 128), BF16),
            pltpu.VMEM((2, H, 48, 128), BF16),
            pltpu.VMEM((NP, 80, 128), BF16),
            pltpu.VMEM((80, 128), F32),
            pltpu.VMEM((S, D), BF16),
            pltpu.VMEM((1, FF + D), F32),
            pltpu.VMEM((8, T0, 128), F32),
            pltpu.VMEM((M, D), BF16),
            pltpu.VMEM((FF,), BF16),
            pltpu.VMEM((D,), BF16),
            pltpu.VMEM((1, D), BF16),
            pltpu.VMEM((5, 4, T0 // 2, 128), BF16),
            pltpu.SemaphoreType.DMA((SEM_N,)),
        ],
        compiler_params=pltpu.CompilerParams(vmem_limit_bytes=120 * 1024 * 1024, disable_bounds_checks=True,
                                             disable_semaphore_checks=True),
    )(
        A_x.reshape(NSEG, SEG, D), A_mem0.reshape(M, D),
        A_Wq.reshape(D // 2, 2, H, DH), A_Wk.reshape(D // 2, 2, H, DH), A_Wv.reshape(D // 2, 2, H, DH),
        A_Wo.reshape(H * DH, D), B_w1, B_b1, B_w2, B_b2, c, w_mod,
    )
    return out.reshape(1, S, D)
```

```python
import contextlib

import jax
import jax.numpy as jnp
from jax import lax
import jax.experimental.pallas as pl
import jax.experimental.pallas.tpu as pltpu

F32 = jnp.float32
BF16 = jnp.bfloat16
U32 = jnp.uint32

S = 2048
D = 1024
H = 32
DH = 128
M = 8
SEG = 32
FF = 3584
NSEG = S // SEG
NP = H // 2
TPS = 24
T0 = S - NSEG * TPS
EPS = 1e-5
P1U = 2
P1ORD = (1, 4, 3, 2, 0, 6, 5)
UPORD = (1, 4, 3, 2, 0, 6, 5)
DNORD = (1, 4, 3, 2, 0, 6, 5)
NEARLY = 4
PA = 4
LNP = (16,) * 8
MODPOS = ((5, 0, 24), (6, 0, 24))
LOG2E = 1.4426950408889634
FB = 256
OC = 128
FC = 256
FH = FF // 2
DH2 = D // 2
T1_ROW = 3 * NP * 2 * T0
T2_ROW = T1_ROW + 5 * (FH // 128) * DH2
LT_ROWS = T2_ROW + 5 * (DH2 // 128) * FH
SSUM = (0, 1, 4, 5, 6)
TSUM = (0, 2, 3, 5, 6)
SEM_W, SEM_A, SEM_M, SEM_MISC, SEM_OUT = 0, 16, 24, 32, 40
SEM_N = SEM_OUT + S // FB


def _make_sched(g):
    out = []

    def rng(a, b):
        return tuple(range(max(a, 0), max(b, 0)))

    for p in range(NP):
        out.append(("proj", p))
        if p % g == 0 and p >= g:
            out.append(("attn", rng(p - 2 * g, p - g), rng(p - g, p)))
    h1 = 2 * (NP - 2 * g)
    h2 = 2 * (NP - g)
    if g == 4:
        out += [("wo", j, 0, h1) for j in (0, 1)]
        out.append(("attn", rng(NP - 2 * g, NP - g), rng(NP - g, NP)))
        out += [("wo", j, 0, h1) for j in (2, 3, 4, 5)]
        out.append(("attn", rng(NP - g, NP), ()))
        out += [("wo", j, 0, h1) for j in (6, 7)]
        out += [("wo", j, h1, h2) for j in range(8)]
        out += [("wo", j, h2, H) for j in range(8)]
    else:
        out += [("wo", 0, 0, h1)]
        out.append(("attn", rng(NP - 2 * g, NP - g), rng(NP - g, NP)))
        out += [("wo", j, 0, h1) for j in (1, 2, 3)]
        out.append(("attn", rng(NP - g, NP), ()))
        out += [("wo", j, 0, h1) for j in (4, 5, 6, 7)]
        out += [("wo", j, h1, H) for j in range(8)]
    return out


SCHED = _make_sched(2)
_SCOPES = False


def _scope(name):
    return jax.named_scope(name) if _SCOPES else contextlib.nullcontext()


def _dot(a, b):
    return jnp.dot(a, b, preferred_element_type=F32)


def _bf(x):
    return pltpu.bitcast(x, BF16)


def _u32(x):
    return pltpu.bitcast(x, U32)


def _ld(ref, idx, r0, n):
    return _bf(ref.bitcast(U32)[(*idx, pl.ds(r0 // 2, n // 2), slice(None))])


def _ln(x):
    m = jnp.mean(x, axis=-1, keepdims=True)
    xc = x - m
    v = jnp.mean(xc * xc, axis=-1, keepdims=True)
    return xc * lax.rsqrt(v + EPS)


def _gelu(x):
    c = 0.7978845608028654
    return 0.5 * x * (1.0 + jnp.tanh(c * (x + 0.044715 * (x * x * x))))


def _strassen_lhs(a11, a12, a21, a22):
    return [a11 + a22, a21 + a22, a11, a22, a11 + a12, a21 - a11, a12 - a22]


def _strassen_rhs(b11, b12, b21, b22):
    return [b11 + b22, b11, b12 - b22, b21 - b11, b22, b11 + b12, b21 + b22]


def _strassen_out(m):
    return (m[0] + m[3] - m[4] + m[6], m[2] + m[4], m[1] + m[3], m[0] - m[1] + m[2] + m[5])


def _interleave(a, b):
    n = a.shape[0] // 8
    parts = []
    for g in range(n):
        parts.append(a[8 * g:8 * g + 8])
        parts.append(b[8 * g:8 * g + 8])
    return jnp.concatenate(parts, axis=0)


def _deinterleave(v):
    n = v.shape[0] // 16
    a = jnp.concatenate([v[16 * g:16 * g + 8] for g in range(n)], axis=0)
    b = jnp.concatenate([v[16 * g + 8:16 * g + 16] for g in range(n)], axis=0)
    return a, b


def _kernel(x_hbm, mem0_hbm, wq_hbm, wk_hbm, wv_hbm, wo_hbm, w1_hbm, b1_hbm, w2_hbm, b2_hbm,
            c_hbm, wmod_hbm, out_hbm,
            x_v, h_v, hn_v, h2_v, x1_v, wmod_v, mod_v, sc_v, w_v, wo_v, w1_v, w2_v, lt_v, fr_v, lo_v, pr_v, fill_v, out_v, bias_v, n_v,
            mem0_ref, b1_ref, b2_ref, c_ref, hs_v,
            sems):
    w32 = [r.bitcast(U32) for r in (wq_hbm, wk_hbm, wv_hbm)]
    wo32 = wo_hbm.bitcast(U32)

    def w_copies(p):
        return [pltpu.make_async_copy(w32[j].at[:, par, p, :], w_v.at[p * 6 + j * 2 + par], sems.at[SEM_W + p])
                for j in range(3) for par in range(2)]

    def _mult(i, m):
        return i * m if isinstance(i, int) else pl.multiple_of(i * m, m)

    def wa_copies(k, pair=None):
        r = pl.ds(_mult(k, 64), 64)
        return [pltpu.make_async_copy(w32[j].at[r, par, p, :], w_v.at[p * 6 + j * 2 + par, r], sems.at[SEM_A + k])
                for p in (range(PA) if pair is None else (pair,)) for j in range(3) for par in range(2)]

    def m_copies(k):
        cols = [pl.ds(_mult(k + 8 * t, 128), 128) for t in range(2)]
        return [pltpu.make_async_copy(wmod_hbm.at[:, cs], wmod_v.at[:, cs], sems.at[SEM_M + k]) for cs in cols]

    def start(cps):
        for cp in cps:
            cp.start()

    def wait(cps):
        for cp in cps:
            cp.wait()

    cp_x0 = pltpu.make_async_copy(x_hbm.at[:, 0:8, :], x_v.at[:, 0:8, :], sems.at[SEM_MISC + 1])

    def wo_copy(j):
        return pltpu.make_async_copy(wo32.at[:, pl.ds(_mult(j, 128), 128)], wo_v.at[j], sems.at[SEM_MISC + 3])

    def late_copies(first):
        sem = sems.at[SEM_MISC + (4 if first else 5)]
        cs = pl.ds(2 * D, NEARLY * 128) if first else pl.ds(2 * D + NEARLY * 128, 4 * D - NEARLY * 128)
        sg = slice(1, 2 * NEARLY + 1) if first else slice(2 * NEARLY + 1, NSEG)
        cps = [(x_hbm.at[sg, 8:SEG, :], x_v.at[sg, 8:SEG, :]), (wmod_hbm.at[:, cs], wmod_v.at[:, cs])]
        for src, dst, nt, kh in ((w1_hbm, w1_v, FF // 128, DH2), (w2_hbm, w2_v, D // 128, FH)):
            for j in range(nt):
                cols = slice(j * 128, (j + 1) * 128)
                if j % (nt // 2):
                    rows = [] if first else [slice(None)]
                else:
                    rows = [slice(a * kh, a * kh + 256) if first else slice(a * kh + 256, (a + 1) * kh)
                            for a in range(2)]
                cps += [(src.at[r, cols], dst.at[j, r]) for r in rows]
        return [pltpu.make_async_copy(src, dst, sem) for src, dst in cps]

    cp_small = [pltpu.make_async_copy(src, dst, sems.at[SEM_MISC])
                for src, dst in ((c_hbm, c_ref), (mem0_hbm, mem0_ref), (b1_hbm, b1_ref), (b2_hbm, b2_ref),
                                 (x_hbm.at[0, 8:SEG, :], x_v.at[0, 8:SEG, :]))]

    start(cp_small)
    cp_x0.start()
    start(m_copies(0))
    for k in range(2):
        start(m_copies(k + 1))
        start(wa_copies(k))

    scale = DH ** -0.5
    ri = lax.broadcasted_iota(jnp.int32, (80, 128), 0)
    ci = lax.broadcasted_iota(jnp.int32, (80, 128), 1)
    same_head = (((ri >> 3) & 1) == ((ci >> 3) & 1)) & (ci < 80)
    rpos = (((ri >> 4) & 3) << 3) + (ri & 7)
    cpos = (((ci >> 4) & 3) << 3) + (ci & 7)
    keep = (ri < 16) | (ci < 16) | (rpos >= cpos)
    fill_v[...] = jnp.where(same_head, jnp.where(keep, 0.0, -1e9 / scale), -jnp.inf).astype(F32)

    wait(cp_small)
    c = c_ref[...].astype(F32)
    sc = jnp.broadcast_to(c * jax.nn.sigmoid(c), (8, D)).astype(BF16)

    sc_v[...] = sc
    bias_v[:, 0:FF] = b1_ref[...].astype(F32).reshape(1, FF)
    bias_v[:, FF:FF + D] = b2_ref[...].astype(F32).reshape(1, D)

    def zero_body(i, carry):
        x1_v[pl.ds(pl.multiple_of(i * 64, 64), 64), :] = jnp.zeros((64, D), F32)
        return carry

    lax.fori_loop(0, PA * 6, zero_body, 0)

    def relayout(c, rows):
        a = w_v[c, rows, :]
        b = w_v[c + 1, rows, :]
        lo = (a & jnp.uint32(0xFFFF)) | (b << 16)
        hi = (a >> 16) | (b & jnp.uint32(0xFFFF0000))
        w_v[c, rows, :] = lo
        w_v[c + 1, rows, :] = hi
        return _bf(lo), _bf(hi)

    def store_lead(p, j, a, b):
        lt_v[pl.ds(_mult(p * 3 + j, 2 * T0), 2 * T0), :] = _interleave(a, b).astype(BF16)

    def mod_tile(ct):
        cs = pl.ds(_mult(ct, 128), 128)
        m = _dot(sc_v[...], wmod_v[:, cs])
        mod_v[:, cs] = m
        return m[0:1]

    with _scope("wait_x0"):
        cp_x0.wait()

    def ln1_body(i, carry):
        r = pl.multiple_of(i * 128, 128)
        n = _ln(x_v[pl.ds(i * 16, 16), 0:8, :].astype(F32).reshape(128, D))
        for k in range(8):
            n_v[k, pl.ds(r, 128), :] = n[:, k * 128:(k + 1) * 128]
        return carry

    with _scope("ln1"):
        lax.fori_loop(0, T0 // 128, ln1_body, 0)
    start(m_copies(3))
    start(wa_copies(2))
    with _scope("wait_m0"):
        wait(m_copies(0))
    h_v[0] = (n_v[0] * (1.0 + mod_tile(8)) + mod_tile(0)).astype(BF16)

    def sa_body(k, carry):
        with _scope("wait_a"):
            wait(wa_copies(k))

            @pl.when(k < 7)
            def _():
                wait(m_copies(k + 1))

        kn = jnp.minimum(k + 1, 7)
        rows = pl.ds(pl.multiple_of(k * 64, 64), 64)
        hk = _ld(h_v, (k,), 0, T0)
        for p in range(PA):
            for j in range(3):
                c = p * 6 + j * 2
                res = []
                for t, w in enumerate(relayout(c, rows)):
                    acc = x1_v.at[(c + t) // 8 * T0:((c + t) // 8 + 1) * T0,
                                  (c + t) % 8 * 128:((c + t) % 8 + 1) * 128]
                    r = _dot(hk, w) + acc[...]
                    acc[...] = r
                    res.append(r)
                store_lead(p, j, *res)
                if c == 2:
                    sh = mod_tile(kn)
                if c == 6:
                    s1 = 1.0 + mod_tile(kn + 8)

                    @pl.when(k + 4 < 8)
                    def _():
                        start(m_copies(k + 4))

            @pl.when(k + 3 < 8)
            def _():
                start(wa_copies(k + 3, p))

        h_v[kn] = (n_v[kn] * s1 + sh).astype(BF16)


        @pl.when(k >= 4)
        def _():
            start(w_copies(PA + k - 4))

        return carry

    with _scope("stageA"):
        lax.fori_loop(0, 8, sa_body, 0)

    def ln1(seg):
        xb = x_v[seg, 8:SEG, :].astype(F32)
        return _ln(xb) * (1.0 + mod_v[0:1, D:2 * D]) + mod_v[0:1, 0:D]

    TH = T0 // 2

    def hs_body(t, carry):
        for r in range(0, TH, 32):
            ss = _strassen_lhs(*[_ld(h_v, (t + 4 * b,), a * TH + r, 32).astype(F32)
                                 for a in range(2) for b in range(2)])
            for k, i in enumerate(SSUM):
                hs_v[k, t, r:r + 32, :] = ss[i].astype(BF16)
        return carry

    lax.fori_loop(0, 4, hs_body, 0)

    def lhs1(i):
        if i == 2:
            tiles = [_ld(h_v, (t,), 0, TH) for t in range(4)]
        elif i == 3:
            tiles = [_ld(h_v, (t + 4,), TH, TH) for t in range(4)]
        else:
            tiles = [_ld(hs_v, (SSUM.index(i), t), 0, TH) for t in range(4)]
        return jnp.concatenate(tiles, axis=1)

    NP1 = (NP - PA) // P1U
    late = late_copies(False)
    nl = -(-len(late) // (3 * P1U))

    def p1_body(i, carry):
        p0 = PA + P1U * i
        with _scope("wait_w"):
            for u in range(P1U):
                wait(w_copies(p0 + u))

        for u in range(3 * P1U):
            p, j = p0 + u // 3, u % 3
            lo, hi = relayout(p * 6 + j * 2, slice(None))
            b = [lo[0:DH2], hi[0:DH2], lo[DH2:D], hi[DH2:D]]
            t = _strassen_rhs(*[x.astype(F32) for x in b])
            t = [b[0] if k == 1 else b[3] if k == 4 else t[k].astype(BF16) for k in range(7)]
            m = {k: _dot(lhs1(k), t[k]) for k in P1ORD}
            c = _strassen_out(m)
            store_lead(p, j, jnp.concatenate([c[0], c[2]], axis=0), jnp.concatenate([c[1], c[3]], axis=0))

            if u < 4:
                @pl.when(i < 2)
                def _():
                    start(w_copies(PA + 4 + 4 * i + u))
            elif u == 4:
                @pl.when(jnp.logical_and(i >= 1, i < 3))
                def _():
                    start([wo_copy(4 * (i - 1) + q) for q in range(4)])
            elif u == 5:
                @pl.when(i == 2)
                def _():
                    start(late_copies(True))

            @pl.when(i == NP1 - 1)
            def _():
                start(late[u * nl:(u + 1) * nl])

        hn_v[...] = ln1(0)
        return carry

    with _scope("phase1"):
        lax.fori_loop(0, NP1, p1_body, 0)

    with _scope("wait_wo"):
        wait([wo_copy(j) for j in range(8)])
        wait(late_copies(True))

    def prep_views(w, t_row, kh, nh, j, r0):
        src = w.at[pl.ds(j, nh + 1), pl.ds(pl.multiple_of(r0, 256), kh + 256), :]
        dst = lt_v.at[pl.ds(pl.multiple_of(t_row + j * kh + r0, 256), 4 * nh * kh + 256), :]
        return src, dst, kh, nh

    def prep(views, r0, n):
        src, dst, kh, nh = views
        t = _strassen_rhs(*[_ld(src, (b * nh,), a * kh + r0, n).astype(F32) for a in range(2) for b in range(2)])
        for k, i in enumerate(TSUM):
            dst[k * nh * kh + r0:k * nh * kh + r0 + n, :] = t[i].astype(BF16)

    def step(it, odd, mem):
        s = 2 * it + int(odd)
        lead = lt_v.at[pl.ds(pl.multiple_of(16 * s, 16), T1_ROW), :]
        lhs = jnp.concatenate([mem, hn_v[...]], axis=0).astype(BF16)
        hn_v[...] = ln1(jnp.minimum(s + 1, NSEG - 1))
        mo = 48 if odd else 32

        def proj(p):
            if p == 0:
                half = [_dot(lhs[:, 0:D // 2], _bf(w_v[c, 0:D // 4, :])) for c in range(6)]
                cols = [_dot(lhs[:, D // 2:D], _bf(w_v[c, D // 4:D // 2, :])) + half[c] for c in range(6)]
            for j in range(3):
                if p == 0:
                    r = _interleave(cols[j * 2], cols[j * 2 + 1])
                else:
                    r = _interleave(_dot(lhs, _bf(w_v[p * 6 + j * 2])), _dot(lhs, _bf(w_v[p * 6 + j * 2 + 1])))
                fr_v[p * 3 + j] = r.astype(BF16)

        def stack(p, j):
            return jnp.concatenate([fr_v[p * 3 + j],
                                    _ld(lead, (), (p * 3 + j) * 2 * T0, 16)], axis=0)

        def attn(pvs, qks):
            os_ = [_dot(pr_v[p, :, 0:80], stack(p, 2)) for p in pvs]
            ss = [lax.dot_general(stack(p, 0), stack(p, 1), (((1,), (1,)), ((), ())),
                                  preferred_element_type=F32) for p in qks]
            for p, o in zip(pvs, os_):
                for t, oh in enumerate(_deinterleave(o)):
                    h = 2 * p + t
                    if odd:
                        lo_v[1, h, 0:8, :] = oh[0:8].astype(BF16)
                        lo_v[1, h, 16:48, :] = oh[8:40].astype(BF16)
                    else:
                        lo_v[0, h, 0:32, :] = oh[0:32].astype(BF16)
                        lo_v[1, h, 8:16, :] = oh[32:40].astype(BF16)
            for p, sc_ in zip(qks, ss):
                fill = fill_v[...]
                sc_ = jnp.concatenate([sc_, jnp.zeros((80, 48), F32)], axis=1)
                sc_ = jnp.where(fill == 0.0, sc_, fill)
                mx = jnp.max(sc_, axis=-1, keepdims=True)
                e = jnp.exp2((sc_ - mx) * (scale * LOG2E))
                l = jnp.sum(e, axis=-1, keepdims=True)
                r = pl.reciprocal(l, approx=True)
                pr_v[p] = (e * (r * (2.0 - l * r))).astype(BF16)

        part = {}

        def wo(j, h0, h1):
            lo = jnp.concatenate([lo_v[int(odd), h, 0:mo, :] for h in range(h0, h1)], axis=1)
            r = _dot(lo, _bf(wo_v[j, h0 * 64:h1 * 64, :]))
            part[j] = r + part[j] if j in part else r

        pc = jnp.maximum(it - 4, 0)
        if odd:
            views = prep_views(w2_v, T2_ROW, FH, DH2 // 128, lax.div(pc, 7), lax.rem(pc, 7) * 256)
        else:
            views = prep_views(w1_v, T1_ROW, DH2, FH // 128, pc >> 1, (pc & 1) * 256)
        npiece = 0
        for op in SCHED:
            if op[0] == "proj":
                proj(op[1])
            elif op[0] == "attn":
                attn(op[1], op[2])
                if npiece < 8:
                    prep(views, npiece * 32, 32)
                    npiece += 1
            else:
                wo(*op[1:])
                if odd and op[1:] in MODPOS:
                    cs = pl.ds(pl.multiple_of((16 + it) * 128, 128), 128)
                    k0 = MODPOS.index(op[1:]) * (D // 2)
                    m = _dot(sc_v[:, k0:k0 + D // 2], wmod_v[k0:k0 + D // 2, cs])
                    if k0 == 0:
                        mhalf = m
                    else:
                        mod_v[:, cs] = m + mhalf
        res = jnp.concatenate([part[j] for j in range(8)], axis=1)
        t0 = pl.multiple_of(SEG * s, SEG)
        if odd:
            x1_v[pl.ds(t0 - SEG, 8), :] = res[8:16]
            x1_v[pl.ds(t0, SEG), :] = jnp.concatenate([res[40:48], res[16:40]], axis=0)
        else:
            x1_v[pl.ds(t0 + 8, TPS), :] = res[8:32]
        return res[0:8]

    with _scope("main"):
        def steps(i, mem):
            with _scope("iter"):
                mem = step(i, True, step(i, False, mem))

            @pl.when(i == NEARLY - 1)
            def _():
                wait(late)

            return mem

        lax.fori_loop(0, NSEG // 2, steps, mem0_ref[...].astype(F32))

    def rhs(w, t_row, kh, nh, i, j, k0, nk):
        if i == 1:
            return _ld(w, (j,), k0, nk)
        if i == 4:
            return _ld(w, (j + nh,), kh + k0, nk)
        return _ld(lt_v, (), t_row + (TSUM.index(i) * nh + j) * kh + k0, nk)

    def out_copy(i, q):
        rows = pl.ds(_mult(i, FB), FB)
        return [pltpu.make_async_copy(out_v.at[rows, cols], out_hbm.at[rows, cols], sems.at[SEM_OUT + i])
                for cols in (pl.ds(q * OC, OC), pl.ds(DH2 + q * OC, OC))]

    HB = FB // 2

    def resid1(r0, k0, n, c0=0, nc=D):
        if n >= SEG:
            xb = x_v[pl.ds((r0 >> 5) + k0 // SEG, n // SEG), :, c0:c0 + nc].astype(F32).reshape(n, nc)
        else:
            xb = x_v[(r0 >> 5) + k0 // SEG, k0 % SEG:k0 % SEG + n, c0:c0 + nc].astype(F32)
        return xb + mod_v[0:1, 2 * D + c0:2 * D + c0 + nc] * x1_v[pl.ds(r0 + k0, n), c0:c0 + nc]

    def ln2(slot, r0, k0, n):
        top, bot = [_ln(resid1(r0, t * HB + k0, n)) * (1.0 + mod_v[0:1, 4 * D:5 * D]) + mod_v[0:1, 3 * D:4 * D]
                    for t in range(2)]
        ss = _strassen_lhs(top[:, 0:DH2], top[:, DH2:D], bot[:, 0:DH2], bot[:, DH2:D])
        for i in range(7):
            for j in range(DH2 // 128):
                h2_v[slot, i, j, k0:k0 + n, :] = ss[i][:, j * 128:(j + 1) * 128].astype(BF16)

    ln2(0, 0, 0, HB)

    def ffn_body(i, carry):
        r0 = pl.multiple_of(i * FB, FB)
        rn = pl.multiple_of(jnp.minimum(r0 + FB, S - FB), FB)
        slot = lax.rem(i, 2)
        nf = FH // FC
        nt = FC // 128
        nq = DH2 // OC
        acc = {}
        gs = {}

        def up(f, t):
            c0 = f * FC + t * 128
            c = _strassen_out({
                k: _dot(jnp.concatenate([_ld(h2_v, (slot, k, j), 0, HB) for j in range(DH2 // 128)], axis=1),
                        rhs(w1_v, T1_ROW, DH2, FH // 128, k, c0 // 128, 0, DH2)) for k in UPORD})
            b1a, b1b = bias_v[0:1, c0:c0 + 128], bias_v[0:1, FH + c0:FH + c0 + 128]
            gs[f, t] = _strassen_lhs(_gelu(c[0] + b1a), _gelu(c[1] + b1b), _gelu(c[2] + b1a), _gelu(c[3] + b1b))
            if t == nt - 1:
                gs[f] = [jnp.concatenate([gs[f, u][k] for u in range(nt)], axis=1).astype(BF16) for k in range(7)]

        def down(f, q):
            for k in DNORD:
                y = _dot(gs[f][k], rhs(w2_v, T2_ROW, FH, DH2 // 128, k, q, f * FC, FC))
                acc[k, q] = y + acc[k, q] if f else y
            if f == nf - 1:
                c = _strassen_out([acc[k, q] for k in range(7)])
                for t in range(4):
                    k0, c0 = (t // 2) * HB, (t % 2) * DH2 + q * OC
                    y = (c[t] + bias_v[0:1, FF + c0:FF + c0 + OC]) * mod_v[0:1, 5 * D + c0:5 * D + c0 + OC]
                    out_v[pl.ds(r0 + k0, HB), c0:c0 + OC] = (resid1(r0, k0, HB, c0, OC) + y).astype(BF16)
                start(out_copy(i, q))

        for t in range(nt):
            up(0, t)
        w = 0
        for f in range(nf):
            for t in range(nt):
                if f + 1 < nf:
                    up(f + 1, t)
                if w < len(LNP) and LNP[w]:
                    ln2(1 - slot, rn, sum(LNP[:w]), LNP[w])
                w += 1
                for q in range(t * nq // nt, (t + 1) * nq // nt):
                    down(f, q)
        return carry

    with _scope("ffn"):
        lax.fori_loop(0, S // FB, ffn_body, 0)
    with _scope("wait_out"):
        for i in range(S // FB):
            for q in range(DH2 // OC):
                wait(out_copy(i, q))


@jax.jit
def pallas_adaLN_cond__memory_aug_recurrent_mem_tr__dense_activation_gelu__prompt_kernel(
    A_x, A_mem0, A_Wq, A_Wk, A_Wv, A_Wo, A_seg_len, B_x, B_w1, B_b1, B_w2, B_b2, c, w_mod,
):
    del A_seg_len, B_x
    assert A_x.shape == (1, S, D)
    hbm = pl.BlockSpec(memory_space=pl.ANY)
    out = pl.pallas_call(
        _kernel,
        out_shape=jax.ShapeDtypeStruct((S, D), BF16),
        in_specs=[hbm] * 12,
        out_specs=hbm,
        scratch_shapes=[
            pltpu.VMEM((NSEG, SEG, D), BF16),
            pltpu.VMEM((8, T0, 128), BF16),
            pltpu.VMEM((TPS, D), F32),
            pltpu.VMEM((2, 7, 4, FB // 2, 128), BF16),
            pltpu.VMEM((S, D), F32),
            pltpu.VMEM((D, 6 * D), BF16),
            pltpu.VMEM((8, 6 * D), F32),
            pltpu.VMEM((8, D), BF16),
            pltpu.VMEM((6 * NP, D // 2, 128), U32),
            pltpu.VMEM((8, H * DH // 2, 128), U32),
            pltpu.VMEM((FF // 128, D, 128), BF16),
            pltpu.VMEM((D // 128, FF, 128), BF16),
            pltpu.VMEM((LT_ROWS, 128), BF16),
            pltpu.VMEM((3 * NP, 64, 128), BF16),
            pltpu.VMEM((2, H, 48, 128), BF16),
            pltpu.VMEM((NP, 80, 128), BF16),
            pltpu.VMEM((80, 128), F32),
            pltpu.VMEM((S, D), BF16),
            pltpu.VMEM((1, FF + D), F32),
            pltpu.VMEM((8, T0, 128), F32),
            pltpu.VMEM((M, D), BF16),
            pltpu.VMEM((FF,), BF16),
            pltpu.VMEM((D,), BF16),
            pltpu.VMEM((1, D), BF16),
            pltpu.VMEM((5, 4, T0 // 2, 128), BF16),
            pltpu.SemaphoreType.DMA((SEM_N,)),
        ],
        compiler_params=pltpu.CompilerParams(vmem_limit_bytes=120 * 1024 * 1024, disable_bounds_checks=True,
                                             disable_semaphore_checks=True),
    )(
        A_x.reshape(NSEG, SEG, D), A_mem0.reshape(M, D),
        A_Wq.reshape(D // 2, 2, H, DH), A_Wk.reshape(D // 2, 2, H, DH), A_Wv.reshape(D // 2, 2, H, DH),
        A_Wo.reshape(H * DH, D), B_w1, B_b1, B_w2, B_b2, c, w_mod,
    )
    return out.reshape(1, S, D)
```

```python
import contextlib

import jax
import jax.numpy as jnp
from jax import lax
import jax.experimental.pallas as pl
import jax.experimental.pallas.tpu as pltpu

F32 = jnp.float32
BF16 = jnp.bfloat16
U32 = jnp.uint32

S = 2048
D = 1024
H = 32
DH = 128
M = 8
SEG = 32
FF = 3584
NSEG = S // SEG
NP = H // 2
TPS = 24
T0 = S - NSEG * TPS
EPS = 1e-5
P1U = 2
P1ORD = (1, 4, 3, 2, 0, 6, 5)
UPORD = (1, 4, 3, 2, 0, 6, 5)
DNORD = (1, 4, 3, 2, 0, 6, 5)
NEARLY = 4
PA = 4
LNP = (16,) * 8
MODK = (1, 3, 0, 6)
LOG2E = 1.4426950408889634
FB = 256
OC = 128
FC = 256
FH = FF // 2
DH2 = D // 2
T1_ROW = 3 * NP * 2 * T0
T2_ROW = T1_ROW + 5 * (FH // 128) * DH2
LT_ROWS = T2_ROW + 5 * (DH2 // 128) * FH
SSUM = (0, 1, 4, 5, 6)
TSUM = (0, 2, 3, 5, 6)
SEM_W, SEM_A, SEM_M, SEM_MISC, SEM_OUT = 0, 16, 24, 32, 40
SEM_N = SEM_OUT + S // FB


def _make_sched(g):
    out = []

    def rng(a, b):
        return tuple(range(max(a, 0), max(b, 0)))

    for p in range(NP):
        out.append(("proj", p))
        if p % g == 0 and p >= g:
            out.append(("attn", rng(p - 2 * g, p - g), rng(p - g, p)))
    h1 = 2 * (NP - 2 * g)
    h2 = 2 * (NP - g)
    if g == 4:
        out += [("wo", j, 0, h1) for j in (0, 1)]
        out.append(("attn", rng(NP - 2 * g, NP - g), rng(NP - g, NP)))
        out += [("wo", j, 0, h1) for j in (2, 3, 4, 5)]
        out.append(("attn", rng(NP - g, NP), ()))
        out += [("wo", j, 0, h1) for j in (6, 7)]
        out += [("wo", j, h1, h2) for j in range(8)]
        out += [("wo", j, h2, H) for j in range(8)]
    else:
        out += [("wo", 0, 0, h1)]
        out.append(("attn", rng(NP - 2 * g, NP - g), rng(NP - g, NP)))
        out += [("wo", j, 0, h1) for j in (1, 2, 3)]
        out.append(("attn", rng(NP - g, NP), ()))
        out += [("wo", j, 0, h1) for j in (4, 5, 6, 7)]
        out += [("wo", j, h1, H) for j in range(8)]
    return out


SCHED = _make_sched(2)
_SCOPES = False


def _scope(name):
    return jax.named_scope(name) if _SCOPES else contextlib.nullcontext()


def _dot(a, b):
    return jnp.dot(a, b, preferred_element_type=F32)


def _bf(x):
    return pltpu.bitcast(x, BF16)


def _u32(x):
    return pltpu.bitcast(x, U32)


def _ld(ref, idx, r0, n):
    return _bf(ref.bitcast(U32)[(*idx, pl.ds(r0 // 2, n // 2), slice(None))])


def _ln(x):
    m = jnp.mean(x, axis=-1, keepdims=True)
    xc = x - m
    v = jnp.mean(xc * xc, axis=-1, keepdims=True)
    return xc * lax.rsqrt(v + EPS)


def _gelu(x):
    c = 0.7978845608028654
    return 0.5 * x * (1.0 + jnp.tanh(c * (x + 0.044715 * (x * x * x))))


def _strassen_lhs(a11, a12, a21, a22):
    return [a11 + a22, a21 + a22, a11, a22, a11 + a12, a21 - a11, a12 - a22]


def _strassen_rhs(b11, b12, b21, b22):
    return [b11 + b22, b11, b12 - b22, b21 - b11, b22, b11 + b12, b21 + b22]


def _strassen_out(m):
    return (m[0] + m[3] - m[4] + m[6], m[2] + m[4], m[1] + m[3], m[0] - m[1] + m[2] + m[5])


def _interleave(a, b):
    n = a.shape[0] // 8
    parts = []
    for g in range(n):
        parts.append(a[8 * g:8 * g + 8])
        parts.append(b[8 * g:8 * g + 8])
    return jnp.concatenate(parts, axis=0)


def _deinterleave(v):
    n = v.shape[0] // 16
    a = jnp.concatenate([v[16 * g:16 * g + 8] for g in range(n)], axis=0)
    b = jnp.concatenate([v[16 * g + 8:16 * g + 16] for g in range(n)], axis=0)
    return a, b


def _kernel(x_hbm, mem0_hbm, wq_hbm, wk_hbm, wv_hbm, wo_hbm, w1_hbm, b1_hbm, w2_hbm, b2_hbm,
            c_hbm, wmod_hbm, out_hbm,
            x_v, h_v, hn_v, h2_v, x1_v, wmod_v, mod_v, sc_v, w_v, wo_v, w1_v, w2_v, lt_v, fr_v, lo_v, pr_v, fill_v, out_v, bias_v, n_v,
            mem0_ref, b1_ref, b2_ref, c_ref, hs_v, so_v, ev_v,
            sems):
    w32 = [r.bitcast(U32) for r in (wq_hbm, wk_hbm, wv_hbm)]
    wo32 = wo_hbm.bitcast(U32)

    def w_copies(p):
        return [pltpu.make_async_copy(w32[j].at[:, par, p, :], w_v.at[p * 6 + j * 2 + par], sems.at[SEM_W + p])
                for j in range(3) for par in range(2)]

    def _mult(i, m):
        return i * m if isinstance(i, int) else pl.multiple_of(i * m, m)

    def wa_copies(k, pair=None):
        r = pl.ds(_mult(k, 64), 64)
        return [pltpu.make_async_copy(w32[j].at[r, par, p, :], w_v.at[p * 6 + j * 2 + par, r], sems.at[SEM_A + k])
                for p in (range(PA) if pair is None else (pair,)) for j in range(3) for par in range(2)]

    def m_copies(k):
        cols = [pl.ds(_mult(k + 8 * t, 128), 128) for t in range(2)]
        return [pltpu.make_async_copy(wmod_hbm.at[:, cs], wmod_v.at[:, cs], sems.at[SEM_M + k]) for cs in cols]

    def start(cps):
        for cp in cps:
            cp.start()

    def wait(cps):
        for cp in cps:
            cp.wait()

    cp_x0 = pltpu.make_async_copy(x_hbm.at[:, 0:8, :], x_v.at[:, 0:8, :], sems.at[SEM_MISC + 1])

    def wo_copy(j):
        return pltpu.make_async_copy(wo32.at[:, pl.ds(_mult(j, 128), 128)], wo_v.at[j], sems.at[SEM_MISC + 3])

    def late_copies(first):
        sem = sems.at[SEM_MISC + (4 if first else 5)]
        sg = slice(1, 2 * NEARLY + 1) if first else slice(2 * NEARLY + 1, NSEG)
        cps = [(x_hbm.at[sg, 8:SEG, :], x_v.at[sg, 8:SEG, :])]
        if not first:
            cps.append((wmod_hbm.at[:, 2 * D:6 * D], wmod_v))
        for src, dst, nt, kh in ((w1_hbm, w1_v, FF // 128, DH2), (w2_hbm, w2_v, D // 128, FH)):
            for j in range(nt):
                cols = slice(j * 128, (j + 1) * 128)
                if j % (nt // 2):
                    rows = [] if first else [slice(None)]
                else:
                    rows = [slice(a * kh, a * kh + 256) if first else slice(a * kh + 256, (a + 1) * kh)
                            for a in range(2)]
                cps += [(src.at[r, cols], dst.at[j, r]) for r in rows]
        return [pltpu.make_async_copy(src, dst, sem) for src, dst in cps]

    cp_small = [pltpu.make_async_copy(src, dst, sems.at[SEM_MISC])
                for src, dst in ((c_hbm, c_ref), (mem0_hbm, mem0_ref), (b1_hbm, b1_ref), (b2_hbm, b2_ref),
                                 (x_hbm.at[0, 8:SEG, :], x_v.at[0, 8:SEG, :]))]

    start(cp_small)
    cp_x0.start()
    start(m_copies(0))
    for k in range(2):
        start(m_copies(k + 1))
        start(wa_copies(k))

    scale = DH ** -0.5
    ri = lax.broadcasted_iota(jnp.int32, (80, 128), 0)
    ci = lax.broadcasted_iota(jnp.int32, (80, 128), 1)
    same_head = (((ri >> 3) & 1) == ((ci >> 3) & 1)) & (ci < 80)
    rpos = (((ri >> 4) & 3) << 3) + (ri & 7)
    cpos = (((ci >> 4) & 3) << 3) + (ci & 7)
    keep = (ri < 16) | (ci < 16) | (rpos >= cpos)
    fill_v[...] = jnp.where(same_head, jnp.where(keep, 0.0, -1e9 / scale), -jnp.inf).astype(F32)

    wait(cp_small)
    c = c_ref[...].astype(F32)
    sc = jnp.broadcast_to(c * jax.nn.sigmoid(c), (8, D)).astype(BF16)

    sc_v[...] = sc
    bias_v[:, 0:FF] = b1_ref[...].astype(F32).reshape(1, FF)
    bias_v[:, FF:FF + D] = b2_ref[...].astype(F32).reshape(1, D)

    def zero_body(i, carry):
        x1_v[pl.ds(pl.multiple_of(i * 64, 64), 64), :] = jnp.zeros((64, D), F32)
        return carry

    lax.fori_loop(0, PA * 6, zero_body, 0)

    def relayout(c, rows):
        a = w_v[c, rows, :]
        b = w_v[c + 1, rows, :]
        lo = (a & jnp.uint32(0xFFFF)) | (b << 16)
        hi = (a >> 16) | (b & jnp.uint32(0xFFFF0000))
        w_v[c, rows, :] = lo
        w_v[c + 1, rows, :] = hi
        return _bf(lo), _bf(hi)

    def store_lead(p, j, a, b):
        lt_v[pl.ds(_mult(p * 3 + j, 2 * T0), 2 * T0), :] = _interleave(a, b).astype(BF16)

    def mod_tile(ct):
        cs = pl.ds(_mult(ct, 128), 128)
        m = _dot(sc_v[...], wmod_v[:, cs])
        mod_v[:, cs] = m
        return m[0:1]

    with _scope("wait_x0"):
        cp_x0.wait()

    def ln1_body(i, carry):
        r = pl.multiple_of(i * 128, 128)
        n = _ln(x_v[pl.ds(i * 16, 16), 0:8, :].astype(F32).reshape(128, D))
        for k in range(8):
            n_v[k, pl.ds(r, 128), :] = n[:, k * 128:(k + 1) * 128]
        return carry

    with _scope("ln1"):
        lax.fori_loop(0, T0 // 128, ln1_body, 0)
    start(m_copies(3))
    start(wa_copies(2))
    with _scope("wait_m0"):
        wait(m_copies(0))
    h_v[0] = (n_v[0] * (1.0 + mod_tile(8)) + mod_tile(0)).astype(BF16)

    def sa_body(k, carry):
        with _scope("wait_a"):
            wait(wa_copies(k))

            @pl.when(k < 7)
            def _():
                wait(m_copies(k + 1))

        kn = jnp.minimum(k + 1, 7)
        rows = pl.ds(pl.multiple_of(k * 64, 64), 64)
        hk = _ld(h_v, (k,), 0, T0)
        for p in range(PA):
            for j in range(3):
                c = p * 6 + j * 2
                res = []
                for t, w in enumerate(relayout(c, rows)):
                    acc = x1_v.at[(c + t) // 8 * T0:((c + t) // 8 + 1) * T0,
                                  (c + t) % 8 * 128:((c + t) % 8 + 1) * 128]
                    r = _dot(hk, w) + acc[...]
                    acc[...] = r
                    res.append(r)
                store_lead(p, j, *res)
                if c == 2:
                    sh = mod_tile(kn)
                if c == 6:
                    s1 = 1.0 + mod_tile(kn + 8)

                    @pl.when(k + 4 < 8)
                    def _():
                        start(m_copies(k + 4))

            @pl.when(k + 3 < 8)
            def _():
                start(wa_copies(k + 3, p))

        h_v[kn] = (n_v[kn] * s1 + sh).astype(BF16)


        @pl.when(k >= 4)
        def _():
            start(w_copies(PA + k - 4))

        return carry

    with _scope("stageA"):
        lax.fori_loop(0, 8, sa_body, 0)

    def ln1(seg):
        xb = x_v[seg, 8:SEG, :].astype(F32)
        return _ln(xb) * (1.0 + mod_v[0:1, D:2 * D]) + mod_v[0:1, 0:D]

    TH = T0 // 2

    def hs_body(t, carry):
        for r in range(0, TH, 32):
            ss = _strassen_lhs(*[_ld(h_v, (t + 4 * b,), a * TH + r, 32).astype(F32)
                                 for a in range(2) for b in range(2)])
            for k, i in enumerate(SSUM):
                hs_v[k, t, r:r + 32, :] = ss[i].astype(BF16)
        return carry

    lax.fori_loop(0, 4, hs_body, 0)

    def lhs1(i):
        if i == 2:
            tiles = [_ld(h_v, (t,), 0, TH) for t in range(4)]
        elif i == 3:
            tiles = [_ld(h_v, (t + 4,), TH, TH) for t in range(4)]
        else:
            tiles = [_ld(hs_v, (SSUM.index(i), t), 0, TH) for t in range(4)]
        return jnp.concatenate(tiles, axis=1)

    NP1 = (NP - PA) // P1U
    late = late_copies(False)
    nl = -(-len(late) // (3 * P1U))

    def p1_body(i, carry):
        p0 = PA + P1U * i
        with _scope("wait_w"):
            for u in range(P1U):
                wait(w_copies(p0 + u))

        for u in range(3 * P1U):
            p, j = p0 + u // 3, u % 3
            lo, hi = relayout(p * 6 + j * 2, slice(None))
            b = [lo[0:DH2], hi[0:DH2], lo[DH2:D], hi[DH2:D]]
            t = _strassen_rhs(*[x.astype(F32) for x in b])
            t = [b[0] if k == 1 else b[3] if k == 4 else t[k].astype(BF16) for k in range(7)]
            m = {k: _dot(lhs1(k), t[k]) for k in P1ORD}
            c = _strassen_out(m)
            store_lead(p, j, jnp.concatenate([c[0], c[2]], axis=0), jnp.concatenate([c[1], c[3]], axis=0))

            if u < 4:
                @pl.when(i < 2)
                def _():
                    start(w_copies(PA + 4 + 4 * i + u))
            elif u == 4:
                @pl.when(jnp.logical_and(i >= 1, i < 3))
                def _():
                    start([wo_copy(4 * (i - 1) + q) for q in range(4)])
            elif u == 5:
                @pl.when(i == 2)
                def _():
                    start(late_copies(True))

            @pl.when(i == NP1 - 1)
            def _():
                start(late[u * nl:(u + 1) * nl])

        hn_v[...] = ln1(0)
        return carry

    with _scope("phase1"):
        lax.fori_loop(0, NP1, p1_body, 0)

    with _scope("wait_wo"):
        wait([wo_copy(j) for j in range(8)])
        wait(late_copies(True))

    def prep_views(w, t_row, kh, nh, j, r0):
        src = w.at[pl.ds(j, nh + 1), pl.ds(pl.multiple_of(r0, 256), kh + 256), :]
        dst = lt_v.at[pl.ds(pl.multiple_of(t_row + j * kh + r0, 256), 4 * nh * kh + 256), :]
        return src, dst, kh, nh

    def prep(views, r0, n):
        src, dst, kh, nh = views
        t = _strassen_rhs(*[_ld(src, (b * nh,), a * kh + r0, n).astype(F32) for a in range(2) for b in range(2)])
        for k, i in enumerate(TSUM):
            dst[k * nh * kh + r0:k * nh * kh + r0 + n, :] = t[i].astype(BF16)

    def step(it, odd, mem):
        s = 2 * it + int(odd)
        lead = lt_v.at[pl.ds(pl.multiple_of(16 * s, 16), T1_ROW), :]
        lhs = jnp.concatenate([mem, hn_v[...]], axis=0).astype(BF16)
        hn_v[...] = ln1(jnp.minimum(s + 1, NSEG - 1))

        def proj(p):
            if p == 0:
                half = [_dot(lhs[:, 0:D // 2], _bf(w_v[c, 0:D // 4, :])) for c in range(6)]
                cols = [_dot(lhs[:, D // 2:D], _bf(w_v[c, D // 4:D // 2, :])) + half[c] for c in range(6)]
            for j in range(3):
                if p == 0:
                    r = _interleave(cols[j * 2], cols[j * 2 + 1])
                else:
                    r = _interleave(_dot(lhs, _bf(w_v[p * 6 + j * 2])), _dot(lhs, _bf(w_v[p * 6 + j * 2 + 1])))
                fr_v[p * 3 + j] = r.astype(BF16)

        def stack(p, j):
            return jnp.concatenate([fr_v[p * 3 + j],
                                    _ld(lead, (), (p * 3 + j) * 2 * T0, 16)], axis=0)

        def attn(pvs, qks):
            os_ = [_dot(pr_v[p, :, 0:80], stack(p, 2)) for p in pvs]
            ss = [lax.dot_general(stack(p, 0), stack(p, 1), (((1,), (1,)), ((), ())),
                                  preferred_element_type=F32) for p in qks]
            for p, o in zip(pvs, os_):
                for t, oh in enumerate(_deinterleave(o[0:64])):
                    lo_v[2 * p + t] = oh.astype(BF16)
                if odd:
                    ev = ev_v[p]
                    for k, sk in enumerate(_strassen_lhs(ev[0:8], ev[8:16], o[64:72], o[72:80])):
                        so_v[k, p, pl.ds(pl.multiple_of(8 * it, 8), 8), :] = sk.astype(BF16)
                else:
                    ev_v[p] = o[64:80]
            for p, sc_ in zip(qks, ss):
                fill = fill_v[...]
                sc_ = jnp.concatenate([sc_, jnp.zeros((80, 48), F32)], axis=1)
                sc_ = jnp.where(fill == 0.0, sc_, fill)
                mx = jnp.max(sc_, axis=-1, keepdims=True)
                e = jnp.exp2((sc_ - mx) * (scale * LOG2E))
                l = jnp.sum(e, axis=-1, keepdims=True)
                r = pl.reciprocal(l, approx=True)
                pr_v[p] = (e * (r * (2.0 - l * r))).astype(BF16)

        part = {}

        def wo(j, h0, h1):
            lo = jnp.concatenate([lo_v[h] for h in range(h0, h1)], axis=1)
            r = _dot(lo, _bf(wo_v[j, h0 * 64:h1 * 64, :]))
            part[j] = r + part[j] if j in part else r

        pc = jnp.maximum(it - 4, 0)
        if odd:
            views = prep_views(w2_v, T2_ROW, FH, DH2 // 128, pc & 3, (pc >> 2) * 256)
        else:
            views = prep_views(w1_v, T1_ROW, DH2, FH // 128, pc >> 1, (pc & 1) * 256)
        npiece = 0
        for op in SCHED:
            if op[0] == "proj":
                proj(op[1])
            elif op[0] == "attn":
                attn(op[1], op[2])
                if npiece < 8:
                    prep(views, npiece * 32, 32)
                    npiece += 1
            else:
                wo(*op[1:])
        res = jnp.concatenate([part[j] for j in range(8)], axis=1)
        x1_v[pl.ds(pl.multiple_of(SEG * s + 8, 8), TPS), :] = res[8:32]
        return res[0:8]

    with _scope("main"):
        def steps(i, mem):
            with _scope("iter"):
                mem = step(i, True, step(i, False, mem))

            @pl.when(i == NEARLY - 1)
            def _():
                wait(late)

            return mem

        lax.fori_loop(0, NSEG // 2, steps, mem0_ref[...].astype(F32))

    def wo_body(j, carry):
        acc = {}
        for kc in range(4):
            b = [jnp.concatenate([_bf(wo_v[j + 4 * n, (2 * p + t) * 64:(2 * p + t + 1) * 64, :])
                                  for p in range(4 * kc, 4 * kc + 4)], axis=0)
                 for t in range(2) for n in range(2)]
            tt = _strassen_rhs(*[x.astype(F32) for x in b])
            tt = [b[0] if k == 1 else b[3] if k == 4 else tt[k].astype(BF16) for k in range(7)]
            for k in P1ORD:
                sk = jnp.concatenate([_ld(so_v, (k, p), 0, TH) for p in range(4 * kc, 4 * kc + 4)], axis=1)
                y = _dot(sk, tt[k])
                acc[k] = y + acc[k] if kc else y
                if k in MODK:
                    q = MODK.index(k)
                    ct = 8 * j + 2 * kc + q // 2
                    k0 = (q % 2) * DH2
                    m = _dot(sc_v[:, k0:k0 + DH2], wmod_v[k0:k0 + DH2, pl.ds(_mult(ct, 128), 128)])
                    if q % 2:
                        mod_v[:, pl.ds(_mult(ct + 16, 128), 128)] = m + mhalf
                    else:
                        mhalf = m
        for t, c in enumerate(_strassen_out(acc)):
            cs = pl.ds(pl.multiple_of((j + 4 * (t % 2)) * 128, 128), 128)
            for g in range(NSEG // 2):
                r0 = (2 * g + t // 2) * SEG
                x1_v[r0:r0 + 8, cs] = c[8 * g:8 * g + 8]
        return carry

    with _scope("p3a"):
        lax.fori_loop(0, 4, wo_body, 0)

    def rhs(w, t_row, kh, nh, i, j, k0, nk):
        if i == 1:
            return _ld(w, (j,), k0, nk)
        if i == 4:
            return _ld(w, (j + nh,), kh + k0, nk)
        return _ld(lt_v, (), t_row + (TSUM.index(i) * nh + j) * kh + k0, nk)

    def out_copy(i, q):
        rows = pl.ds(_mult(i, FB), FB)
        return [pltpu.make_async_copy(out_v.at[rows, cols], out_hbm.at[rows, cols], sems.at[SEM_OUT + i])
                for cols in (pl.ds(q * OC, OC), pl.ds(DH2 + q * OC, OC))]

    HB = FB // 2

    def resid1(r0, k0, n, c0=0, nc=D):
        if n >= SEG:
            xb = x_v[pl.ds((r0 >> 5) + k0 // SEG, n // SEG), :, c0:c0 + nc].astype(F32).reshape(n, nc)
        else:
            xb = x_v[(r0 >> 5) + k0 // SEG, k0 % SEG:k0 % SEG + n, c0:c0 + nc].astype(F32)
        return xb + mod_v[0:1, 2 * D + c0:2 * D + c0 + nc] * x1_v[pl.ds(r0 + k0, n), c0:c0 + nc]

    def ln2(slot, r0, k0, n):
        top, bot = [_ln(resid1(r0, t * HB + k0, n)) * (1.0 + mod_v[0:1, 4 * D:5 * D]) + mod_v[0:1, 3 * D:4 * D]
                    for t in range(2)]
        ss = _strassen_lhs(top[:, 0:DH2], top[:, DH2:D], bot[:, 0:DH2], bot[:, DH2:D])
        for i in range(7):
            for j in range(DH2 // 128):
                h2_v[slot, i, j, k0:k0 + n, :] = ss[i][:, j * 128:(j + 1) * 128].astype(BF16)

    ln2(0, 0, 0, HB)

    def ffn_body(i, carry):
        r0 = pl.multiple_of(i * FB, FB)
        rn = pl.multiple_of(jnp.minimum(r0 + FB, S - FB), FB)
        slot = lax.rem(i, 2)
        nf = FH // FC
        nt = FC // 128
        nq = DH2 // OC
        acc = {}
        gs = {}

        def up(f, t):
            c0 = f * FC + t * 128
            c = _strassen_out({
                k: _dot(jnp.concatenate([_ld(h2_v, (slot, k, j), 0, HB) for j in range(DH2 // 128)], axis=1),
                        rhs(w1_v, T1_ROW, DH2, FH // 128, k, c0 // 128, 0, DH2)) for k in UPORD})
            b1a, b1b = bias_v[0:1, c0:c0 + 128], bias_v[0:1, FH + c0:FH + c0 + 128]
            gs[f, t] = _strassen_lhs(_gelu(c[0] + b1a), _gelu(c[1] + b1b), _gelu(c[2] + b1a), _gelu(c[3] + b1b))
            if t == nt - 1:
                gs[f] = [jnp.concatenate([gs[f, u][k] for u in range(nt)], axis=1).astype(BF16) for k in range(7)]

        def down(f, q):
            for k in DNORD:
                y = _dot(gs[f][k], rhs(w2_v, T2_ROW, FH, DH2 // 128, k, q, f * FC, FC))
                acc[k, q] = y + acc[k, q] if f else y
            if f == nf - 1:
                c = _strassen_out([acc[k, q] for k in range(7)])
                for t in range(4):
                    k0, c0 = (t // 2) * HB, (t % 2) * DH2 + q * OC
                    y = (c[t] + bias_v[0:1, FF + c0:FF + c0 + OC]) * mod_v[0:1, 5 * D + c0:5 * D + c0 + OC]
                    out_v[pl.ds(r0 + k0, HB), c0:c0 + OC] = (resid1(r0, k0, HB, c0, OC) + y).astype(BF16)
                start(out_copy(i, q))

        for t in range(nt):
            up(0, t)
        w = 0
        for f in range(nf):
            for t in range(nt):
                if f + 1 < nf:
                    up(f + 1, t)
                if w < len(LNP) and LNP[w]:
                    ln2(1 - slot, rn, sum(LNP[:w]), LNP[w])
                w += 1
                for q in range(t * nq // nt, (t + 1) * nq // nt):
                    down(f, q)
        return carry

    with _scope("ffn"):
        lax.fori_loop(0, S // FB, ffn_body, 0)
    with _scope("wait_out"):
        for i in range(S // FB):
            for q in range(DH2 // OC):
                wait(out_copy(i, q))


@jax.jit
def pallas_adaLN_cond__memory_aug_recurrent_mem_tr__dense_activation_gelu__prompt_kernel(
    A_x, A_mem0, A_Wq, A_Wk, A_Wv, A_Wo, A_seg_len, B_x, B_w1, B_b1, B_w2, B_b2, c, w_mod,
):
    del A_seg_len, B_x
    assert A_x.shape == (1, S, D)
    hbm = pl.BlockSpec(memory_space=pl.ANY)
    out = pl.pallas_call(
        _kernel,
        out_shape=jax.ShapeDtypeStruct((S, D), BF16),
        in_specs=[hbm] * 12,
        out_specs=hbm,
        scratch_shapes=[
            pltpu.VMEM((NSEG, SEG, D), BF16),
            pltpu.VMEM((8, T0, 128), BF16),
            pltpu.VMEM((TPS, D), F32),
            pltpu.VMEM((2, 7, 4, FB // 2, 128), BF16),
            pltpu.VMEM((S, D), F32),
            pltpu.VMEM((D, 4 * D), BF16),
            pltpu.VMEM((8, 6 * D), F32),
            pltpu.VMEM((8, D), BF16),
            pltpu.VMEM((6 * NP, D // 2, 128), U32),
            pltpu.VMEM((8, H * DH // 2, 128), U32),
            pltpu.VMEM((FF // 128, D, 128), BF16),
            pltpu.VMEM((D // 128, FF, 128), BF16),
            pltpu.VMEM((LT_ROWS, 128), BF16),
            pltpu.VMEM((3 * NP, 64, 128), BF16),
            pltpu.VMEM((H, 32, 128), BF16),
            pltpu.VMEM((NP, 80, 128), BF16),
            pltpu.VMEM((80, 128), F32),
            pltpu.VMEM((S, D), BF16),
            pltpu.VMEM((1, FF + D), F32),
            pltpu.VMEM((8, T0, 128), F32),
            pltpu.VMEM((M, D), BF16),
            pltpu.VMEM((FF,), BF16),
            pltpu.VMEM((D,), BF16),
            pltpu.VMEM((1, D), BF16),
            pltpu.VMEM((5, 4, T0 // 2, 128), BF16),
            pltpu.VMEM((7, NP, T0 // 2, 128), BF16),
            pltpu.VMEM((NP, 16, 128), F32),
            pltpu.SemaphoreType.DMA((SEM_N,)),
        ],
        compiler_params=pltpu.CompilerParams(vmem_limit_bytes=120 * 1024 * 1024, disable_bounds_checks=True,
                                             disable_semaphore_checks=True),
    )(
        A_x.reshape(NSEG, SEG, D), A_mem0.reshape(M, D),
        A_Wq.reshape(D // 2, 2, H, DH), A_Wk.reshape(D // 2, 2, H, DH), A_Wv.reshape(D // 2, 2, H, DH),
        A_Wo.reshape(H * DH, D), B_w1, B_b1, B_w2, B_b2, c, w_mod,
    )
    return out.reshape(1, S, D)
```

```python
import contextlib

import jax
import jax.numpy as jnp
from jax import lax
import jax.experimental.pallas as pl
import jax.experimental.pallas.tpu as pltpu

F32 = jnp.float32
BF16 = jnp.bfloat16
U32 = jnp.uint32

S = 2048
D = 1024
H = 32
DH = 128
M = 8
SEG = 32
FF = 3584
NSEG = S // SEG
NP = H // 2
TPS = 24
T0 = S - NSEG * TPS
EPS = 1e-5
P1U = 2
P1ORD = (1, 4, 3, 2, 0, 6, 5)
UPORD = (1, 4, 3, 2, 0, 6, 5)
DNORD = (1, 4, 3, 2, 0, 6, 5)
NEARLY = 4
PA = 4
LNP = (16,) * 8
MODK = (1, 3, 0, 6)
LOG2E = 1.4426950408889634
FB = 256
OC = 128
FC = 256
FH = FF // 2
DH2 = D // 2
T1_ROW = 3 * NP * 2 * T0
T2_ROW = T1_ROW + 5 * (FH // 128) * DH2
LT_ROWS = T2_ROW + 5 * (DH2 // 128) * FH
SSUM = (0, 1, 4, 5, 6)
TSUM = (0, 2, 3, 5, 6)
SEM_W, SEM_A, SEM_M, SEM_MISC, SEM_OUT = 0, 16, 24, 32, 40
SEM_N = SEM_OUT + S // FB


def _make_sched(g):
    out = []

    def rng(a, b):
        return tuple(range(max(a, 0), max(b, 0)))

    for p in range(NP):
        out.append(("proj", p))
        if p % g == 0 and p >= g:
            out.append(("attn", rng(p - 2 * g, p - g), rng(p - g, p)))
    h1 = 2 * (NP - 2 * g)
    h2 = 2 * (NP - g)
    if g == 4:
        out += [("wo", j, 0, h1) for j in (0, 1)]
        out.append(("attn", rng(NP - 2 * g, NP - g), rng(NP - g, NP)))
        out += [("wo", j, 0, h1) for j in (2, 3, 4, 5)]
        out.append(("attn", rng(NP - g, NP), ()))
        out += [("wo", j, 0, h1) for j in (6, 7)]
        out += [("wo", j, h1, h2) for j in range(8)]
        out += [("wo", j, h2, H) for j in range(8)]
    else:
        out += [("wo", 0, 0, h1)]
        out.append(("attn", rng(NP - 2 * g, NP - g), rng(NP - g, NP)))
        out += [("wo", j, 0, h1) for j in (1, 2, 3)]
        out.append(("attn", rng(NP - g, NP), ()))
        out += [("wo", j, 0, h1) for j in (4, 5, 6, 7)]
        out += [("wo", j, h1, H) for j in range(8)]
    return out


SCHED = _make_sched(2)
_SCOPES = False


def _scope(name):
    return jax.named_scope(name) if _SCOPES else contextlib.nullcontext()


def _dot(a, b):
    return jnp.dot(a, b, preferred_element_type=F32)


def _bf(x):
    return pltpu.bitcast(x, BF16)


def _u32(x):
    return pltpu.bitcast(x, U32)


def _ld(ref, idx, r0, n):
    return _bf(ref.at[(*idx, pl.ds(r0, n), slice(None))].bitcast(U32)[...])


def _ln(x):
    m = jnp.mean(x, axis=-1, keepdims=True)
    xc = x - m
    v = jnp.mean(xc * xc, axis=-1, keepdims=True)
    return xc * lax.rsqrt(v + EPS)


def _gelu(x):
    c = 0.7978845608028654
    return 0.5 * x * (1.0 + jnp.tanh(c * (x + 0.044715 * (x * x * x))))


def _strassen_lhs(a11, a12, a21, a22):
    return [a11 + a22, a21 + a22, a11, a22, a11 + a12, a21 - a11, a12 - a22]


def _strassen_rhs(b11, b12, b21, b22):
    return [b11 + b22, b11, b12 - b22, b21 - b11, b22, b11 + b12, b21 + b22]


def _strassen_out(m):
    return (m[0] + m[3] - m[4] + m[6], m[2] + m[4], m[1] + m[3], m[0] - m[1] + m[2] + m[5])


def _interleave(a, b):
    n = a.shape[0] // 8
    parts = []
    for g in range(n):
        parts.append(a[8 * g:8 * g + 8])
        parts.append(b[8 * g:8 * g + 8])
    return jnp.concatenate(parts, axis=0)


def _deinterleave(v):
    n = v.shape[0] // 16
    a = jnp.concatenate([v[16 * g:16 * g + 8] for g in range(n)], axis=0)
    b = jnp.concatenate([v[16 * g + 8:16 * g + 16] for g in range(n)], axis=0)
    return a, b


def _kernel(x_hbm, mem0_hbm, wq_hbm, wk_hbm, wv_hbm, wo_hbm, w1_hbm, b1_hbm, w2_hbm, b2_hbm,
            c_hbm, wmod_hbm, out_hbm,
            x_v, h_v, hn_v, h2_v, x1_v, wmod_v, mod_v, sc_v, w_v, wo_v, w1_v, w2_v, lt_v, fr_v, lo_v, pr_v, fill_v, bias_v, n_v,
            mem0_ref, b1_ref, b2_ref, c_ref, hs_v, so_v, ev_v,
            sems):
    w32 = [r.bitcast(U32) for r in (wq_hbm, wk_hbm, wv_hbm)]
    wo32 = wo_hbm.bitcast(U32)

    def w_copies(p):
        return [pltpu.make_async_copy(w32[j].at[:, par, p, :], w_v.at[p * 6 + j * 2 + par], sems.at[SEM_W + p])
                for j in range(3) for par in range(2)]

    def _mult(i, m):
        return i * m if isinstance(i, int) else pl.multiple_of(i * m, m)

    def wa_copies(k, pair=None):
        r = pl.ds(_mult(k, 64), 64)
        return [pltpu.make_async_copy(w32[j].at[r, par, p, :], w_v.at[p * 6 + j * 2 + par, r], sems.at[SEM_A + k])
                for p in (range(PA) if pair is None else (pair,)) for j in range(3) for par in range(2)]

    def m_copies(k):
        cols = [pl.ds(_mult(k + 8 * t, 128), 128) for t in range(2)]
        return [pltpu.make_async_copy(wmod_hbm.at[:, cs], wmod_v.at[:, cs], sems.at[SEM_M + k]) for cs in cols]

    def start(cps):
        for cp in cps:
            cp.start()

    def wait(cps):
        for cp in cps:
            cp.wait()

    cp_x0 = pltpu.make_async_copy(x_hbm.at[:, 0:8, :], x_v.at[:, 0:8, :], sems.at[SEM_MISC + 1])

    def wo_copy(j):
        return pltpu.make_async_copy(wo32.at[:, pl.ds(_mult(j, 128), 128)], wo_v.at[j], sems.at[SEM_MISC + 3])

    def late_copies(first):
        sem = sems.at[SEM_MISC + (4 if first else 5)]
        sg = slice(1, 2 * NEARLY + 1) if first else slice(2 * NEARLY + 1, NSEG)
        cps = [(x_hbm.at[sg, 8:SEG, :], x_v.at[sg, 8:SEG, :])]
        if not first:
            cps.append((wmod_hbm.at[:, 2 * D:6 * D], wmod_v))
        for src, dst, nt, kh in ((w1_hbm, w1_v, FF // 128, DH2), (w2_hbm, w2_v, D // 128, FH)):
            for j in range(nt):
                cols = slice(j * 128, (j + 1) * 128)
                if j % (nt // 2):
                    rows = [] if first else [slice(None)]
                else:
                    rows = [slice(a * kh, a * kh + 256) if first else slice(a * kh + 256, (a + 1) * kh)
                            for a in range(2)]
                cps += [(src.at[r, cols], dst.at[j, r]) for r in rows]
        return [pltpu.make_async_copy(src, dst, sem) for src, dst in cps]

    cp_small = [pltpu.make_async_copy(src, dst, sems.at[SEM_MISC])
                for src, dst in ((c_hbm, c_ref), (mem0_hbm, mem0_ref), (b1_hbm, b1_ref), (b2_hbm, b2_ref),
                                 (x_hbm.at[0, 8:SEG, :], x_v.at[0, 8:SEG, :]))]

    start(cp_small)
    cp_x0.start()
    start(m_copies(0))
    for k in range(2):
        start(m_copies(k + 1))
        start(wa_copies(k))

    scale = DH ** -0.5
    ri = lax.broadcasted_iota(jnp.int32, (80, 128), 0)
    ci = lax.broadcasted_iota(jnp.int32, (80, 128), 1)
    same_head = (((ri >> 3) & 1) == ((ci >> 3) & 1)) & (ci < 80)
    rpos = (((ri >> 4) & 3) << 3) + (ri & 7)
    cpos = (((ci >> 4) & 3) << 3) + (ci & 7)
    keep = (ri < 16) | (ci < 16) | (rpos >= cpos)
    fill_v[...] = jnp.where(same_head, jnp.where(keep, 0.0, -1e9 / scale), -jnp.inf).astype(F32)

    wait(cp_small)
    c = c_ref[...].astype(F32)
    sc = jnp.broadcast_to(c * jax.nn.sigmoid(c), (8, D)).astype(BF16)

    sc_v[...] = sc
    bias_v[:, 0:FF] = b1_ref[...].astype(F32).reshape(1, FF)
    bias_v[:, FF:FF + D] = b2_ref[...].astype(F32).reshape(1, D)

    def zero_body(i, carry):
        x1_v[pl.ds(pl.multiple_of(i * 64, 64), 64), :] = jnp.zeros((64, D), F32)
        return carry

    lax.fori_loop(0, PA * 6, zero_body, 0)

    def relayout(c, rows):
        a = w_v[c, rows, :]
        b = w_v[c + 1, rows, :]
        lo = (a & jnp.uint32(0xFFFF)) | (b << 16)
        hi = (a >> 16) | (b & jnp.uint32(0xFFFF0000))
        w_v[c, rows, :] = lo
        w_v[c + 1, rows, :] = hi
        return _bf(lo), _bf(hi)

    def store_lead(p, j, a, b):
        lt_v[pl.ds(_mult(p * 3 + j, 2 * T0), 2 * T0), :] = _interleave(a, b).astype(BF16)

    def mod_tile(ct):
        cs = pl.ds(_mult(ct, 128), 128)
        m = _dot(sc_v[...], wmod_v[:, cs])
        mod_v[:, cs] = m
        return m[0:1]

    with _scope("wait_x0"):
        cp_x0.wait()

    def ln1_body(i, carry):
        r = pl.multiple_of(i * 128, 128)
        n = _ln(x_v[pl.ds(i * 16, 16), 0:8, :].astype(F32).reshape(128, D))
        for k in range(8):
            n_v[k, pl.ds(r, 128), :] = n[:, k * 128:(k + 1) * 128]
        return carry

    with _scope("ln1"):
        lax.fori_loop(0, T0 // 128, ln1_body, 0)
    start(m_copies(3))
    start(wa_copies(2))
    with _scope("wait_m0"):
        wait(m_copies(0))
    h_v[0] = (n_v[0] * (1.0 + mod_tile(8)) + mod_tile(0)).astype(BF16)

    def sa_body(k, carry):
        with _scope("wait_a"):
            wait(wa_copies(k))

            @pl.when(k < 7)
            def _():
                wait(m_copies(k + 1))

        kn = jnp.minimum(k + 1, 7)
        rows = pl.ds(pl.multiple_of(k * 64, 64), 64)
        hk = _ld(h_v, (k,), 0, T0)
        for p in range(PA):
            for j in range(3):
                c = p * 6 + j * 2
                res = []
                for t, w in enumerate(relayout(c, rows)):
                    acc = x1_v.at[(c + t) // 8 * T0:((c + t) // 8 + 1) * T0,
                                  (c + t) % 8 * 128:((c + t) % 8 + 1) * 128]
                    r = _dot(hk, w) + acc[...]
                    acc[...] = r
                    res.append(r)
                store_lead(p, j, *res)
                if c == 2:
                    sh = mod_tile(kn)
                if c == 6:
                    s1 = 1.0 + mod_tile(kn + 8)

                    @pl.when(k + 4 < 8)
                    def _():
                        start(m_copies(k + 4))

            @pl.when(k + 3 < 8)
            def _():
                start(wa_copies(k + 3, p))

        h_v[kn] = (n_v[kn] * s1 + sh).astype(BF16)


        @pl.when(k >= 4)
        def _():
            start(w_copies(PA + k - 4))

        return carry

    with _scope("stageA"):
        lax.fori_loop(0, 8, sa_body, 0)

    def ln1(seg):
        xb = x_v[seg, 8:SEG, :].astype(F32)
        return _ln(xb) * (1.0 + mod_v[0:1, D:2 * D]) + mod_v[0:1, 0:D]

    TH = T0 // 2

    def hs_body(t, carry):
        for r in range(0, TH, 32):
            ss = _strassen_lhs(*[_ld(h_v, (t + 4 * b,), a * TH + r, 32).astype(F32)
                                 for a in range(2) for b in range(2)])
            for k, i in enumerate(SSUM):
                hs_v[k, t, r:r + 32, :] = ss[i].astype(BF16)
        return carry

    lax.fori_loop(0, 4, hs_body, 0)

    def lhs1(i):
        if i == 2:
            tiles = [_ld(h_v, (t,), 0, TH) for t in range(4)]
        elif i == 3:
            tiles = [_ld(h_v, (t + 4,), TH, TH) for t in range(4)]
        else:
            tiles = [_ld(hs_v, (SSUM.index(i), t), 0, TH) for t in range(4)]
        return jnp.concatenate(tiles, axis=1)

    NP1 = (NP - PA) // P1U
    late = late_copies(False)
    nl = -(-len(late) // (3 * P1U))

    def p1_body(i, carry):
        p0 = PA + P1U * i
        with _scope("wait_w"):
            for u in range(P1U):
                wait(w_copies(p0 + u))

        for u in range(3 * P1U):
            p, j = p0 + u // 3, u % 3
            lo, hi = relayout(p * 6 + j * 2, slice(None))
            b = [lo[0:DH2], hi[0:DH2], lo[DH2:D], hi[DH2:D]]
            t = _strassen_rhs(*[x.astype(F32) for x in b])
            t = [b[0] if k == 1 else b[3] if k == 4 else t[k].astype(BF16) for k in range(7)]
            m = {k: _dot(lhs1(k), t[k]) for k in P1ORD}
            c = _strassen_out(m)
            store_lead(p, j, jnp.concatenate([c[0], c[2]], axis=0), jnp.concatenate([c[1], c[3]], axis=0))

            if u < 4:
                @pl.when(i < 2)
                def _():
                    start(w_copies(PA + 4 + 4 * i + u))
            elif u == 4:
                @pl.when(jnp.logical_and(i >= 1, i < 3))
                def _():
                    start([wo_copy(4 * (i - 1) + q) for q in range(4)])
            elif u == 5:
                @pl.when(i == 2)
                def _():
                    start(late_copies(True))

            @pl.when(i == NP1 - 1)
            def _():
                start(late[u * nl:(u + 1) * nl])

        hn_v[...] = ln1(0)
        return carry

    with _scope("phase1"):
        lax.fori_loop(0, NP1, p1_body, 0)

    with _scope("wait_wo"):
        wait([wo_copy(j) for j in range(8)])
        wait(late_copies(True))

    def prep_views(w, t_row, kh, nh, j, r0):
        src = w.at[pl.ds(j, nh + 1), pl.ds(pl.multiple_of(r0, 256), kh + 256), :]
        dst = lt_v.at[pl.ds(pl.multiple_of(t_row + j * kh + r0, 256), 4 * nh * kh + 256), :]
        return src, dst, kh, nh

    def prep(views, r0, n):
        src, dst, kh, nh = views
        t = _strassen_rhs(*[_ld(src, (b * nh,), a * kh + r0, n).astype(F32) for a in range(2) for b in range(2)])
        for k, i in enumerate(TSUM):
            dst[k * nh * kh + r0:k * nh * kh + r0 + n, :] = t[i].astype(BF16)

    def step(it, odd, mem):
        s = 2 * it + int(odd)
        lead = lt_v.at[pl.ds(pl.multiple_of(16 * s, 16), T1_ROW), :]
        lhs = jnp.concatenate([mem, hn_v[...]], axis=0).astype(BF16)
        hn_v[...] = ln1(jnp.minimum(s + 1, NSEG - 1))

        def proj(p):
            if p == 0:
                half = [_dot(lhs[:, 0:D // 2], _bf(w_v[c, 0:D // 4, :])) for c in range(6)]
                cols = [_dot(lhs[:, D // 2:D], _bf(w_v[c, D // 4:D // 2, :])) + half[c] for c in range(6)]
            for j in range(3):
                if p == 0:
                    r = _interleave(cols[j * 2], cols[j * 2 + 1])
                else:
                    r = _interleave(_dot(lhs, _bf(w_v[p * 6 + j * 2])), _dot(lhs, _bf(w_v[p * 6 + j * 2 + 1])))
                fr_v[p * 3 + j] = r.astype(BF16)

        def stack(p, j):
            return jnp.concatenate([fr_v[p * 3 + j],
                                    _ld(lead, (), (p * 3 + j) * 2 * T0, 16)], axis=0)

        def attn(pvs, qks):
            os_ = [_dot(pr_v[p, :, 0:80], stack(p, 2)) for p in pvs]
            ss = [lax.dot_general(stack(p, 0), stack(p, 1), (((1,), (1,)), ((), ())),
                                  preferred_element_type=F32) for p in qks]
            for p, o in zip(pvs, os_):
                for t, oh in enumerate(_deinterleave(o[0:64])):
                    lo_v[2 * p + t] = oh.astype(BF16)
                if odd:
                    ev = ev_v[p]
                    for k, sk in enumerate(_strassen_lhs(ev[0:8], ev[8:16], o[64:72], o[72:80])):
                        so_v[k, p, pl.ds(pl.multiple_of(8 * it, 8), 8), :] = sk.astype(BF16)
                else:
                    ev_v[p] = o[64:80]
            for p, sc_ in zip(qks, ss):
                fill = fill_v[...]
                sc_ = jnp.concatenate([sc_, jnp.zeros((80, 48), F32)], axis=1)
                sc_ = jnp.where(fill == 0.0, sc_, fill)
                mx = jnp.max(sc_, axis=-1, keepdims=True)
                e = jnp.exp2((sc_ - mx) * (scale * LOG2E))
                l = jnp.sum(e, axis=-1, keepdims=True)
                r = pl.reciprocal(l, approx=True)
                pr_v[p] = (e * (r * (2.0 - l * r))).astype(BF16)

        part = {}

        def wo(j, h0, h1):
            lo = jnp.concatenate([lo_v[h] for h in range(h0, h1)], axis=1)
            r = _dot(lo, _bf(wo_v[j, h0 * 64:h1 * 64, :]))
            part[j] = r + part[j] if j in part else r

        pc = jnp.maximum(it - 4, 0)
        if odd:
            views = prep_views(w2_v, T2_ROW, FH, DH2 // 128, pc & 3, (pc >> 2) * 256)
        else:
            views = prep_views(w1_v, T1_ROW, DH2, FH // 128, pc >> 1, (pc & 1) * 256)
        npiece = 0
        for op in SCHED:
            if op[0] == "proj":
                proj(op[1])
            elif op[0] == "attn":
                attn(op[1], op[2])
                if npiece < 8:
                    prep(views, npiece * 32, 32)
                    npiece += 1
            else:
                wo(*op[1:])
        res = jnp.concatenate([part[j] for j in range(8)], axis=1)
        x1_v[pl.ds(pl.multiple_of(SEG * s + 8, 8), TPS), :] = res[8:32]
        return res[0:8]

    with _scope("main"):
        def steps(i, mem):
            with _scope("iter"):
                mem = step(i, True, step(i, False, mem))

            @pl.when(i == NEARLY - 1)
            def _():
                wait(late)

            return mem

        lax.fori_loop(0, NSEG // 2, steps, mem0_ref[...].astype(F32))

    def wo_body(j, carry):
        acc = {}
        for kc in range(4):
            b = [jnp.concatenate([_bf(wo_v[j + 4 * n, (2 * p + t) * 64:(2 * p + t + 1) * 64, :])
                                  for p in range(4 * kc, 4 * kc + 4)], axis=0)
                 for t in range(2) for n in range(2)]
            tt = _strassen_rhs(*[x.astype(F32) for x in b])
            tt = [b[0] if k == 1 else b[3] if k == 4 else tt[k].astype(BF16) for k in range(7)]
            for k in P1ORD:
                sk = jnp.concatenate([_ld(so_v, (k, p), 0, TH) for p in range(4 * kc, 4 * kc + 4)], axis=1)
                y = _dot(sk, tt[k])
                acc[k] = y + acc[k] if kc else y
                if k in MODK:
                    q = MODK.index(k)
                    ct = 8 * j + 2 * kc + q // 2
                    k0 = (q % 2) * DH2
                    m = _dot(sc_v[:, k0:k0 + DH2], wmod_v[k0:k0 + DH2, pl.ds(_mult(ct, 128), 128)])
                    if q % 2:
                        mod_v[:, pl.ds(_mult(ct + 16, 128), 128)] = m + mhalf
                    else:
                        mhalf = m
        for t, c in enumerate(_strassen_out(acc)):
            cs = pl.ds(pl.multiple_of((j + 4 * (t % 2)) * 128, 128), 128)
            for g in range(NSEG // 2):
                r0 = (2 * g + t // 2) * SEG
                x1_v[r0:r0 + 8, cs] = c[8 * g:8 * g + 8]
        return carry

    with _scope("p3a"):
        lax.fori_loop(0, 4, wo_body, 0)

    def rhs(w, t_row, kh, nh, i, j, k0, nk):
        if i == 1:
            return _ld(w, (j,), k0, nk)
        if i == 4:
            return _ld(w, (j + nh,), kh + k0, nk)
        return _ld(lt_v, (), t_row + (TSUM.index(i) * nh + j) * kh + k0, nk)

    def out_copy(i, q):
        segs = pl.ds(i * (FB // SEG), FB // SEG)
        return [pltpu.make_async_copy(x_v.at[segs, :, cols], out_hbm.at[segs, :, cols], sems.at[SEM_OUT + i])
                for cols in (pl.ds(q * OC, OC), pl.ds(DH2 + q * OC, OC))]

    HB = FB // 2

    def resid1(r0, k0, n, c0=0, nc=D):
        if n >= SEG:
            xb = x_v[pl.ds((r0 >> 5) + k0 // SEG, n // SEG), :, c0:c0 + nc].astype(F32).reshape(n, nc)
        else:
            xb = x_v[(r0 >> 5) + k0 // SEG, k0 % SEG:k0 % SEG + n, c0:c0 + nc].astype(F32)
        return xb + mod_v[0:1, 2 * D + c0:2 * D + c0 + nc] * x1_v[pl.ds(r0 + k0, n), c0:c0 + nc]

    def ln2(slot, r0, k0, n):
        top, bot = [_ln(resid1(r0, t * HB + k0, n)) * (1.0 + mod_v[0:1, 4 * D:5 * D]) + mod_v[0:1, 3 * D:4 * D]
                    for t in range(2)]
        ss = _strassen_lhs(top[:, 0:DH2], top[:, DH2:D], bot[:, 0:DH2], bot[:, DH2:D])
        for i in range(7):
            for j in range(DH2 // 128):
                h2_v[slot, i, j, k0:k0 + n, :] = ss[i][:, j * 128:(j + 1) * 128].astype(BF16)

    ln2(0, 0, 0, HB)

    def ffn_body(i, carry):
        r0 = pl.multiple_of(i * FB, FB)
        rn = pl.multiple_of(jnp.minimum(r0 + FB, S - FB), FB)
        slot = lax.rem(i, 2)
        nf = FH // FC
        nt = FC // 128
        nq = DH2 // OC
        acc = {}
        gs = {}

        def up(f, t):
            c0 = f * FC + t * 128
            c = _strassen_out({
                k: _dot(jnp.concatenate([_ld(h2_v, (slot, k, j), 0, HB) for j in range(DH2 // 128)], axis=1),
                        rhs(w1_v, T1_ROW, DH2, FH // 128, k, c0 // 128, 0, DH2)) for k in UPORD})
            b1a, b1b = bias_v[0:1, c0:c0 + 128], bias_v[0:1, FH + c0:FH + c0 + 128]
            gs[f, t] = _strassen_lhs(_gelu(c[0] + b1a), _gelu(c[1] + b1b), _gelu(c[2] + b1a), _gelu(c[3] + b1b))
            if t == nt - 1:
                gs[f] = [jnp.concatenate([gs[f, u][k] for u in range(nt)], axis=1).astype(BF16) for k in range(7)]

        def down(f, q):
            for k in DNORD:
                y = _dot(gs[f][k], rhs(w2_v, T2_ROW, FH, DH2 // 128, k, q, f * FC, FC))
                acc[k, q] = y + acc[k, q] if f else y
            if f == nf - 1:
                c = _strassen_out([acc[k, q] for k in range(7)])
                for t in range(4):
                    k0, c0 = (t // 2) * HB, (t % 2) * DH2 + q * OC
                    y = (c[t] + bias_v[0:1, FF + c0:FF + c0 + OC]) * mod_v[0:1, 5 * D + c0:5 * D + c0 + OC]
                    o = (resid1(r0, k0, HB, c0, OC) + y).reshape(HB // SEG, SEG, OC).astype(BF16)
                    x_v[pl.ds((r0 >> 5) + k0 // SEG, HB // SEG), :, c0:c0 + OC] = o
                start(out_copy(i, q))

        for t in range(nt):
            up(0, t)
        w = 0
        for f in range(nf):
            for t in range(nt):
                if f + 1 < nf:
                    up(f + 1, t)
                if w < len(LNP) and LNP[w]:
                    ln2(1 - slot, rn, sum(LNP[:w]), LNP[w])
                w += 1
                for q in range(t * nq // nt, (t + 1) * nq // nt):
                    down(f, q)
        return carry

    with _scope("ffn"):
        lax.fori_loop(0, S // FB, ffn_body, 0)
    with _scope("wait_out"):
        for i in range(S // FB):
            for q in range(DH2 // OC):
                wait(out_copy(i, q))


@jax.jit
def pallas_adaLN_cond__memory_aug_recurrent_mem_tr__dense_activation_gelu__prompt_kernel(
    A_x, A_mem0, A_Wq, A_Wk, A_Wv, A_Wo, A_seg_len, B_x, B_w1, B_b1, B_w2, B_b2, c, w_mod,
):
    del A_seg_len, B_x
    assert A_x.shape == (1, S, D)
    hbm = pl.BlockSpec(memory_space=pl.ANY)
    out = pl.pallas_call(
        _kernel,
        out_shape=jax.ShapeDtypeStruct((NSEG, SEG, D), BF16),
        in_specs=[hbm] * 12,
        out_specs=hbm,
        scratch_shapes=[
            pltpu.VMEM((NSEG, SEG, D), BF16),
            pltpu.VMEM((8, T0, 128), BF16),
            pltpu.VMEM((TPS, D), F32),
            pltpu.VMEM((2, 7, 4, FB // 2, 128), BF16),
            pltpu.VMEM((S, D), F32),
            pltpu.VMEM((D, 4 * D), BF16),
            pltpu.VMEM((8, 6 * D), F32),
            pltpu.VMEM((8, D), BF16),
            pltpu.VMEM((6 * NP, D // 2, 128), U32),
            pltpu.VMEM((8, H * DH // 2, 128), U32),
            pltpu.VMEM((FF // 128, D, 128), BF16),
            pltpu.VMEM((D // 128, FF, 128), BF16),
            pltpu.VMEM((LT_ROWS, 128), BF16),
            pltpu.VMEM((3 * NP, 64, 128), BF16),
            pltpu.VMEM((H, 32, 128), BF16),
            pltpu.VMEM((NP, 80, 128), BF16),
            pltpu.VMEM((80, 128), F32),
            pltpu.VMEM((1, FF + D), F32),
            pltpu.VMEM((8, T0, 128), F32),
            pltpu.VMEM((M, D), BF16),
            pltpu.VMEM((FF,), BF16),
            pltpu.VMEM((D,), BF16),
            pltpu.VMEM((1, D), BF16),
            pltpu.VMEM((5, 4, T0 // 2, 128), BF16),
            pltpu.VMEM((7, NP, T0 // 2, 128), BF16),
            pltpu.VMEM((NP, 16, 128), F32),
            pltpu.SemaphoreType.DMA((SEM_N,)),
        ],
        compiler_params=pltpu.CompilerParams(vmem_limit_bytes=122 * 1024 * 1024, disable_bounds_checks=True,
                                             disable_semaphore_checks=True),
    )(
        A_x.reshape(NSEG, SEG, D), A_mem0.reshape(M, D),
        A_Wq.reshape(D // 2, 2, H, DH), A_Wk.reshape(D // 2, 2, H, DH), A_Wv.reshape(D // 2, 2, H, DH),
        A_Wo.reshape(H * DH, D), B_w1, B_b1, B_w2, B_b2, c, w_mod,
    )
    return out.reshape(1, S, D)
```

```python
import contextlib

import jax
import jax.numpy as jnp
from jax import lax
import jax.experimental.pallas as pl
import jax.experimental.pallas.tpu as pltpu

F32 = jnp.float32
BF16 = jnp.bfloat16
U32 = jnp.uint32

S = 2048
D = 1024
H = 32
DH = 128
M = 8
SEG = 32
FF = 3584
NSEG = S // SEG
NP = H // 2
TPS = 24
T0 = S - NSEG * TPS
EPS = 1e-5
P1U = 2
P1ORD = (1, 4, 3, 2, 0, 6, 5)
UPORD = (1, 4, 3, 2, 0, 6, 5)
DNORD = (1, 4, 3, 2, 0, 6, 5)
NEARLY = 4
PA = 4
LNP = (16,) * 8
MODK = (1, 3, 0, 6)
LOG2E = 1.4426950408889634
FB = 256
OC = 128
FC = 256
FH = FF // 2
DH2 = D // 2
T1_ROW = 3 * NP * 2 * T0
T2_ROW = T1_ROW + 5 * (FH // 128) * DH2
LT_ROWS = T2_ROW + 5 * (DH2 // 128) * FH + 16
SSUM = (0, 1, 4, 5, 6)
TSUM = (0, 2, 3, 5, 6)
SEM_W, SEM_A, SEM_M, SEM_MISC, SEM_OUT = 0, 16, 24, 32, 40
SEM_N = SEM_OUT + S // FB


def _make_sched(g):
    out = []

    def rng(a, b):
        return tuple(range(max(a, 0), max(b, 0)))

    for p in range(NP):
        out.append(("proj", p))
        if p % g == 0 and p >= g:
            out.append(("attn", rng(p - 2 * g, p - g), rng(p - g, p)))
    h1 = 2 * (NP - 2 * g)
    h2 = 2 * (NP - g)
    if g == 4:
        out += [("wo", j, 0, h1) for j in (0, 1)]
        out.append(("attn", rng(NP - 2 * g, NP - g), rng(NP - g, NP)))
        out += [("wo", j, 0, h1) for j in (2, 3, 4, 5)]
        out.append(("attn", rng(NP - g, NP), ()))
        out += [("wo", j, 0, h1) for j in (6, 7)]
        out += [("wo", j, h1, h2) for j in range(8)]
        out += [("wo", j, h2, H) for j in range(8)]
    else:
        out += [("wo", 0, 0, h1)]
        out.append(("attn", rng(NP - 2 * g, NP - g), rng(NP - g, NP)))
        out += [("wo", j, 0, h1) for j in (1, 2, 3)]
        out.append(("attn", rng(NP - g, NP), ()))
        out += [("wo", j, 0, h1) for j in (4, 5, 6, 7)]
        out += [("wo", j, h1, H) for j in range(8)]
    return out


SCHED = _make_sched(2)
_SCOPES = False


def _scope(name):
    return jax.named_scope(name) if _SCOPES else contextlib.nullcontext()


def _dot(a, b):
    return jnp.dot(a, b, preferred_element_type=F32)


def _bf(x):
    return pltpu.bitcast(x, BF16)


def _u32(x):
    return pltpu.bitcast(x, U32)


def _u32f(x):
    return pltpu.bitcast(x, U32)


def _ld(ref, idx, r0, n):
    return _bf(ref.at[(*idx, pl.ds(r0, n), slice(None))].bitcast(U32)[...])


def _ln(x):
    m = jnp.mean(x, axis=-1, keepdims=True)
    xc = x - m
    v = jnp.mean(xc * xc, axis=-1, keepdims=True)
    return xc * lax.rsqrt(v + EPS)


def _gelu(x):
    c = 0.7978845608028654
    return 0.5 * x * (1.0 + jnp.tanh(c * (x + 0.044715 * (x * x * x))))


def _strassen_lhs(a11, a12, a21, a22):
    return [a11 + a22, a21 + a22, a11, a22, a11 + a12, a21 - a11, a12 - a22]


def _strassen_rhs(b11, b12, b21, b22):
    return [b11 + b22, b11, b12 - b22, b21 - b11, b22, b11 + b12, b21 + b22]


def _strassen_out(m):
    return (m[0] + m[3] - m[4] + m[6], m[2] + m[4], m[1] + m[3], m[0] - m[1] + m[2] + m[5])


def _interleave(a, b):
    n = a.shape[0] // 8
    parts = []
    for g in range(n):
        parts.append(a[8 * g:8 * g + 8])
        parts.append(b[8 * g:8 * g + 8])
    return jnp.concatenate(parts, axis=0)


def _deinterleave(v):
    n = v.shape[0] // 16
    a = jnp.concatenate([v[16 * g:16 * g + 8] for g in range(n)], axis=0)
    b = jnp.concatenate([v[16 * g + 8:16 * g + 16] for g in range(n)], axis=0)
    return a, b


def _kernel(x_hbm, mem0_hbm, wq_hbm, wk_hbm, wv_hbm, wo_hbm, w1_hbm, b1_hbm, w2_hbm, b2_hbm,
            c_hbm, wmod_hbm, out_hbm,
            x_v, h_v, hn_v, h2_v, x1_v, wmod_v, mod_v, sc_v, w_v, wo_v, w1_v, w2_v, lt_v, fr_v, lo_v, pr_v, fill_v, bias_v, n_v,
            mem0_ref, b1_ref, b2_ref, c_ref, hs_v, so_v, ev_v, st_v,
            sems):
    w32 = [r.bitcast(U32) for r in (wq_hbm, wk_hbm, wv_hbm)]
    wo32 = wo_hbm.bitcast(U32)

    def w_copies(p):
        return [pltpu.make_async_copy(w32[j].at[:, par, p, :], w_v.at[p * 6 + j * 2 + par], sems.at[SEM_W + p])
                for j in range(3) for par in range(2)]

    def _mult(i, m):
        return i * m if isinstance(i, int) else pl.multiple_of(i * m, m)

    def wa_copies(k, pair=None):
        r = pl.ds(_mult(k, 64), 64)
        return [pltpu.make_async_copy(w32[j].at[r, par, p, :], w_v.at[p * 6 + j * 2 + par, r], sems.at[SEM_A + k])
                for p in (range(PA) if pair is None else (pair,)) for j in range(3) for par in range(2)]

    def m_copies(k):
        return [pltpu.make_async_copy(wmod_hbm.at[:, pl.ds(_mult(k + 8 * t, 128), 128)], wmod_v.at[16 + k + 8 * t],
                                      sems.at[SEM_M + k]) for t in range(2)]

    def start(cps):
        for cp in cps:
            cp.start()

    def wait(cps):
        for cp in cps:
            cp.wait()

    cp_x0 = pltpu.make_async_copy(x_hbm.at[:, 0:8, :], x_v.at[:, 0:8, :], sems.at[SEM_MISC + 1])

    def wo_copy(j):
        return pltpu.make_async_copy(wo32.at[:, pl.ds(_mult(j, 128), 128)], wo_v.at[j], sems.at[SEM_MISC + 3])

    def late_copies(first):
        sem = sems.at[SEM_MISC + (4 if first else 5)]
        sg = slice(1, 2 * NEARLY + 1) if first else slice(2 * NEARLY + 1, NSEG)
        cps = [(x_hbm.at[sg, 8:SEG, :], x_v.at[sg, 8:SEG, :])]
        cps += [(wmod_hbm.at[:, (16 + j) * 128:(17 + j) * 128], wmod_v.at[j])
                for j in (range(NEARLY) if first else range(NEARLY, 32))]
        for src, dst, nt, kh in ((w1_hbm, w1_v, FF // 128, DH2), (w2_hbm, w2_v, D // 128, FH)):
            for j in range(nt):
                cols = slice(j * 128, (j + 1) * 128)
                if j % (nt // 2):
                    rows = [] if first else [slice(None)]
                else:
                    rows = [slice(a * kh, a * kh + 256) if first else slice(a * kh + 256, (a + 1) * kh)
                            for a in range(2)]
                cps += [(src.at[r, cols], dst.at[j, r]) for r in rows]
        return [pltpu.make_async_copy(src, dst, sem) for src, dst in cps]

    cp_small = [pltpu.make_async_copy(src, dst, sems.at[SEM_MISC])
                for src, dst in ((c_hbm, c_ref), (mem0_hbm, mem0_ref), (b1_hbm, b1_ref), (b2_hbm, b2_ref),
                                 (x_hbm.at[0, 8:SEG, :], x_v.at[0, 8:SEG, :]))]

    start(cp_small)
    cp_x0.start()
    start(m_copies(0))
    for k in range(2):
        start(m_copies(k + 1))
        start(wa_copies(k))

    scale = DH ** -0.5
    ri = lax.broadcasted_iota(jnp.int32, (80, 128), 0)
    ci = lax.broadcasted_iota(jnp.int32, (80, 128), 1)
    same_head = (((ri >> 3) & 1) == ((ci >> 3) & 1)) & (ci < 80)
    rpos = (((ri >> 4) & 3) << 3) + (ri & 7)
    cpos = (((ci >> 4) & 3) << 3) + (ci & 7)
    keep = (ri < 16) | (ci < 16) | (rpos >= cpos)
    fill_v[...] = jnp.where(same_head, jnp.where(keep, 0.0, -1e9 / scale), -jnp.inf).astype(F32)

    wait(cp_small)
    c = c_ref[...].astype(F32)
    sc = jnp.broadcast_to(c * jax.nn.sigmoid(c), (8, D)).astype(BF16)

    sc_v[...] = sc
    for k in range(8):
        st_v[k * 128:(k + 1) * 128, :] = jnp.broadcast_to(sc[0:1, k * 128:(k + 1) * 128].astype(F32), (128, 128)).T
    bias_v[:, 0:FF] = b1_ref[...].astype(F32).reshape(1, FF)
    bias_v[:, FF:FF + D] = b2_ref[...].astype(F32).reshape(1, D)

    def zero_body(i, carry):
        x1_v[pl.ds(pl.multiple_of(i * 64, 64), 64), :] = jnp.zeros((64, D), F32)
        return carry

    lax.fori_loop(0, PA * 6, zero_body, 0)

    def relayout(c, rows):
        a = w_v[c, rows, :]
        b = w_v[c + 1, rows, :]
        lo = (a & jnp.uint32(0xFFFF)) | (b << 16)
        hi = (a >> 16) | (b & jnp.uint32(0xFFFF0000))
        w_v[c, rows, :] = lo
        w_v[c + 1, rows, :] = hi
        return _bf(lo), _bf(hi)

    def store_lead(p, j, a, b):
        lt_v[pl.ds(_mult(p * 3 + j, 2 * T0), 2 * T0), :] = _interleave(a, b).astype(BF16)

    def mod_tile(ct):
        m = _dot(sc_v[...], _ld(wmod_v, (16 + ct,), 0, D))
        mod_v[:, pl.ds(_mult(ct, 128), 128)] = m
        return m[0:1]

    with _scope("wait_x0"):
        cp_x0.wait()

    def ln1_body(i, carry):
        r = pl.multiple_of(i * 128, 128)
        n = _ln(x_v[pl.ds(i * 16, 16), 0:8, :].astype(F32).reshape(128, D))
        for k in range(8):
            n_v[k, pl.ds(r, 128), :] = n[:, k * 128:(k + 1) * 128]
        return carry

    with _scope("ln1"):
        lax.fori_loop(0, T0 // 128, ln1_body, 0)
    start(m_copies(3))
    start(wa_copies(2))
    with _scope("wait_m0"):
        wait(m_copies(0))
    h_v[0] = (n_v[0] * (1.0 + mod_tile(8)) + mod_tile(0)).astype(BF16)

    def sa_body(k, carry):
        with _scope("wait_a"):
            wait(wa_copies(k))

            @pl.when(k < 7)
            def _():
                wait(m_copies(k + 1))

        kn = jnp.minimum(k + 1, 7)
        rows = pl.ds(pl.multiple_of(k * 64, 64), 64)
        hk = _ld(h_v, (k,), 0, T0)
        for p in range(PA):
            for j in range(3):
                c = p * 6 + j * 2
                res = []
                for t, w in enumerate(relayout(c, rows)):
                    acc = x1_v.at[(c + t) // 8 * T0:((c + t) // 8 + 1) * T0,
                                  (c + t) % 8 * 128:((c + t) % 8 + 1) * 128]
                    r = _dot(hk, w) + acc[...]
                    acc[...] = r
                    res.append(r)
                store_lead(p, j, *res)
                if c == 2:
                    sh = mod_tile(kn)
                if c == 6:
                    s1 = 1.0 + mod_tile(kn + 8)

                    @pl.when(k + 4 < 8)
                    def _():
                        start(m_copies(k + 4))

            @pl.when(k + 3 < 8)
            def _():
                start(wa_copies(k + 3, p))

        h_v[kn] = (n_v[kn] * s1 + sh).astype(BF16)


        @pl.when(k >= 4)
        def _():
            start(w_copies(PA + k - 4))

        return carry

    with _scope("stageA"):
        lax.fori_loop(0, 8, sa_body, 0)

    def ln1(seg):
        xb = x_v[seg, 8:SEG, :].astype(F32)
        return _ln(xb) * (1.0 + mod_v[0:1, D:2 * D]) + mod_v[0:1, 0:D]

    TH = T0 // 2

    def hs_body(t, carry):
        for r in range(0, TH, 32):
            ss = _strassen_lhs(*[_ld(h_v, (t + 4 * b,), a * TH + r, 32).astype(F32)
                                 for a in range(2) for b in range(2)])
            for k, i in enumerate(SSUM):
                hs_v[k, t, r:r + 32, :] = ss[i].astype(BF16)
        return carry

    lax.fori_loop(0, 4, hs_body, 0)

    def lhs1(i):
        if i == 2:
            tiles = [_ld(h_v, (t,), 0, TH) for t in range(4)]
        elif i == 3:
            tiles = [_ld(h_v, (t + 4,), TH, TH) for t in range(4)]
        else:
            tiles = [_ld(hs_v, (SSUM.index(i), t), 0, TH) for t in range(4)]
        return jnp.concatenate(tiles, axis=1)

    NP1 = (NP - PA) // P1U
    late = late_copies(False)
    nl = -(-len(late) // (3 * P1U))

    def p1_body(i, carry):
        p0 = PA + P1U * i
        with _scope("wait_w"):
            for u in range(P1U):
                wait(w_copies(p0 + u))

        for u in range(3 * P1U):
            p, j = p0 + u // 3, u % 3
            lo, hi = relayout(p * 6 + j * 2, slice(None))
            b = [lo[0:DH2], hi[0:DH2], lo[DH2:D], hi[DH2:D]]
            t = _strassen_rhs(*[x.astype(F32) for x in b])
            t = [b[0] if k == 1 else b[3] if k == 4 else t[k].astype(BF16) for k in range(7)]
            m = {k: _dot(lhs1(k), t[k]) for k in P1ORD}
            c = _strassen_out(m)
            store_lead(p, j, jnp.concatenate([c[0], c[2]], axis=0), jnp.concatenate([c[1], c[3]], axis=0))

            if u < 4:
                @pl.when(i < 2)
                def _():
                    start(w_copies(PA + 4 + 4 * i + u))
            elif u == 4:
                @pl.when(jnp.logical_and(i >= 1, i < 3))
                def _():
                    start([wo_copy(4 * (i - 1) + q) for q in range(4)])
            elif u == 5:
                @pl.when(i == 2)
                def _():
                    start(late_copies(True))

            @pl.when(i == NP1 - 1)
            def _():
                start(late[u * nl:(u + 1) * nl])

        hn_v[...] = ln1(0)
        return carry

    with _scope("phase1"):
        lax.fori_loop(0, NP1, p1_body, 0)

    with _scope("wait_wo"):
        wait([wo_copy(j) for j in range(8)])
        wait(late_copies(True))

    def prep_views(w, t_row, kh, nh, j, r0):
        src = w.at[pl.ds(j, nh + 1), pl.ds(pl.multiple_of(r0, 256), kh + 256), :]
        dst = lt_v.at[pl.ds(pl.multiple_of(t_row + j * kh + r0, 256), 4 * nh * kh + 256), :]
        return src, dst, kh, nh

    def prep(views, r0, n):
        src, dst, kh, nh = views
        t = _strassen_rhs(*[_ld(src, (b * nh,), a * kh + r0, n).astype(F32) for a in range(2) for b in range(2)])
        for k, i in enumerate(TSUM):
            dst[k * nh * kh + r0:k * nh * kh + r0 + n, :] = t[i].astype(BF16)

    def step(it, odd, mem, macc):
        s = 2 * it + int(odd)
        lead = lt_v.at[pl.ds(pl.multiple_of(16 * s, 16), T1_ROW), :]
        lhs = jnp.concatenate([mem, hn_v[...]], axis=0).astype(BF16)
        hn_v[...] = ln1(jnp.minimum(s + 1, NSEG - 1))

        def proj(p):
            if p == 0:
                half = [_dot(lhs[:, 0:D // 2], _bf(w_v[c, 0:D // 4, :])) for c in range(6)]
                cols = [_dot(lhs[:, D // 2:D], _bf(w_v[c, D // 4:D // 2, :])) + half[c] for c in range(6)]
            for j in range(3):
                if p == 0:
                    r = _interleave(cols[j * 2], cols[j * 2 + 1])
                else:
                    r = _interleave(_dot(lhs, _bf(w_v[p * 6 + j * 2])), _dot(lhs, _bf(w_v[p * 6 + j * 2 + 1])))
                fr_v[p * 3 + j] = r.astype(BF16)

        def stack(p, j):
            return jnp.concatenate([fr_v[p * 3 + j],
                                    _ld(lead, (), (p * 3 + j) * 2 * T0, 16)], axis=0)

        def attn(pvs, qks):
            os_ = [_dot(pr_v[p, :, 0:80], stack(p, 2)) for p in pvs]
            ss = [lax.dot_general(stack(p, 0), stack(p, 1), (((1,), (1,)), ((), ())),
                                  preferred_element_type=F32) for p in qks]
            for p, o in zip(pvs, os_):
                for t, oh in enumerate(_deinterleave(o[0:64])):
                    lo_v[2 * p + t] = oh.astype(BF16)
                if odd:
                    ev = ev_v[p]
                    for k, sk in enumerate(_strassen_lhs(ev[0:8], ev[8:16], o[64:72], o[72:80])):
                        so_v[k, p, pl.ds(pl.multiple_of(8 * it, 8), 8), :] = sk.astype(BF16)
                else:
                    ev_v[p] = o[64:80]
            for p, sc_ in zip(qks, ss):
                fill = fill_v[...]
                sc_ = jnp.concatenate([sc_, jnp.zeros((80, 48), F32)], axis=1)
                sc_ = jnp.where(fill == 0.0, sc_, fill)
                mx = jnp.max(sc_, axis=-1, keepdims=True)
                e = jnp.exp2((sc_ - mx) * (scale * LOG2E))
                l = jnp.sum(e, axis=-1, keepdims=True)
                r = pl.reciprocal(l, approx=True)
                pr_v[p] = (e * (r * (2.0 - l * r))).astype(BF16)

        part = {}

        def wo(j, h0, h1):
            lo = jnp.concatenate([lo_v[h] for h in range(h0, h1)], axis=1)
            r = _dot(lo, _bf(wo_v[j, h0 * 64:h1 * 64, :]))
            part[j] = r + part[j] if j in part else r

        pc = jnp.maximum(it - 4, 0)
        if odd:
            views = prep_views(w2_v, T2_ROW, FH, DH2 // 128, pc & 3, (pc >> 2) * 256)
        else:
            views = prep_views(w1_v, T1_ROW, DH2, FH // 128, pc >> 1, (pc & 1) * 256)
        npiece = 0
        for op in SCHED:
            if op[0] == "proj":
                proj(op[1])
            elif op[0] == "attn":
                attn(op[1], op[2])
                if npiece < 8:
                    prep(views, npiece * 32, 32)
                    k0 = (8 * int(odd) + npiece) * 64
                    pr = _ld(wmod_v, (it,), k0, 64).astype(F32) * st_v[k0:k0 + 64, :]
                    for g in range(8):
                        macc = pr[8 * g:8 * g + 8] if macc is None else macc + pr[8 * g:8 * g + 8]
                    lt_v[LT_ROWS - 16:LT_ROWS, :] = _bf(_u32f(macc))
                    npiece += 1
            else:
                wo(*op[1:])
        res = jnp.concatenate([part[j] for j in range(8)], axis=1)
        x1_v[pl.ds(pl.multiple_of(SEG * s + 8, 8), TPS), :] = res[8:32]
        return res[0:8], macc

    with _scope("main"):
        def steps(i, mem):
            with _scope("iter"):
                mem, macc = step(i, True, *step(i, False, mem, None))
                mod_v[0:1, pl.ds(pl.multiple_of((16 + i) * 128, 128), 128)] = jnp.sum(macc, axis=0, keepdims=True)

            @pl.when(i == NEARLY - 1)
            def _():
                wait(late)

            return mem

        lax.fori_loop(0, NSEG // 2, steps, mem0_ref[...].astype(F32))

    def wo_body(j, carry):
        acc = {}
        for kc in range(4):
            b = [jnp.concatenate([_bf(wo_v[j + 4 * n, (2 * p + t) * 64:(2 * p + t + 1) * 64, :])
                                  for p in range(4 * kc, 4 * kc + 4)], axis=0)
                 for t in range(2) for n in range(2)]
            tt = _strassen_rhs(*[x.astype(F32) for x in b])
            tt = [b[0] if k == 1 else b[3] if k == 4 else tt[k].astype(BF16) for k in range(7)]
            for k in P1ORD:
                sk = jnp.concatenate([_ld(so_v, (k, p), 0, TH) for p in range(4 * kc, 4 * kc + 4)], axis=1)
                y = _dot(sk, tt[k])
                acc[k] = y + acc[k] if kc else y
        for t, c in enumerate(_strassen_out(acc)):
            cs = pl.ds(pl.multiple_of((j + 4 * (t % 2)) * 128, 128), 128)
            for g in range(NSEG // 2):
                r0 = (2 * g + t // 2) * SEG
                x1_v[r0:r0 + 8, cs] = c[8 * g:8 * g + 8]
        return carry

    with _scope("p3a"):
        lax.fori_loop(0, 4, wo_body, 0)

    def rhs(w, t_row, kh, nh, i, j, k0, nk):
        if i == 1:
            return _ld(w, (j,), k0, nk)
        if i == 4:
            return _ld(w, (j + nh,), kh + k0, nk)
        return _ld(lt_v, (), t_row + (TSUM.index(i) * nh + j) * kh + k0, nk)

    def out_copy(i, q):
        segs = pl.ds(i * (FB // SEG), FB // SEG)
        return [pltpu.make_async_copy(x_v.at[segs, :, cols], out_hbm.at[segs, :, cols], sems.at[SEM_OUT + i])
                for cols in (pl.ds(q * OC, OC), pl.ds(DH2 + q * OC, OC))]

    HB = FB // 2

    def resid1(r0, k0, n, c0=0, nc=D):
        if n >= SEG:
            xb = x_v[pl.ds((r0 >> 5) + k0 // SEG, n // SEG), :, c0:c0 + nc].astype(F32).reshape(n, nc)
        else:
            xb = x_v[(r0 >> 5) + k0 // SEG, k0 % SEG:k0 % SEG + n, c0:c0 + nc].astype(F32)
        return xb + mod_v[0:1, 2 * D + c0:2 * D + c0 + nc] * x1_v[pl.ds(r0 + k0, n), c0:c0 + nc]

    def ln2(slot, r0, k0, n):
        top, bot = [_ln(resid1(r0, t * HB + k0, n)) * (1.0 + mod_v[0:1, 4 * D:5 * D]) + mod_v[0:1, 3 * D:4 * D]
                    for t in range(2)]
        ss = _strassen_lhs(top[:, 0:DH2], top[:, DH2:D], bot[:, 0:DH2], bot[:, DH2:D])
        for i in range(7):
            for j in range(DH2 // 128):
                h2_v[slot, i, j, k0:k0 + n, :] = ss[i][:, j * 128:(j + 1) * 128].astype(BF16)

    ln2(0, 0, 0, HB)

    def ffn_body(i, carry):
        r0 = pl.multiple_of(i * FB, FB)
        rn = pl.multiple_of(jnp.minimum(r0 + FB, S - FB), FB)
        slot = lax.rem(i, 2)
        nf = FH // FC
        nt = FC // 128
        nq = DH2 // OC
        acc = {}
        gs = {}

        def up(f, t):
            c0 = f * FC + t * 128
            c = _strassen_out({
                k: _dot(jnp.concatenate([_ld(h2_v, (slot, k, j), 0, HB) for j in range(DH2 // 128)], axis=1),
                        rhs(w1_v, T1_ROW, DH2, FH // 128, k, c0 // 128, 0, DH2)) for k in UPORD})
            b1a, b1b = bias_v[0:1, c0:c0 + 128], bias_v[0:1, FH + c0:FH + c0 + 128]
            gs[f, t] = _strassen_lhs(_gelu(c[0] + b1a), _gelu(c[1] + b1b), _gelu(c[2] + b1a), _gelu(c[3] + b1b))
            if t == nt - 1:
                gs[f] = [jnp.concatenate([gs[f, u][k] for u in range(nt)], axis=1).astype(BF16) for k in range(7)]

        def down(f, q):
            for k in DNORD:
                y = _dot(gs[f][k], rhs(w2_v, T2_ROW, FH, DH2 // 128, k, q, f * FC, FC))
                acc[k, q] = y + acc[k, q] if f else y
            if f == nf - 1:
                c = _strassen_out([acc[k, q] for k in range(7)])
                for t in range(4):
                    k0, c0 = (t // 2) * HB, (t % 2) * DH2 + q * OC
                    y = (c[t] + bias_v[0:1, FF + c0:FF + c0 + OC]) * mod_v[0:1, 5 * D + c0:5 * D + c0 + OC]
                    o = (resid1(r0, k0, HB, c0, OC) + y).reshape(HB // SEG, SEG, OC).astype(BF16)
                    x_v[pl.ds((r0 >> 5) + k0 // SEG, HB // SEG), :, c0:c0 + OC] = o
                start(out_copy(i, q))

        for t in range(nt):
            up(0, t)
        w = 0
        for f in range(nf):
            for t in range(nt):
                if f + 1 < nf:
                    up(f + 1, t)
                if w < len(LNP) and LNP[w]:
                    ln2(1 - slot, rn, sum(LNP[:w]), LNP[w])
                w += 1
                for q in range(t * nq // nt, (t + 1) * nq // nt):
                    down(f, q)
        return carry

    with _scope("ffn"):
        lax.fori_loop(0, S // FB, ffn_body, 0)
    with _scope("wait_out"):
        for i in range(S // FB):
            for q in range(DH2 // OC):
                wait(out_copy(i, q))


@jax.jit
def pallas_adaLN_cond__memory_aug_recurrent_mem_tr__dense_activation_gelu__prompt_kernel(
    A_x, A_mem0, A_Wq, A_Wk, A_Wv, A_Wo, A_seg_len, B_x, B_w1, B_b1, B_w2, B_b2, c, w_mod,
):
    del A_seg_len, B_x
    assert A_x.shape == (1, S, D)
    hbm = pl.BlockSpec(memory_space=pl.ANY)
    out = pl.pallas_call(
        _kernel,
        out_shape=jax.ShapeDtypeStruct((NSEG, SEG, D), BF16),
        in_specs=[hbm] * 12,
        out_specs=hbm,
        scratch_shapes=[
            pltpu.VMEM((NSEG, SEG, D), BF16),
            pltpu.VMEM((8, T0, 128), BF16),
            pltpu.VMEM((TPS, D), F32),
            pltpu.VMEM((2, 7, 4, FB // 2, 128), BF16),
            pltpu.VMEM((S, D), F32),
            pltpu.VMEM((32, D, 128), BF16),
            pltpu.VMEM((8, 6 * D), F32),
            pltpu.VMEM((8, D), BF16),
            pltpu.VMEM((6 * NP, D // 2, 128), U32),
            pltpu.VMEM((8, H * DH // 2, 128), U32),
            pltpu.VMEM((FF // 128, D, 128), BF16),
            pltpu.VMEM((D // 128, FF, 128), BF16),
            pltpu.VMEM((LT_ROWS, 128), BF16),
            pltpu.VMEM((3 * NP, 64, 128), BF16),
            pltpu.VMEM((H, 32, 128), BF16),
            pltpu.VMEM((NP, 80, 128), BF16),
            pltpu.VMEM((80, 128), F32),
            pltpu.VMEM((1, FF + D), F32),
            pltpu.VMEM((8, T0, 128), F32),
            pltpu.VMEM((M, D), BF16),
            pltpu.VMEM((FF,), BF16),
            pltpu.VMEM((D,), BF16),
            pltpu.VMEM((1, D), BF16),
            pltpu.VMEM((5, 4, T0 // 2, 128), BF16),
            pltpu.VMEM((7, NP, T0 // 2, 128), BF16),
            pltpu.VMEM((NP, 16, 128), F32),
            pltpu.VMEM((D, 128), F32),
            pltpu.SemaphoreType.DMA((SEM_N,)),
        ],
        compiler_params=pltpu.CompilerParams(vmem_limit_bytes=122 * 1024 * 1024, disable_bounds_checks=True,
                                             disable_semaphore_checks=True),
    )(
        A_x.reshape(NSEG, SEG, D), A_mem0.reshape(M, D),
        A_Wq.reshape(D // 2, 2, H, DH), A_Wk.reshape(D // 2, 2, H, DH), A_Wv.reshape(D // 2, 2, H, DH),
        A_Wo.reshape(H * DH, D), B_w1, B_b1, B_w2, B_b2, c, w_mod,
    )
    return out.reshape(1, S, D)
```

```python
import contextlib

import jax
import jax.numpy as jnp
from jax import lax
import jax.experimental.pallas as pl
import jax.experimental.pallas.tpu as pltpu

F32 = jnp.float32
BF16 = jnp.bfloat16
U32 = jnp.uint32

S = 2048
D = 1024
H = 32
DH = 128
M = 8
SEG = 32
FF = 3584
NSEG = S // SEG
NP = H // 2
TPS = 24
T0 = S - NSEG * TPS
EPS = 1e-5
P1ORD = (1, 4, 3, 2, 0, 6, 5)
UPORD = (1, 4, 3, 2, 0, 6, 5)
DNORD = (1, 4, 3, 2, 0, 6, 5)
NEARLY = 4
UA = 8
P1N = 5
LNP = (16,) * 8
MODK = (1, 3, 0, 6)
LOG2E = 1.4426950408889634
FB = 256
OC = 128
FC = 256
FH = FF // 2
DH2 = D // 2
T1_ROW = 3 * NP * 2 * T0
T2_ROW = T1_ROW + 5 * (FH // 128) * DH2
LT_ROWS = T2_ROW + 5 * (DH2 // 128) * FH + 16
SSUM = (0, 1, 4, 5, 6)
TSUM = (0, 2, 3, 5, 6)
SEM_W, SEM_A, SEM_M, SEM_MISC, SEM_OUT = 0, 48, 56, 64, 72
SEM_N = SEM_OUT + S // FB


def _make_sched(g):
    out = []

    def rng(a, b):
        return tuple(range(max(a, 0), max(b, 0)))

    for p in range(NP):
        out.append(("proj", p))
        if p % g == 0 and p >= g:
            out.append(("attn", rng(p - 2 * g, p - g), rng(p - g, p)))
    h1 = 2 * (NP - 2 * g)
    h2 = 2 * (NP - g)
    if g == 4:
        out += [("wo", j, 0, h1) for j in (0, 1)]
        out.append(("attn", rng(NP - 2 * g, NP - g), rng(NP - g, NP)))
        out += [("wo", j, 0, h1) for j in (2, 3, 4, 5)]
        out.append(("attn", rng(NP - g, NP), ()))
        out += [("wo", j, 0, h1) for j in (6, 7)]
        out += [("wo", j, h1, h2) for j in range(8)]
        out += [("wo", j, h2, H) for j in range(8)]
    else:
        out += [("wo", 0, 0, h1)]
        out.append(("attn", rng(NP - 2 * g, NP - g), rng(NP - g, NP)))
        out += [("wo", j, 0, h1) for j in (1, 2, 3)]
        out.append(("attn", rng(NP - g, NP), ()))
        out += [("wo", j, 0, h1) for j in (4, 5, 6, 7)]
        out += [("wo", j, h1, H) for j in range(8)]
    return out


SCHED = _make_sched(2)
_SCOPES = False


def _scope(name):
    return jax.named_scope(name) if _SCOPES else contextlib.nullcontext()


def _dot(a, b):
    return jnp.dot(a, b, preferred_element_type=F32)


def _bf(x):
    return pltpu.bitcast(x, BF16)


def _u32(x):
    return pltpu.bitcast(x, U32)


def _u32f(x):
    return pltpu.bitcast(x, U32)


def _ld(ref, idx, r0, n):
    return _bf(ref.at[(*idx, pl.ds(r0, n), slice(None))].bitcast(U32)[...])


def _ln(x):
    m = jnp.mean(x, axis=-1, keepdims=True)
    xc = x - m
    v = jnp.mean(xc * xc, axis=-1, keepdims=True)
    return xc * lax.rsqrt(v + EPS)


def _gelu(x):
    c = 0.7978845608028654
    return 0.5 * x * (1.0 + jnp.tanh(c * (x + 0.044715 * (x * x * x))))


def _strassen_lhs(a11, a12, a21, a22):
    return [a11 + a22, a21 + a22, a11, a22, a11 + a12, a21 - a11, a12 - a22]


def _strassen_rhs(b11, b12, b21, b22):
    return [b11 + b22, b11, b12 - b22, b21 - b11, b22, b11 + b12, b21 + b22]


def _strassen_out(m):
    return (m[0] + m[3] - m[4] + m[6], m[2] + m[4], m[1] + m[3], m[0] - m[1] + m[2] + m[5])


def _interleave(a, b):
    n = a.shape[0] // 8
    parts = []
    for g in range(n):
        parts.append(a[8 * g:8 * g + 8])
        parts.append(b[8 * g:8 * g + 8])
    return jnp.concatenate(parts, axis=0)


def _deinterleave(v):
    n = v.shape[0] // 16
    a = jnp.concatenate([v[16 * g:16 * g + 8] for g in range(n)], axis=0)
    b = jnp.concatenate([v[16 * g + 8:16 * g + 16] for g in range(n)], axis=0)
    return a, b


def _kernel(x_hbm, mem0_hbm, wq_hbm, wk_hbm, wv_hbm, wo_hbm, w1_hbm, b1_hbm, w2_hbm, b2_hbm,
            c_hbm, wmod_hbm, out_hbm,
            x_v, h_v, hn_v, h2_v, x1_v, wmod_v, mod_v, sc_v, w_v, wo_v, w1_v, w2_v, lt_v, fr_v, lo_v, pr_v, fill_v, bias_v, n_v,
            mem0_ref, b1_ref, b2_ref, c_ref, hs_v, so_v, ev_v, st_v,
            sems):
    w32 = [r.bitcast(U32) for r in (wq_hbm, wk_hbm, wv_hbm)]
    wo32 = wo_hbm.bitcast(U32)

    def w_copies(p, js=range(3)):
        return [pltpu.make_async_copy(w32[j].at[:, par, p, :], w_v.at[p * 6 + j * 2 + par],
                                      sems.at[SEM_W + 3 * p + j]) for j in js for par in range(2)]

    def w_wait(u):
        both = w_v.at[pl.ds(2 * u, 2)]
        pltpu.make_async_copy(both, both, sems.at[SEM_W + u]).wait()

    def _mult(i, m):
        return i * m if isinstance(i, int) else pl.multiple_of(i * m, m)

    def wa_copies(k, units=range(UA)):
        r = pl.ds(_mult(k, 64), 64)
        return [pltpu.make_async_copy(w32[u % 3].at[r, par, u // 3, :], w_v.at[2 * u + par, r], sems.at[SEM_A + k])
                for u in units for par in range(2)]

    def m_copies(k):
        return [pltpu.make_async_copy(wmod_hbm.at[:, pl.ds(_mult(k + 8 * t, 128), 128)], wmod_v.at[16 + k + 8 * t],
                                      sems.at[SEM_M + k]) for t in range(2)]

    def start(cps):
        for cp in cps:
            cp.start()

    def wait(cps):
        for cp in cps:
            cp.wait()

    cp_x0 = pltpu.make_async_copy(x_hbm.at[:, 0:8, :], x_v.at[:, 0:8, :], sems.at[SEM_MISC + 1])

    def wo_copy(j):
        return pltpu.make_async_copy(wo32.at[:, pl.ds(_mult(j, 128), 128)], wo_v.at[j], sems.at[SEM_MISC + 3])

    def late_copies(first):
        sem = sems.at[SEM_MISC + (4 if first else 5)]
        sg = slice(1, 2 * NEARLY + 1) if first else slice(2 * NEARLY + 1, NSEG)
        cps = [(x_hbm.at[sg, 8:SEG, :], x_v.at[sg, 8:SEG, :])]
        cps += [(wmod_hbm.at[:, (16 + j) * 128:(17 + j) * 128], wmod_v.at[j])
                for j in (range(NEARLY) if first else range(NEARLY, 32))]
        for src, dst, nt, kh in ((w1_hbm, w1_v, FF // 128, DH2), (w2_hbm, w2_v, D // 128, FH)):
            for j in range(nt):
                cols = slice(j * 128, (j + 1) * 128)
                if j % (nt // 2):
                    rows = [] if first else [slice(None)]
                else:
                    rows = [slice(a * kh, a * kh + 256) if first else slice(a * kh + 256, (a + 1) * kh)
                            for a in range(2)]
                cps += [(src.at[r, cols], dst.at[j, r]) for r in rows]
        return [pltpu.make_async_copy(src, dst, sem) for src, dst in cps]

    cp_small = [pltpu.make_async_copy(src, dst, sems.at[SEM_MISC])
                for src, dst in ((c_hbm, c_ref), (mem0_hbm, mem0_ref), (b1_hbm, b1_ref), (b2_hbm, b2_ref),
                                 (x_hbm.at[0, 8:SEG, :], x_v.at[0, 8:SEG, :]))]

    start(cp_small)
    cp_x0.start()
    start(m_copies(0))
    for k in range(2):
        start(m_copies(k + 1))
        start(wa_copies(k))

    scale = DH ** -0.5
    ri = lax.broadcasted_iota(jnp.int32, (80, 128), 0)
    ci = lax.broadcasted_iota(jnp.int32, (80, 128), 1)
    same_head = (((ri >> 3) & 1) == ((ci >> 3) & 1)) & (ci < 80)
    rpos = (((ri >> 4) & 3) << 3) + (ri & 7)
    cpos = (((ci >> 4) & 3) << 3) + (ci & 7)
    keep = (ri < 16) | (ci < 16) | (rpos >= cpos)
    fill_v[...] = jnp.where(same_head, jnp.where(keep, 0.0, -1e9 / scale), -jnp.inf).astype(F32)

    wait(cp_small)
    c = c_ref[...].astype(F32)
    sc = jnp.broadcast_to(c * jax.nn.sigmoid(c), (8, D)).astype(BF16)

    sc_v[...] = sc
    for k in range(8):
        st_v[k * 128:(k + 1) * 128, :] = jnp.broadcast_to(sc[0:1, k * 128:(k + 1) * 128].astype(F32), (128, 128)).T
    bias_v[:, 0:FF] = b1_ref[...].astype(F32).reshape(1, FF)
    bias_v[:, FF:FF + D] = b2_ref[...].astype(F32).reshape(1, D)

    def zero_body(i, carry):
        x1_v[pl.ds(pl.multiple_of(i * 64, 64), 64), :] = jnp.zeros((64, D), F32)
        return carry

    lax.fori_loop(0, -(-UA // 4) * 8, zero_body, 0)

    def relayout(c, rows):
        a = w_v[c, rows, :]
        b = w_v[c + 1, rows, :]
        lo = (a & jnp.uint32(0xFFFF)) | (b << 16)
        hi = (a >> 16) | (b & jnp.uint32(0xFFFF0000))
        w_v[c, rows, :] = lo
        w_v[c + 1, rows, :] = hi
        return _bf(lo), _bf(hi)

    def store_lead(u, a, b):
        lt_v[pl.ds(_mult(u, 2 * T0), 2 * T0), :] = _interleave(a, b).astype(BF16)

    def mod_tile(ct):
        m = _dot(sc_v[...], _ld(wmod_v, (16 + ct,), 0, D))
        mod_v[:, pl.ds(_mult(ct, 128), 128)] = m
        return m[0:1]

    with _scope("wait_x0"):
        cp_x0.wait()

    def ln1_body(i, carry):
        r = pl.multiple_of(i * 128, 128)
        n = _ln(x_v[pl.ds(i * 16, 16), 0:8, :].astype(F32).reshape(128, D))
        for k in range(8):
            n_v[k, pl.ds(r, 128), :] = n[:, k * 128:(k + 1) * 128]
        return carry

    with _scope("ln1"):
        lax.fori_loop(0, T0 // 128, ln1_body, 0)
    start(m_copies(3))
    start(wa_copies(2))
    with _scope("wait_m0"):
        wait(m_copies(0))
    h_v[0] = (n_v[0] * (1.0 + mod_tile(8)) + mod_tile(0)).astype(BF16)

    def sa_body(k, carry):
        with _scope("wait_a"):
            wait(wa_copies(k))

            @pl.when(k < 7)
            def _():
                wait(m_copies(k + 1))

        kn = jnp.minimum(k + 1, 7)
        rows = pl.ds(pl.multiple_of(k * 64, 64), 64)
        hk = _ld(h_v, (k,), 0, T0)
        for u in range(UA):
            res = []
            for t, w in enumerate(relayout(2 * u, rows)):
                c = 2 * u + t
                acc = x1_v.at[c // 8 * T0:(c // 8 + 1) * T0, c % 8 * 128:(c % 8 + 1) * 128]
                r = _dot(hk, w) + acc[...]
                acc[...] = r
                res.append(r)
            store_lead(u, *res)
            if u == 1:
                sh = mod_tile(kn)
            if u == 3:
                s1 = 1.0 + mod_tile(kn + 8)

                @pl.when(k + 4 < 8)
                def _():
                    start(m_copies(k + 4))

            if u >= 4 and u % 2 == 0:
                @pl.when(k + 3 < 8)
                def _():
                    start(wa_copies(k + 3, range((u - 4) * 2, (u - 4) * 2 + 4)))

        h_v[kn] = (n_v[kn] * s1 + sh).astype(BF16)

        @pl.when(k == 4)
        def _():
            start(w_copies(UA // 3, range(UA % 3, 3)))

        @pl.when(k >= 4)
        def _():
            start(w_copies(UA // 3 + 1 + k - 4))

        return carry

    with _scope("stageA"):
        lax.fori_loop(0, 8, sa_body, 0)

    def ln1(seg):
        xb = x_v[seg, 8:SEG, :].astype(F32)
        return _ln(xb) * (1.0 + mod_v[0:1, D:2 * D]) + mod_v[0:1, 0:D]

    TH = T0 // 2

    def hs_body(t, carry):
        for r in range(0, TH, 32):
            ss = _strassen_lhs(*[_ld(h_v, (t + 4 * b,), a * TH + r, 32).astype(F32)
                                 for a in range(2) for b in range(2)])
            for k, i in enumerate(SSUM):
                hs_v[k, t, r:r + 32, :] = ss[i].astype(BF16)
        return carry

    lax.fori_loop(0, 4, hs_body, 0)

    def lhs1(i):
        if i == 2:
            tiles = [_ld(h_v, (t,), 0, TH) for t in range(4)]
        elif i == 3:
            tiles = [_ld(h_v, (t + 4,), TH, TH) for t in range(4)]
        else:
            tiles = [_ld(hs_v, (SSUM.index(i), t), 0, TH) for t in range(4)]
        return jnp.concatenate(tiles, axis=1)

    NP1 = (3 * NP - UA) // P1N
    late = late_copies(False)
    nl = -(-len(late) // P1N)
    PW = UA // 3 + 5

    def p1_body(i, carry):
        u0 = UA + P1N * i
        with _scope("wait_w"):
            for q in range(P1N):
                w_wait(u0 + q)

        for q in range(P1N):
            lo, hi = relayout(2 * (u0 + q), slice(None))
            b = [lo[0:DH2], hi[0:DH2], lo[DH2:D], hi[DH2:D]]
            t = _strassen_rhs(*[x.astype(F32) for x in b])
            t = [b[0] if k == 1 else b[3] if k == 4 else t[k].astype(BF16) for k in range(7)]
            c = _strassen_out({k: _dot(lhs1(k), t[k]) for k in P1ORD})
            store_lead(u0 + q, jnp.concatenate([c[0], c[2]], axis=0), jnp.concatenate([c[1], c[3]], axis=0))

            if q < 3:
                @pl.when(PW + 3 * i + q < NP)
                def _():
                    start(w_copies(PW + 3 * i + q))
            elif q == 3:
                @pl.when(jnp.logical_and(i >= 2, i < 4))
                def _():
                    start([wo_copy(4 * (i - 2) + r) for r in range(4)])
            else:
                @pl.when(i == 3)
                def _():
                    start(late_copies(True))

            @pl.when(i == NP1 - 1)
            def _():
                start(late[q * nl:(q + 1) * nl])

        hn_v[...] = ln1(0)
        return carry

    with _scope("phase1"):
        lax.fori_loop(0, NP1, p1_body, 0)

    with _scope("wait_wo"):
        wait([wo_copy(j) for j in range(8)])
        wait(late_copies(True))

    def prep_views(w, t_row, kh, nh, j, r0):
        src = w.at[pl.ds(j, nh + 1), pl.ds(pl.multiple_of(r0, 256), kh + 256), :]
        dst = lt_v.at[pl.ds(pl.multiple_of(t_row + j * kh + r0, 256), 4 * nh * kh + 256), :]
        return src, dst, kh, nh

    def prep(views, r0, n):
        src, dst, kh, nh = views
        t = _strassen_rhs(*[_ld(src, (b * nh,), a * kh + r0, n).astype(F32) for a in range(2) for b in range(2)])
        for k, i in enumerate(TSUM):
            dst[k * nh * kh + r0:k * nh * kh + r0 + n, :] = t[i].astype(BF16)

    def step(it, odd, mem, macc):
        s = 2 * it + int(odd)
        lead = lt_v.at[pl.ds(pl.multiple_of(16 * s, 16), T1_ROW), :]
        lhs = jnp.concatenate([mem, hn_v[...]], axis=0).astype(BF16)
        hn_v[...] = ln1(jnp.minimum(s + 1, NSEG - 1))

        def proj(p):
            if p == 0:
                half = [_dot(lhs[:, 0:D // 2], _bf(w_v[c, 0:D // 4, :])) for c in range(6)]
                cols = [_dot(lhs[:, D // 2:D], _bf(w_v[c, D // 4:D // 2, :])) + half[c] for c in range(6)]
            for j in range(3):
                if p == 0:
                    r = _interleave(cols[j * 2], cols[j * 2 + 1])
                else:
                    r = _interleave(_dot(lhs, _bf(w_v[p * 6 + j * 2])), _dot(lhs, _bf(w_v[p * 6 + j * 2 + 1])))
                fr_v[p * 3 + j] = r.astype(BF16)

        def stack(p, j):
            return jnp.concatenate([fr_v[p * 3 + j],
                                    _ld(lead, (), (p * 3 + j) * 2 * T0, 16)], axis=0)

        def attn(pvs, qks):
            os_ = [_dot(pr_v[p, :, 0:80], stack(p, 2)) for p in pvs]
            ss = [lax.dot_general(stack(p, 0), stack(p, 1), (((1,), (1,)), ((), ())),
                                  preferred_element_type=F32) for p in qks]
            for p, o in zip(pvs, os_):
                for t, oh in enumerate(_deinterleave(o[0:64])):
                    lo_v[2 * p + t] = oh.astype(BF16)
                if odd:
                    ev = ev_v[p]
                    for k, sk in enumerate(_strassen_lhs(ev[0:8], ev[8:16], o[64:72], o[72:80])):
                        so_v[k, p, pl.ds(pl.multiple_of(8 * it, 8), 8), :] = sk.astype(BF16)
                else:
                    ev_v[p] = o[64:80]
            for p, sc_ in zip(qks, ss):
                fill = fill_v[...]
                sc_ = jnp.concatenate([sc_, jnp.zeros((80, 48), F32)], axis=1)
                sc_ = jnp.where(fill == 0.0, sc_, fill)
                mx = jnp.max(sc_, axis=-1, keepdims=True)
                e = jnp.exp2((sc_ - mx) * (scale * LOG2E))
                l = jnp.sum(e, axis=-1, keepdims=True)
                r = pl.reciprocal(l, approx=True)
                pr_v[p] = (e * (r * (2.0 - l * r))).astype(BF16)

        part = {}

        def wo(j, h0, h1):
            lo = jnp.concatenate([lo_v[h] for h in range(h0, h1)], axis=1)
            r = _dot(lo, _bf(wo_v[j, h0 * 64:h1 * 64, :]))
            part[j] = r + part[j] if j in part else r

        pc = jnp.maximum(it - 4, 0)
        if odd:
            views = prep_views(w2_v, T2_ROW, FH, DH2 // 128, pc & 3, (pc >> 2) * 256)
        else:
            views = prep_views(w1_v, T1_ROW, DH2, FH // 128, pc >> 1, (pc & 1) * 256)
        npiece = 0
        for op in SCHED:
            if op[0] == "proj":
                proj(op[1])
            elif op[0] == "attn":
                attn(op[1], op[2])
                if npiece < 8:
                    prep(views, npiece * 32, 32)
                    k0 = (8 * int(odd) + npiece) * 64
                    pr = _ld(wmod_v, (it,), k0, 64).astype(F32) * st_v[k0:k0 + 64, :]
                    for g in range(8):
                        macc = pr[8 * g:8 * g + 8] if macc is None else macc + pr[8 * g:8 * g + 8]
                    lt_v[LT_ROWS - 16:LT_ROWS, :] = _bf(_u32f(macc))
                    npiece += 1
            else:
                wo(*op[1:])
        res = jnp.concatenate([part[j] for j in range(8)], axis=1)
        x1_v[pl.ds(pl.multiple_of(SEG * s + 8, 8), TPS), :] = res[8:32]
        return res[0:8], macc

    with _scope("main"):
        def steps(i, mem):
            with _scope("iter"):
                mem, macc = step(i, True, *step(i, False, mem, None))
                mod_v[0:1, pl.ds(pl.multiple_of((16 + i) * 128, 128), 128)] = jnp.sum(macc, axis=0, keepdims=True)

            @pl.when(i == NEARLY - 1)
            def _():
                wait(late)

            return mem

        lax.fori_loop(0, NSEG // 2, steps, mem0_ref[...].astype(F32))

    def wo_body(j, carry):
        acc = {}
        for kc in range(4):
            b = [jnp.concatenate([_bf(wo_v[j + 4 * n, (2 * p + t) * 64:(2 * p + t + 1) * 64, :])
                                  for p in range(4 * kc, 4 * kc + 4)], axis=0)
                 for t in range(2) for n in range(2)]
            tt = _strassen_rhs(*[x.astype(F32) for x in b])
            tt = [b[0] if k == 1 else b[3] if k == 4 else tt[k].astype(BF16) for k in range(7)]
            for k in P1ORD:
                sk = jnp.concatenate([_ld(so_v, (k, p), 0, TH) for p in range(4 * kc, 4 * kc + 4)], axis=1)
                y = _dot(sk, tt[k])
                acc[k] = y + acc[k] if kc else y
        for t, c in enumerate(_strassen_out(acc)):
            cs = pl.ds(pl.multiple_of((j + 4 * (t % 2)) * 128, 128), 128)
            for g in range(NSEG // 2):
                r0 = (2 * g + t // 2) * SEG
                x1_v[r0:r0 + 8, cs] = c[8 * g:8 * g + 8]
        return carry

    with _scope("p3a"):
        lax.fori_loop(0, 4, wo_body, 0)

    def rhs(w, t_row, kh, nh, i, j, k0, nk):
        if i == 1:
            return _ld(w, (j,), k0, nk)
        if i == 4:
            return _ld(w, (j + nh,), kh + k0, nk)
        return _ld(lt_v, (), t_row + (TSUM.index(i) * nh + j) * kh + k0, nk)

    def out_copy(i, q):
        segs = pl.ds(i * (FB // SEG), FB // SEG)
        return [pltpu.make_async_copy(x_v.at[segs, :, cols], out_hbm.at[segs, :, cols], sems.at[SEM_OUT + i])
                for cols in (pl.ds(q * OC, OC), pl.ds(DH2 + q * OC, OC))]

    HB = FB // 2

    def resid1(r0, k0, n, c0=0, nc=D):
        if n >= SEG:
            xb = x_v[pl.ds((r0 >> 5) + k0 // SEG, n // SEG), :, c0:c0 + nc].astype(F32).reshape(n, nc)
        else:
            xb = x_v[(r0 >> 5) + k0 // SEG, k0 % SEG:k0 % SEG + n, c0:c0 + nc].astype(F32)
        return xb + mod_v[0:1, 2 * D + c0:2 * D + c0 + nc] * x1_v[pl.ds(r0 + k0, n), c0:c0 + nc]

    def ln2(slot, r0, k0, n):
        top, bot = [_ln(resid1(r0, t * HB + k0, n)) * (1.0 + mod_v[0:1, 4 * D:5 * D]) + mod_v[0:1, 3 * D:4 * D]
                    for t in range(2)]
        ss = _strassen_lhs(top[:, 0:DH2], top[:, DH2:D], bot[:, 0:DH2], bot[:, DH2:D])
        for i in range(7):
            for j in range(DH2 // 128):
                h2_v[slot, i, j, k0:k0 + n, :] = ss[i][:, j * 128:(j + 1) * 128].astype(BF16)

    ln2(0, 0, 0, HB)

    def ffn_body(i, carry):
        r0 = pl.multiple_of(i * FB, FB)
        rn = pl.multiple_of(jnp.minimum(r0 + FB, S - FB), FB)
        slot = lax.rem(i, 2)
        nf = FH // FC
        nt = FC // 128
        nq = DH2 // OC
        acc = {}
        gs = {}

        def up(f, t):
            c0 = f * FC + t * 128
            c = _strassen_out({
                k: _dot(jnp.concatenate([_ld(h2_v, (slot, k, j), 0, HB) for j in range(DH2 // 128)], axis=1),
                        rhs(w1_v, T1_ROW, DH2, FH // 128, k, c0 // 128, 0, DH2)) for k in UPORD})
            b1a, b1b = bias_v[0:1, c0:c0 + 128], bias_v[0:1, FH + c0:FH + c0 + 128]
            gs[f, t] = _strassen_lhs(_gelu(c[0] + b1a), _gelu(c[1] + b1b), _gelu(c[2] + b1a), _gelu(c[3] + b1b))
            if t == nt - 1:
                gs[f] = [jnp.concatenate([gs[f, u][k] for u in range(nt)], axis=1).astype(BF16) for k in range(7)]

        def down(f, q):
            for k in DNORD:
                y = _dot(gs[f][k], rhs(w2_v, T2_ROW, FH, DH2 // 128, k, q, f * FC, FC))
                acc[k, q] = y + acc[k, q] if f else y
            if f == nf - 1:
                c = _strassen_out([acc[k, q] for k in range(7)])
                for t in range(4):
                    k0, c0 = (t // 2) * HB, (t % 2) * DH2 + q * OC
                    y = (c[t] + bias_v[0:1, FF + c0:FF + c0 + OC]) * mod_v[0:1, 5 * D + c0:5 * D + c0 + OC]
                    o = (resid1(r0, k0, HB, c0, OC) + y).reshape(HB // SEG, SEG, OC).astype(BF16)
                    x_v[pl.ds((r0 >> 5) + k0 // SEG, HB // SEG), :, c0:c0 + OC] = o
                start(out_copy(i, q))

        for t in range(nt):
            up(0, t)
        w = 0
        for f in range(nf):
            for t in range(nt):
                if f + 1 < nf:
                    up(f + 1, t)
                if w < len(LNP) and LNP[w]:
                    ln2(1 - slot, rn, sum(LNP[:w]), LNP[w])
                w += 1
                for q in range(t * nq // nt, (t + 1) * nq // nt):
                    down(f, q)
        return carry

    with _scope("ffn"):
        lax.fori_loop(0, S // FB, ffn_body, 0)
    with _scope("wait_out"):
        for i in range(S // FB):
            for q in range(DH2 // OC):
                wait(out_copy(i, q))


@jax.jit
def pallas_adaLN_cond__memory_aug_recurrent_mem_tr__dense_activation_gelu__prompt_kernel(
    A_x, A_mem0, A_Wq, A_Wk, A_Wv, A_Wo, A_seg_len, B_x, B_w1, B_b1, B_w2, B_b2, c, w_mod,
):
    del A_seg_len, B_x
    assert A_x.shape == (1, S, D)
    hbm = pl.BlockSpec(memory_space=pl.ANY)
    out = pl.pallas_call(
        _kernel,
        out_shape=jax.ShapeDtypeStruct((NSEG, SEG, D), BF16),
        in_specs=[hbm] * 12,
        out_specs=hbm,
        scratch_shapes=[
            pltpu.VMEM((NSEG, SEG, D), BF16),
            pltpu.VMEM((8, T0, 128), BF16),
            pltpu.VMEM((TPS, D), F32),
            pltpu.VMEM((2, 7, 4, FB // 2, 128), BF16),
            pltpu.VMEM((S, D), F32),
            pltpu.VMEM((32, D, 128), BF16),
            pltpu.VMEM((8, 6 * D), F32),
            pltpu.VMEM((8, D), BF16),
            pltpu.VMEM((6 * NP, D // 2, 128), U32),
            pltpu.VMEM((8, H * DH // 2, 128), U32),
            pltpu.VMEM((FF // 128, D, 128), BF16),
            pltpu.VMEM((D // 128, FF, 128), BF16),
            pltpu.VMEM((LT_ROWS, 128), BF16),
            pltpu.VMEM((3 * NP, 64, 128), BF16),
            pltpu.VMEM((H, 32, 128), BF16),
            pltpu.VMEM((NP, 80, 128), BF16),
            pltpu.VMEM((80, 128), F32),
            pltpu.VMEM((1, FF + D), F32),
            pltpu.VMEM((8, T0, 128), F32),
            pltpu.VMEM((M, D), BF16),
            pltpu.VMEM((FF,), BF16),
            pltpu.VMEM((D,), BF16),
            pltpu.VMEM((1, D), BF16),
            pltpu.VMEM((5, 4, T0 // 2, 128), BF16),
            pltpu.VMEM((7, NP, T0 // 2, 128), BF16),
            pltpu.VMEM((NP, 16, 128), F32),
            pltpu.VMEM((D, 128), F32),
            pltpu.SemaphoreType.DMA((SEM_N,)),
        ],
        compiler_params=pltpu.CompilerParams(vmem_limit_bytes=122 * 1024 * 1024, disable_bounds_checks=True,
                                             disable_semaphore_checks=True),
    )(
        A_x.reshape(NSEG, SEG, D), A_mem0.reshape(M, D),
        A_Wq.reshape(D // 2, 2, H, DH), A_Wk.reshape(D // 2, 2, H, DH), A_Wv.reshape(D // 2, 2, H, DH),
        A_Wo.reshape(H * DH, D), B_w1, B_b1, B_w2, B_b2, c, w_mod,
    )
    return out.reshape(1, S, D)
```

```python
import contextlib

import jax
import jax.numpy as jnp
from jax import lax
import jax.experimental.pallas as pl
import jax.experimental.pallas.tpu as pltpu

F32 = jnp.float32
BF16 = jnp.bfloat16
U32 = jnp.uint32

S = 2048
D = 1024
H = 32
DH = 128
M = 8
SEG = 32
FF = 3584
EPS = 1e-5
LOG2E = 1.4426950408889634

NSEG = S // SEG
NP = H // 2
TPS = SEG - 8
T0 = 8 * NSEG
TH = T0 // 2
FH = FF // 2
DH2 = D // 2
UA = 8
P1N = 5
NEARLY = 4
FB = 256
HB = FB // 2
OC = 128
FC = 256
LNP = 16

SSUM = (0, 1, 4, 5, 6)
TSUM = (0, 2, 3, 5, 6)
SORD = (1, 4, 3, 2, 0, 6, 5)

T1_ROW = 3 * NP * 2 * T0
T2_ROW = T1_ROW + 5 * (FH // 128) * DH2
LT_ROWS = T2_ROW + 5 * (DH2 // 128) * FH + 16

SEM_W, SEM_A, SEM_M, SEM_MISC, SEM_OUT = 0, 48, 56, 64, 72
SEM_N = SEM_OUT + S // FB


def _make_sched(h1=24, n1=1, n2=4):
    out = []

    def pairs(a):
        return tuple(p for p in (a, a + 1) if 0 <= p < NP)

    nxt = 0
    for p in range(NP):
        out.append(("proj", p))
        if p >= 2 and p % 2 == 0:
            out.append(("attn", pairs(nxt - 2), pairs(nxt)))
            nxt += 2
    out += [("wo", j, 0, h1) for j in range(n1)]
    out.append(("attn", pairs(nxt - 2), pairs(nxt)))
    out += [("wo", j, 0, h1) for j in range(n1, n2)]
    out.append(("attn", pairs(nxt), ()))
    out += [("wo", j, 0, h1) for j in range(n2, 8)]
    out += [("wo", j, h1, H) for j in range(8)]
    return out


SCHED = _make_sched()
_SCOPES = False


def _scope(name):
    return jax.named_scope(name) if _SCOPES else contextlib.nullcontext()


def _dot(a, b):
    return jnp.dot(a, b, preferred_element_type=F32)


def _bf(x):
    return pltpu.bitcast(x, BF16)


def _ld(ref, idx, r0, n):
    return _bf(ref.at[(*idx, pl.ds(r0, n), slice(None))].bitcast(U32)[...])


def _ln(x):
    m = jnp.mean(x, axis=-1, keepdims=True)
    xc = x - m
    v = jnp.mean(xc * xc, axis=-1, keepdims=True)
    return xc * lax.rsqrt(v + EPS)


def _gelu(x):
    c = 0.7978845608028654
    return 0.5 * x * (1.0 + jnp.tanh(c * (x + 0.044715 * (x * x * x))))


def _strassen_lhs(a11, a12, a21, a22):
    return [a11 + a22, a21 + a22, a11, a22, a11 + a12, a21 - a11, a12 - a22]


def _strassen_rhs(b11, b12, b21, b22):
    return [b11 + b22, b11, b12 - b22, b21 - b11, b22, b11 + b12, b21 + b22]


def _strassen_out(m):
    return (m[0] + m[3] - m[4] + m[6], m[2] + m[4], m[1] + m[3], m[0] - m[1] + m[2] + m[5])


def _interleave(a, b):
    n = a.shape[0] // 8
    parts = []
    for g in range(n):
        parts.append(a[8 * g:8 * g + 8])
        parts.append(b[8 * g:8 * g + 8])
    return jnp.concatenate(parts, axis=0)


def _deinterleave(v):
    n = v.shape[0] // 16
    a = jnp.concatenate([v[16 * g:16 * g + 8] for g in range(n)], axis=0)
    b = jnp.concatenate([v[16 * g + 8:16 * g + 16] for g in range(n)], axis=0)
    return a, b


def _kernel(x_hbm, mem0_hbm, wq_hbm, wk_hbm, wv_hbm, wo_hbm, w1_hbm, b1_hbm, w2_hbm, b2_hbm,
            c_hbm, wmod_hbm, out_hbm,
            x_v, h_v, hn_v, h2_v, x1_v, wmod_v, mod_v, sc_v, w_v, wo_v, w1_v, w2_v,
            lt_v, fr_v, lo_v, pr_v, fill_v, bias_v, n_v,
            mem0_ref, b1_ref, b2_ref, c_ref, hs_v, so_v, ev_v, st_v,
            sems):
    w32 = [r.bitcast(U32) for r in (wq_hbm, wk_hbm, wv_hbm)]
    wo32 = wo_hbm.bitcast(U32)

    def w_copies(p, js=range(3)):
        return [pltpu.make_async_copy(w32[j].at[:, par, p, :], w_v.at[p * 6 + j * 2 + par],
                                      sems.at[SEM_W + 3 * p + j]) for j in js for par in range(2)]

    def w_wait(u):
        both = w_v.at[pl.ds(2 * u, 2)]
        pltpu.make_async_copy(both, both, sems.at[SEM_W + u]).wait()

    def _mult(i, m):
        return i * m if isinstance(i, int) else pl.multiple_of(i * m, m)

    def wa_copies(k, units=range(UA)):
        r = pl.ds(_mult(k, 64), 64)
        return [pltpu.make_async_copy(w32[u % 3].at[r, par, u // 3, :], w_v.at[2 * u + par, r], sems.at[SEM_A + k])
                for u in units for par in range(2)]

    def m_copies(k):
        return [pltpu.make_async_copy(wmod_hbm.at[:, pl.ds(_mult(k + 8 * t, 128), 128)], wmod_v.at[16 + k + 8 * t],
                                      sems.at[SEM_M + k]) for t in range(2)]

    def start(cps):
        for cp in cps:
            cp.start()

    def wait(cps):
        for cp in cps:
            cp.wait()

    cp_x0 = pltpu.make_async_copy(x_hbm.at[:, 0:8, :], x_v.at[:, 0:8, :], sems.at[SEM_MISC + 1])

    def wo_copy(j):
        return pltpu.make_async_copy(wo32.at[:, pl.ds(_mult(j, 128), 128)], wo_v.at[j], sems.at[SEM_MISC + 3])

    def late_copies(first):
        sem = sems.at[SEM_MISC + (4 if first else 5)]
        sg = slice(1, 2 * NEARLY + 1) if first else slice(2 * NEARLY + 1, NSEG)
        cps = [(x_hbm.at[sg, 8:SEG, :], x_v.at[sg, 8:SEG, :])]
        cps += [(wmod_hbm.at[:, (16 + j) * 128:(17 + j) * 128], wmod_v.at[j])
                for j in (range(NEARLY) if first else range(NEARLY, 32))]
        for src, dst, nt, kh in ((w1_hbm, w1_v, FF // 128, DH2), (w2_hbm, w2_v, D // 128, FH)):
            for j in range(nt):
                cols = slice(j * 128, (j + 1) * 128)
                if j % (nt // 2):
                    rows = [] if first else [slice(None)]
                else:
                    rows = [slice(a * kh, a * kh + 256) if first else slice(a * kh + 256, (a + 1) * kh)
                            for a in range(2)]
                cps += [(src.at[r, cols], dst.at[j, r]) for r in rows]
        return [pltpu.make_async_copy(src, dst, sem) for src, dst in cps]

    cp_small = [pltpu.make_async_copy(src, dst, sems.at[SEM_MISC])
                for src, dst in ((c_hbm, c_ref), (mem0_hbm, mem0_ref), (b1_hbm, b1_ref), (b2_hbm, b2_ref),
                                 (x_hbm.at[0, 8:SEG, :], x_v.at[0, 8:SEG, :]))]

    start(cp_small)
    cp_x0.start()
    start(m_copies(0))
    for k in range(2):
        start(m_copies(k + 1))
        start(wa_copies(k))

    scale = DH ** -0.5
    ri = lax.broadcasted_iota(jnp.int32, (80, 128), 0)
    ci = lax.broadcasted_iota(jnp.int32, (80, 128), 1)
    same_head = (((ri >> 3) & 1) == ((ci >> 3) & 1)) & (ci < 80)
    rpos = (((ri >> 4) & 3) << 3) + (ri & 7)
    cpos = (((ci >> 4) & 3) << 3) + (ci & 7)
    keep = (ri < 16) | (ci < 16) | (rpos >= cpos)
    fill_v[...] = jnp.where(same_head, jnp.where(keep, 0.0, -1e9 / scale), -jnp.inf).astype(F32)

    wait(cp_small)
    c = c_ref[...].astype(F32)
    sc = jnp.broadcast_to(c * jax.nn.sigmoid(c), (8, D)).astype(BF16)

    sc_v[...] = sc
    for k in range(8):
        st_v[k * 128:(k + 1) * 128, :] = jnp.broadcast_to(sc[0:1, k * 128:(k + 1) * 128].astype(F32), (128, 128)).T
    bias_v[:, 0:FF] = b1_ref[...].astype(F32).reshape(1, FF)
    bias_v[:, FF:FF + D] = b2_ref[...].astype(F32).reshape(1, D)

    def zero_body(i, carry):
        x1_v[pl.ds(pl.multiple_of(i * 64, 64), 64), :] = jnp.zeros((64, D), F32)
        return carry

    lax.fori_loop(0, -(-UA // 4) * 8, zero_body, 0)

    def relayout(c, rows):
        a = w_v[c, rows, :]
        b = w_v[c + 1, rows, :]
        lo = (a & jnp.uint32(0xFFFF)) | (b << 16)
        hi = (a >> 16) | (b & jnp.uint32(0xFFFF0000))
        w_v[c, rows, :] = lo
        w_v[c + 1, rows, :] = hi
        return _bf(lo), _bf(hi)

    def store_lead(u, a, b):
        lt_v[pl.ds(_mult(u, 2 * T0), 2 * T0), :] = _interleave(a, b).astype(BF16)

    def mod_tile(ct):
        m = _dot(sc_v[...], _ld(wmod_v, (16 + ct,), 0, D))
        mod_v[:, pl.ds(_mult(ct, 128), 128)] = m
        return m[0:1]

    with _scope("wait_x0"):
        cp_x0.wait()

    def ln1_body(i, carry):
        r = pl.multiple_of(i * 128, 128)
        n = _ln(x_v[pl.ds(i * 16, 16), 0:8, :].astype(F32).reshape(128, D))
        for k in range(8):
            n_v[k, pl.ds(r, 128), :] = n[:, k * 128:(k + 1) * 128]
        return carry

    with _scope("ln1"):
        lax.fori_loop(0, T0 // 128, ln1_body, 0)
    start(m_copies(3))
    start(wa_copies(2))
    with _scope("wait_m0"):
        wait(m_copies(0))
    h_v[0] = (n_v[0] * (1.0 + mod_tile(8)) + mod_tile(0)).astype(BF16)

    def sa_body(k, carry):
        with _scope("wait_a"):
            wait(wa_copies(k))

            @pl.when(k < 7)
            def _():
                wait(m_copies(k + 1))

        kn = jnp.minimum(k + 1, 7)
        rows = pl.ds(pl.multiple_of(k * 64, 64), 64)
        hk = _ld(h_v, (k,), 0, T0)
        for u in range(UA):
            res = []
            for t, w in enumerate(relayout(2 * u, rows)):
                c = 2 * u + t
                acc = x1_v.at[c // 8 * T0:(c // 8 + 1) * T0, c % 8 * 128:(c % 8 + 1) * 128]
                r = _dot(hk, w) + acc[...]
                acc[...] = r
                res.append(r)
            store_lead(u, *res)
            if u == 1:
                sh = mod_tile(kn)
            if u == 3:
                s1 = 1.0 + mod_tile(kn + 8)

                @pl.when(k + 4 < 8)
                def _():
                    start(m_copies(k + 4))

            if u >= 4 and u % 2 == 0:
                @pl.when(k + 3 < 8)
                def _():
                    start(wa_copies(k + 3, range((u - 4) * 2, (u - 4) * 2 + 4)))

        h_v[kn] = (n_v[kn] * s1 + sh).astype(BF16)

        @pl.when(k == 4)
        def _():
            start(w_copies(UA // 3, range(UA % 3, 3)))

        @pl.when(k >= 4)
        def _():
            start(w_copies(UA // 3 + 1 + k - 4))

        return carry

    with _scope("stageA"):
        lax.fori_loop(0, 8, sa_body, 0)

    def ln1(seg):
        xb = x_v[seg, 8:SEG, :].astype(F32)
        return _ln(xb) * (1.0 + mod_v[0:1, D:2 * D]) + mod_v[0:1, 0:D]

    def hs_body(t, carry):
        for r in range(0, TH, 32):
            ss = _strassen_lhs(*[_ld(h_v, (t + 4 * b,), a * TH + r, 32).astype(F32)
                                 for a in range(2) for b in range(2)])
            for k, i in enumerate(SSUM):
                hs_v[k, t, r:r + 32, :] = ss[i].astype(BF16)
        return carry

    lax.fori_loop(0, 4, hs_body, 0)

    def lhs1(i):
        if i == 2:
            tiles = [_ld(h_v, (t,), 0, TH) for t in range(4)]
        elif i == 3:
            tiles = [_ld(h_v, (t + 4,), TH, TH) for t in range(4)]
        else:
            tiles = [_ld(hs_v, (SSUM.index(i), t), 0, TH) for t in range(4)]
        return jnp.concatenate(tiles, axis=1)

    NP1 = (3 * NP - UA) // P1N
    late = late_copies(False)
    nl = -(-len(late) // P1N)
    PW = UA // 3 + 5

    def p1_body(i, carry):
        u0 = UA + P1N * i
        with _scope("wait_w"):
            for q in range(P1N):
                w_wait(u0 + q)

        for q in range(P1N):
            lo, hi = relayout(2 * (u0 + q), slice(None))
            b = [lo[0:DH2], hi[0:DH2], lo[DH2:D], hi[DH2:D]]
            t = _strassen_rhs(*[x.astype(F32) for x in b])
            t = [b[0] if k == 1 else b[3] if k == 4 else t[k].astype(BF16) for k in range(7)]
            c = _strassen_out({k: _dot(lhs1(k), t[k]) for k in SORD})
            store_lead(u0 + q, jnp.concatenate([c[0], c[2]], axis=0), jnp.concatenate([c[1], c[3]], axis=0))

            if q < 3:
                @pl.when(PW + 3 * i + q < NP)
                def _():
                    start(w_copies(PW + 3 * i + q))
            elif q == 3:
                @pl.when(jnp.logical_and(i >= 2, i < 4))
                def _():
                    start([wo_copy(4 * (i - 2) + r) for r in range(4)])
            elif q == 4:
                @pl.when(i == 3)
                def _():
                    start(late_copies(True))

            @pl.when(i == NP1 - 1)
            def _():
                start(late[q * nl:(q + 1) * nl])

        hn_v[...] = ln1(0)
        return carry

    with _scope("phase1"):
        lax.fori_loop(0, NP1, p1_body, 0)

    with _scope("wait_wo"):
        wait([wo_copy(j) for j in range(8)])
        wait(late_copies(True))

    def prep_views(w, t_row, kh, nh, j, r0):
        src = w.at[pl.ds(j, nh + 1), pl.ds(pl.multiple_of(r0, 256), kh + 256), :]
        dst = lt_v.at[pl.ds(pl.multiple_of(t_row + j * kh + r0, 256), 4 * nh * kh + 256), :]
        return src, dst, kh, nh

    def prep(views, r0, n):
        src, dst, kh, nh = views
        t = _strassen_rhs(*[_ld(src, (b * nh,), a * kh + r0, n).astype(F32) for a in range(2) for b in range(2)])
        for k, i in enumerate(TSUM):
            dst[k * nh * kh + r0:k * nh * kh + r0 + n, :] = t[i].astype(BF16)

    def step(it, odd, mem, macc):
        s = 2 * it + int(odd)
        lead = lt_v.at[pl.ds(pl.multiple_of(16 * s, 16), T1_ROW), :]
        lhs = jnp.concatenate([mem, hn_v[...]], axis=0).astype(BF16)
        hn_v[...] = ln1(jnp.minimum(s + 1, NSEG - 1))

        def proj(p):
            if p == 0:
                half = [_dot(lhs[:, 0:D // 2], _bf(w_v[c, 0:D // 4, :])) for c in range(6)]
                cols = [_dot(lhs[:, D // 2:D], _bf(w_v[c, D // 4:D // 2, :])) + half[c] for c in range(6)]
            for j in range(3):
                if p == 0:
                    r = _interleave(cols[j * 2], cols[j * 2 + 1])
                else:
                    r = _interleave(_dot(lhs, _bf(w_v[p * 6 + j * 2])), _dot(lhs, _bf(w_v[p * 6 + j * 2 + 1])))
                fr_v[p * 3 + j] = r.astype(BF16)

        def stack(p, j):
            return jnp.concatenate([fr_v[p * 3 + j],
                                    _ld(lead, (), (p * 3 + j) * 2 * T0, 16)], axis=0)

        def attn(pvs, qks):
            os_ = [_dot(pr_v[p, :, 0:80], stack(p, 2)) for p in pvs]
            ss = [lax.dot_general(stack(p, 0), stack(p, 1), (((1,), (1,)), ((), ())),
                                  preferred_element_type=F32) for p in qks]
            for p, o in zip(pvs, os_):
                for t, oh in enumerate(_deinterleave(o[0:64])):
                    lo_v[2 * p + t] = oh.astype(BF16)
                if odd:
                    ev = ev_v[p]
                    for k, sk in enumerate(_strassen_lhs(ev[0:8], ev[8:16], o[64:72], o[72:80])):
                        so_v[k, p, pl.ds(pl.multiple_of(8 * it, 8), 8), :] = sk.astype(BF16)
                else:
                    ev_v[p] = o[64:80]
            for p, sc_ in zip(qks, ss):
                fill = fill_v[...]
                sc_ = jnp.concatenate([sc_, jnp.zeros((80, 48), F32)], axis=1)
                sc_ = jnp.where(fill == 0.0, sc_, fill)
                mx = jnp.max(sc_, axis=-1, keepdims=True)
                e = jnp.exp2((sc_ - mx) * (scale * LOG2E))
                l = jnp.sum(e, axis=-1, keepdims=True)
                r = pl.reciprocal(l, approx=True)
                pr_v[p] = (e * (r * (2.0 - l * r))).astype(BF16)

        part = {}

        def wo(j, h0, h1):
            lo = jnp.concatenate([lo_v[h] for h in range(h0, h1)], axis=1)
            r = _dot(lo, _bf(wo_v[j, h0 * 64:h1 * 64, :]))
            part[j] = r + part[j] if j in part else r

        pc = jnp.maximum(it - NEARLY, 0)
        if odd:
            views = prep_views(w2_v, T2_ROW, FH, DH2 // 128, pc & 3, (pc >> 2) * 256)
        else:
            views = prep_views(w1_v, T1_ROW, DH2, FH // 128, pc >> 1, (pc & 1) * 256)
        npiece = 0
        for op in SCHED:
            if op[0] == "proj":
                proj(op[1])
            elif op[0] == "attn":
                attn(op[1], op[2])
                if npiece < 8:
                    prep(views, npiece * 32, 32)
                    k0 = (8 * int(odd) + npiece) * 64
                    pr = _ld(wmod_v, (it,), k0, 64).astype(F32) * st_v[k0:k0 + 64, :]
                    for g in range(8):
                        macc = pr[8 * g:8 * g + 8] if macc is None else macc + pr[8 * g:8 * g + 8]
                    lt_v[LT_ROWS - 16:LT_ROWS, :] = _bf(macc)
                    npiece += 1
            else:
                wo(*op[1:])
        res = jnp.concatenate([part[j] for j in range(8)], axis=1)
        x1_v[pl.ds(pl.multiple_of(SEG * s + 8, 8), TPS), :] = res[8:32]
        return res[0:8], macc

    with _scope("main"):
        def steps(i, mem):
            @pl.when(i == NEARLY)
            def _():
                wait(late)

            with _scope("iter"):
                mem, macc = step(i, True, *step(i, False, mem, None))
                mod_v[0:1, pl.ds(pl.multiple_of((16 + i) * 128, 128), 128)] = jnp.sum(macc, axis=0, keepdims=True)

            return mem

        lax.fori_loop(0, NSEG // 2, steps, mem0_ref[...].astype(F32))

    def wo_body(j, carry):
        acc = {}
        for kc in range(4):
            b = [jnp.concatenate([_bf(wo_v[j + 4 * n, (2 * p + t) * 64:(2 * p + t + 1) * 64, :])
                                  for p in range(4 * kc, 4 * kc + 4)], axis=0)
                 for t in range(2) for n in range(2)]
            tt = _strassen_rhs(*[x.astype(F32) for x in b])
            tt = [b[0] if k == 1 else b[3] if k == 4 else tt[k].astype(BF16) for k in range(7)]
            for k in SORD:
                sk = jnp.concatenate([_ld(so_v, (k, p), 0, TH) for p in range(4 * kc, 4 * kc + 4)], axis=1)
                y = _dot(sk, tt[k])
                acc[k] = y + acc[k] if kc else y
        for t, c in enumerate(_strassen_out(acc)):
            cs = pl.ds(pl.multiple_of((j + 4 * (t % 2)) * 128, 128), 128)
            for g in range(NSEG // 2):
                r0 = (2 * g + t // 2) * SEG
                x1_v[r0:r0 + 8, cs] = c[8 * g:8 * g + 8]
        return carry

    with _scope("p3a"):
        lax.fori_loop(0, 4, wo_body, 0)

    def rhs(w, t_row, kh, nh, i, j, k0, nk):
        if i == 1:
            return _ld(w, (j,), k0, nk)
        if i == 4:
            return _ld(w, (j + nh,), kh + k0, nk)
        return _ld(lt_v, (), t_row + (TSUM.index(i) * nh + j) * kh + k0, nk)

    def out_copy(i, q):
        segs = pl.ds(i * (FB // SEG), FB // SEG)
        return [pltpu.make_async_copy(x_v.at[segs, :, cols], out_hbm.at[segs, :, cols], sems.at[SEM_OUT + i])
                for cols in (pl.ds(q * OC, OC), pl.ds(DH2 + q * OC, OC))]

    def resid1(r0, k0, n, c0=0, nc=D):
        if n >= SEG:
            xb = x_v[pl.ds((r0 >> 5) + k0 // SEG, n // SEG), :, c0:c0 + nc].astype(F32).reshape(n, nc)
        else:
            xb = x_v[(r0 >> 5) + k0 // SEG, k0 % SEG:k0 % SEG + n, c0:c0 + nc].astype(F32)
        return xb + mod_v[0:1, 2 * D + c0:2 * D + c0 + nc] * x1_v[pl.ds(r0 + k0, n), c0:c0 + nc]

    def ln2(slot, r0, k0, n):
        top, bot = [_ln(resid1(r0, t * HB + k0, n)) * (1.0 + mod_v[0:1, 4 * D:5 * D]) + mod_v[0:1, 3 * D:4 * D]
                    for t in range(2)]
        ss = _strassen_lhs(top[:, 0:DH2], top[:, DH2:D], bot[:, 0:DH2], bot[:, DH2:D])
        for i in range(7):
            for j in range(DH2 // 128):
                h2_v[slot, i, j, k0:k0 + n, :] = ss[i][:, j * 128:(j + 1) * 128].astype(BF16)

    ln2(0, 0, 0, HB)

    def ffn_body(i, carry):
        r0 = pl.multiple_of(i * FB, FB)
        rn = pl.multiple_of(jnp.minimum(r0 + FB, S - FB), FB)
        slot = lax.rem(i, 2)
        nf = FH // FC
        nt = FC // 128
        nq = DH2 // OC
        acc = {}
        gs = {}

        def up(f, t):
            c0 = f * FC + t * 128
            c = _strassen_out({
                k: _dot(jnp.concatenate([_ld(h2_v, (slot, k, j), 0, HB) for j in range(DH2 // 128)], axis=1),
                        rhs(w1_v, T1_ROW, DH2, FH // 128, k, c0 // 128, 0, DH2)) for k in SORD})
            b1a, b1b = bias_v[0:1, c0:c0 + 128], bias_v[0:1, FH + c0:FH + c0 + 128]
            gs[f, t] = _strassen_lhs(_gelu(c[0] + b1a), _gelu(c[1] + b1b), _gelu(c[2] + b1a), _gelu(c[3] + b1b))
            if t == nt - 1:
                gs[f] = [jnp.concatenate([gs[f, u][k] for u in range(nt)], axis=1).astype(BF16) for k in range(7)]

        def down(f, q):
            for k in SORD:
                y = _dot(gs[f][k], rhs(w2_v, T2_ROW, FH, DH2 // 128, k, q, f * FC, FC))
                acc[k, q] = y + acc[k, q] if f else y
            if f == nf - 1:
                c = _strassen_out([acc[k, q] for k in range(7)])
                for t in range(4):
                    k0, c0 = (t // 2) * HB, (t % 2) * DH2 + q * OC
                    y = (c[t] + bias_v[0:1, FF + c0:FF + c0 + OC]) * mod_v[0:1, 5 * D + c0:5 * D + c0 + OC]
                    o = (resid1(r0, k0, HB, c0, OC) + y).reshape(HB // SEG, SEG, OC).astype(BF16)
                    x_v[pl.ds((r0 >> 5) + k0 // SEG, HB // SEG), :, c0:c0 + OC] = o
                start(out_copy(i, q))

        for t in range(nt):
            up(0, t)
        w = 0
        for f in range(nf):
            for t in range(nt):
                if f + 1 < nf:
                    up(f + 1, t)
                if w * LNP < HB:
                    ln2(1 - slot, rn, w * LNP, LNP)
                w += 1
                for q in range(t * nq // nt, (t + 1) * nq // nt):
                    down(f, q)
        return carry

    with _scope("ffn"):
        lax.fori_loop(0, S // FB, ffn_body, 0)
    with _scope("wait_out"):
        for i in range(S // FB):
            for q in range(DH2 // OC):
                wait(out_copy(i, q))


@jax.jit
def pallas_adaLN_cond__memory_aug_recurrent_mem_tr__dense_activation_gelu__prompt_kernel(
    A_x, A_mem0, A_Wq, A_Wk, A_Wv, A_Wo, A_seg_len, B_x, B_w1, B_b1, B_w2, B_b2, c, w_mod,
):
    del A_seg_len, B_x
    assert A_x.shape == (1, S, D)
    hbm = pl.BlockSpec(memory_space=pl.ANY)
    out = pl.pallas_call(
        _kernel,
        out_shape=jax.ShapeDtypeStruct((NSEG, SEG, D), BF16),
        in_specs=[hbm] * 12,
        out_specs=hbm,
        scratch_shapes=[
            pltpu.VMEM((NSEG, SEG, D), BF16),
            pltpu.VMEM((8, T0, 128), BF16),
            pltpu.VMEM((TPS, D), F32),
            pltpu.VMEM((2, 7, 4, FB // 2, 128), BF16),
            pltpu.VMEM((S, D), F32),
            pltpu.VMEM((32, D, 128), BF16),
            pltpu.VMEM((8, 6 * D), F32),
            pltpu.VMEM((8, D), BF16),
            pltpu.VMEM((6 * NP, D // 2, 128), U32),
            pltpu.VMEM((8, H * DH // 2, 128), U32),
            pltpu.VMEM((FF // 128, D, 128), BF16),
            pltpu.VMEM((D // 128, FF, 128), BF16),
            pltpu.VMEM((LT_ROWS, 128), BF16),
            pltpu.VMEM((3 * NP, 64, 128), BF16),
            pltpu.VMEM((H, 32, 128), BF16),
            pltpu.VMEM((NP, 80, 128), BF16),
            pltpu.VMEM((80, 128), F32),
            pltpu.VMEM((1, FF + D), F32),
            pltpu.VMEM((8, T0, 128), F32),
            pltpu.VMEM((M, D), BF16),
            pltpu.VMEM((FF,), BF16),
            pltpu.VMEM((D,), BF16),
            pltpu.VMEM((1, D), BF16),
            pltpu.VMEM((5, 4, T0 // 2, 128), BF16),
            pltpu.VMEM((7, NP, T0 // 2, 128), BF16),
            pltpu.VMEM((NP, 16, 128), F32),
            pltpu.VMEM((D, 128), F32),
            pltpu.SemaphoreType.DMA((SEM_N,)),
        ],
        compiler_params=pltpu.CompilerParams(vmem_limit_bytes=122 * 1024 * 1024, disable_bounds_checks=True,
                                             disable_semaphore_checks=True),
    )(
        A_x.reshape(NSEG, SEG, D), A_mem0.reshape(M, D),
        A_Wq.reshape(D // 2, 2, H, DH), A_Wk.reshape(D // 2, 2, H, DH), A_Wv.reshape(D // 2, 2, H, DH),
        A_Wo.reshape(H * DH, D), B_w1, B_b1, B_w2, B_b2, c, w_mod,
    )
    return out.reshape(1, S, D)
```

```python
import contextlib

import jax
import jax.numpy as jnp
from jax import lax
import jax.experimental.pallas as pl
import jax.experimental.pallas.tpu as pltpu

F32 = jnp.float32
BF16 = jnp.bfloat16
U32 = jnp.uint32

S = 2048
D = 1024
H = 32
DH = 128
M = 8
SEG = 32
FF = 3584
EPS = 1e-5
LOG2E = 1.4426950408889634

NSEG = S // SEG
NP = H // 2
TPS = SEG - 8
T0 = 8 * NSEG
TH = T0 // 2
FH = FF // 2
DH2 = D // 2
UA = 8
P1N = 5
NEARLY = 4
FB = 256
HB = FB // 2
OC = 128
FC = 256
GROUPS = ((0, 1), (2, 3), (4, 5), (6,))
PIECE = 28
LNP = 16

SSUM = (0, 1, 4, 5, 6)
TSUM = (0, 2, 3, 5, 6)
SORD = (1, 4, 3, 2, 0, 6, 5)

HK = (
    (((0, 0, 1), (1, 0, -1)), ((0, 0, 1), (0, 1, 1), (2, 0, -1)), ((0, 0, 1),)),
    (((1, 0, 1),), ((0, 0, 1), (0, 2, 1), (1, 0, -1)), ((0, 0, 1), (1, 0, 1))),
    (((0, 1, 1),), ((1, 1, 1), (1, 2, 1), (0, 1, -1), (3, 1, -1)), ((0, 1, 1), (1, 1, 1))),
    (((1, 1, 1), (0, 1, -1)), ((1, 0, 1), (1, 1, 1), (1, 3, 1), (2, 1, -1)), ((1, 1, 1),)),
    (((0, 2, 1),), ((2, 1, 1), (2, 2, 1), (0, 2, -1), (3, 2, -1)), ((0, 2, 1),)),
    (((1, 2, 1),), ((2, 0, 1), (2, 2, 1), (2, 3, 1), (1, 2, -1)), ((1, 2, 1),)),
    (((0, 3, 1), (1, 3, -1)), ((3, 1, 1), (3, 3, 1), (2, 3, -1)), ((0, 3, 1),)),
    (((1, 3, 1),), ((3, 2, 1), (3, 3, 1), (1, 3, -1)), ((0, 3, 1), (1, 3, 1))),
    (((0, 1, 1), (1, 0, 1)), ((0, 1, 1), (1, 0, 1)), ((0, 0, 1), (1, 1, 1))),
    (((0, 0, 1), (0, 1, 1)), ((0, 1, 1),), ((0, 0, -1), (0, 1, 1))),
    (((1, 0, 1), (1, 1, 1)), ((1, 0, 1),), ((1, 0, 1), (1, 1, -1))),
    (((0, 0, 1), (0, 2, 1), (1, 0, -1)), ((0, 2, 1), (2, 0, 1)), ((0, 0, 1), (1, 0, 1), (1, 2, -1))),
    (((0, 0, 1), (0, 2, 1)), ((0, 2, 1),), ((0, 0, -1), (0, 2, 1), (1, 0, -1), (1, 2, 1))),
    (((0, 0, 1), (0, 2, 1), (1, 0, -1), (1, 2, -1)), ((2, 0, 1),), ((1, 0, -1), (1, 2, 1))),
    (((0, 3, 1),), ((3, 0, 1),), ((0, 0, 1),)),
    (((1, 3, 1),), ((3, 0, 1),), ((1, 0, 1),)),
    (((0, 0, 1),), ((0, 3, 1),), ((0, 3, 1),)),
    (((1, 0, 1),), ((0, 3, 1),), ((1, 3, 1),)),
    (((1, 1, 1), (1, 2, 1), (0, 1, -1)), ((1, 2, 1), (2, 1, 1)), ((0, 1, 1), (0, 2, -1), (1, 1, 1))),
    (((1, 1, 1), (1, 2, 1)), ((1, 2, 1),), ((0, 1, -1), (0, 2, 1), (1, 1, -1), (1, 2, 1))),
    (((1, 1, 1), (1, 2, 1), (0, 1, -1), (0, 2, -1)), ((2, 1, 1),), ((0, 1, -1), (0, 2, 1))),
    (((0, 1, 1), (1, 3, 1)), ((1, 3, 1), (3, 1, 1)), ((0, 3, 1), (1, 1, 1))),
    (((1, 1, 1), (1, 3, 1)), ((1, 3, 1),), ((1, 1, -1), (1, 3, 1))),
    (((0, 1, 1), (0, 3, 1)), ((3, 1, 1),), ((0, 1, 1), (0, 3, -1))),
    (((0, 2, 1), (0, 3, 1), (1, 3, -1)), ((2, 3, 1), (3, 2, 1)), ((0, 3, 1), (1, 2, -1), (1, 3, 1))),
    (((0, 2, 1), (0, 3, 1), (1, 3, -1), (1, 2, -1)), ((2, 3, 1),), ((1, 2, 1), (1, 3, -1))),
    (((0, 2, 1), (0, 3, 1)), ((3, 2, 1),), ((0, 2, 1), (0, 3, -1), (1, 2, 1), (1, 3, -1))),
)
HKSUM = tuple(r for r, t in enumerate(HK) if len(t[1]) > 1)
HKORD = tuple(sorted(range(len(HK)), key=lambda r: min(n for _, n, _ in HK[r][2])))
KT2 = (0, 128, FH, FH + 128)

T1_ROW = 3 * NP * 2 * T0
T2_ROW = T1_ROW + 5 * (FH // 128) * DH2
LT_ROWS = T2_ROW + len(HKSUM) * 2 * (FF // 4) + 16

SEM_W, SEM_A, SEM_M, SEM_MISC, SEM_OUT = 0, 48, 56, 64, 72
SEM_N = SEM_OUT + S // FB


def _make_sched(h1=24, n1=1, n2=4):
    out = []

    def pairs(a):
        return tuple(p for p in (a, a + 1) if 0 <= p < NP)

    nxt = 0
    for p in range(NP):
        out.append(("proj", p))
        if p >= 2 and p % 2 == 0:
            out.append(("attn", pairs(nxt - 2), pairs(nxt)))
            nxt += 2
    out += [("wo", j, 0, h1) for j in range(n1)]
    out.append(("attn", pairs(nxt - 2), pairs(nxt)))
    out += [("wo", j, 0, h1) for j in range(n1, n2)]
    out.append(("attn", pairs(nxt), ()))
    out += [("wo", j, 0, h1) for j in range(n2, 8)]
    out += [("wo", j, h1, H) for j in range(8)]
    return out


SCHED = _make_sched()
_SCOPES = False


def _scope(name):
    return jax.named_scope(name) if _SCOPES else contextlib.nullcontext()


def _dot(a, b):
    return jnp.dot(a, b, preferred_element_type=F32)


def _bf(x):
    return pltpu.bitcast(x, BF16)


def _ld(ref, idx, r0, n):
    return _bf(ref.at[(*idx, pl.ds(r0, n), slice(None))].bitcast(U32)[...])


def _ln(x):
    m = jnp.mean(x, axis=-1, keepdims=True)
    xc = x - m
    v = jnp.mean(xc * xc, axis=-1, keepdims=True)
    return xc * lax.rsqrt(v + EPS)


def _gelu(x):
    c = 0.7978845608028654
    return 0.5 * x * (1.0 + jnp.tanh(c * (x + 0.044715 * (x * x * x))))


def _strassen_lhs(a11, a12, a21, a22):
    return [a11 + a22, a21 + a22, a11, a22, a11 + a12, a21 - a11, a12 - a22]


def _strassen_rhs(b11, b12, b21, b22):
    return [b11 + b22, b11, b12 - b22, b21 - b11, b22, b11 + b12, b21 + b22]


def _strassen_out(m):
    return (m[0] + m[3] - m[4] + m[6], m[2] + m[4], m[1] + m[3], m[0] - m[1] + m[2] + m[5])


def _comb(terms, blocks, memo=None):
    memo = {} if memo is None else memo
    for n in range(1, len(terms) + 1):
        key = terms[:n]
        if key not in memo:
            i, j, sg = terms[n - 1]
            b = blocks[i, j]
            memo[key] = b if n == 1 else (memo[terms[:n - 1]] + b if sg > 0 else memo[terms[:n - 1]] - b)
    return memo[terms]


def _interleave(a, b):
    n = a.shape[0] // 8
    parts = []
    for g in range(n):
        parts.append(a[8 * g:8 * g + 8])
        parts.append(b[8 * g:8 * g + 8])
    return jnp.concatenate(parts, axis=0)


def _deinterleave(v):
    n = v.shape[0] // 16
    a = jnp.concatenate([v[16 * g:16 * g + 8] for g in range(n)], axis=0)
    b = jnp.concatenate([v[16 * g + 8:16 * g + 16] for g in range(n)], axis=0)
    return a, b


def _kernel(x_hbm, mem0_hbm, wq_hbm, wk_hbm, wv_hbm, wo_hbm, w1_hbm, b1_hbm, w2_hbm, b2_hbm,
            c_hbm, wmod_hbm, out_hbm,
            x_v, h_v, hn_v, h2_v, x1_v, wmod_v, mod_v, sc_v, w_v, wo_v, w1_v, w2_v,
            lt_v, fr_v, lo_v, pr_v, fill_v, bias_v, n_v,
            mem0_ref, b1_ref, b2_ref, c_ref, hs_v, so_v, ev_v, st_v,
            sems):
    w32 = [r.bitcast(U32) for r in (wq_hbm, wk_hbm, wv_hbm)]
    wo32 = wo_hbm.bitcast(U32)

    def w_copies(p, js=range(3)):
        return [pltpu.make_async_copy(w32[j].at[:, par, p, :], w_v.at[p * 6 + j * 2 + par],
                                      sems.at[SEM_W + 3 * p + j]) for j in js for par in range(2)]

    def w_wait(u):
        both = w_v.at[pl.ds(2 * u, 2)]
        pltpu.make_async_copy(both, both, sems.at[SEM_W + u]).wait()

    def _mult(i, m):
        return i * m if isinstance(i, int) else pl.multiple_of(i * m, m)

    def wa_copies(k, units=range(UA)):
        r = pl.ds(_mult(k, 64), 64)
        return [pltpu.make_async_copy(w32[u % 3].at[r, par, u // 3, :], w_v.at[2 * u + par, r], sems.at[SEM_A + k])
                for u in units for par in range(2)]

    def m_copies(k):
        return [pltpu.make_async_copy(wmod_hbm.at[:, pl.ds(_mult(k + 8 * t, 128), 128)], wmod_v.at[16 + k + 8 * t],
                                      sems.at[SEM_M + k]) for t in range(2)]

    def start(cps):
        for cp in cps:
            cp.start()

    def wait(cps):
        for cp in cps:
            cp.wait()

    cp_x0 = pltpu.make_async_copy(x_hbm.at[:, 0:8, :], x_v.at[:, 0:8, :], sems.at[SEM_MISC + 1])

    def wo_copy(j):
        return pltpu.make_async_copy(wo32.at[:, pl.ds(_mult(j, 128), 128)], wo_v.at[j], sems.at[SEM_MISC + 3])

    def late_copies(first):
        sem = sems.at[SEM_MISC + (4 if first else 5)]
        sg = slice(1, 2 * NEARLY + 1) if first else slice(2 * NEARLY + 1, NSEG)
        cps = [(x_hbm.at[sg, 8:SEG, :], x_v.at[sg, 8:SEG, :])]
        cps += [(wmod_hbm.at[:, (16 + j) * 128:(17 + j) * 128], wmod_v.at[j])
                for j in (range(NEARLY) if first else range(NEARLY, 32))]
        for src, dst, nt, kh in ((w1_hbm, w1_v, FF // 128, DH2), (w2_hbm, w2_v, D // 128, FH)):
            for j in range(nt):
                cols = slice(j * 128, (j + 1) * 128)
                if (j % (nt // 2) if dst is w1_v else j >= 4):
                    rows = [] if first else [slice(None)]
                else:
                    rows = [slice(a * kh, a * kh + 256) if first else slice(a * kh + 256, (a + 1) * kh)
                            for a in range(2)]
                cps += [(src.at[r, cols], dst.at[j, r]) for r in rows]
        return [pltpu.make_async_copy(src, dst, sem) for src, dst in cps]

    cp_small = [pltpu.make_async_copy(src, dst, sems.at[SEM_MISC])
                for src, dst in ((c_hbm, c_ref), (mem0_hbm, mem0_ref), (b1_hbm, b1_ref), (b2_hbm, b2_ref),
                                 (x_hbm.at[0, 8:SEG, :], x_v.at[0, 8:SEG, :]))]

    start(cp_small)
    cp_x0.start()
    start(m_copies(0))
    for k in range(2):
        start(m_copies(k + 1))
        start(wa_copies(k))

    scale = DH ** -0.5
    ri = lax.broadcasted_iota(jnp.int32, (80, 128), 0)
    ci = lax.broadcasted_iota(jnp.int32, (80, 128), 1)
    same_head = (((ri >> 3) & 1) == ((ci >> 3) & 1)) & (ci < 80)
    rpos = (((ri >> 4) & 3) << 3) + (ri & 7)
    cpos = (((ci >> 4) & 3) << 3) + (ci & 7)
    keep = (ri < 16) | (ci < 16) | (rpos >= cpos)
    fill_v[...] = jnp.where(same_head, jnp.where(keep, 0.0, -1e9 / scale), -jnp.inf).astype(F32)

    wait(cp_small)
    c = c_ref[...].astype(F32)
    sc = jnp.broadcast_to(c * jax.nn.sigmoid(c), (8, D)).astype(BF16)

    sc_v[...] = sc
    for k in range(8):
        st_v[k * 128:(k + 1) * 128, :] = jnp.broadcast_to(sc[0:1, k * 128:(k + 1) * 128].astype(F32), (128, 128)).T
    bias_v[:, 0:FF] = b1_ref[...].astype(F32).reshape(1, FF)
    bias_v[:, FF:FF + D] = b2_ref[...].astype(F32).reshape(1, D)

    def zero_body(i, carry):
        x1_v[pl.ds(pl.multiple_of(i * 64, 64), 64), :] = jnp.zeros((64, D), F32)
        return carry

    lax.fori_loop(0, -(-UA // 4) * 8, zero_body, 0)

    def relayout(c, rows):
        a = w_v[c, rows, :]
        b = w_v[c + 1, rows, :]
        lo = (a & jnp.uint32(0xFFFF)) | (b << 16)
        hi = (a >> 16) | (b & jnp.uint32(0xFFFF0000))
        w_v[c, rows, :] = lo
        w_v[c + 1, rows, :] = hi
        return _bf(lo), _bf(hi)

    def store_lead(u, a, b):
        lt_v[pl.ds(_mult(u, 2 * T0), 2 * T0), :] = _interleave(a, b).astype(BF16)

    def mod_tile(ct):
        m = _dot(sc_v[...], _ld(wmod_v, (16 + ct,), 0, D))
        mod_v[:, pl.ds(_mult(ct, 128), 128)] = m
        return m[0:1]

    with _scope("wait_x0"):
        cp_x0.wait()

    def ln1_body(i, carry):
        r = pl.multiple_of(i * 128, 128)
        n = _ln(x_v[pl.ds(i * 16, 16), 0:8, :].astype(F32).reshape(128, D))
        for k in range(8):
            n_v[k, pl.ds(r, 128), :] = n[:, k * 128:(k + 1) * 128]
        return carry

    with _scope("ln1"):
        lax.fori_loop(0, T0 // 128, ln1_body, 0)
    start(m_copies(3))
    start(wa_copies(2))
    with _scope("wait_m0"):
        wait(m_copies(0))
    h_v[0] = (n_v[0] * (1.0 + mod_tile(8)) + mod_tile(0)).astype(BF16)

    def sa_body(k, carry):
        with _scope("wait_a"):
            wait(wa_copies(k))

            @pl.when(k < 7)
            def _():
                wait(m_copies(k + 1))

        kn = jnp.minimum(k + 1, 7)
        rows = pl.ds(pl.multiple_of(k * 64, 64), 64)
        hk = _ld(h_v, (k,), 0, T0)
        for u in range(UA):
            res = []
            for t, w in enumerate(relayout(2 * u, rows)):
                c = 2 * u + t
                acc = x1_v.at[c // 8 * T0:(c // 8 + 1) * T0, c % 8 * 128:(c % 8 + 1) * 128]
                r = _dot(hk, w) + acc[...]
                acc[...] = r
                res.append(r)
            store_lead(u, *res)
            if u == 1:
                sh = mod_tile(kn)
            if u == 3:
                s1 = 1.0 + mod_tile(kn + 8)

                @pl.when(k + 4 < 8)
                def _():
                    start(m_copies(k + 4))

            if u >= 4 and u % 2 == 0:
                @pl.when(k + 3 < 8)
                def _():
                    start(wa_copies(k + 3, range((u - 4) * 2, (u - 4) * 2 + 4)))

        h_v[kn] = (n_v[kn] * s1 + sh).astype(BF16)

        @pl.when(k == 4)
        def _():
            start(w_copies(UA // 3, range(UA % 3, 3)))

        @pl.when(k >= 4)
        def _():
            start(w_copies(UA // 3 + 1 + k - 4))

        return carry

    with _scope("stageA"):
        lax.fori_loop(0, 8, sa_body, 0)

    def ln1(seg):
        xb = x_v[seg, 8:SEG, :].astype(F32)
        return _ln(xb) * (1.0 + mod_v[0:1, D:2 * D]) + mod_v[0:1, 0:D]

    def hs_body(t, carry):
        for r in range(0, TH, 32):
            ss = _strassen_lhs(*[_ld(h_v, (t + 4 * b,), a * TH + r, 32).astype(F32)
                                 for a in range(2) for b in range(2)])
            for k, i in enumerate(SSUM):
                hs_v[k, t, r:r + 32, :] = ss[i].astype(BF16)
        return carry

    lax.fori_loop(0, 4, hs_body, 0)

    def lhs1(i):
        if i == 2:
            tiles = [_ld(h_v, (t,), 0, TH) for t in range(4)]
        elif i == 3:
            tiles = [_ld(h_v, (t + 4,), TH, TH) for t in range(4)]
        else:
            tiles = [_ld(hs_v, (SSUM.index(i), t), 0, TH) for t in range(4)]
        return jnp.concatenate(tiles, axis=1)

    NP1 = (3 * NP - UA) // P1N
    late = late_copies(False)
    nl = -(-len(late) // P1N)
    PW = UA // 3 + 5

    def p1_body(i, carry):
        u0 = UA + P1N * i
        with _scope("wait_w"):
            for q in range(P1N):
                w_wait(u0 + q)

        for q in range(P1N):
            lo, hi = relayout(2 * (u0 + q), slice(None))
            b = [lo[0:DH2], hi[0:DH2], lo[DH2:D], hi[DH2:D]]
            t = _strassen_rhs(*[x.astype(F32) for x in b])
            t = [b[0] if k == 1 else b[3] if k == 4 else t[k].astype(BF16) for k in range(7)]
            c = _strassen_out({k: _dot(lhs1(k), t[k]) for k in SORD})
            store_lead(u0 + q, jnp.concatenate([c[0], c[2]], axis=0), jnp.concatenate([c[1], c[3]], axis=0))

            if q < 3:
                @pl.when(PW + 3 * i + q < NP)
                def _():
                    start(w_copies(PW + 3 * i + q))
            elif q == 3:
                @pl.when(jnp.logical_and(i >= 2, i < 4))
                def _():
                    start([wo_copy(4 * (i - 2) + r) for r in range(4)])
            elif q == 4:
                @pl.when(i == 3)
                def _():
                    start(late_copies(True))

            @pl.when(i == NP1 - 1)
            def _():
                start(late[q * nl:(q + 1) * nl])

        hn_v[...] = ln1(0)
        return carry

    with _scope("phase1"):
        lax.fori_loop(0, NP1, p1_body, 0)

    with _scope("wait_wo"):
        wait([wo_copy(j) for j in range(8)])
        wait(late_copies(True))

    def prep_views(w, t_row, kh, nh, j, r0):
        src = w.at[pl.ds(j, nh + 1), pl.ds(pl.multiple_of(r0, 256), kh + 256), :]
        dst = lt_v.at[pl.ds(pl.multiple_of(t_row + j * kh + r0, 256), 4 * nh * kh + 256), :]
        return src, dst, kh, nh

    def prep(views, r0, n):
        src, dst, kh, nh = views
        t = _strassen_rhs(*[_ld(src, (b * nh,), a * kh + r0, n).astype(F32) for a in range(2) for b in range(2)])
        for k, i in enumerate(TSUM):
            dst[k * nh * kh + r0:k * nh * kh + r0 + n, :] = t[i].astype(BF16)

    def prep2_views(pc):
        f, q, half = pc >> 2, (pc >> 1) & 1, pc & 1
        src = w2_v.at[pl.ds(4 * q, 4), pl.ds(pl.multiple_of(256 * f + 64 * half, 64), KT2[3] + 64), :]
        dst = lt_v.at[pl.ds(pl.multiple_of(T2_ROW + q * (FF // 4) + 128 * f + 64 * half, 64),
                            (len(HKSUM) - 1) * (FF // 2) + 64), :]
        return src, dst

    def prep2(views, piece):
        src, dst = views
        r0 = (piece // 2) * 16
        sel = HKSUM[:6] if piece % 2 == 0 else HKSUM[6:]
        need = sorted({(k, n) for r in sel for k, n, _ in HK[r][1]})
        blocks = {(k, n): _ld(src, (n,), KT2[k] + r0, 16).astype(F32) for k, n in need}
        for r in sel:
            o = HKSUM.index(r) * (FF // 2) + r0
            dst[o:o + 16, :] = _comb(HK[r][1], blocks).astype(BF16)

    def step(it, odd, mem, macc):
        s = 2 * it + int(odd)
        lead = lt_v.at[pl.ds(pl.multiple_of(16 * s, 16), T1_ROW), :]
        lhs = jnp.concatenate([mem, hn_v[...]], axis=0).astype(BF16)
        hn_v[...] = ln1(jnp.minimum(s + 1, NSEG - 1))

        def proj(p):
            if p == 0:
                half = [_dot(lhs[:, 0:D // 2], _bf(w_v[c, 0:D // 4, :])) for c in range(6)]
                cols = [_dot(lhs[:, D // 2:D], _bf(w_v[c, D // 4:D // 2, :])) + half[c] for c in range(6)]
            for j in range(3):
                if p == 0:
                    r = _interleave(cols[j * 2], cols[j * 2 + 1])
                else:
                    r = _interleave(_dot(lhs, _bf(w_v[p * 6 + j * 2])), _dot(lhs, _bf(w_v[p * 6 + j * 2 + 1])))
                fr_v[p * 3 + j] = r.astype(BF16)

        def stack(p, j):
            return jnp.concatenate([fr_v[p * 3 + j],
                                    _ld(lead, (), (p * 3 + j) * 2 * T0, 16)], axis=0)

        def attn(pvs, qks):
            os_ = [_dot(pr_v[p, :, 0:80], stack(p, 2)) for p in pvs]
            ss = [lax.dot_general(stack(p, 0), stack(p, 1), (((1,), (1,)), ((), ())),
                                  preferred_element_type=F32) for p in qks]
            for p, o in zip(pvs, os_):
                for t, oh in enumerate(_deinterleave(o[0:64])):
                    lo_v[2 * p + t] = oh.astype(BF16)
                if odd:
                    ev = ev_v[p]
                    for k, sk in enumerate(_strassen_lhs(ev[0:8], ev[8:16], o[64:72], o[72:80])):
                        so_v[k, p, pl.ds(pl.multiple_of(8 * it, 8), 8), :] = sk.astype(BF16)
                else:
                    ev_v[p] = o[64:80]
            for p, sc_ in zip(qks, ss):
                fill = fill_v[...]
                sc_ = jnp.concatenate([sc_, jnp.zeros((80, 48), F32)], axis=1)
                sc_ = jnp.where(fill == 0.0, sc_, fill)
                mx = jnp.max(sc_, axis=-1, keepdims=True)
                e = jnp.exp2((sc_ - mx) * (scale * LOG2E))
                l = jnp.sum(e, axis=-1, keepdims=True)
                r = pl.reciprocal(l, approx=True)
                pr_v[p] = (e * (r * (2.0 - l * r))).astype(BF16)

        part = {}

        def wo(j, h0, h1):
            lo = jnp.concatenate([lo_v[h] for h in range(h0, h1)], axis=1)
            r = _dot(lo, _bf(wo_v[j, h0 * 64:h1 * 64, :]))
            part[j] = r + part[j] if j in part else r

        pc = jnp.maximum(it - NEARLY, 0)
        if odd:
            views = prep2_views(pc)
        else:
            views = prep_views(w1_v, T1_ROW, DH2, FH // 128, pc >> 1, (pc & 1) * 256)
        npiece = 0
        for op in SCHED:
            if op[0] == "proj":
                proj(op[1])
            elif op[0] == "attn":
                attn(op[1], op[2])
                if npiece < 8:
                    if odd:
                        prep2(views, npiece)
                    else:
                        prep(views, npiece * 32, 32)
                    k0 = (8 * int(odd) + npiece) * 64
                    pr = _ld(wmod_v, (it,), k0, 64).astype(F32) * st_v[k0:k0 + 64, :]
                    for g in range(8):
                        macc = pr[8 * g:8 * g + 8] if macc is None else macc + pr[8 * g:8 * g + 8]
                    lt_v[LT_ROWS - 16:LT_ROWS, :] = _bf(macc)
                    npiece += 1
            else:
                wo(*op[1:])
        res = jnp.concatenate([part[j] for j in range(8)], axis=1)
        x1_v[pl.ds(pl.multiple_of(SEG * s + 8, 8), TPS), :] = res[8:32]
        return res[0:8], macc

    with _scope("main"):
        def steps(i, mem):
            @pl.when(i == NEARLY)
            def _():
                wait(late)

            with _scope("iter"):
                mem, macc = step(i, True, *step(i, False, mem, None))
                mod_v[0:1, pl.ds(pl.multiple_of((16 + i) * 128, 128), 128)] = jnp.sum(macc, axis=0, keepdims=True)

            return mem

        lax.fori_loop(0, NSEG // 2, steps, mem0_ref[...].astype(F32))

    def wo_body(j, carry):
        acc = {}
        for kc in range(4):
            b = [jnp.concatenate([_bf(wo_v[j + 4 * n, (2 * p + t) * 64:(2 * p + t + 1) * 64, :])
                                  for p in range(4 * kc, 4 * kc + 4)], axis=0)
                 for t in range(2) for n in range(2)]
            tt = _strassen_rhs(*[x.astype(F32) for x in b])
            tt = [b[0] if k == 1 else b[3] if k == 4 else tt[k].astype(BF16) for k in range(7)]
            for k in SORD:
                sk = jnp.concatenate([_ld(so_v, (k, p), 0, TH) for p in range(4 * kc, 4 * kc + 4)], axis=1)
                y = _dot(sk, tt[k])
                acc[k] = y + acc[k] if kc else y
        for t, c in enumerate(_strassen_out(acc)):
            cs = pl.ds(pl.multiple_of((j + 4 * (t % 2)) * 128, 128), 128)
            for g in range(NSEG // 2):
                r0 = (2 * g + t // 2) * SEG
                x1_v[r0:r0 + 8, cs] = c[8 * g:8 * g + 8]
        return carry

    with _scope("p3a"):
        lax.fori_loop(0, 4, wo_body, 0)

    def rhs(w, t_row, kh, nh, i, j, k0, nk):
        if i == 1:
            return _ld(w, (j,), k0, nk)
        if i == 4:
            return _ld(w, (j + nh,), kh + k0, nk)
        return _ld(lt_v, (), t_row + (TSUM.index(i) * nh + j) * kh + k0, nk)

    def out_copy(i, q):
        segs = pl.ds(i * (FB // SEG), FB // SEG)
        cols = pl.ds(q * 256, 256)
        return [pltpu.make_async_copy(x_v.at[segs, :, cols], out_hbm.at[segs, :, cols], sems.at[SEM_OUT + i])]

    def resid1(r0, k0, n, c0=0, nc=D):
        if n >= SEG:
            xb = x_v[pl.ds((r0 >> 5) + k0 // SEG, n // SEG), :, c0:c0 + nc].astype(F32).reshape(n, nc)
        else:
            xb = x_v[(r0 >> 5) + k0 // SEG, k0 % SEG:k0 % SEG + n, c0:c0 + nc].astype(F32)
        return xb + mod_v[0:1, 2 * D + c0:2 * D + c0 + nc] * x1_v[pl.ds(r0 + k0, n), c0:c0 + nc]

    def ln2(slot, r0, k0, n):
        top, bot = [_ln(resid1(r0, t * HB + k0, n)) * (1.0 + mod_v[0:1, 4 * D:5 * D]) + mod_v[0:1, 3 * D:4 * D]
                    for t in range(2)]
        ss = _strassen_lhs(top[:, 0:DH2], top[:, DH2:D], bot[:, 0:DH2], bot[:, DH2:D])
        for i in range(7):
            for j in range(DH2 // 128):
                h2_v[slot, i, j, k0:k0 + n, :] = ss[i][:, j * 128:(j + 1) * 128].astype(BF16)

    ln2(0, 0, 0, HB)

    def ffn_body(i, carry):
        r0 = pl.multiple_of(i * FB, FB)
        rn = pl.multiple_of(jnp.minimum(r0 + FB, S - FB), FB)
        slot = lax.rem(i, 2)
        nf = FH // 256
        acc = {}
        gb = {}
        gl = {}

        def up(f, t):
            c0 = f * 256 + t * 128
            c = _strassen_out({
                k: _dot(jnp.concatenate([_ld(h2_v, (slot, k, j), 0, HB) for j in range(DH2 // 128)], axis=1),
                        rhs(w1_v, T1_ROW, DH2, FH // 128, k, c0 // 128, 0, DH2)) for k in SORD})
            b1a, b1b = bias_v[0:1, c0:c0 + 128], bias_v[0:1, FH + c0:FH + c0 + 128]
            blk = gb.setdefault(f, {})
            blk[0, t], blk[0, 2 + t] = _gelu(c[0] + b1a), _gelu(c[1] + b1b)
            blk[1, t], blk[1, 2 + t] = _gelu(c[2] + b1a), _gelu(c[3] + b1b)

        def lhs2(fs, r):
            key = (fs, HK[r][0])
            if key not in gl:
                gl[key] = jnp.concatenate([_comb(HK[r][0], gb[f], gl.setdefault(f, {})) for f in fs],
                                          axis=1).astype(BF16)
            return gl[key]

        def rhs2(fs, r, q):
            if r in HKSUM:
                return _ld(lt_v, (), T2_ROW + HKSUM.index(r) * (FF // 2) + q * (FF // 4) + 128 * fs[0], 128 * len(fs))
            k, n, _ = HK[r][1][0]
            return jnp.concatenate([_ld(w2_v, (4 * q + n,), 256 * f + KT2[k], 128) for f in fs], axis=0)

        def down(fs, q, r):
            y = _dot(lhs2(fs, r), rhs2(fs, r, q))
            key = (HK[r][2], q)
            acc[key] = y + acc[key] if key in acc else y

        def finish(q, n):
            for m in range(2):
                c = None
                for pat in dict.fromkeys(HK[r][2] for r in HKORD):
                    for mm, nn, sg in pat:
                        if (mm, nn) == (m, n):
                            a_ = acc[pat, q]
                            c = (a_ if sg > 0 else -a_) if c is None else (c + a_ if sg > 0 else c - a_)
                k0, c0 = m * HB, (4 * q + n) * 128
                y = (c + bias_v[0:1, FF + c0:FF + c0 + 128]) * mod_v[0:1, 5 * D + c0:5 * D + c0 + 128]
                o = (resid1(r0, k0, HB, c0, 128) + y).reshape(HB // SEG, SEG, 128).astype(BF16)
                x_v[pl.ds((r0 >> 5) + k0 // SEG, HB // SEG), :, c0:c0 + 128] = o
            if n % 2:
                start(out_copy(i, 2 * q + n // 2))

        groups = GROUPS
        work = [(fs, q, r) for fs in groups[:-1] for q in range(2) for r in HKORD]
        calls = [(f, t) for f in range(nf) for t in range(2)]
        done = 0
        w = 0
        for ci, (f, t) in enumerate(calls):
            up(f, t)
            ready = [x for x in work[done:] if 2 * x[0][-1] + 1 < ci]
            if ready:
                if w * LNP < HB:
                    ln2(1 - slot, rn, w * LNP, LNP)
                w += 1
                npc = min(len(ready), PIECE // len(ready[0][0]))
                for x in ready[:npc]:
                    down(*x)
                done += npc
        for x in work[done:]:
            down(*x)
        for q in range(2):
            for idx, r in enumerate(HKORD):
                down(groups[-1], q, r)
                for n in range(4):
                    last = max(j for j, rr in enumerate(HKORD) if any(nn == n for _, nn, _ in HK[rr][2]))
                    if idx == last:
                        finish(q, n)
        return carry

    with _scope("ffn"):
        lax.fori_loop(0, S // FB, ffn_body, 0)
    with _scope("wait_out"):
        for i in range(S // FB):
            for q in range(4):
                wait(out_copy(i, q))


@jax.jit
def pallas_adaLN_cond__memory_aug_recurrent_mem_tr__dense_activation_gelu__prompt_kernel(
    A_x, A_mem0, A_Wq, A_Wk, A_Wv, A_Wo, A_seg_len, B_x, B_w1, B_b1, B_w2, B_b2, c, w_mod,
):
    del A_seg_len, B_x
    assert A_x.shape == (1, S, D)
    hbm = pl.BlockSpec(memory_space=pl.ANY)
    out = pl.pallas_call(
        _kernel,
        out_shape=jax.ShapeDtypeStruct((NSEG, SEG, D), BF16),
        in_specs=[hbm] * 12,
        out_specs=hbm,
        scratch_shapes=[
            pltpu.VMEM((NSEG, SEG, D), BF16),
            pltpu.VMEM((8, T0, 128), BF16),
            pltpu.VMEM((TPS, D), F32),
            pltpu.VMEM((2, 7, 4, FB // 2, 128), BF16),
            pltpu.VMEM((S, D), F32),
            pltpu.VMEM((32, D, 128), BF16),
            pltpu.VMEM((8, 6 * D), F32),
            pltpu.VMEM((8, D), BF16),
            pltpu.VMEM((6 * NP, D // 2, 128), U32),
            pltpu.VMEM((8, H * DH // 2, 128), U32),
            pltpu.VMEM((FF // 128, D, 128), BF16),
            pltpu.VMEM((D // 128, FF, 128), BF16),
            pltpu.VMEM((LT_ROWS, 128), BF16),
            pltpu.VMEM((3 * NP, 64, 128), BF16),
            pltpu.VMEM((H, 32, 128), BF16),
            pltpu.VMEM((NP, 80, 128), BF16),
            pltpu.VMEM((80, 128), F32),
            pltpu.VMEM((1, FF + D), F32),
            pltpu.VMEM((8, T0, 128), F32),
            pltpu.VMEM((M, D), BF16),
            pltpu.VMEM((FF,), BF16),
            pltpu.VMEM((D,), BF16),
            pltpu.VMEM((1, D), BF16),
            pltpu.VMEM((5, 4, T0 // 2, 128), BF16),
            pltpu.VMEM((7, NP, T0 // 2, 128), BF16),
            pltpu.VMEM((NP, 16, 128), F32),
            pltpu.VMEM((D, 128), F32),
            pltpu.SemaphoreType.DMA((SEM_N,)),
        ],
        compiler_params=pltpu.CompilerParams(vmem_limit_bytes=122 * 1024 * 1024, disable_bounds_checks=True,
                                             disable_semaphore_checks=True),
    )(
        A_x.reshape(NSEG, SEG, D), A_mem0.reshape(M, D),
        A_Wq.reshape(D // 2, 2, H, DH), A_Wk.reshape(D // 2, 2, H, DH), A_Wv.reshape(D // 2, 2, H, DH),
        A_Wo.reshape(H * DH, D), B_w1, B_b1, B_w2, B_b2, c, w_mod,
    )
    return out.reshape(1, S, D)
```

```python
import contextlib

import jax
import jax.numpy as jnp
from jax import lax
import jax.experimental.pallas as pl
import jax.experimental.pallas.tpu as pltpu

F32 = jnp.float32
BF16 = jnp.bfloat16
U32 = jnp.uint32

S = 2048
D = 1024
H = 32
DH = 128
M = 8
SEG = 32
FF = 3584
EPS = 1e-5
LOG2E = 1.4426950408889634

NSEG = S // SEG
NP = H // 2
TPS = SEG - 8
T0 = 8 * NSEG
TH = T0 // 2
DH2 = D // 2
UA = 8
P1N = 5
NEARLY = 4
FB = 256
HB = FB // 2
LNP = 16

SSUM = (0, 1, 4, 5, 6)
SORD = (1, 4, 3, 2, 0, 6, 5)

HK = (
    (((0, 0, 1), (1, 0, -1)), ((0, 0, 1), (0, 1, 1), (2, 0, -1)), ((0, 0, 1),)),
    (((1, 0, 1),), ((0, 0, 1), (0, 2, 1), (1, 0, -1)), ((0, 0, 1), (1, 0, 1))),
    (((0, 1, 1),), ((1, 1, 1), (1, 2, 1), (0, 1, -1), (3, 1, -1)), ((0, 1, 1), (1, 1, 1))),
    (((1, 1, 1), (0, 1, -1)), ((1, 0, 1), (1, 1, 1), (1, 3, 1), (2, 1, -1)), ((1, 1, 1),)),
    (((0, 2, 1),), ((2, 1, 1), (2, 2, 1), (0, 2, -1), (3, 2, -1)), ((0, 2, 1),)),
    (((1, 2, 1),), ((2, 0, 1), (2, 2, 1), (2, 3, 1), (1, 2, -1)), ((1, 2, 1),)),
    (((0, 3, 1), (1, 3, -1)), ((3, 1, 1), (3, 3, 1), (2, 3, -1)), ((0, 3, 1),)),
    (((1, 3, 1),), ((3, 2, 1), (3, 3, 1), (1, 3, -1)), ((0, 3, 1), (1, 3, 1))),
    (((0, 1, 1), (1, 0, 1)), ((0, 1, 1), (1, 0, 1)), ((0, 0, 1), (1, 1, 1))),
    (((0, 0, 1), (0, 1, 1)), ((0, 1, 1),), ((0, 0, -1), (0, 1, 1))),
    (((1, 0, 1), (1, 1, 1)), ((1, 0, 1),), ((1, 0, 1), (1, 1, -1))),
    (((0, 0, 1), (0, 2, 1), (1, 0, -1)), ((0, 2, 1), (2, 0, 1)), ((0, 0, 1), (1, 0, 1), (1, 2, -1))),
    (((0, 0, 1), (0, 2, 1)), ((0, 2, 1),), ((0, 0, -1), (0, 2, 1), (1, 0, -1), (1, 2, 1))),
    (((0, 0, 1), (0, 2, 1), (1, 0, -1), (1, 2, -1)), ((2, 0, 1),), ((1, 0, -1), (1, 2, 1))),
    (((0, 3, 1),), ((3, 0, 1),), ((0, 0, 1),)),
    (((1, 3, 1),), ((3, 0, 1),), ((1, 0, 1),)),
    (((0, 0, 1),), ((0, 3, 1),), ((0, 3, 1),)),
    (((1, 0, 1),), ((0, 3, 1),), ((1, 3, 1),)),
    (((1, 1, 1), (1, 2, 1), (0, 1, -1)), ((1, 2, 1), (2, 1, 1)), ((0, 1, 1), (0, 2, -1), (1, 1, 1))),
    (((1, 1, 1), (1, 2, 1)), ((1, 2, 1),), ((0, 1, -1), (0, 2, 1), (1, 1, -1), (1, 2, 1))),
    (((1, 1, 1), (1, 2, 1), (0, 1, -1), (0, 2, -1)), ((2, 1, 1),), ((0, 1, -1), (0, 2, 1))),
    (((0, 1, 1), (1, 3, 1)), ((1, 3, 1), (3, 1, 1)), ((0, 3, 1), (1, 1, 1))),
    (((1, 1, 1), (1, 3, 1)), ((1, 3, 1),), ((1, 1, -1), (1, 3, 1))),
    (((0, 1, 1), (0, 3, 1)), ((3, 1, 1),), ((0, 1, 1), (0, 3, -1))),
    (((0, 2, 1), (0, 3, 1), (1, 3, -1)), ((2, 3, 1), (3, 2, 1)), ((0, 3, 1), (1, 2, -1), (1, 3, 1))),
    (((0, 2, 1), (0, 3, 1), (1, 3, -1), (1, 2, -1)), ((2, 3, 1),), ((1, 2, 1), (1, 3, -1))),
    (((0, 2, 1), (0, 3, 1)), ((3, 2, 1),), ((0, 2, 1), (0, 3, -1), (1, 2, 1), (1, 3, -1))),
)
HKSUM = tuple(r for r, t in enumerate(HK) if len(t[1]) > 1)
HKCOL = tuple(sorted(range(len(HK)), key=lambda r: min(n for _, n, _ in HK[r][2])))
HKBLK = (2, 9, 18, 19, 20, 23, 4, 12, 26, 0, 1, 8, 11, 14, 10, 13, 15, 3, 21, 22, 5, 24, 25, 7, 17, 6, 16)
HKL = tuple(dict.fromkeys(t[0] for t in HK))
TS = FF // 2

T1_ROW = 3 * NP * 2 * T0
T2_ROW = T1_ROW + len(HKSUM) * TS
LT_ROWS = T2_ROW + len(HKSUM) * TS + 16

SEM_W, SEM_A, SEM_M, SEM_MISC, SEM_OUT = 0, 48, 56, 64, 72
SEM_N = SEM_OUT + S // FB


def _make_sched(h1=24, n1=1, n2=4):
    out = []

    def pairs(a):
        return tuple(p for p in (a, a + 1) if 0 <= p < NP)

    nxt = 0
    for p in range(NP):
        out.append(("proj", p))
        if p >= 2 and p % 2 == 0:
            out.append(("attn", pairs(nxt - 2), pairs(nxt)))
            nxt += 2
    out += [("wo", j, 0, h1) for j in range(n1)]
    out.append(("attn", pairs(nxt - 2), pairs(nxt)))
    out += [("wo", j, 0, h1) for j in range(n1, n2)]
    out.append(("attn", pairs(nxt), ()))
    out += [("wo", j, 0, h1) for j in range(n2, 8)]
    out += [("wo", j, h1, H) for j in range(8)]
    return out


SCHED = _make_sched()
_SCOPES = False


def _scope(name):
    return jax.named_scope(name) if _SCOPES else contextlib.nullcontext()


def _dot(a, b):
    return jnp.dot(a, b, preferred_element_type=F32)


def _bf(x):
    return pltpu.bitcast(x, BF16)


def _ld(ref, idx, r0, n):
    return _bf(ref.at[(*idx, pl.ds(r0, n), slice(None))].bitcast(U32)[...])


def _ln(x):
    m = jnp.mean(x, axis=-1, keepdims=True)
    xc = x - m
    v = jnp.mean(xc * xc, axis=-1, keepdims=True)
    return xc * lax.rsqrt(v + EPS)


def _gelu(x):
    c = 0.7978845608028654
    return 0.5 * x * (1.0 + jnp.tanh(c * (x + 0.044715 * (x * x * x))))


def _strassen_lhs(a11, a12, a21, a22):
    return [a11 + a22, a21 + a22, a11, a22, a11 + a12, a21 - a11, a12 - a22]


def _strassen_rhs(b11, b12, b21, b22):
    return [b11 + b22, b11, b12 - b22, b21 - b11, b22, b11 + b12, b21 + b22]


def _strassen_out(m):
    return (m[0] + m[3] - m[4] + m[6], m[2] + m[4], m[1] + m[3], m[0] - m[1] + m[2] + m[5])


def _comb(terms, blocks, memo=None):
    memo = {} if memo is None else memo
    for n in range(1, len(terms) + 1):
        key = terms[:n]
        if key not in memo:
            i, j, sg = terms[n - 1]
            b = blocks[i, j]
            memo[key] = b if n == 1 else (memo[terms[:n - 1]] + b if sg > 0 else memo[terms[:n - 1]] - b)
    return memo[terms]


def _interleave(a, b):
    n = a.shape[0] // 8
    parts = []
    for g in range(n):
        parts.append(a[8 * g:8 * g + 8])
        parts.append(b[8 * g:8 * g + 8])
    return jnp.concatenate(parts, axis=0)


def _deinterleave(v):
    n = v.shape[0] // 16
    a = jnp.concatenate([v[16 * g:16 * g + 8] for g in range(n)], axis=0)
    b = jnp.concatenate([v[16 * g + 8:16 * g + 16] for g in range(n)], axis=0)
    return a, b


def _kernel(x_hbm, mem0_hbm, wq_hbm, wk_hbm, wv_hbm, wo_hbm, w1_hbm, b1_hbm, w2_hbm, b2_hbm,
            c_hbm, wmod_hbm, out_hbm,
            x_v, h_v, hn_v, h2_v, x1_v, wmod_v, mod_v, sc_v, w_v, wo_v, w1_v, w2_v,
            lt_v, fr_v, lo_v, pr_v, fill_v, bias_v, n_v,
            mem0_ref, b1_ref, b2_ref, c_ref, hs_v, so_v, ev_v, st_v,
            sems):
    w32 = [r.bitcast(U32) for r in (wq_hbm, wk_hbm, wv_hbm)]
    wo32 = wo_hbm.bitcast(U32)

    def w_copies(p, js=range(3)):
        return [pltpu.make_async_copy(w32[j].at[:, par, p, :], w_v.at[p * 6 + j * 2 + par],
                                      sems.at[SEM_W + 3 * p + j]) for j in js for par in range(2)]

    def w_wait(u):
        both = w_v.at[pl.ds(2 * u, 2)]
        pltpu.make_async_copy(both, both, sems.at[SEM_W + u]).wait()

    def _mult(i, m):
        return i * m if isinstance(i, int) else pl.multiple_of(i * m, m)

    def wa_copies(k, units=range(UA)):
        r = pl.ds(_mult(k, 64), 64)
        return [pltpu.make_async_copy(w32[u % 3].at[r, par, u // 3, :], w_v.at[2 * u + par, r], sems.at[SEM_A + k])
                for u in units for par in range(2)]

    def m_copies(k):
        return [pltpu.make_async_copy(wmod_hbm.at[:, pl.ds(_mult(k + 8 * t, 128), 128)], wmod_v.at[16 + k + 8 * t],
                                      sems.at[SEM_M + k]) for t in range(2)]

    def start(cps):
        for cp in cps:
            cp.start()

    def wait(cps):
        for cp in cps:
            cp.wait()

    cp_x0 = pltpu.make_async_copy(x_hbm.at[:, 0:8, :], x_v.at[:, 0:8, :], sems.at[SEM_MISC + 1])

    def wo_copy(j):
        return pltpu.make_async_copy(wo32.at[:, pl.ds(_mult(j, 128), 128)], wo_v.at[j], sems.at[SEM_MISC + 3])

    def late_copies(first):
        sem = sems.at[SEM_MISC + (4 if first else 5)]
        sg = slice(1, 2 * NEARLY + 1) if first else slice(2 * NEARLY + 1, NSEG)
        cps = [(x_hbm.at[sg, 8:SEG, :], x_v.at[sg, 8:SEG, :])]
        cps += [(wmod_hbm.at[:, (16 + j) * 128:(17 + j) * 128], wmod_v.at[j])
                for j in (range(NEARLY) if first else range(NEARLY, 32))]
        for src, dst, nt, nr in ((w1_hbm, w1_v, FF // 128, D), (w2_hbm, w2_v, D // 128, 512)):
            for j in range(nt):
                if j < 4:
                    rows = slice(0, nr) if first else slice(nr, src.shape[0])
                else:
                    rows = slice(0, 0) if first else slice(0, src.shape[0])
                if rows.stop > rows.start:
                    cps.append((src.at[rows, j * 128:(j + 1) * 128], dst.at[j, rows]))
        return [pltpu.make_async_copy(src, dst, sem) for src, dst in cps]

    cp_small = [pltpu.make_async_copy(src, dst, sems.at[SEM_MISC])
                for src, dst in ((c_hbm, c_ref), (mem0_hbm, mem0_ref), (b1_hbm, b1_ref), (b2_hbm, b2_ref),
                                 (x_hbm.at[0, 8:SEG, :], x_v.at[0, 8:SEG, :]))]

    start(cp_small)
    cp_x0.start()
    start(m_copies(0))
    for k in range(2):
        start(m_copies(k + 1))
        start(wa_copies(k))

    scale = DH ** -0.5
    ri = lax.broadcasted_iota(jnp.int32, (80, 128), 0)
    ci = lax.broadcasted_iota(jnp.int32, (80, 128), 1)
    same_head = (((ri >> 3) & 1) == ((ci >> 3) & 1)) & (ci < 80)
    rpos = (((ri >> 4) & 3) << 3) + (ri & 7)
    cpos = (((ci >> 4) & 3) << 3) + (ci & 7)
    keep = (ri < 16) | (ci < 16) | (rpos >= cpos)
    fill_v[...] = jnp.where(same_head, jnp.where(keep, 0.0, -1e9 / scale), -jnp.inf).astype(F32)

    wait(cp_small)
    c = c_ref[...].astype(F32)
    sc = jnp.broadcast_to(c * jax.nn.sigmoid(c), (8, D)).astype(BF16)

    sc_v[...] = sc
    for k in range(8):
        st_v[k * 128:(k + 1) * 128, :] = jnp.broadcast_to(sc[0:1, k * 128:(k + 1) * 128].astype(F32), (128, 128)).T
    bias_v[:, 0:FF] = b1_ref[...].astype(F32).reshape(1, FF)
    bias_v[:, FF:FF + D] = b2_ref[...].astype(F32).reshape(1, D)

    def zero_body(i, carry):
        x1_v[pl.ds(pl.multiple_of(i * 64, 64), 64), :] = jnp.zeros((64, D), F32)
        return carry

    lax.fori_loop(0, -(-UA // 4) * 8, zero_body, 0)

    def relayout(c, rows):
        a = w_v[c, rows, :]
        b = w_v[c + 1, rows, :]
        lo = (a & jnp.uint32(0xFFFF)) | (b << 16)
        hi = (a >> 16) | (b & jnp.uint32(0xFFFF0000))
        w_v[c, rows, :] = lo
        w_v[c + 1, rows, :] = hi
        return _bf(lo), _bf(hi)

    def store_lead(u, a, b):
        lt_v[pl.ds(_mult(u, 2 * T0), 2 * T0), :] = _interleave(a, b).astype(BF16)

    def mod_tile(ct):
        m = _dot(sc_v[...], _ld(wmod_v, (16 + ct,), 0, D))
        mod_v[:, pl.ds(_mult(ct, 128), 128)] = m
        return m[0:1]

    with _scope("wait_x0"):
        cp_x0.wait()

    def ln1_body(i, carry):
        r = pl.multiple_of(i * 128, 128)
        n = _ln(x_v[pl.ds(i * 16, 16), 0:8, :].astype(F32).reshape(128, D))
        for k in range(8):
            n_v[k, pl.ds(r, 128), :] = n[:, k * 128:(k + 1) * 128]
        return carry

    with _scope("ln1"):
        lax.fori_loop(0, T0 // 128, ln1_body, 0)
    start(m_copies(3))
    start(wa_copies(2))
    with _scope("wait_m0"):
        wait(m_copies(0))
    h_v[0] = (n_v[0] * (1.0 + mod_tile(8)) + mod_tile(0)).astype(BF16)

    def sa_body(k, carry):
        with _scope("wait_a"):
            wait(wa_copies(k))

            @pl.when(k < 7)
            def _():
                wait(m_copies(k + 1))

        kn = jnp.minimum(k + 1, 7)
        rows = pl.ds(pl.multiple_of(k * 64, 64), 64)
        hk = _ld(h_v, (k,), 0, T0)
        for u in range(UA):
            res = []
            for t, w in enumerate(relayout(2 * u, rows)):
                c = 2 * u + t
                acc = x1_v.at[c // 8 * T0:(c // 8 + 1) * T0, c % 8 * 128:(c % 8 + 1) * 128]
                r = _dot(hk, w) + acc[...]
                acc[...] = r
                res.append(r)
            store_lead(u, *res)
            if u == 1:
                sh = mod_tile(kn)
            if u == 3:
                s1 = 1.0 + mod_tile(kn + 8)

                @pl.when(k + 4 < 8)
                def _():
                    start(m_copies(k + 4))

            if u >= 4 and u % 2 == 0:
                @pl.when(k + 3 < 8)
                def _():
                    start(wa_copies(k + 3, range((u - 4) * 2, (u - 4) * 2 + 4)))

        h_v[kn] = (n_v[kn] * s1 + sh).astype(BF16)

        @pl.when(k == 4)
        def _():
            start(w_copies(UA // 3, range(UA % 3, 3)))

        @pl.when(k >= 4)
        def _():
            start(w_copies(UA // 3 + 1 + k - 4))

        return carry

    with _scope("stageA"):
        lax.fori_loop(0, 8, sa_body, 0)

    def ln1(seg):
        xb = x_v[seg, 8:SEG, :].astype(F32)
        return _ln(xb) * (1.0 + mod_v[0:1, D:2 * D]) + mod_v[0:1, 0:D]

    def hs_body(t, carry):
        for r in range(0, TH, 32):
            ss = _strassen_lhs(*[_ld(h_v, (t + 4 * b,), a * TH + r, 32).astype(F32)
                                 for a in range(2) for b in range(2)])
            for k, i in enumerate(SSUM):
                hs_v[k, t, r:r + 32, :] = ss[i].astype(BF16)
        return carry

    lax.fori_loop(0, 4, hs_body, 0)

    def lhs1(i):
        if i == 2:
            tiles = [_ld(h_v, (t,), 0, TH) for t in range(4)]
        elif i == 3:
            tiles = [_ld(h_v, (t + 4,), TH, TH) for t in range(4)]
        else:
            tiles = [_ld(hs_v, (SSUM.index(i), t), 0, TH) for t in range(4)]
        return jnp.concatenate(tiles, axis=1)

    NP1 = (3 * NP - UA) // P1N
    late = late_copies(False)
    nl = -(-len(late) // P1N)
    PW = UA // 3 + 5

    def p1_body(i, carry):
        u0 = UA + P1N * i
        with _scope("wait_w"):
            for q in range(P1N):
                w_wait(u0 + q)

        for q in range(P1N):
            lo, hi = relayout(2 * (u0 + q), slice(None))
            b = [lo[0:DH2], hi[0:DH2], lo[DH2:D], hi[DH2:D]]
            t = _strassen_rhs(*[x.astype(F32) for x in b])
            t = [b[0] if k == 1 else b[3] if k == 4 else t[k].astype(BF16) for k in range(7)]
            c = _strassen_out({k: _dot(lhs1(k), t[k]) for k in SORD})
            store_lead(u0 + q, jnp.concatenate([c[0], c[2]], axis=0), jnp.concatenate([c[1], c[3]], axis=0))

            if q < 3:
                @pl.when(PW + 3 * i + q < NP)
                def _():
                    start(w_copies(PW + 3 * i + q))
            elif q == 3:
                @pl.when(jnp.logical_and(i >= 2, i < 4))
                def _():
                    start([wo_copy(4 * (i - 2) + r) for r in range(4)])
            elif q == 4:
                @pl.when(i == 3)
                def _():
                    start(late_copies(True))

            @pl.when(i == NP1 - 1)
            def _():
                start(late[q * nl:(q + 1) * nl])

        hn_v[...] = ln1(0)
        return carry

    with _scope("phase1"):
        lax.fori_loop(0, NP1, p1_body, 0)

    with _scope("wait_wo"):
        wait([wo_copy(j) for j in range(8)])
        wait(late_copies(True))

    def prep_views(odd, pc):
        f = pc >> 2
        if odd:
            q, half = (pc >> 1) & 1, pc & 1
            kb, w, tile0, r0 = 128, w2_v, 4 * q, 512 * f + 64 * half
            d0 = T2_ROW + q * (FF // 4) + 128 * f + 64 * half
        else:
            kb, w, tile0, r0 = 256, w1_v, 4 * f, 64 * (pc & 3)
            d0 = T1_ROW + 64 * pc
        src = w.at[pl.ds(tile0, 4), pl.ds(pl.multiple_of(r0, 64), 3 * kb + 64), :]
        dst = lt_v.at[pl.ds(pl.multiple_of(d0, 64), (len(HKSUM) - 1) * TS + 64), :]
        return src, dst, kb

    def prep(views, piece):
        src, dst, kb = views
        r0 = (piece // 2) * 16
        sel = HKSUM[:6] if piece % 2 == 0 else HKSUM[6:]
        need = sorted({(k, n) for r in sel for k, n, _ in HK[r][1]})
        blocks = {(k, n): _ld(src, (n,), k * kb + r0, 16).astype(F32) for k, n in need}
        for r in sel:
            o = HKSUM.index(r) * TS + r0
            dst[o:o + 16, :] = _comb(HK[r][1], blocks).astype(BF16)

    def step(it, odd, mem, macc):
        s = 2 * it + int(odd)
        lead = lt_v.at[pl.ds(pl.multiple_of(16 * s, 16), T1_ROW), :]
        lhs = jnp.concatenate([mem, hn_v[...]], axis=0).astype(BF16)
        hn_v[...] = ln1(jnp.minimum(s + 1, NSEG - 1))

        def proj(p):
            if p == 0:
                half = [_dot(lhs[:, 0:D // 2], _bf(w_v[c, 0:D // 4, :])) for c in range(6)]
                cols = [_dot(lhs[:, D // 2:D], _bf(w_v[c, D // 4:D // 2, :])) + half[c] for c in range(6)]
            for j in range(3):
                if p == 0:
                    r = _interleave(cols[j * 2], cols[j * 2 + 1])
                else:
                    r = _interleave(_dot(lhs, _bf(w_v[p * 6 + j * 2])), _dot(lhs, _bf(w_v[p * 6 + j * 2 + 1])))
                fr_v[p * 3 + j] = r.astype(BF16)

        def stack(p, j):
            return jnp.concatenate([fr_v[p * 3 + j],
                                    _ld(lead, (), (p * 3 + j) * 2 * T0, 16)], axis=0)

        def attn(pvs, qks):
            os_ = [_dot(pr_v[p, :, 0:80], stack(p, 2)) for p in pvs]
            ss = [lax.dot_general(stack(p, 0), stack(p, 1), (((1,), (1,)), ((), ())),
                                  preferred_element_type=F32) for p in qks]
            for p, o in zip(pvs, os_):
                for t, oh in enumerate(_deinterleave(o[0:64])):
                    lo_v[2 * p + t] = oh.astype(BF16)
                if odd:
                    ev = ev_v[p]
                    for k, sk in enumerate(_strassen_lhs(ev[0:8], ev[8:16], o[64:72], o[72:80])):
                        so_v[k, p, pl.ds(pl.multiple_of(8 * it, 8), 8), :] = sk.astype(BF16)
                else:
                    ev_v[p] = o[64:80]
            for p, sc_ in zip(qks, ss):
                fill = fill_v[...]
                sc_ = jnp.concatenate([sc_, jnp.zeros((80, 48), F32)], axis=1)
                sc_ = jnp.where(fill == 0.0, sc_, fill)
                mx = jnp.max(sc_, axis=-1, keepdims=True)
                e = jnp.exp2((sc_ - mx) * (scale * LOG2E))
                l = jnp.sum(e, axis=-1, keepdims=True)
                r = pl.reciprocal(l, approx=True)
                pr_v[p] = (e * (r * (2.0 - l * r))).astype(BF16)

        part = {}

        def wo(j, h0, h1):
            lo = jnp.concatenate([lo_v[h] for h in range(h0, h1)], axis=1)
            r = _dot(lo, _bf(wo_v[j, h0 * 64:h1 * 64, :]))
            part[j] = r + part[j] if j in part else r

        pc = jnp.maximum(it - NEARLY, 0)
        views = prep_views(odd, pc)
        npiece = 0
        for op in SCHED:
            if op[0] == "proj":
                proj(op[1])
            elif op[0] == "attn":
                attn(op[1], op[2])
                if npiece < 8:
                    prep(views, npiece)
                    k0 = (8 * int(odd) + npiece) * 64
                    pr = _ld(wmod_v, (it,), k0, 64).astype(F32) * st_v[k0:k0 + 64, :]
                    for g in range(8):
                        macc = pr[8 * g:8 * g + 8] if macc is None else macc + pr[8 * g:8 * g + 8]
                    lt_v[LT_ROWS - 16:LT_ROWS, :] = _bf(macc)
                    npiece += 1
            else:
                wo(*op[1:])
        res = jnp.concatenate([part[j] for j in range(8)], axis=1)
        x1_v[pl.ds(pl.multiple_of(SEG * s + 8, 8), TPS), :] = res[8:32]
        return res[0:8], macc

    with _scope("main"):
        def steps(i, mem):
            @pl.when(i == NEARLY)
            def _():
                wait(late)

            with _scope("iter"):
                mem, macc = step(i, True, *step(i, False, mem, None))
                mod_v[0:1, pl.ds(pl.multiple_of((16 + i) * 128, 128), 128)] = jnp.sum(macc, axis=0, keepdims=True)

            return mem

        lax.fori_loop(0, NSEG // 2, steps, mem0_ref[...].astype(F32))

    def wo_body(j, carry):
        acc = {}
        for kc in range(4):
            b = [jnp.concatenate([_bf(wo_v[j + 4 * n, (2 * p + t) * 64:(2 * p + t + 1) * 64, :])
                                  for p in range(4 * kc, 4 * kc + 4)], axis=0)
                 for t in range(2) for n in range(2)]
            tt = _strassen_rhs(*[x.astype(F32) for x in b])
            tt = [b[0] if k == 1 else b[3] if k == 4 else tt[k].astype(BF16) for k in range(7)]
            for k in SORD:
                sk = jnp.concatenate([_ld(so_v, (k, p), 0, TH) for p in range(4 * kc, 4 * kc + 4)], axis=1)
                y = _dot(sk, tt[k])
                acc[k] = y + acc[k] if kc else y
        for t, c in enumerate(_strassen_out(acc)):
            cs = pl.ds(pl.multiple_of((j + 4 * (t % 2)) * 128, 128), 128)
            for g in range(NSEG // 2):
                r0 = (2 * g + t // 2) * SEG
                x1_v[r0:r0 + 8, cs] = c[8 * g:8 * g + 8]
        return carry

    with _scope("p3a"):
        lax.fori_loop(0, 4, wo_body, 0)

    def out_copy(i, q):
        segs = pl.ds(i * (FB // SEG), FB // SEG)
        cols = pl.ds(q * 256, 256)
        return pltpu.make_async_copy(x_v.at[segs, :, cols], out_hbm.at[segs, :, cols], sems.at[SEM_OUT + i])

    def resid1(r0, k0, n, c0=0, nc=D):
        if n >= SEG:
            xb = x_v[pl.ds((r0 >> 5) + k0 // SEG, n // SEG), :, c0:c0 + nc].astype(F32).reshape(n, nc)
        else:
            xb = x_v[(r0 >> 5) + k0 // SEG, k0 % SEG:k0 % SEG + n, c0:c0 + nc].astype(F32)
        return xb + mod_v[0:1, 2 * D + c0:2 * D + c0 + nc] * x1_v[pl.ds(r0 + k0, n), c0:c0 + nc]

    def ln2(slot, r0, k0, n):
        hm = [_ln(resid1(r0, m * HB + k0, n)) * (1.0 + mod_v[0:1, 4 * D:5 * D]) + mod_v[0:1, 3 * D:4 * D]
              for m in range(2)]
        for j in range(2):
            blocks = {(m, k): hm[m][:, k * 256 + j * 128:k * 256 + (j + 1) * 128]
                      for m in range(2) for k in range(4)}
            memo = {}
            for i, terms in enumerate(HKL):
                h2_v[slot, i, j, k0:k0 + n, :] = _comb(terms, blocks, memo).astype(BF16)

    ln2(0, 0, 0, HB)

    def ffn_body(i, carry):
        r0 = pl.multiple_of(i * FB, FB)
        rn = pl.multiple_of(jnp.minimum(r0 + FB, S - FB), FB)
        slot = lax.rem(i, 2)
        acc = {}
        act = {}
        memo = {}

        def accumulate(key, r, y):
            key = (HK[r][2], key)
            acc[key] = y + acc[key] if key in acc else y

        def collect(key, m, n, order):
            c = None
            for pat in dict.fromkeys(HK[r][2] for r in order):
                for mm, nn, sg in pat:
                    if (mm, nn) == (m, n):
                        y = acc[pat, key]
                        c = (y if sg > 0 else -y) if c is None else (c + y if sg > 0 else c - y)
            return c

        def up(f, lo, hi):
            for idx in range(lo, hi):
                r = HKBLK[idx]
                lhs = jnp.concatenate([_ld(h2_v, (slot, HKL.index(HK[r][0]), j), 0, HB) for j in range(2)], axis=1)
                if r in HKSUM:
                    w = _ld(lt_v, (), T1_ROW + HKSUM.index(r) * TS + 256 * f, 256)
                else:
                    k, n, _ = HK[r][1][0]
                    w = _ld(w1_v, (4 * f + n,), 256 * k, 256)
                accumulate(("up", f), r, _dot(lhs, w))
                for m, n, _ in HK[r][2]:
                    if not any((m, n) == t[0:2] for rr in HKBLK[idx + 1:] for t in HK[rr][2]):
                        c0 = (4 * f + n) * 128
                        act.setdefault(f, {})[m, n] = _gelu(
                            collect(("up", f), m, n, HKBLK) + bias_v[0:1, c0:c0 + 128])

        def down(fs, q, r):
            if (fs, HK[r][0]) not in memo:
                memo[fs, HK[r][0]] = jnp.concatenate(
                    [_comb(HK[r][0], act[f], memo.setdefault(f, {})) for f in fs], axis=1).astype(BF16)
            if r in HKSUM:
                w = _ld(lt_v, (), T2_ROW + HKSUM.index(r) * TS + q * (FF // 4) + 128 * fs[0], 128 * len(fs))
            else:
                k, n, _ = HK[r][1][0]
                w = jnp.concatenate([_ld(w2_v, (4 * q + n,), 512 * f + 128 * k, 128) for f in fs], axis=0)
            accumulate(q, r, _dot(memo[fs, HK[r][0]], w))

        def finish(q, n):
            c0 = (4 * q + n) * 128
            for m in range(2):
                y = (collect(q, m, n, HKCOL) + bias_v[0:1, FF + c0:FF + c0 + 128]) * mod_v[0:1, 5 * D + c0:5 * D + c0 + 128]
                o = (resid1(r0, m * HB, HB, c0, 128) + y).reshape(HB // SEG, SEG, 128).astype(BF16)
                x_v[pl.ds((r0 >> 5) + m * (HB // SEG), HB // SEG), :, c0:c0 + 128] = o
            if n % 2:
                out_copy(i, 2 * q + n // 2).start()

        work = [(fs, q, r) for fs in ((0, 1), (2, 3), (4, 5)) for r in range(len(HK)) for q in range(2)]
        piece = 0
        for f in range(FF // 512):
            for lo, hi in ((0, 14), (14, len(HK))):
                up(f, lo, hi)
                ready = [x for x in work[:14] if x[0][-1] < f]
                if ready and piece * LNP < HB:
                    ln2(1 - slot, rn, piece * LNP, LNP)
                    piece += 1
                for x in ready:
                    down(*x)
                work = work[len(ready):]
        assert piece * LNP == HB
        for x in work:
            down(*x)
        for q in range(2):
            for idx, r in enumerate(HKCOL):
                down((6,), q, r)
                for n in range(4):
                    if idx == max(j for j, rr in enumerate(HKCOL) if any(t[1] == n for t in HK[rr][2])):
                        finish(q, n)
        return carry

    with _scope("ffn"):
        lax.fori_loop(0, S // FB, ffn_body, 0)
    with _scope("wait_out"):
        for i in range(S // FB):
            for q in range(4):
                out_copy(i, q).wait()


@jax.jit
def pallas_adaLN_cond__memory_aug_recurrent_mem_tr__dense_activation_gelu__prompt_kernel(
    A_x, A_mem0, A_Wq, A_Wk, A_Wv, A_Wo, A_seg_len, B_x, B_w1, B_b1, B_w2, B_b2, c, w_mod,
):
    del A_seg_len, B_x
    assert A_x.shape == (1, S, D)
    hbm = pl.BlockSpec(memory_space=pl.ANY)
    out = pl.pallas_call(
        _kernel,
        out_shape=jax.ShapeDtypeStruct((NSEG, SEG, D), BF16),
        in_specs=[hbm] * 12,
        out_specs=hbm,
        scratch_shapes=[
            pltpu.VMEM((NSEG, SEG, D), BF16),
            pltpu.VMEM((8, T0, 128), BF16),
            pltpu.VMEM((TPS, D), F32),
            pltpu.VMEM((2, len(HKL), 2, HB, 128), BF16),
            pltpu.VMEM((S, D), F32),
            pltpu.VMEM((32, D, 128), BF16),
            pltpu.VMEM((8, 6 * D), F32),
            pltpu.VMEM((8, D), BF16),
            pltpu.VMEM((6 * NP, D // 2, 128), U32),
            pltpu.VMEM((8, H * DH // 2, 128), U32),
            pltpu.VMEM((FF // 128, D, 128), BF16),
            pltpu.VMEM((D // 128, FF, 128), BF16),
            pltpu.VMEM((LT_ROWS, 128), BF16),
            pltpu.VMEM((3 * NP, 64, 128), BF16),
            pltpu.VMEM((H, 32, 128), BF16),
            pltpu.VMEM((NP, 80, 128), BF16),
            pltpu.VMEM((80, 128), F32),
            pltpu.VMEM((1, FF + D), F32),
            pltpu.VMEM((8, T0, 128), F32),
            pltpu.VMEM((M, D), BF16),
            pltpu.VMEM((FF,), BF16),
            pltpu.VMEM((D,), BF16),
            pltpu.VMEM((1, D), BF16),
            pltpu.VMEM((5, 4, T0 // 2, 128), BF16),
            pltpu.VMEM((7, NP, T0 // 2, 128), BF16),
            pltpu.VMEM((NP, 16, 128), F32),
            pltpu.VMEM((D, 128), F32),
            pltpu.SemaphoreType.DMA((SEM_N,)),
        ],
        compiler_params=pltpu.CompilerParams(vmem_limit_bytes=122 * 1024 * 1024, disable_bounds_checks=True,
                                             disable_semaphore_checks=True),
    )(
        A_x.reshape(NSEG, SEG, D), A_mem0.reshape(M, D),
        A_Wq.reshape(D // 2, 2, H, DH), A_Wk.reshape(D // 2, 2, H, DH), A_Wv.reshape(D // 2, 2, H, DH),
        A_Wo.reshape(H * DH, D), B_w1, B_b1, B_w2, B_b2, c, w_mod,
    )
    return out.reshape(1, S, D)
```

```python
import contextlib

import jax
import jax.numpy as jnp
from jax import lax
import jax.experimental.pallas as pl
import jax.experimental.pallas.tpu as pltpu

F32 = jnp.float32
BF16 = jnp.bfloat16
U32 = jnp.uint32

S = 2048
D = 1024
H = 32
DH = 128
M = 8
SEG = 32
FF = 3584
EPS = 1e-5
LOG2E = 1.4426950408889634

NSEG = S // SEG
NP = H // 2
TPS = SEG - 8
T0 = 8 * NSEG
TH = T0 // 2
DH2 = D // 2
UA = 8
P1N = 5
NEARLY = 4
FB = 256
HB = FB // 2
LNP = 16

SSUM = (0, 1, 4, 5, 6)
SORD = (1, 4, 3, 2, 0, 6, 5)

HK = (
    (((0, 0, 1), (1, 0, -1)), ((0, 0, 1), (0, 1, 1), (2, 0, -1)), ((0, 0, 1),)),
    (((1, 0, 1),), ((0, 0, 1), (0, 2, 1), (1, 0, -1)), ((0, 0, 1), (1, 0, 1))),
    (((0, 1, 1),), ((1, 1, 1), (1, 2, 1), (0, 1, -1), (3, 1, -1)), ((0, 1, 1), (1, 1, 1))),
    (((1, 1, 1), (0, 1, -1)), ((1, 0, 1), (1, 1, 1), (1, 3, 1), (2, 1, -1)), ((1, 1, 1),)),
    (((0, 2, 1),), ((2, 1, 1), (2, 2, 1), (0, 2, -1), (3, 2, -1)), ((0, 2, 1),)),
    (((1, 2, 1),), ((2, 0, 1), (2, 2, 1), (2, 3, 1), (1, 2, -1)), ((1, 2, 1),)),
    (((0, 3, 1), (1, 3, -1)), ((3, 1, 1), (3, 3, 1), (2, 3, -1)), ((0, 3, 1),)),
    (((1, 3, 1),), ((3, 2, 1), (3, 3, 1), (1, 3, -1)), ((0, 3, 1), (1, 3, 1))),
    (((0, 1, 1), (1, 0, 1)), ((0, 1, 1), (1, 0, 1)), ((0, 0, 1), (1, 1, 1))),
    (((0, 0, 1), (0, 1, 1)), ((0, 1, 1),), ((0, 0, -1), (0, 1, 1))),
    (((1, 0, 1), (1, 1, 1)), ((1, 0, 1),), ((1, 0, 1), (1, 1, -1))),
    (((0, 0, 1), (0, 2, 1), (1, 0, -1)), ((0, 2, 1), (2, 0, 1)), ((0, 0, 1), (1, 0, 1), (1, 2, -1))),
    (((0, 0, 1), (0, 2, 1)), ((0, 2, 1),), ((0, 0, -1), (0, 2, 1), (1, 0, -1), (1, 2, 1))),
    (((0, 0, 1), (0, 2, 1), (1, 0, -1), (1, 2, -1)), ((2, 0, 1),), ((1, 0, -1), (1, 2, 1))),
    (((0, 3, 1),), ((3, 0, 1),), ((0, 0, 1),)),
    (((1, 3, 1),), ((3, 0, 1),), ((1, 0, 1),)),
    (((0, 0, 1),), ((0, 3, 1),), ((0, 3, 1),)),
    (((1, 0, 1),), ((0, 3, 1),), ((1, 3, 1),)),
    (((1, 1, 1), (1, 2, 1), (0, 1, -1)), ((1, 2, 1), (2, 1, 1)), ((0, 1, 1), (0, 2, -1), (1, 1, 1))),
    (((1, 1, 1), (1, 2, 1)), ((1, 2, 1),), ((0, 1, -1), (0, 2, 1), (1, 1, -1), (1, 2, 1))),
    (((1, 1, 1), (1, 2, 1), (0, 1, -1), (0, 2, -1)), ((2, 1, 1),), ((0, 1, -1), (0, 2, 1))),
    (((0, 1, 1), (1, 3, 1)), ((1, 3, 1), (3, 1, 1)), ((0, 3, 1), (1, 1, 1))),
    (((1, 1, 1), (1, 3, 1)), ((1, 3, 1),), ((1, 1, -1), (1, 3, 1))),
    (((0, 1, 1), (0, 3, 1)), ((3, 1, 1),), ((0, 1, 1), (0, 3, -1))),
    (((0, 2, 1), (0, 3, 1), (1, 3, -1)), ((2, 3, 1), (3, 2, 1)), ((0, 3, 1), (1, 2, -1), (1, 3, 1))),
    (((0, 2, 1), (0, 3, 1), (1, 3, -1), (1, 2, -1)), ((2, 3, 1),), ((1, 2, 1), (1, 3, -1))),
    (((0, 2, 1), (0, 3, 1)), ((3, 2, 1),), ((0, 2, 1), (0, 3, -1), (1, 2, 1), (1, 3, -1))),
)
HKSUM = tuple(r for r, t in enumerate(HK) if len(t[1]) > 1)
HKCOL = tuple(sorted(range(len(HK)), key=lambda r: min(n for _, n, _ in HK[r][2])))
HKBLK = (7, 17, 22, 24, 25, 26, 6, 16, 21, 23, 5, 11, 12, 13, 19, 4, 18, 20, 2, 9, 3, 8, 10, 1, 15, 0, 14)
HKL = tuple(dict.fromkeys(t[0] for t in HK))
TS = FF // 2

T1_ROW = 3 * NP * 2 * T0
T2_ROW = T1_ROW + len(HKSUM) * TS
LT_ROWS = T2_ROW + len(HKSUM) * TS + 16

H2_SLOT = len(HKL) * 2 * HB

SEM_W, SEM_A, SEM_M, SEM_MISC, SEM_OUT = 0, 48, 56, 64, 72
SEM_N = SEM_OUT + S // FB


def _make_sched(h1=24, n1=1, n2=4):
    out = []

    def pairs(a):
        return tuple(p for p in (a, a + 1) if 0 <= p < NP)

    nxt = 0
    for p in range(NP):
        out.append(("proj", p))
        if p >= 2 and p % 2 == 0:
            out.append(("attn", pairs(nxt - 2), pairs(nxt)))
            nxt += 2
    out += [("wo", j, 0, h1) for j in range(n1)]
    out.append(("attn", pairs(nxt - 2), pairs(nxt)))
    out += [("wo", j, 0, h1) for j in range(n1, n2)]
    out.append(("attn", pairs(nxt), ()))
    out += [("wo", j, 0, h1) for j in range(n2, 8)]
    out += [("wo", j, h1, H) for j in range(8)]
    return out


SCHED = _make_sched()
_SCOPES = False


def _scope(name):
    return jax.named_scope(name) if _SCOPES else contextlib.nullcontext()


def _dot(a, b):
    return jnp.dot(a, b, preferred_element_type=F32)


def _bf(x):
    return pltpu.bitcast(x, BF16)


def _ld(ref, idx, r0, n):
    return _bf(ref.at[(*idx, pl.ds(r0, n), slice(None))].bitcast(U32)[...])


def _ln(x):
    m = jnp.mean(x, axis=-1, keepdims=True)
    xc = x - m
    v = jnp.mean(xc * xc, axis=-1, keepdims=True)
    return xc * lax.rsqrt(v + EPS)


def _gelu(x):
    c = 0.7978845608028654
    hx = 0.5 * x
    return hx + hx * jnp.tanh(x * (c + (c * 0.044715) * (x * x)))


def _strassen_lhs(a11, a12, a21, a22):
    return [a11 + a22, a21 + a22, a11, a22, a11 + a12, a21 - a11, a12 - a22]


def _strassen_rhs(b11, b12, b21, b22):
    return [b11 + b22, b11, b12 - b22, b21 - b11, b22, b11 + b12, b21 + b22]


def _strassen_out(m):
    return (m[0] + m[3] - m[4] + m[6], m[2] + m[4], m[1] + m[3], m[0] - m[1] + m[2] + m[5])


def _comb(terms, blocks, memo=None):
    memo = {} if memo is None else memo
    for n in range(1, len(terms) + 1):
        key = terms[:n]
        if key not in memo:
            i, j, sg = terms[n - 1]
            b = blocks[i, j]
            memo[key] = b if n == 1 else (memo[terms[:n - 1]] + b if sg > 0 else memo[terms[:n - 1]] - b)
    return memo[terms]


def _interleave(a, b):
    n = a.shape[0] // 8
    parts = []
    for g in range(n):
        parts.append(a[8 * g:8 * g + 8])
        parts.append(b[8 * g:8 * g + 8])
    return jnp.concatenate(parts, axis=0)


def _deinterleave(v):
    n = v.shape[0] // 16
    a = jnp.concatenate([v[16 * g:16 * g + 8] for g in range(n)], axis=0)
    b = jnp.concatenate([v[16 * g + 8:16 * g + 16] for g in range(n)], axis=0)
    return a, b


def _kernel(x_hbm, mem0_hbm, wq_hbm, wk_hbm, wv_hbm, wo_hbm, w1_hbm, b1_hbm, w2_hbm, b2_hbm,
            c_hbm, wmod_hbm, out_hbm,
            x_v, h_v, hn_v, h2_v, x1_v, wmod_v, mod_v, sc_v, w_v, wo_v, w1_v, w2_v,
            lt_v, fr_v, lo_v, pr_v, fill_v, bias_v, n_v,
            mem0_ref, b1_ref, b2_ref, c_ref, hs_v, so_v, ev_v, st_v,
            sems):
    w32 = [r.bitcast(U32) for r in (wq_hbm, wk_hbm, wv_hbm)]

    def w_copies(p, js=range(3)):
        return [pltpu.make_async_copy(w32[j].at[:, par, p, :], w_v.at[p * 6 + j * 2 + par],
                                      sems.at[SEM_W + 3 * p + j]) for j in js for par in range(2)]

    def w_wait(u):
        both = w_v.at[pl.ds(2 * u, 2)]
        pltpu.make_async_copy(both, both, sems.at[SEM_W + u]).wait()

    def _mult(i, m):
        return i * m if isinstance(i, int) else pl.multiple_of(i * m, m)

    def wa_copies(k, units=range(UA)):
        r = pl.ds(_mult(k, 64), 64)
        return [pltpu.make_async_copy(w32[u % 3].at[r, par, u // 3, :], w_v.at[2 * u + par, r], sems.at[SEM_A + k])
                for u in units for par in range(2)]

    def m_copies(k):
        return [pltpu.make_async_copy(wmod_hbm.at[:, pl.ds(_mult(k + 8 * t, 128), 128)], wmod_v.at[16 + k + 8 * t],
                                      sems.at[SEM_M + k]) for t in range(2)]

    def start(cps):
        for cp in cps:
            cp.start()

    def wait(cps):
        for cp in cps:
            cp.wait()

    cp_x0 = pltpu.make_async_copy(x_hbm.at[:, 0], x_v.at[3 * NSEG:4 * NSEG], sems.at[SEM_MISC + 1])

    def x_pairs(s0, s1):
        return [(x_hbm.at[s0:s1, g + 1], x_v.at[g * NSEG + s0:g * NSEG + s1]) for g in range(3)]

    def wo_copy(j):
        return pltpu.make_async_copy(wo_hbm.at[:, pl.ds(_mult(j, 128), 128)], wo_v.at[j], sems.at[SEM_MISC + 3])

    def late_copies(first):
        sem = sems.at[SEM_MISC + (4 if first else 5)]
        cps = x_pairs(1, 2 * NEARLY + 1) if first else x_pairs(2 * NEARLY + 1, NSEG)
        cps += [(wmod_hbm.at[:, (16 + j) * 128:(17 + j) * 128], wmod_v.at[j])
                for j in (range(NEARLY) if first else range(NEARLY, 32))]
        for src, dst, nt, nr in ((w1_hbm, w1_v, FF // 128, D), (w2_hbm, w2_v, D // 128, 512)):
            for j in range(nt):
                if j < 4:
                    rows = slice(0, nr) if first else slice(nr, src.shape[0])
                else:
                    rows = slice(0, 0) if first else slice(0, src.shape[0])
                if rows.stop > rows.start:
                    cps.append((src.at[rows, j * 128:(j + 1) * 128], dst.at[j, rows]))
        return [pltpu.make_async_copy(src, dst, sem) for src, dst in cps]

    cp_small = [pltpu.make_async_copy(src, dst, sems.at[SEM_MISC])
                for src, dst in [(c_hbm, c_ref), (mem0_hbm, mem0_ref), (b1_hbm, b1_ref), (b2_hbm, b2_ref)]
                + x_pairs(0, 1)]

    start(cp_small)
    cp_x0.start()
    start(m_copies(0))
    for k in range(2):
        start(m_copies(k + 1))
        start(wa_copies(k))

    scale = DH ** -0.5
    ri = lax.broadcasted_iota(jnp.int32, (80, 128), 0)
    ci = lax.broadcasted_iota(jnp.int32, (80, 128), 1)
    same_head = (((ri >> 3) & 1) == ((ci >> 3) & 1)) & (ci < 80)
    rpos = (((ri >> 4) & 3) << 3) + (ri & 7)
    cpos = (((ci >> 4) & 3) << 3) + (ci & 7)
    keep = (ri < 16) | (ci < 16) | (rpos >= cpos)
    fill_v[...] = jnp.where(same_head, jnp.where(keep, 0.0, -1e9 / scale), -jnp.inf).astype(F32)

    wait(cp_small)
    c = c_ref[...].astype(F32)
    sc = jnp.broadcast_to(c * jax.nn.sigmoid(c), (8, D)).astype(BF16)

    sc_v[...] = sc
    for k in range(8):
        st_v[k * 128:(k + 1) * 128, :] = jnp.broadcast_to(sc[0:1, k * 128:(k + 1) * 128].astype(F32), (128, 128)).T
    bias_v[:, 0:FF] = b1_ref[...].astype(F32).reshape(1, FF)
    bias_v[:, FF:FF + D] = b2_ref[...].astype(F32).reshape(1, D)

    def zero_body(i, carry):
        x1_v[pl.ds(pl.multiple_of(i * 64, 64), 64), :] = jnp.zeros((64, D), F32)
        return carry

    lax.fori_loop(0, -(-UA // 4) * 8, zero_body, 0)

    def relayout(c, rows):
        a = w_v[c, rows, :]
        b = w_v[c + 1, rows, :]
        lo = (a & jnp.uint32(0xFFFF)) | (b << 16)
        hi = (a >> 16) | (b & jnp.uint32(0xFFFF0000))
        w_v[c, rows, :] = lo
        w_v[c + 1, rows, :] = hi
        return _bf(lo), _bf(hi)

    def store_lead(u, a, b):
        lt_v[pl.ds(_mult(u, 2 * T0), 2 * T0), :] = _interleave(a, b).astype(BF16)

    def mod_tile(ct):
        m = _dot(sc_v[...], _ld(wmod_v, (16 + ct,), 0, D))
        mod_v[:, pl.ds(_mult(ct, 128), 128)] = m
        return m[0:1]

    with _scope("wait_x0"):
        cp_x0.wait()

    def ln1_body(i, carry):
        r = pl.multiple_of(i * 128, 128)
        n = _ln(x_v[pl.ds(3 * NSEG + i * 16, 16)].astype(F32).reshape(128, D))
        for k in range(8):
            n_v[k, pl.ds(r, 128), :] = n[:, k * 128:(k + 1) * 128]
        return carry

    with _scope("ln1"):
        lax.fori_loop(0, T0 // 128, ln1_body, 0)
    start(m_copies(3))
    start(wa_copies(2))
    with _scope("wait_m0"):
        wait(m_copies(0))
    h_v[0] = (n_v[0] * (1.0 + mod_tile(8)) + mod_tile(0)).astype(BF16)

    def sa_body(k, carry):
        with _scope("wait_a"):
            wait(wa_copies(k))

            @pl.when(k < 7)
            def _():
                wait(m_copies(k + 1))

        kn = jnp.minimum(k + 1, 7)
        rows = pl.ds(pl.multiple_of(k * 64, 64), 64)
        hk = _ld(h_v, (k,), 0, T0)
        for u in range(UA):
            res = []
            for t, w in enumerate(relayout(2 * u, rows)):
                c = 2 * u + t
                acc = x1_v.at[c // 8 * T0:(c // 8 + 1) * T0, c % 8 * 128:(c % 8 + 1) * 128]
                r = _dot(hk, w) + acc[...]
                acc[...] = r
                res.append(r)
            store_lead(u, *res)
            if u == 1:
                sh = mod_tile(kn)
            if u == 3:
                s1 = 1.0 + mod_tile(kn + 8)

                @pl.when(k + 4 < 8)
                def _():
                    start(m_copies(k + 4))

            if u >= 4 and u % 2 == 0:
                @pl.when(k + 3 < 8)
                def _():
                    start(wa_copies(k + 3, range((u - 4) * 2, (u - 4) * 2 + 4)))

        h_v[kn] = (n_v[kn] * s1 + sh).astype(BF16)

        @pl.when(k == 4)
        def _():
            start(w_copies(UA // 3, range(UA % 3, 3)))

        @pl.when(k >= 4)
        def _():
            start(w_copies(UA // 3 + 1 + k - 4))

        return carry

    with _scope("stageA"):
        lax.fori_loop(0, 8, sa_body, 0)

    def ln1(seg):
        xb = jnp.concatenate([x_v[g * NSEG + seg].astype(F32) for g in range(3)], axis=0)
        return _ln(xb) * (1.0 + mod_v[0:1, D:2 * D]) + mod_v[0:1, 0:D]

    def hs_body(t, carry):
        for r in range(0, TH, 32):
            ss = _strassen_lhs(*[_ld(h_v, (t + 4 * b,), a * TH + r, 32).astype(F32)
                                 for a in range(2) for b in range(2)])
            for k, i in enumerate(SSUM):
                hs_v[k, t, r:r + 32, :] = ss[i].astype(BF16)
        return carry

    lax.fori_loop(0, 4, hs_body, 0)

    def lhs1(i):
        if i == 2:
            tiles = [_ld(h_v, (t,), 0, TH) for t in range(4)]
        elif i == 3:
            tiles = [_ld(h_v, (t + 4,), TH, TH) for t in range(4)]
        else:
            tiles = [_ld(hs_v, (SSUM.index(i), t), 0, TH) for t in range(4)]
        return jnp.concatenate(tiles, axis=1)

    NP1 = (3 * NP - UA) // P1N
    late = late_copies(False)
    nl = -(-len(late) // P1N)
    PW = UA // 3 + 5

    def p1_body(i, carry):
        u0 = UA + P1N * i
        with _scope("wait_w"):
            for q in range(P1N):
                w_wait(u0 + q)

        for q in range(P1N):
            lo, hi = relayout(2 * (u0 + q), slice(None))
            b = [lo[0:DH2], hi[0:DH2], lo[DH2:D], hi[DH2:D]]
            t = _strassen_rhs(*[x.astype(F32) for x in b])
            t = [b[0] if k == 1 else b[3] if k == 4 else t[k].astype(BF16) for k in range(7)]
            c = _strassen_out({k: _dot(lhs1(k), t[k]) for k in SORD})
            store_lead(u0 + q, jnp.concatenate([c[0], c[2]], axis=0), jnp.concatenate([c[1], c[3]], axis=0))

            if q < 3:
                @pl.when(PW + 3 * i + q < NP)
                def _():
                    start(w_copies(PW + 3 * i + q))
            elif q == 3:
                @pl.when(jnp.logical_and(i >= 2, i < 4))
                def _():
                    start([wo_copy(4 * (i - 2) + r) for r in range(4)])
            elif q == 4:
                @pl.when(i == 3)
                def _():
                    start(late_copies(True))

            @pl.when(i == NP1 - 1)
            def _():
                start(late[q * nl:(q + 1) * nl])

        hn_v[...] = ln1(0)
        return carry

    with _scope("phase1"):
        lax.fori_loop(0, NP1, p1_body, 0)

    with _scope("wait_wo"):
        wait([wo_copy(j) for j in range(8)])
        wait(late_copies(True))

    def prep_views(odd, pc):
        f = pc >> 2
        if odd:
            q, half = (pc >> 1) & 1, pc & 1
            kb, w, tile0, r0 = 128, w2_v, 4 * q, 512 * f + 64 * half
            d0 = T2_ROW + q * (FF // 4) + 128 * f + 64 * half
        else:
            kb, w, tile0, r0 = 256, w1_v, 4 * f, 64 * (pc & 3)
            d0 = T1_ROW + 64 * pc
        src = w.at[pl.ds(tile0, 4), pl.ds(pl.multiple_of(r0, 64), 3 * kb + 64), :]
        dst = lt_v.at[pl.ds(pl.multiple_of(d0, 64), (len(HKSUM) - 1) * TS + 64), :]
        return src, dst, kb

    def prep(views, piece):
        src, dst, kb = views
        r0 = (piece // 2) * 16
        sel = HKSUM[:6] if piece % 2 == 0 else HKSUM[6:]
        need = sorted({(k, n) for r in sel for k, n, _ in HK[r][1]})
        blocks = {(k, n): _ld(src, (n,), k * kb + r0, 16).astype(F32) for k, n in need}
        for r in sel:
            o = HKSUM.index(r) * TS + r0
            dst[o:o + 16, :] = _comb(HK[r][1], blocks).astype(BF16)

    def step(it, odd, mem, macc):
        s = 2 * it + int(odd)
        lead = lt_v.at[pl.ds(pl.multiple_of(16 * s, 16), T1_ROW), :]
        lhs = jnp.concatenate([mem, hn_v[...]], axis=0).astype(BF16)
        hn_v[...] = ln1(jnp.minimum(s + 1, NSEG - 1))

        def proj(p):
            if p == 0:
                half = [_dot(lhs[:, 0:D // 2], _bf(w_v[c, 0:D // 4, :])) for c in range(6)]
                cols = [_dot(lhs[:, D // 2:D], _bf(w_v[c, D // 4:D // 2, :])) + half[c] for c in range(6)]
            for j in range(3):
                if p == 0:
                    r = _interleave(cols[j * 2], cols[j * 2 + 1])
                else:
                    r = _interleave(_dot(lhs, _bf(w_v[p * 6 + j * 2])), _dot(lhs, _bf(w_v[p * 6 + j * 2 + 1])))
                fr_v[p * 3 + j] = r.astype(BF16)

        def stack(p, j):
            return jnp.concatenate([fr_v[p * 3 + j],
                                    _ld(lead, (), (p * 3 + j) * 2 * T0, 16)], axis=0)

        def attn(pvs, qks):
            os_ = [_dot(pr_v[p, :, 0:80], stack(p, 2)) for p in pvs]
            ss = [lax.dot_general(stack(p, 0), stack(p, 1), (((1,), (1,)), ((), ())),
                                  preferred_element_type=F32) for p in qks]
            for p, o in zip(pvs, os_):
                for t, oh in enumerate(_deinterleave(o[0:64])):
                    lo_v[2 * p + t] = oh.astype(BF16)
                if odd:
                    ev = ev_v[p]
                    for k, sk in enumerate(_strassen_lhs(ev[0:8], ev[8:16], o[64:72], o[72:80])):
                        so_v[k, p, pl.ds(pl.multiple_of(8 * it, 8), 8), :] = sk.astype(BF16)
                else:
                    ev_v[p] = o[64:80]
            for p, sc_ in zip(qks, ss):
                fill = fill_v[...]
                sc_ = jnp.concatenate([sc_, jnp.zeros((80, 48), F32)], axis=1)
                sc_ = jnp.where(fill == 0.0, sc_, fill)
                mx = jnp.max(sc_, axis=-1, keepdims=True)
                e = jnp.exp2((sc_ - mx) * (scale * LOG2E))
                l = jnp.sum(e, axis=-1, keepdims=True)
                r = pl.reciprocal(l, approx=True)
                pr_v[p] = (e * (r * (2.0 - l * r))).astype(BF16)

        part = {}

        def wo(j, h0, h1):
            lo = jnp.concatenate([lo_v[h] for h in range(h0, h1)], axis=1)
            r = _dot(lo, _ld(wo_v, (j,), h0 * DH, (h1 - h0) * DH))
            part[j] = r + part[j] if j in part else r

        pc = jnp.maximum(it - NEARLY, 0)
        views = prep_views(odd, pc)
        npiece = 0
        for op in SCHED:
            if op[0] == "proj":
                proj(op[1])
            elif op[0] == "attn":
                attn(op[1], op[2])
                if npiece < 8:
                    prep(views, npiece)
                    k0 = (8 * int(odd) + npiece) * 64
                    pr = _ld(wmod_v, (it,), k0, 64).astype(F32) * st_v[k0:k0 + 64, :]
                    for g in range(8):
                        macc = pr[8 * g:8 * g + 8] if macc is None else macc + pr[8 * g:8 * g + 8]
                    lt_v[LT_ROWS - 16:LT_ROWS, :] = _bf(macc)
                    npiece += 1
            else:
                wo(*op[1:])
        res = jnp.concatenate([part[j] for j in range(8)], axis=1)
        for g in range(3):
            x1_v[pl.ds(pl.multiple_of(g * T0 + 8 * s, 8), 8), :] = res[8 * g + 8:8 * g + 16]
        return res[0:8], macc

    with _scope("main"):
        def steps(i, mem):
            @pl.when(i == NEARLY)
            def _():
                wait(late)

            with _scope("iter"):
                mem, macc = step(i, True, *step(i, False, mem, None))
                mod_v[0:1, pl.ds(pl.multiple_of((16 + i) * 128, 128), 128)] = jnp.sum(macc, axis=0, keepdims=True)

            return mem

        lax.fori_loop(0, NSEG // 2, steps, mem0_ref[...].astype(F32))

    def resid1(r, k0, n, c0=0, nc=D):
        xb = x_v[pl.ds((r >> 3) + k0 // 8, n // 8), :, c0:c0 + nc].astype(F32).reshape(n, nc)
        return xb + mod_v[0:1, 2 * D + c0:2 * D + c0 + nc] * x1_v[pl.ds(r + k0, n), c0:c0 + nc]

    def h2_view(slot, k0=0):
        r = slot * H2_SLOT + k0
        return h2_v.at[pl.ds(pl.multiple_of(r, LNP), H2_SLOT - HB + (HB if isinstance(k0, int) else LNP)), :]

    def ln2(dst, r, k0):
        hm = [_ln(resid1(r, k0 + m * HB, LNP)) * (1.0 + mod_v[0:1, 4 * D:5 * D])
              + mod_v[0:1, 3 * D:4 * D] for m in range(2)]
        for j in range(2):
            blocks = {(m, k): hm[m][:, k * 256 + j * 128:k * 256 + (j + 1) * 128]
                      for m in range(2) for k in range(4)}
            memo = {}
            for i, terms in enumerate(HKL):
                o = (2 * i + j) * HB + k0
                dst[o:o + LNP, :] = _comb(terms, blocks, memo).astype(BF16)

    def wo_body(j, carry):
        acc = {}
        for kc in range(4):
            b = [jnp.concatenate([_ld(wo_v, (j + 4 * n,), (2 * p + t) * DH, DH)
                                  for p in range(4 * kc, 4 * kc + 4)], axis=0)
                 for t in range(2) for n in range(2)]
            tt = _strassen_rhs(*[x.astype(F32) for x in b])
            tt = [b[0] if k == 1 else b[3] if k == 4 else tt[k].astype(BF16) for k in range(7)]
            for k in SORD:
                sk = jnp.concatenate([_ld(so_v, (k, p), 0, TH) for p in range(4 * kc, 4 * kc + 4)], axis=1)
                y = _dot(sk, tt[k])
                acc[k] = y + acc[k] if kc else y
        for e in range(2):
            k0 = (2 * j + e) * LNP
            ln2(h2_view(0, k0), pl.multiple_of(k0, LNP), 0)
        for t, c in enumerate(_strassen_out(acc)):
            cs = pl.ds(pl.multiple_of((j + 4 * (t % 2)) * 128, 128), 128)
            for g in range(NSEG // 2):
                r0 = 3 * T0 + (2 * g + t // 2) * 8
                x1_v[r0:r0 + 8, cs] = c[8 * g:8 * g + 8]
        return carry

    with _scope("p3a"):
        lax.fori_loop(0, 4, wo_body, 0)

    def out_copy(i, q):
        cols = pl.ds(q * 256, 256)
        return pltpu.make_async_copy(x_v.at[pl.ds(i * (FB // 8), FB // 8), :, cols],
                                     out_hbm.at[pl.ds((i & 1) * (FB // 8), FB // 8), ((i >> 1) + 1) & 3, :, cols],
                                     sems.at[SEM_OUT + i])

    def ffn_body(i, carry):
        r0 = pl.multiple_of(i * FB, FB)
        rn = pl.multiple_of(jnp.minimum(r0 + FB, S - FB), FB)
        h2_cur, h2_nxt = h2_view(i & 1), h2_view(1 - (i & 1))
        acc = {}
        act = {}
        memo = {}

        def accumulate(key, r, y):
            key = (HK[r][2], key)
            acc[key] = y + acc[key] if key in acc else y

        def collect(key, m, n, order):
            c = None
            for pat in dict.fromkeys(HK[r][2] for r in order):
                for mm, nn, sg in pat:
                    if (mm, nn) == (m, n):
                        y = acc[pat, key]
                        c = (y if sg > 0 else -y) if c is None else (c + y if sg > 0 else c - y)
            return c

        def up(f, lo, hi):
            for idx in range(lo, hi):
                r = HKBLK[idx]
                lhs = jnp.concatenate([_ld(h2_cur, (), (2 * HKL.index(HK[r][0]) + j) * HB, HB) for j in range(2)], axis=1)
                if r in HKSUM:
                    w = _ld(lt_v, (), T1_ROW + HKSUM.index(r) * TS + 256 * f, 256)
                else:
                    k, n, _ = HK[r][1][0]
                    w = _ld(w1_v, (4 * f + n,), 256 * k, 256)
                accumulate(("up", f), r, _dot(lhs, w))
                for m, n, _ in HK[r][2]:
                    if not any((m, n) == t[0:2] for rr in HKBLK[idx + 1:] for t in HK[rr][2]):
                        c0 = (4 * f + n) * 128
                        act.setdefault(f, {})[m, n] = _gelu(
                            collect(("up", f), m, n, HKBLK) + bias_v[0:1, c0:c0 + 128])

        def down(fs, q, r):
            if (fs, HK[r][0]) not in memo:
                memo[fs, HK[r][0]] = jnp.concatenate(
                    [_comb(HK[r][0], act[f], memo.setdefault(f, {})) for f in fs], axis=1).astype(BF16)
            if r in HKSUM:
                w = _ld(lt_v, (), T2_ROW + HKSUM.index(r) * TS + q * (FF // 4) + 128 * fs[0], 128 * len(fs))
            else:
                k, n, _ = HK[r][1][0]
                w = jnp.concatenate([_ld(w2_v, (4 * q + n,), 512 * f + 128 * k, 128) for f in fs], axis=0)
            accumulate(q, r, _dot(memo[fs, HK[r][0]], w))

        def finish(q, n):
            c0 = (4 * q + n) * 128
            for m in range(2):
                y = (collect(q, m, n, HKCOL) + bias_v[0:1, FF + c0:FF + c0 + 128]) * mod_v[0:1, 5 * D + c0:5 * D + c0 + 128]
                o = (resid1(r0, m * HB, HB, c0, 128) + y).reshape(HB // 8, 8, 128).astype(BF16)
                x_v[pl.ds((r0 >> 3) + m * (HB // 8), HB // 8), :, c0:c0 + 128] = o
            if n % 2:
                out_copy(i, 2 * q + n // 2).start()

        work = [(fs, q, r) for fs in ((0, 1), (2, 3), (4, 5)) for r in range(len(HK)) for q in range(2)]
        piece = 0
        for f in range(FF // 512):
            for lo, hi in ((0, 14), (14, len(HK))):
                up(f, lo, hi)
                ready = [x for x in work[:14] if x[0][-1] < f]
                if ready and piece * LNP < HB:
                    ln2(h2_nxt, rn, piece * LNP)
                    piece += 1
                for x in ready:
                    down(*x)
                work = work[len(ready):]
        assert piece * LNP == HB
        for x in work:
            down(*x)
        for q in range(2):
            for idx, r in enumerate(HKCOL):
                down((6,), q, r)
                for n in range(4):
                    if idx == max(j for j, rr in enumerate(HKCOL) if any(t[1] == n for t in HK[rr][2])):
                        finish(q, n)
        return carry

    with _scope("ffn"):
        lax.fori_loop(0, S // FB, ffn_body, 0)
    with _scope("wait_out"):
        for i in range(S // FB):
            for q in range(4):
                out_copy(i, q).wait()


@jax.jit
def pallas_adaLN_cond__memory_aug_recurrent_mem_tr__dense_activation_gelu__prompt_kernel(
    A_x, A_mem0, A_Wq, A_Wk, A_Wv, A_Wo, A_seg_len, B_x, B_w1, B_b1, B_w2, B_b2, c, w_mod,
):
    del A_seg_len, B_x
    assert A_x.shape == (1, S, D)
    hbm = pl.BlockSpec(memory_space=pl.ANY)
    out = pl.pallas_call(
        _kernel,
        out_shape=jax.ShapeDtypeStruct((NSEG, 4, 8, D), BF16),
        in_specs=[hbm] * 12,
        out_specs=hbm,
        scratch_shapes=[
            pltpu.VMEM((4 * NSEG, 8, D), BF16),
            pltpu.VMEM((8, T0, 128), BF16),
            pltpu.VMEM((TPS, D), F32),
            pltpu.VMEM((2 * H2_SLOT, 128), BF16),
            pltpu.VMEM((S, D), F32),
            pltpu.VMEM((32, D, 128), BF16),
            pltpu.VMEM((8, 6 * D), F32),
            pltpu.VMEM((8, D), BF16),
            pltpu.VMEM((6 * NP, D // 2, 128), U32),
            pltpu.VMEM((8, H * DH, 128), BF16),
            pltpu.VMEM((FF // 128, D, 128), BF16),
            pltpu.VMEM((D // 128, FF, 128), BF16),
            pltpu.VMEM((LT_ROWS, 128), BF16),
            pltpu.VMEM((3 * NP, 64, 128), BF16),
            pltpu.VMEM((H, 32, 128), BF16),
            pltpu.VMEM((NP, 80, 128), BF16),
            pltpu.VMEM((80, 128), F32),
            pltpu.VMEM((1, FF + D), F32),
            pltpu.VMEM((8, T0, 128), F32),
            pltpu.VMEM((M, D), BF16),
            pltpu.VMEM((FF,), BF16),
            pltpu.VMEM((D,), BF16),
            pltpu.VMEM((1, D), BF16),
            pltpu.VMEM((5, 4, T0 // 2, 128), BF16),
            pltpu.VMEM((7, NP, T0 // 2, 128), BF16),
            pltpu.VMEM((NP, 16, 128), F32),
            pltpu.VMEM((D, 128), F32),
            pltpu.SemaphoreType.DMA((SEM_N,)),
        ],
        compiler_params=pltpu.CompilerParams(vmem_limit_bytes=122 * 1024 * 1024, disable_bounds_checks=True,
                                             disable_semaphore_checks=True),
    )(
        A_x.reshape(NSEG, 4, 8, D), A_mem0.reshape(M, D),
        A_Wq.reshape(D // 2, 2, H, DH), A_Wk.reshape(D // 2, 2, H, DH), A_Wv.reshape(D // 2, 2, H, DH),
        A_Wo.reshape(H * DH, D), B_w1, B_b1, B_w2, B_b2, c, w_mod,
    )
    return out.reshape(1, S, D)
```

```python
import contextlib

import jax
import jax.numpy as jnp
from jax import lax
import jax.experimental.pallas as pl
import jax.experimental.pallas.tpu as pltpu

F32 = jnp.float32
BF16 = jnp.bfloat16
U32 = jnp.uint32

S = 2048
D = 1024
H = 32
DH = 128
M = 8
SEG = 32
FF = 3584
EPS = 1e-5
LOG2E = 1.4426950408889634

NSEG = S // SEG
NP = H // 2
TPS = SEG - 8
T0 = 8 * NSEG
TH = T0 // 2
DH2 = D // 2
UA = 8
P1N = 4
NEARLY = 4
FB = 256
HB = FB // 2
LNP = 16

SORD = (1, 4, 3, 2, 0, 6, 5)

HK = (
    (((0, 0, 1), (1, 0, -1)), ((0, 0, 1), (0, 1, 1), (2, 0, -1)), ((0, 0, 1),)),
    (((1, 0, 1),), ((0, 0, 1), (0, 2, 1), (1, 0, -1)), ((0, 0, 1), (1, 0, 1))),
    (((0, 1, 1),), ((1, 1, 1), (1, 2, 1), (0, 1, -1), (3, 1, -1)), ((0, 1, 1), (1, 1, 1))),
    (((1, 1, 1), (0, 1, -1)), ((1, 0, 1), (1, 1, 1), (1, 3, 1), (2, 1, -1)), ((1, 1, 1),)),
    (((0, 2, 1),), ((2, 1, 1), (2, 2, 1), (0, 2, -1), (3, 2, -1)), ((0, 2, 1),)),
    (((1, 2, 1),), ((2, 0, 1), (2, 2, 1), (2, 3, 1), (1, 2, -1)), ((1, 2, 1),)),
    (((0, 3, 1), (1, 3, -1)), ((3, 1, 1), (3, 3, 1), (2, 3, -1)), ((0, 3, 1),)),
    (((1, 3, 1),), ((3, 2, 1), (3, 3, 1), (1, 3, -1)), ((0, 3, 1), (1, 3, 1))),
    (((0, 1, 1), (1, 0, 1)), ((0, 1, 1), (1, 0, 1)), ((0, 0, 1), (1, 1, 1))),
    (((0, 0, 1), (0, 1, 1)), ((0, 1, 1),), ((0, 0, -1), (0, 1, 1))),
    (((1, 0, 1), (1, 1, 1)), ((1, 0, 1),), ((1, 0, 1), (1, 1, -1))),
    (((0, 0, 1), (0, 2, 1), (1, 0, -1)), ((0, 2, 1), (2, 0, 1)), ((0, 0, 1), (1, 0, 1), (1, 2, -1))),
    (((0, 0, 1), (0, 2, 1)), ((0, 2, 1),), ((0, 0, -1), (0, 2, 1), (1, 0, -1), (1, 2, 1))),
    (((0, 0, 1), (0, 2, 1), (1, 0, -1), (1, 2, -1)), ((2, 0, 1),), ((1, 0, -1), (1, 2, 1))),
    (((0, 3, 1),), ((3, 0, 1),), ((0, 0, 1),)),
    (((1, 3, 1),), ((3, 0, 1),), ((1, 0, 1),)),
    (((0, 0, 1),), ((0, 3, 1),), ((0, 3, 1),)),
    (((1, 0, 1),), ((0, 3, 1),), ((1, 3, 1),)),
    (((1, 1, 1), (1, 2, 1), (0, 1, -1)), ((1, 2, 1), (2, 1, 1)), ((0, 1, 1), (0, 2, -1), (1, 1, 1))),
    (((1, 1, 1), (1, 2, 1)), ((1, 2, 1),), ((0, 1, -1), (0, 2, 1), (1, 1, -1), (1, 2, 1))),
    (((1, 1, 1), (1, 2, 1), (0, 1, -1), (0, 2, -1)), ((2, 1, 1),), ((0, 1, -1), (0, 2, 1))),
    (((0, 1, 1), (1, 3, 1)), ((1, 3, 1), (3, 1, 1)), ((0, 3, 1), (1, 1, 1))),
    (((1, 1, 1), (1, 3, 1)), ((1, 3, 1),), ((1, 1, -1), (1, 3, 1))),
    (((0, 1, 1), (0, 3, 1)), ((3, 1, 1),), ((0, 1, 1), (0, 3, -1))),
    (((0, 2, 1), (0, 3, 1), (1, 3, -1)), ((2, 3, 1), (3, 2, 1)), ((0, 3, 1), (1, 2, -1), (1, 3, 1))),
    (((0, 2, 1), (0, 3, 1), (1, 3, -1), (1, 2, -1)), ((2, 3, 1),), ((1, 2, 1), (1, 3, -1))),
    (((0, 2, 1), (0, 3, 1)), ((3, 2, 1),), ((0, 2, 1), (0, 3, -1), (1, 2, 1), (1, 3, -1))),
)
HKSUM = tuple(r for r, t in enumerate(HK) if len(t[1]) > 1)
HKCOL = tuple(sorted(range(len(HK)), key=lambda r: min(n for _, n, _ in HK[r][2])))
HKBLK = (7, 17, 22, 24, 25, 26, 6, 16, 21, 23, 5, 11, 12, 13, 19, 4, 18, 20, 2, 9, 3, 8, 10, 1, 15, 0, 14)
HKL = tuple(dict.fromkeys(t[0] for t in HK))
HKLS = tuple(t for t in HKL if len(t) > 1)
P1ORD = (9, 10, 14, 15, 13, 12, 1, 11, 0, 8, 19, 20, 23, 2, 18, 22, 3, 21, 25, 5, 24, 17, 7, 26, 16, 6, 4)
TS = FF // 2

T1_ROW = 3 * NP * 2 * T0
T2_ROW = T1_ROW + len(HKSUM) * TS
LT_ROWS = T2_ROW + len(HKSUM) * TS + 16

H2_SLOT = len(HKL) * 2 * HB

SEM_W, SEM_A, SEM_M, SEM_MISC, SEM_OUT = 0, 48, 56, 64, 72
SEM_N = SEM_OUT + S // FB


def _make_sched(h1=24, n1=1, n2=4):
    out = []

    def pairs(a):
        return tuple(p for p in (a, a + 1) if 0 <= p < NP)

    nxt = 0
    for p in range(NP):
        out.append(("proj", p))
        if p >= 2 and p % 2 == 0:
            out.append(("attn", pairs(nxt - 2), pairs(nxt)))
            nxt += 2
    out += [("wo", j, 0, h1) for j in range(n1)]
    out.append(("attn", pairs(nxt - 2), pairs(nxt)))
    out += [("wo", j, 0, h1) for j in range(n1, n2)]
    out.append(("attn", pairs(nxt), ()))
    out += [("wo", j, 0, h1) for j in range(n2, 8)]
    out += [("wo", j, h1, H) for j in range(8)]
    return out


SCHED = _make_sched()
_SCOPES = False


def _scope(name):
    return jax.named_scope(name) if _SCOPES else contextlib.nullcontext()


def _dot(a, b):
    return jnp.dot(a, b, preferred_element_type=F32)


def _bf(x):
    return pltpu.bitcast(x, BF16)


def _ld(ref, idx, r0, n):
    return _bf(ref.at[(*idx, pl.ds(r0, n), slice(None))].bitcast(U32)[...])


def _ln(x):
    m = jnp.mean(x, axis=-1, keepdims=True)
    xc = x - m
    v = jnp.mean(xc * xc, axis=-1, keepdims=True)
    return xc * lax.rsqrt(v + EPS)


def _gelu(x):
    c = 0.7978845608028654
    hx = 0.5 * x
    return hx + hx * jnp.tanh(x * (c + (c * 0.044715) * (x * x)))


def _strassen_lhs(a11, a12, a21, a22):
    return [a11 + a22, a21 + a22, a11, a22, a11 + a12, a21 - a11, a12 - a22]


def _strassen_rhs(b11, b12, b21, b22):
    return [b11 + b22, b11, b12 - b22, b21 - b11, b22, b11 + b12, b21 + b22]


def _strassen_out(m):
    return (m[0] + m[3] - m[4] + m[6], m[2] + m[4], m[1] + m[3], m[0] - m[1] + m[2] + m[5])


def _comb(terms, blocks, memo=None):
    memo = {} if memo is None else memo
    for n in range(1, len(terms) + 1):
        key = terms[:n]
        if key not in memo:
            i, j, sg = terms[n - 1]
            b = blocks[i, j]
            memo[key] = b if n == 1 else (memo[terms[:n - 1]] + b if sg > 0 else memo[terms[:n - 1]] - b)
    return memo[terms]


def _collect(acc, m, n):
    c = None
    for pat, y in acc.items():
        for mm, nn, sg in pat:
            if (mm, nn) == (m, n):
                c = (y if sg > 0 else -y) if c is None else (c + y if sg > 0 else c - y)
    return c


def _interleave(a, b):
    n = a.shape[0] // 8
    parts = []
    for g in range(n):
        parts.append(a[8 * g:8 * g + 8])
        parts.append(b[8 * g:8 * g + 8])
    return jnp.concatenate(parts, axis=0)


def _deinterleave(v):
    n = v.shape[0] // 16
    a = jnp.concatenate([v[16 * g:16 * g + 8] for g in range(n)], axis=0)
    b = jnp.concatenate([v[16 * g + 8:16 * g + 16] for g in range(n)], axis=0)
    return a, b


def _kernel(x_hbm, mem0_hbm, wq_hbm, wk_hbm, wv_hbm, wo_hbm, w1_hbm, b1_hbm, w2_hbm, b2_hbm,
            c_hbm, wmod_hbm, out_hbm,
            x_v, h_v, hn_v, h2_v, x1_v, wmod_v, mod_v, sc_v, w_v, wo_v, w1_v, w2_v,
            lt_v, fr_v, lo_v, pr_v, fill_v, bias_v, n_v,
            mem0_ref, b1_ref, b2_ref, c_ref, hs_v, so_v, ev_v, st_v,
            sems):
    w32 = [r.bitcast(U32) for r in (wq_hbm, wk_hbm, wv_hbm)]

    def w_copies(p, js=range(3)):
        return [pltpu.make_async_copy(w32[j].at[:, par, p, :], w_v.at[p * 6 + j * 2 + par],
                                      sems.at[SEM_W + 3 * p + j]) for j in js for par in range(2)]

    def w_wait(u):
        both = w_v.at[pl.ds(2 * u, 2)]
        pltpu.make_async_copy(both, both, sems.at[SEM_W + u]).wait()

    def _mult(i, m):
        return i * m if isinstance(i, int) else pl.multiple_of(i * m, m)

    def wa_copies(k, units=range(UA)):
        r = pl.ds(_mult(k, 64), 64)
        return [pltpu.make_async_copy(w32[u % 3].at[r, par, u // 3, :], w_v.at[2 * u + par, r], sems.at[SEM_A + k])
                for u in units for par in range(2)]

    def m_copies(k):
        return [pltpu.make_async_copy(wmod_hbm.at[:, pl.ds(_mult(k + 8 * t, 128), 128)], wmod_v.at[16 + k + 8 * t],
                                      sems.at[SEM_M + k]) for t in range(2)]

    def start(cps):
        for cp in cps:
            cp.start()

    def wait(cps):
        for cp in cps:
            cp.wait()

    cp_x0 = pltpu.make_async_copy(x_hbm.at[:, 0], x_v.at[3 * NSEG:4 * NSEG], sems.at[SEM_MISC + 1])

    def x_pairs(s0, s1):
        return [(x_hbm.at[s0:s1, g + 1], x_v.at[g * NSEG + s0:g * NSEG + s1]) for g in range(3)]

    def wo_copy(j):
        return pltpu.make_async_copy(wo_hbm.at[:, pl.ds(_mult(j, 128), 128)], wo_v.at[j], sems.at[SEM_MISC + 3])

    def late_copies(first):
        sem = sems.at[SEM_MISC + (4 if first else 5)]
        cps = x_pairs(1, 2 * NEARLY + 1) if first else x_pairs(2 * NEARLY + 1, NSEG)
        cps += [(wmod_hbm.at[:, (16 + j) * 128:(17 + j) * 128], wmod_v.at[j])
                for j in (range(NEARLY) if first else range(NEARLY, 32))]
        for src, dst, nt, nr in ((w1_hbm, w1_v, FF // 128, D), (w2_hbm, w2_v, D // 128, 512)):
            for j in range(nt):
                if j < 4:
                    rows = slice(0, nr) if first else slice(nr, src.shape[0])
                else:
                    rows = slice(0, 0) if first else slice(0, src.shape[0])
                if rows.stop > rows.start:
                    cps.append((src.at[rows, j * 128:(j + 1) * 128], dst.at[j, rows]))
        return [pltpu.make_async_copy(src, dst, sem) for src, dst in cps]

    cp_small = [pltpu.make_async_copy(src, dst, sems.at[SEM_MISC])
                for src, dst in [(c_hbm, c_ref), (mem0_hbm, mem0_ref), (b1_hbm, b1_ref), (b2_hbm, b2_ref)]
                + x_pairs(0, 1)]

    start(cp_small)
    cp_x0.start()
    start(m_copies(0))
    for k in range(2):
        start(m_copies(k + 1))
        start(wa_copies(k))

    scale = DH ** -0.5
    ri = lax.broadcasted_iota(jnp.int32, (80, 128), 0)
    ci = lax.broadcasted_iota(jnp.int32, (80, 128), 1)
    same_head = (((ri >> 3) & 1) == ((ci >> 3) & 1)) & (ci < 80)
    rpos = (((ri >> 4) & 3) << 3) + (ri & 7)
    cpos = (((ci >> 4) & 3) << 3) + (ci & 7)
    keep = (ri < 16) | (ci < 16) | (rpos >= cpos)
    fill_v[...] = jnp.where(same_head, jnp.where(keep, 0.0, -1e9 / scale), -jnp.inf).astype(F32)

    wait(cp_small)
    c = c_ref[...].astype(F32)
    sc = jnp.broadcast_to(c * jax.nn.sigmoid(c), (8, D)).astype(BF16)

    sc_v[...] = sc
    for k in range(8):
        st_v[k * 128:(k + 1) * 128, :] = jnp.broadcast_to(sc[0:1, k * 128:(k + 1) * 128].astype(F32), (128, 128)).T
    bias_v[:, 0:FF] = b1_ref[...].astype(F32).reshape(1, FF)
    bias_v[:, FF:FF + D] = b2_ref[...].astype(F32).reshape(1, D)

    def zero_body(i, carry):
        x1_v[pl.ds(pl.multiple_of(i * 64, 64), 64), :] = jnp.zeros((64, D), F32)
        return carry

    lax.fori_loop(0, -(-UA // 4) * 8, zero_body, 0)

    def relayout(c, rows):
        a = w_v[c, rows, :]
        b = w_v[c + 1, rows, :]
        lo = (a & jnp.uint32(0xFFFF)) | (b << 16)
        hi = (a >> 16) | (b & jnp.uint32(0xFFFF0000))
        w_v[c, rows, :] = lo
        w_v[c + 1, rows, :] = hi
        return _bf(lo), _bf(hi)

    def store_lead(u, a, b):
        lt_v[pl.ds(_mult(u, 2 * T0), 2 * T0), :] = _interleave(a, b).astype(BF16)

    def mod_tile(ct):
        m = _dot(sc_v[...], _ld(wmod_v, (16 + ct,), 0, D))
        mod_v[:, pl.ds(_mult(ct, 128), 128)] = m
        return m[0:1]

    with _scope("wait_x0"):
        cp_x0.wait()

    def ln1_body(i, carry):
        r = pl.multiple_of(i * 128, 128)
        n = _ln(x_v[pl.ds(3 * NSEG + i * 16, 16)].astype(F32).reshape(128, D))
        for k in range(8):
            n_v[k, pl.ds(r, 128), :] = n[:, k * 128:(k + 1) * 128]
        return carry

    with _scope("ln1"):
        lax.fori_loop(0, T0 // 128, ln1_body, 0)
    start(m_copies(3))
    start(wa_copies(2))
    with _scope("wait_m0"):
        wait(m_copies(0))
    h_v[0] = (n_v[0] * (1.0 + mod_tile(8)) + mod_tile(0)).astype(BF16)

    def sa_body(k, carry):
        with _scope("wait_a"):
            wait(wa_copies(k))

            @pl.when(k < 7)
            def _():
                wait(m_copies(k + 1))

        kn = jnp.minimum(k + 1, 7)
        rows = pl.ds(pl.multiple_of(k * 64, 64), 64)
        hk = _ld(h_v, (k,), 0, T0)
        for u in range(UA):
            res = []
            for t, w in enumerate(relayout(2 * u, rows)):
                c = 2 * u + t
                acc = x1_v.at[c // 8 * T0:(c // 8 + 1) * T0, c % 8 * 128:(c % 8 + 1) * 128]
                r = _dot(hk, w) + acc[...]
                acc[...] = r
                res.append(r)
            store_lead(u, *res)
            if u == 1:
                sh = mod_tile(kn)
            if u == 3:
                s1 = 1.0 + mod_tile(kn + 8)

                @pl.when(k + 4 < 8)
                def _():
                    start(m_copies(k + 4))

            if u >= 4 and u % 2 == 0:
                @pl.when(k + 3 < 8)
                def _():
                    start(wa_copies(k + 3, range((u - 4) * 2, (u - 4) * 2 + 4)))

        h_v[kn] = (n_v[kn] * s1 + sh).astype(BF16)

        @pl.when(k == 4)
        def _():
            start(w_copies(UA // 3, range(UA % 3, 3)))

        @pl.when(k >= 4)
        def _():
            start(w_copies(UA // 3 + 1 + k - 4))

        return carry

    with _scope("stageA"):
        lax.fori_loop(0, 8, sa_body, 0)

    def ln1(seg):
        xb = jnp.concatenate([x_v[g * NSEG + seg].astype(F32) for g in range(3)], axis=0)
        return _ln(xb) * (1.0 + mod_v[0:1, D:2 * D]) + mod_v[0:1, 0:D]

    def hs_body(t, carry):
        j, r = t & 1, pl.multiple_of((t >> 1) * 64, 64)
        src = h_v.at[pl.ds(j, 7), pl.ds(r, TH + 64), :]
        dst = hs_v.at[:, j, pl.ds(r, 64), :]
        for r0 in range(0, 64, 16):
            blocks = {(m, k): _ld(src, (2 * k,), m * TH + r0, 16).astype(F32) for m in range(2) for k in range(4)}
            memo = {}
            for i, terms in enumerate(HKLS):
                dst[i, r0:r0 + 16, :] = _comb(terms, blocks, memo).astype(BF16)
        return carry

    lax.fori_loop(0, 8, hs_body, 0)

    def lhs1(terms):
        if len(terms) == 1:
            m, k, _ = terms[0]
            tiles = [_ld(h_v, (2 * k + j,), m * TH, TH) for j in range(2)]
        else:
            tiles = [_ld(hs_v, (HKLS.index(terms), j), 0, TH) for j in range(2)]
        return jnp.concatenate(tiles, axis=1)

    NP1 = (3 * NP - UA) // P1N
    late = late_copies(False)
    nl = -(-len(late) // 6)
    PW = UA // 3 + 5

    def p1_body(i, carry):
        u0 = UA + P1N * i
        with _scope("wait_w"):
            for q in range(P1N):
                w_wait(u0 + q)

        def dma_slot(q):
            if q < 2:
                @pl.when(PW + 2 * i + q < NP)
                def _():
                    start(w_copies(PW + 2 * i + q))
            elif q == 2:
                @pl.when(jnp.logical_and(i >= 3, i < 7))
                def _():
                    start([wo_copy(2 * (i - 3) + r) for r in range(2)])
            elif q == 3:
                @pl.when(i == 6)
                def _():
                    start(late_copies(True))

            @pl.when(i == NP1 - 1)
            def _():
                start(late[q * nl:(q + 1) * nl])

        for g in range(P1N // 2):
            u = u0 + 2 * g
            tiles = relayout(2 * u, slice(None)) + relayout(2 * u + 2, slice(None))
            b = {(k, n): tiles[n][256 * k:256 * (k + 1)] for k in range(4) for n in range(4)}
            bf = {key: x.astype(F32) for key, x in b.items()}
            acc = {}
            for idx, r in enumerate(P1ORD):
                terms = HK[r][1]
                w = b[terms[0][0:2]] if len(terms) == 1 else _comb(terms, bf).astype(BF16)
                y = _dot(lhs1(HK[r][0]), w)
                acc[HK[r][2]] = y + acc[HK[r][2]] if HK[r][2] in acc else y
                if idx % 9 == 8:
                    dma_slot(3 * g + idx // 9)
            c = {(m, n): _collect(acc, m, n) for m in range(2) for n in range(4)}
            col = [jnp.concatenate([c[0, n], c[1, n]], axis=0) for n in range(4)]
            store_lead(u, col[0], col[1])
            store_lead(u + 1, col[2], col[3])

        hn_v[...] = ln1(0)
        return carry

    with _scope("phase1"):
        lax.fori_loop(0, NP1, p1_body, 0)

    with _scope("wait_wo"):
        wait([wo_copy(j) for j in range(8)])
        wait(late_copies(True))

    def prep_views(odd, pc):
        f = pc >> 2
        if odd:
            q, half = (pc >> 1) & 1, pc & 1
            kb, w, tile0, r0 = 128, w2_v, 4 * q, 512 * f + 64 * half
            d0 = T2_ROW + q * (FF // 4) + 128 * f + 64 * half
        else:
            kb, w, tile0, r0 = 256, w1_v, 4 * f, 64 * (pc & 3)
            d0 = T1_ROW + 64 * pc
        src = w.at[pl.ds(tile0, 4), pl.ds(pl.multiple_of(r0, 64), 3 * kb + 64), :]
        dst = lt_v.at[pl.ds(pl.multiple_of(d0, 64), (len(HKSUM) - 1) * TS + 64), :]
        return src, dst, kb

    def prep(views, piece):
        src, dst, kb = views
        r0 = (piece // 2) * 16
        sel = HKSUM[:6] if piece % 2 == 0 else HKSUM[6:]
        need = sorted({(k, n) for r in sel for k, n, _ in HK[r][1]})
        blocks = {(k, n): _ld(src, (n,), k * kb + r0, 16).astype(F32) for k, n in need}
        for r in sel:
            o = HKSUM.index(r) * TS + r0
            dst[o:o + 16, :] = _comb(HK[r][1], blocks).astype(BF16)

    def step(it, odd, mem, macc):
        s = 2 * it + int(odd)
        lead = lt_v.at[pl.ds(pl.multiple_of(16 * s, 16), T1_ROW), :]
        lhs = jnp.concatenate([mem, hn_v[...]], axis=0).astype(BF16)
        hn_v[...] = ln1(jnp.minimum(s + 1, NSEG - 1))

        def proj(p):
            if p == 0:
                half = [_dot(lhs[:, 0:D // 2], _bf(w_v[c, 0:D // 4, :])) for c in range(6)]
                cols = [_dot(lhs[:, D // 2:D], _bf(w_v[c, D // 4:D // 2, :])) + half[c] for c in range(6)]
            for j in range(3):
                if p == 0:
                    r = _interleave(cols[j * 2], cols[j * 2 + 1])
                else:
                    r = _interleave(_dot(lhs, _bf(w_v[p * 6 + j * 2])), _dot(lhs, _bf(w_v[p * 6 + j * 2 + 1])))
                fr_v[p * 3 + j] = r.astype(BF16)

        def stack(p, j):
            return jnp.concatenate([fr_v[p * 3 + j],
                                    _ld(lead, (), (p * 3 + j) * 2 * T0, 16)], axis=0)

        def attn(pvs, qks):
            os_ = [_dot(pr_v[p, :, 0:80], stack(p, 2)) for p in pvs]
            ss = [lax.dot_general(stack(p, 0), stack(p, 1), (((1,), (1,)), ((), ())),
                                  preferred_element_type=F32) for p in qks]
            for p, o in zip(pvs, os_):
                for t, oh in enumerate(_deinterleave(o[0:64])):
                    lo_v[2 * p + t] = oh.astype(BF16)
                if odd:
                    ev = ev_v[p]
                    for k, sk in enumerate(_strassen_lhs(ev[0:8], ev[8:16], o[64:72], o[72:80])):
                        so_v[k, p, pl.ds(pl.multiple_of(8 * it, 8), 8), :] = sk.astype(BF16)
                else:
                    ev_v[p] = o[64:80]
            for p, sc_ in zip(qks, ss):
                fill = fill_v[...]
                sc_ = jnp.concatenate([sc_, jnp.zeros((80, 48), F32)], axis=1)
                sc_ = jnp.where(fill == 0.0, sc_, fill)
                mx = jnp.max(sc_, axis=-1, keepdims=True)
                e = jnp.exp2((sc_ - mx) * (scale * LOG2E))
                l = jnp.sum(e, axis=-1, keepdims=True)
                r = pl.reciprocal(l, approx=True)
                pr_v[p] = (e * (r * (2.0 - l * r))).astype(BF16)

        part = {}

        def wo(j, h0, h1):
            lo = jnp.concatenate([lo_v[h] for h in range(h0, h1)], axis=1)
            r = _dot(lo, _ld(wo_v, (j,), h0 * DH, (h1 - h0) * DH))
            part[j] = r + part[j] if j in part else r

        pc = jnp.maximum(it - NEARLY, 0)
        views = prep_views(odd, pc)
        npiece = 0
        for op in SCHED:
            if op[0] == "proj":
                proj(op[1])
            elif op[0] == "attn":
                attn(op[1], op[2])
                if npiece < 8:
                    prep(views, npiece)
                    k0 = (8 * int(odd) + npiece) * 64
                    pr = _ld(wmod_v, (it,), k0, 64).astype(F32) * st_v[k0:k0 + 64, :]
                    for g in range(8):
                        macc = pr[8 * g:8 * g + 8] if macc is None else macc + pr[8 * g:8 * g + 8]
                    lt_v[LT_ROWS - 16:LT_ROWS, :] = _bf(macc)
                    npiece += 1
            else:
                wo(*op[1:])
        res = jnp.concatenate([part[j] for j in range(8)], axis=1)
        for g in range(3):
            x1_v[pl.ds(pl.multiple_of(g * T0 + 8 * s, 8), 8), :] = res[8 * g + 8:8 * g + 16]
        return res[0:8], macc

    with _scope("main"):
        def steps(i, mem):
            @pl.when(i == NEARLY)
            def _():
                wait(late)

            with _scope("iter"):
                mem, macc = step(i, True, *step(i, False, mem, None))
                mod_v[0:1, pl.ds(pl.multiple_of((16 + i) * 128, 128), 128)] = jnp.sum(macc, axis=0, keepdims=True)

            return mem

        lax.fori_loop(0, NSEG // 2, steps, mem0_ref[...].astype(F32))

    def resid1(r, k0, n, c0=0, nc=D):
        xb = x_v[pl.ds((r >> 3) + k0 // 8, n // 8), :, c0:c0 + nc].astype(F32).reshape(n, nc)
        return xb + mod_v[0:1, 2 * D + c0:2 * D + c0 + nc] * x1_v[pl.ds(r + k0, n), c0:c0 + nc]

    def h2_view(slot, k0=0):
        r = slot * H2_SLOT + k0
        return h2_v.at[pl.ds(pl.multiple_of(r, LNP), H2_SLOT - HB + (HB if isinstance(k0, int) else LNP)), :]

    def ln2(dst, r, k0):
        hm = [_ln(resid1(r, k0 + m * HB, LNP)) * (1.0 + mod_v[0:1, 4 * D:5 * D])
              + mod_v[0:1, 3 * D:4 * D] for m in range(2)]
        for j in range(2):
            blocks = {(m, k): hm[m][:, k * 256 + j * 128:k * 256 + (j + 1) * 128]
                      for m in range(2) for k in range(4)}
            memo = {}
            for i, terms in enumerate(HKL):
                o = (2 * i + j) * HB + k0
                dst[o:o + LNP, :] = _comb(terms, blocks, memo).astype(BF16)

    def wo_body(j, carry):
        acc = {}
        for kc in range(4):
            b = [jnp.concatenate([_ld(wo_v, (j + 4 * n,), (2 * p + t) * DH, DH)
                                  for p in range(4 * kc, 4 * kc + 4)], axis=0)
                 for t in range(2) for n in range(2)]
            tt = _strassen_rhs(*[x.astype(F32) for x in b])
            tt = [b[0] if k == 1 else b[3] if k == 4 else tt[k].astype(BF16) for k in range(7)]
            for k in SORD:
                sk = jnp.concatenate([_ld(so_v, (k, p), 0, TH) for p in range(4 * kc, 4 * kc + 4)], axis=1)
                y = _dot(sk, tt[k])
                acc[k] = y + acc[k] if kc else y
        for e in range(2):
            k0 = (2 * j + e) * LNP
            ln2(h2_view(0, k0), pl.multiple_of(k0, LNP), 0)
        for t, c in enumerate(_strassen_out(acc)):
            cs = pl.ds(pl.multiple_of((j + 4 * (t % 2)) * 128, 128), 128)
            for g in range(NSEG // 2):
                r0 = 3 * T0 + (2 * g + t // 2) * 8
                x1_v[r0:r0 + 8, cs] = c[8 * g:8 * g + 8]
        return carry

    with _scope("p3a"):
        lax.fori_loop(0, 4, wo_body, 0)

    def out_copy(i, q):
        cols = pl.ds(q * 256, 256)
        return pltpu.make_async_copy(x_v.at[pl.ds(i * (FB // 8), FB // 8), :, cols],
                                     out_hbm.at[pl.ds((i & 1) * (FB // 8), FB // 8), ((i >> 1) + 1) & 3, :, cols],
                                     sems.at[SEM_OUT + i])

    def ffn_body(i, carry):
        r0 = pl.multiple_of(i * FB, FB)
        rn = pl.multiple_of(jnp.minimum(r0 + FB, S - FB), FB)
        h2_cur, h2_nxt = h2_view(i & 1), h2_view(1 - (i & 1))
        acc = {}
        act = {}
        memo = {}

        def accumulate(key, r, y):
            a = acc.setdefault(key, {})
            a[HK[r][2]] = y + a[HK[r][2]] if HK[r][2] in a else y

        def up(f, lo, hi):
            for idx in range(lo, hi):
                r = HKBLK[idx]
                lhs = jnp.concatenate([_ld(h2_cur, (), (2 * HKL.index(HK[r][0]) + j) * HB, HB) for j in range(2)], axis=1)
                if r in HKSUM:
                    w = _ld(lt_v, (), T1_ROW + HKSUM.index(r) * TS + 256 * f, 256)
                else:
                    k, n, _ = HK[r][1][0]
                    w = _ld(w1_v, (4 * f + n,), 256 * k, 256)
                accumulate(("up", f), r, _dot(lhs, w))
                for m, n, _ in HK[r][2]:
                    if not any((m, n) == t[0:2] for rr in HKBLK[idx + 1:] for t in HK[rr][2]):
                        c0 = (4 * f + n) * 128
                        act.setdefault(f, {})[m, n] = _gelu(
                            _collect(acc["up", f], m, n) + bias_v[0:1, c0:c0 + 128])

        def down(fs, q, r):
            if (fs, HK[r][0]) not in memo:
                memo[fs, HK[r][0]] = jnp.concatenate(
                    [_comb(HK[r][0], act[f], memo.setdefault(f, {})) for f in fs], axis=1).astype(BF16)
            if r in HKSUM:
                w = _ld(lt_v, (), T2_ROW + HKSUM.index(r) * TS + q * (FF // 4) + 128 * fs[0], 128 * len(fs))
            else:
                k, n, _ = HK[r][1][0]
                w = jnp.concatenate([_ld(w2_v, (4 * q + n,), 512 * f + 128 * k, 128) for f in fs], axis=0)
            accumulate(q, r, _dot(memo[fs, HK[r][0]], w))

        def finish(q, n):
            c0 = (4 * q + n) * 128
            for m in range(2):
                y = (_collect({HK[r][2]: acc[q][HK[r][2]] for r in HKCOL}, m, n) + bias_v[0:1, FF + c0:FF + c0 + 128]) * mod_v[0:1, 5 * D + c0:5 * D + c0 + 128]
                o = (resid1(r0, m * HB, HB, c0, 128) + y).reshape(HB // 8, 8, 128).astype(BF16)
                x_v[pl.ds((r0 >> 3) + m * (HB // 8), HB // 8), :, c0:c0 + 128] = o
            if n % 2:
                out_copy(i, 2 * q + n // 2).start()

        work = [(fs, q, r) for fs in ((0, 1), (2, 3), (4, 5)) for r in range(len(HK)) for q in range(2)]
        piece = 0
        for f in range(FF // 512):
            for lo, hi in ((0, 14), (14, len(HK))):
                up(f, lo, hi)
                ready = [x for x in work[:14] if x[0][-1] < f]
                if ready and piece * LNP < HB:
                    ln2(h2_nxt, rn, piece * LNP)
                    piece += 1
                for x in ready:
                    down(*x)
                work = work[len(ready):]
        assert piece * LNP == HB
        for x in work:
            down(*x)
        for q in range(2):
            for idx, r in enumerate(HKCOL):
                down((6,), q, r)
                for n in range(4):
                    if idx == max(j for j, rr in enumerate(HKCOL) if any(t[1] == n for t in HK[rr][2])):
                        finish(q, n)
        return carry

    with _scope("ffn"):
        lax.fori_loop(0, S // FB, ffn_body, 0)
    with _scope("wait_out"):
        for i in range(S // FB):
            for q in range(4):
                out_copy(i, q).wait()


@jax.jit
def pallas_adaLN_cond__memory_aug_recurrent_mem_tr__dense_activation_gelu__prompt_kernel(
    A_x, A_mem0, A_Wq, A_Wk, A_Wv, A_Wo, A_seg_len, B_x, B_w1, B_b1, B_w2, B_b2, c, w_mod,
):
    del A_seg_len, B_x
    assert A_x.shape == (1, S, D)
    hbm = pl.BlockSpec(memory_space=pl.ANY)
    out = pl.pallas_call(
        _kernel,
        out_shape=jax.ShapeDtypeStruct((NSEG, 4, 8, D), BF16),
        in_specs=[hbm] * 12,
        out_specs=hbm,
        scratch_shapes=[
            pltpu.VMEM((4 * NSEG, 8, D), BF16),
            pltpu.VMEM((8, T0, 128), BF16),
            pltpu.VMEM((TPS, D), F32),
            pltpu.VMEM((2 * H2_SLOT, 128), BF16),
            pltpu.VMEM((S, D), F32),
            pltpu.VMEM((32, D, 128), BF16),
            pltpu.VMEM((8, 6 * D), F32),
            pltpu.VMEM((8, D), BF16),
            pltpu.VMEM((6 * NP, D // 2, 128), U32),
            pltpu.VMEM((8, H * DH, 128), BF16),
            pltpu.VMEM((FF // 128, D, 128), BF16),
            pltpu.VMEM((D // 128, FF, 128), BF16),
            pltpu.VMEM((LT_ROWS, 128), BF16),
            pltpu.VMEM((3 * NP, 64, 128), BF16),
            pltpu.VMEM((H, 32, 128), BF16),
            pltpu.VMEM((NP, 80, 128), BF16),
            pltpu.VMEM((80, 128), F32),
            pltpu.VMEM((1, FF + D), F32),
            pltpu.VMEM((8, T0, 128), F32),
            pltpu.VMEM((M, D), BF16),
            pltpu.VMEM((FF,), BF16),
            pltpu.VMEM((D,), BF16),
            pltpu.VMEM((1, D), BF16),
            pltpu.VMEM((len(HKLS), 2, TH, 128), BF16),
            pltpu.VMEM((7, NP, T0 // 2, 128), BF16),
            pltpu.VMEM((NP, 16, 128), F32),
            pltpu.VMEM((D, 128), F32),
            pltpu.SemaphoreType.DMA((SEM_N,)),
        ],
        compiler_params=pltpu.CompilerParams(vmem_limit_bytes=122 * 1024 * 1024, disable_bounds_checks=True,
                                             disable_semaphore_checks=True),
    )(
        A_x.reshape(NSEG, 4, 8, D), A_mem0.reshape(M, D),
        A_Wq.reshape(D // 2, 2, H, DH), A_Wk.reshape(D // 2, 2, H, DH), A_Wv.reshape(D // 2, 2, H, DH),
        A_Wo.reshape(H * DH, D), B_w1, B_b1, B_w2, B_b2, c, w_mod,
    )
    return out.reshape(1, S, D)
```

```python
import contextlib

import jax
import jax.numpy as jnp
from jax import lax
import jax.experimental.pallas as pl
import jax.experimental.pallas.tpu as pltpu

F32 = jnp.float32
BF16 = jnp.bfloat16
U32 = jnp.uint32

S = 2048
D = 1024
H = 32
DH = 128
M = 8
SEG = 32
FF = 3584
EPS = 1e-5
LOG2E = 1.4426950408889634

NSEG = S // SEG
NP = H // 2
TPS = SEG - 8
T0 = 8 * NSEG
TH = T0 // 2
DH2 = D // 2
UA = 8
P1N = 4
NEARLY = 4
FB = 256
HB = FB // 2
MROWS = (0, 336, 688, 1024)
LNP = 16

SORD = (1, 4, 3, 2, 0, 6, 5)

HK = (
    (((0, 0, 1), (1, 0, -1)), ((0, 0, 1), (0, 1, 1), (2, 0, -1)), ((0, 0, 1),)),
    (((1, 0, 1),), ((0, 0, 1), (0, 2, 1), (1, 0, -1)), ((0, 0, 1), (1, 0, 1))),
    (((0, 1, 1),), ((1, 1, 1), (1, 2, 1), (0, 1, -1), (3, 1, -1)), ((0, 1, 1), (1, 1, 1))),
    (((1, 1, 1), (0, 1, -1)), ((1, 0, 1), (1, 1, 1), (1, 3, 1), (2, 1, -1)), ((1, 1, 1),)),
    (((0, 2, 1),), ((2, 1, 1), (2, 2, 1), (0, 2, -1), (3, 2, -1)), ((0, 2, 1),)),
    (((1, 2, 1),), ((2, 0, 1), (2, 2, 1), (2, 3, 1), (1, 2, -1)), ((1, 2, 1),)),
    (((0, 3, 1), (1, 3, -1)), ((3, 1, 1), (3, 3, 1), (2, 3, -1)), ((0, 3, 1),)),
    (((1, 3, 1),), ((3, 2, 1), (3, 3, 1), (1, 3, -1)), ((0, 3, 1), (1, 3, 1))),
    (((0, 1, 1), (1, 0, 1)), ((0, 1, 1), (1, 0, 1)), ((0, 0, 1), (1, 1, 1))),
    (((0, 0, 1), (0, 1, 1)), ((0, 1, 1),), ((0, 0, -1), (0, 1, 1))),
    (((1, 0, 1), (1, 1, 1)), ((1, 0, 1),), ((1, 0, 1), (1, 1, -1))),
    (((0, 0, 1), (0, 2, 1), (1, 0, -1)), ((0, 2, 1), (2, 0, 1)), ((0, 0, 1), (1, 0, 1), (1, 2, -1))),
    (((0, 0, 1), (0, 2, 1)), ((0, 2, 1),), ((0, 0, -1), (0, 2, 1), (1, 0, -1), (1, 2, 1))),
    (((0, 0, 1), (0, 2, 1), (1, 0, -1), (1, 2, -1)), ((2, 0, 1),), ((1, 0, -1), (1, 2, 1))),
    (((0, 3, 1),), ((3, 0, 1),), ((0, 0, 1),)),
    (((1, 3, 1),), ((3, 0, 1),), ((1, 0, 1),)),
    (((0, 0, 1),), ((0, 3, 1),), ((0, 3, 1),)),
    (((1, 0, 1),), ((0, 3, 1),), ((1, 3, 1),)),
    (((1, 1, 1), (1, 2, 1), (0, 1, -1)), ((1, 2, 1), (2, 1, 1)), ((0, 1, 1), (0, 2, -1), (1, 1, 1))),
    (((1, 1, 1), (1, 2, 1)), ((1, 2, 1),), ((0, 1, -1), (0, 2, 1), (1, 1, -1), (1, 2, 1))),
    (((1, 1, 1), (1, 2, 1), (0, 1, -1), (0, 2, -1)), ((2, 1, 1),), ((0, 1, -1), (0, 2, 1))),
    (((0, 1, 1), (1, 3, 1)), ((1, 3, 1), (3, 1, 1)), ((0, 3, 1), (1, 1, 1))),
    (((1, 1, 1), (1, 3, 1)), ((1, 3, 1),), ((1, 1, -1), (1, 3, 1))),
    (((0, 1, 1), (0, 3, 1)), ((3, 1, 1),), ((0, 1, 1), (0, 3, -1))),
    (((0, 2, 1), (0, 3, 1), (1, 3, -1)), ((2, 3, 1), (3, 2, 1)), ((0, 3, 1), (1, 2, -1), (1, 3, 1))),
    (((0, 2, 1), (0, 3, 1), (1, 3, -1), (1, 2, -1)), ((2, 3, 1),), ((1, 2, 1), (1, 3, -1))),
    (((0, 2, 1), (0, 3, 1)), ((3, 2, 1),), ((0, 2, 1), (0, 3, -1), (1, 2, 1), (1, 3, -1))),
)
HKSUM = tuple(r for r, t in enumerate(HK) if len(t[1]) > 1)
HKCOL = tuple(sorted(range(len(HK)), key=lambda r: min(n for _, n, _ in HK[r][2])))
HKBLK = (7, 17, 22, 24, 25, 26, 6, 16, 21, 23, 5, 11, 12, 13, 19, 4, 18, 20, 2, 9, 3, 8, 10, 1, 15, 0, 14)
HKL = tuple(dict.fromkeys(t[0] for t in HK))
HKLS = tuple(t for t in HKL if len(t) > 1)
P1ORD = (9, 10, 14, 15, 13, 12, 1, 11, 0, 8, 19, 20, 23, 2, 18, 22, 3, 21, 25, 5, 24, 17, 7, 26, 16, 6, 4)
TS = FF // 2

T1_ROW = 3 * NP * 2 * T0
T2_ROW = T1_ROW + len(HKSUM) * TS
LT_ROWS = T2_ROW + len(HKSUM) * TS + 16

H2_SLOT = len(HKL) * 2 * HB

SEM_W, SEM_A, SEM_M, SEM_MISC, SEM_OUT = 0, 48, 56, 64, 72
SEM_N = SEM_OUT + S // FB


def _make_sched(h1=24, n1=1, n2=4):
    out = []

    def pairs(a):
        return tuple(p for p in (a, a + 1) if 0 <= p < NP)

    nxt = 0
    for p in range(NP):
        out.append(("proj", p))
        if p >= 2 and p % 2 == 0:
            out.append(("attn", pairs(nxt - 2), pairs(nxt)))
            nxt += 2
    out += [("wo", j, 0, h1) for j in range(n1)]
    out.append(("attn", pairs(nxt - 2), pairs(nxt)))
    out += [("wo", j, 0, h1) for j in range(n1, n2)]
    out.append(("attn", pairs(nxt), ()))
    out += [("wo", j, 0, h1) for j in range(n2, 8)]
    out += [("wo", j, h1, H) for j in range(8)]
    return out


SCHED = _make_sched()
_SCOPES = False


def _scope(name):
    return jax.named_scope(name) if _SCOPES else contextlib.nullcontext()


def _dot(a, b):
    return jnp.dot(a, b, preferred_element_type=F32)


def _bf(x):
    return pltpu.bitcast(x, BF16)


def _ld(ref, idx, r0, n):
    return _bf(ref.at[(*idx, pl.ds(r0, n), slice(None))].bitcast(U32)[...])


def _ln(x):
    m = jnp.mean(x, axis=-1, keepdims=True)
    xc = x - m
    v = jnp.mean(xc * xc, axis=-1, keepdims=True)
    return xc * lax.rsqrt(v + EPS)


def _gelu(x):
    c = 0.7978845608028654
    hx = 0.5 * x
    return hx + hx * jnp.tanh(x * (c + (c * 0.044715) * (x * x)))


def _strassen_lhs(a11, a12, a21, a22):
    return [a11 + a22, a21 + a22, a11, a22, a11 + a12, a21 - a11, a12 - a22]


def _strassen_rhs(b11, b12, b21, b22):
    return [b11 + b22, b11, b12 - b22, b21 - b11, b22, b11 + b12, b21 + b22]


def _strassen_out(m):
    return (m[0] + m[3] - m[4] + m[6], m[2] + m[4], m[1] + m[3], m[0] - m[1] + m[2] + m[5])


def _comb(terms, blocks, memo=None):
    memo = {} if memo is None else memo
    for n in range(1, len(terms) + 1):
        key = terms[:n]
        if key not in memo:
            i, j, sg = terms[n - 1]
            b = blocks[i, j]
            memo[key] = b if n == 1 else (memo[terms[:n - 1]] + b if sg > 0 else memo[terms[:n - 1]] - b)
    return memo[terms]


def _collect(acc, m, n):
    c = None
    for pat, y in acc.items():
        for mm, nn, sg in pat:
            if (mm, nn) == (m, n):
                c = (y if sg > 0 else -y) if c is None else (c + y if sg > 0 else c - y)
    return c


def _interleave(a, b):
    n = a.shape[0] // 8
    parts = []
    for g in range(n):
        parts.append(a[8 * g:8 * g + 8])
        parts.append(b[8 * g:8 * g + 8])
    return jnp.concatenate(parts, axis=0)


def _deinterleave(v):
    n = v.shape[0] // 16
    a = jnp.concatenate([v[16 * g:16 * g + 8] for g in range(n)], axis=0)
    b = jnp.concatenate([v[16 * g + 8:16 * g + 16] for g in range(n)], axis=0)
    return a, b


def _kernel(x_hbm, mem0_hbm, wq_hbm, wk_hbm, wv_hbm, wo_hbm, w1_hbm, b1_hbm, w2_hbm, b2_hbm,
            c_hbm, wmod_hbm, out_hbm,
            x_v, h_v, hn_v, h2_v, x1_v, wmod_v, mod_v, sc_v, w_v, wo_v, w1_v, w2_v,
            lt_v, fr_v, lo_v, pr_v, fill_v, bias_v, n_v,
            mem0_ref, b1_ref, b2_ref, c_ref, hs_v, so_v, ev_v, st_v,
            sems):
    w32 = [r.bitcast(U32) for r in (wq_hbm, wk_hbm, wv_hbm)]

    def w_copies(p, js=range(3)):
        return [pltpu.make_async_copy(w32[j].at[:, par, p, :], w_v.at[p * 6 + j * 2 + par],
                                      sems.at[SEM_W + 3 * p + j]) for j in js for par in range(2)]

    def w_wait(u):
        both = w_v.at[pl.ds(2 * u, 2)]
        pltpu.make_async_copy(both, both, sems.at[SEM_W + u]).wait()

    def _mult(i, m):
        return i * m if isinstance(i, int) else pl.multiple_of(i * m, m)

    def wa_copies(k, units=range(UA)):
        r = pl.ds(_mult(k, 64), 64)
        return [pltpu.make_async_copy(w32[u % 3].at[r, par, u // 3, :], w_v.at[2 * u + par, r], sems.at[SEM_A + k])
                for u in units for par in range(2)]

    def m_copies(k):
        return [pltpu.make_async_copy(wmod_hbm.at[:, pl.ds(_mult(k + 8 * t, 128), 128)], wmod_v.at[16 + k + 8 * t],
                                      sems.at[SEM_M + k]) for t in range(2)]

    def start(cps):
        for cp in cps:
            cp.start()

    def wait(cps):
        for cp in cps:
            cp.wait()

    cp_x0 = pltpu.make_async_copy(x_hbm.at[:, 0], x_v.at[3 * NSEG:4 * NSEG], sems.at[SEM_MISC + 1])

    def x_pairs(s0, s1):
        return [(x_hbm.at[s0:s1, g + 1], x_v.at[g * NSEG + s0:g * NSEG + s1]) for g in range(3)]

    def wo_copy(j):
        return pltpu.make_async_copy(wo_hbm.at[:, pl.ds(_mult(j, 128), 128)], wo_v.at[j], sems.at[SEM_MISC + 3])

    def late_copies(first):
        sem = sems.at[SEM_MISC + (4 if first else 5)]
        cps = x_pairs(1, 2 * NEARLY + 1) if first else x_pairs(2 * NEARLY + 1, NSEG)
        cps += [(wmod_hbm.at[:, (16 + j) * 128:(17 + j) * 128], wmod_v.at[j])
                for j in (range(NEARLY) if first else range(NEARLY, 32))]
        for src, dst, nt, nr in ((w1_hbm, w1_v, FF // 128, D), (w2_hbm, w2_v, D // 128, 512)):
            for j in range(nt):
                if j < 4:
                    rows = slice(0, nr) if first else slice(nr, src.shape[0])
                else:
                    rows = slice(0, 0) if first else slice(0, src.shape[0])
                if rows.stop > rows.start:
                    cps.append((src.at[rows, j * 128:(j + 1) * 128], dst.at[j, rows]))
        return [pltpu.make_async_copy(src, dst, sem) for src, dst in cps]

    cp_small = [pltpu.make_async_copy(src, dst, sems.at[SEM_MISC])
                for src, dst in [(c_hbm, c_ref), (mem0_hbm, mem0_ref), (b1_hbm, b1_ref), (b2_hbm, b2_ref)]
                + x_pairs(0, 1)]

    start(cp_small)
    cp_x0.start()
    start(m_copies(0))
    for k in range(2):
        start(m_copies(k + 1))
        start(wa_copies(k))

    scale = DH ** -0.5
    ri = lax.broadcasted_iota(jnp.int32, (80, 128), 0)
    ci = lax.broadcasted_iota(jnp.int32, (80, 128), 1)
    same_head = (((ri >> 3) & 1) == ((ci >> 3) & 1)) & (ci < 80)
    rpos = (((ri >> 4) & 3) << 3) + (ri & 7)
    cpos = (((ci >> 4) & 3) << 3) + (ci & 7)
    keep = (ri < 16) | (ci < 16) | (rpos >= cpos)
    fill_v[...] = jnp.where(same_head, jnp.where(keep, 0.0, -1e9 / scale), -jnp.inf).astype(F32)

    wait(cp_small)
    c = c_ref[...].astype(F32)
    sc = jnp.broadcast_to(c * jax.nn.sigmoid(c), (8, D)).astype(BF16)

    sc_v[...] = sc
    for k in range(8):
        st_v[k * 128:(k + 1) * 128, :] = jnp.broadcast_to(sc[0:1, k * 128:(k + 1) * 128].astype(F32), (128, 128)).T
    bias_v[:, 0:FF] = b1_ref[...].astype(F32).reshape(1, FF)
    bias_v[:, FF:FF + D] = b2_ref[...].astype(F32).reshape(1, D)

    def zero_body(i, carry):
        x1_v[pl.ds(pl.multiple_of(i * 64, 64), 64), :] = jnp.zeros((64, D), F32)
        return carry

    lax.fori_loop(0, -(-UA // 4) * 8, zero_body, 0)

    def relayout(c, rows):
        a = w_v[c, rows, :]
        b = w_v[c + 1, rows, :]
        lo = (a & jnp.uint32(0xFFFF)) | (b << 16)
        hi = (a >> 16) | (b & jnp.uint32(0xFFFF0000))
        w_v[c, rows, :] = lo
        w_v[c + 1, rows, :] = hi
        return _bf(lo), _bf(hi)

    def store_lead(u, a, b):
        lt_v[pl.ds(_mult(u, 2 * T0), 2 * T0), :] = _interleave(a, b).astype(BF16)

    def mod_tile(ct):
        m = _dot(sc_v[...], _ld(wmod_v, (16 + ct,), 0, D))
        mod_v[:, pl.ds(_mult(ct, 128), 128)] = m
        return m[0:1]

    with _scope("wait_x0"):
        cp_x0.wait()

    def ln1_body(i, carry):
        r = pl.multiple_of(i * 128, 128)
        n = _ln(x_v[pl.ds(3 * NSEG + i * 16, 16)].astype(F32).reshape(128, D))
        for k in range(8):
            n_v[k, pl.ds(r, 128), :] = n[:, k * 128:(k + 1) * 128]
        return carry

    with _scope("ln1"):
        lax.fori_loop(0, T0 // 128, ln1_body, 0)
    start(m_copies(3))
    start(wa_copies(2))
    with _scope("wait_m0"):
        wait(m_copies(0))
    h_v[0] = (n_v[0] * (1.0 + mod_tile(8)) + mod_tile(0)).astype(BF16)

    def hs_piece(j, r):
        blocks = {(m, k): _ld(h_v, (2 * k + j,), m * TH + r, 16).astype(F32) for m in range(2) for k in range(4)}
        memo = {}
        for i, terms in enumerate(HKLS):
            hs_v[i, j, r:r + 16, :] = _comb(terms, blocks, memo).astype(BF16)

    def sa_body(k, carry):
        last = isinstance(k, int)
        with _scope("wait_a"):
            wait(wa_copies(k))
            if not last:
                wait(m_copies(k + 1))

        rows = pl.ds(_mult(k, 64), 64)
        hk = _ld(h_v, (k,), 0, T0)
        macc = [None, None]
        for u in range(UA):
            res = []
            for t, w in enumerate(relayout(2 * u, rows)):
                c = 2 * u + t
                acc = x1_v.at[c // 8 * T0:(c // 8 + 1) * T0, c % 8 * 128:(c % 8 + 1) * 128]
                r = _dot(hk, w) + acc[...]
                if not last:
                    acc[...] = r
                res.append(r)
            if last:
                store_lead(u, *res)
                for e in range(4 * u, 4 * u + 4):
                    hs_piece(e % 2, (e // 2) * 16)
                continue
            if u in (1, 3, 5):
                r0, nr = MROWS[u // 2], MROWS[u // 2 + 1] - MROWS[u // 2]
                sb = st_v[r0:r0 + nr, :]
                for t in range(2):
                    pr = _ld(wmod_v, (17 + k + 8 * t,), r0, nr).astype(F32) * sb
                    for g in range(nr // 8):
                        macc[t] = pr[8 * g:8 * g + 8] if macc[t] is None else macc[t] + pr[8 * g:8 * g + 8]
                    w_v[6 * NP, 8 * t:8 * t + 8, :] = pltpu.bitcast(macc[t], U32)
            if u == 5:
                sh, sc1 = [jnp.sum(m_, axis=0, keepdims=True) for m_ in macc]
                mod_v[0:1, pl.ds(_mult(k + 1, 128), 128)] = sh
                mod_v[0:1, pl.ds(_mult(k + 9, 128), 128)] = sc1
            if u == 6:
                @pl.when(k + 4 < 8)
                def _():
                    start(m_copies(k + 4))

            if u >= 4 and u % 2 == 0:
                @pl.when(k + 3 < 8)
                def _():
                    start(wa_copies(k + 3, range((u - 4) * 2, (u - 4) * 2 + 4)))

        if last:
            start(w_copies(UA // 3 + 4))
            return carry
        h_v[k + 1] = (n_v[k + 1] * (1.0 + sc1) + sh).astype(BF16)

        @pl.when(k == 4)
        def _():
            start(w_copies(UA // 3, range(UA % 3, 3)))

        @pl.when(k >= 4)
        def _():
            start(w_copies(UA // 3 + 1 + k - 4))

        return carry

    with _scope("stageA"):
        lax.fori_loop(0, 7, sa_body, 0)
        sa_body(7, 0)

    def ln1(seg):
        xb = jnp.concatenate([x_v[g * NSEG + seg].astype(F32) for g in range(3)], axis=0)
        return _ln(xb) * (1.0 + mod_v[0:1, D:2 * D]) + mod_v[0:1, 0:D]

    def lhs1(terms):
        if len(terms) == 1:
            m, k, _ = terms[0]
            tiles = [_ld(h_v, (2 * k + j,), m * TH, TH) for j in range(2)]
        else:
            tiles = [_ld(hs_v, (HKLS.index(terms), j), 0, TH) for j in range(2)]
        return jnp.concatenate(tiles, axis=1)

    NP1 = (3 * NP - UA) // P1N
    late = late_copies(False)
    nl = -(-len(late) // 6)
    PW = UA // 3 + 5

    def p1_body(i, carry):
        u0 = UA + P1N * i
        with _scope("wait_w"):
            for q in range(P1N):
                w_wait(u0 + q)

        def dma_slot(q):
            if q < 2:
                @pl.when(PW + 2 * i + q < NP)
                def _():
                    start(w_copies(PW + 2 * i + q))
            elif q == 2:
                @pl.when(jnp.logical_and(i >= 3, i < 7))
                def _():
                    start([wo_copy(2 * (i - 3) + r) for r in range(2)])
            elif q == 3:
                @pl.when(i == 6)
                def _():
                    start(late_copies(True))

            @pl.when(i == NP1 - 1)
            def _():
                start(late[q * nl:(q + 1) * nl])

        for g in range(P1N // 2):
            u = u0 + 2 * g
            tiles = relayout(2 * u, slice(None)) + relayout(2 * u + 2, slice(None))
            b = {(k, n): tiles[n][256 * k:256 * (k + 1)] for k in range(4) for n in range(4)}
            bf = {key: x.astype(F32) for key, x in b.items()}
            acc = {}
            for idx, r in enumerate(P1ORD):
                terms = HK[r][1]
                w = b[terms[0][0:2]] if len(terms) == 1 else _comb(terms, bf).astype(BF16)
                y = _dot(lhs1(HK[r][0]), w)
                acc[HK[r][2]] = y + acc[HK[r][2]] if HK[r][2] in acc else y
                if idx % 9 == 8:
                    dma_slot(3 * g + idx // 9)
            c = {(m, n): _collect(acc, m, n) for m in range(2) for n in range(4)}
            col = [jnp.concatenate([c[0, n], c[1, n]], axis=0) for n in range(4)]
            store_lead(u, col[0], col[1])
            store_lead(u + 1, col[2], col[3])

        hn_v[...] = ln1(0)
        return carry

    with _scope("phase1"):
        lax.fori_loop(0, NP1, p1_body, 0)

    with _scope("wait_wo"):
        wait([wo_copy(j) for j in range(8)])
        wait(late_copies(True))

    def prep_views(odd, pc):
        f = pc >> 2
        if odd:
            q, half = (pc >> 1) & 1, pc & 1
            kb, w, tile0, r0 = 128, w2_v, 4 * q, 512 * f + 64 * half
            d0 = T2_ROW + q * (FF // 4) + 128 * f + 64 * half
        else:
            kb, w, tile0, r0 = 256, w1_v, 4 * f, 64 * (pc & 3)
            d0 = T1_ROW + 64 * pc
        src = w.at[pl.ds(tile0, 4), pl.ds(pl.multiple_of(r0, 64), 3 * kb + 64), :]
        dst = lt_v.at[pl.ds(pl.multiple_of(d0, 64), (len(HKSUM) - 1) * TS + 64), :]
        return src, dst, kb

    def prep(views, piece):
        src, dst, kb = views
        r0 = (piece // 2) * 16
        sel = HKSUM[:6] if piece % 2 == 0 else HKSUM[6:]
        need = sorted({(k, n) for r in sel for k, n, _ in HK[r][1]})
        blocks = {(k, n): _ld(src, (n,), k * kb + r0, 16).astype(F32) for k, n in need}
        for r in sel:
            o = HKSUM.index(r) * TS + r0
            dst[o:o + 16, :] = _comb(HK[r][1], blocks).astype(BF16)

    def step(it, odd, mem, macc):
        s = 2 * it + int(odd)
        lead = lt_v.at[pl.ds(pl.multiple_of(16 * s, 16), T1_ROW), :]
        lhs = jnp.concatenate([mem, hn_v[...]], axis=0).astype(BF16)
        hn_v[...] = ln1(jnp.minimum(s + 1, NSEG - 1))

        def proj(p):
            if p == 0:
                half = [_dot(lhs[:, 0:D // 2], _bf(w_v[c, 0:D // 4, :])) for c in range(6)]
                cols = [_dot(lhs[:, D // 2:D], _bf(w_v[c, D // 4:D // 2, :])) + half[c] for c in range(6)]
            for j in range(3):
                if p == 0:
                    r = _interleave(cols[j * 2], cols[j * 2 + 1])
                else:
                    r = _interleave(_dot(lhs, _bf(w_v[p * 6 + j * 2])), _dot(lhs, _bf(w_v[p * 6 + j * 2 + 1])))
                fr_v[p * 3 + j] = r.astype(BF16)

        def stack(p, j):
            return jnp.concatenate([fr_v[p * 3 + j],
                                    _ld(lead, (), (p * 3 + j) * 2 * T0, 16)], axis=0)

        def attn(pvs, qks):
            os_ = [_dot(pr_v[p, :, 0:80], stack(p, 2)) for p in pvs]
            ss = [lax.dot_general(stack(p, 0), stack(p, 1), (((1,), (1,)), ((), ())),
                                  preferred_element_type=F32) for p in qks]
            for p, o in zip(pvs, os_):
                for t, oh in enumerate(_deinterleave(o[0:64])):
                    lo_v[2 * p + t] = oh.astype(BF16)
                if odd:
                    ev = ev_v[p]
                    for k, sk in enumerate(_strassen_lhs(ev[0:8], ev[8:16], o[64:72], o[72:80])):
                        so_v[k, p, pl.ds(pl.multiple_of(8 * it, 8), 8), :] = sk.astype(BF16)
                else:
                    ev_v[p] = o[64:80]
            for p, sc_ in zip(qks, ss):
                fill = fill_v[...]
                sc_ = jnp.concatenate([sc_, jnp.zeros((80, 48), F32)], axis=1)
                sc_ = jnp.where(fill == 0.0, sc_, fill)
                mx = jnp.max(sc_, axis=-1, keepdims=True)
                e = jnp.exp2((sc_ - mx) * (scale * LOG2E))
                l = jnp.sum(e, axis=-1, keepdims=True)
                r = pl.reciprocal(l, approx=True)
                pr_v[p] = (e * (r * (2.0 - l * r))).astype(BF16)

        part = {}

        def wo(j, h0, h1):
            lo = jnp.concatenate([lo_v[h] for h in range(h0, h1)], axis=1)
            r = _dot(lo, _ld(wo_v, (j,), h0 * DH, (h1 - h0) * DH))
            part[j] = r + part[j] if j in part else r

        pc = jnp.maximum(it - NEARLY, 0)
        views = prep_views(odd, pc)
        npiece = 0
        for op in SCHED:
            if op[0] == "proj":
                proj(op[1])
            elif op[0] == "attn":
                attn(op[1], op[2])
                if npiece < 8:
                    prep(views, npiece)
                    k0 = (8 * int(odd) + npiece) * 64
                    pr = _ld(wmod_v, (it,), k0, 64).astype(F32) * st_v[k0:k0 + 64, :]
                    for g in range(8):
                        macc = pr[8 * g:8 * g + 8] if macc is None else macc + pr[8 * g:8 * g + 8]
                    lt_v[LT_ROWS - 16:LT_ROWS, :] = _bf(macc)
                    npiece += 1
            else:
                wo(*op[1:])
        res = jnp.concatenate([part[j] for j in range(8)], axis=1)
        for g in range(3):
            x1_v[pl.ds(pl.multiple_of(g * T0 + 8 * s, 8), 8), :] = res[8 * g + 8:8 * g + 16]
        return res[0:8], macc

    with _scope("main"):
        def steps(i, mem):
            @pl.when(i == NEARLY)
            def _():
                wait(late)

            with _scope("iter"):
                mem, macc = step(i, True, *step(i, False, mem, None))
                mod_v[0:1, pl.ds(pl.multiple_of((16 + i) * 128, 128), 128)] = jnp.sum(macc, axis=0, keepdims=True)

            return mem

        lax.fori_loop(0, NSEG // 2, steps, mem0_ref[...].astype(F32))

    def resid1(r, k0, n, c0=0, nc=D):
        xb = x_v[pl.ds((r >> 3) + k0 // 8, n // 8), :, c0:c0 + nc].astype(F32).reshape(n, nc)
        return xb + mod_v[0:1, 2 * D + c0:2 * D + c0 + nc] * x1_v[pl.ds(r + k0, n), c0:c0 + nc]

    def h2_view(slot, k0=0):
        r = slot * H2_SLOT + k0
        return h2_v.at[pl.ds(pl.multiple_of(r, LNP), H2_SLOT - HB + (HB if isinstance(k0, int) else LNP)), :]

    def ln2(dst, r, k0):
        hm = [_ln(resid1(r, k0 + m * HB, LNP)) * (1.0 + mod_v[0:1, 4 * D:5 * D])
              + mod_v[0:1, 3 * D:4 * D] for m in range(2)]
        for j in range(2):
            blocks = {(m, k): hm[m][:, k * 256 + j * 128:k * 256 + (j + 1) * 128]
                      for m in range(2) for k in range(4)}
            memo = {}
            for i, terms in enumerate(HKL):
                o = (2 * i + j) * HB + k0
                dst[o:o + LNP, :] = _comb(terms, blocks, memo).astype(BF16)

    def wo_body(j, carry):
        acc = {}
        for kc in range(4):
            b = [jnp.concatenate([_ld(wo_v, (j + 4 * n,), (2 * p + t) * DH, DH)
                                  for p in range(4 * kc, 4 * kc + 4)], axis=0)
                 for t in range(2) for n in range(2)]
            tt = _strassen_rhs(*[x.astype(F32) for x in b])
            tt = [b[0] if k == 1 else b[3] if k == 4 else tt[k].astype(BF16) for k in range(7)]
            for k in SORD:
                sk = jnp.concatenate([_ld(so_v, (k, p), 0, TH) for p in range(4 * kc, 4 * kc + 4)], axis=1)
                y = _dot(sk, tt[k])
                acc[k] = y + acc[k] if kc else y
        for e in range(2):
            k0 = (2 * j + e) * LNP
            ln2(h2_view(0, k0), pl.multiple_of(k0, LNP), 0)
        for t, c in enumerate(_strassen_out(acc)):
            cs = pl.ds(pl.multiple_of((j + 4 * (t % 2)) * 128, 128), 128)
            for g in range(NSEG // 2):
                r0 = 3 * T0 + (2 * g + t // 2) * 8
                x1_v[r0:r0 + 8, cs] = c[8 * g:8 * g + 8]
        return carry

    with _scope("p3a"):
        lax.fori_loop(0, 4, wo_body, 0)

    def out_copy(i, q):
        cols = pl.ds(q * 256, 256)
        return pltpu.make_async_copy(x_v.at[pl.ds(i * (FB // 8), FB // 8), :, cols],
                                     out_hbm.at[pl.ds((i & 1) * (FB // 8), FB // 8), ((i >> 1) + 1) & 3, :, cols],
                                     sems.at[SEM_OUT + i])

    def ffn_body(i, carry):
        r0 = pl.multiple_of(i * FB, FB)
        rn = pl.multiple_of(jnp.minimum(r0 + FB, S - FB), FB)
        h2_cur, h2_nxt = h2_view(i & 1), h2_view(1 - (i & 1))
        acc = {}
        act = {}
        memo = {}

        def accumulate(key, r, y):
            a = acc.setdefault(key, {})
            a[HK[r][2]] = y + a[HK[r][2]] if HK[r][2] in a else y

        def up(f, lo, hi):
            for idx in range(lo, hi):
                r = HKBLK[idx]
                lhs = jnp.concatenate([_ld(h2_cur, (), (2 * HKL.index(HK[r][0]) + j) * HB, HB) for j in range(2)], axis=1)
                if r in HKSUM:
                    w = _ld(lt_v, (), T1_ROW + HKSUM.index(r) * TS + 256 * f, 256)
                else:
                    k, n, _ = HK[r][1][0]
                    w = _ld(w1_v, (4 * f + n,), 256 * k, 256)
                accumulate(("up", f), r, _dot(lhs, w))
                for m, n, _ in HK[r][2]:
                    if not any((m, n) == t[0:2] for rr in HKBLK[idx + 1:] for t in HK[rr][2]):
                        c0 = (4 * f + n) * 128
                        act.setdefault(f, {})[m, n] = _gelu(
                            _collect(acc["up", f], m, n) + bias_v[0:1, c0:c0 + 128])

        def down(fs, q, r):
            if (fs, HK[r][0]) not in memo:
                memo[fs, HK[r][0]] = jnp.concatenate(
                    [_comb(HK[r][0], act[f], memo.setdefault(f, {})) for f in fs], axis=1).astype(BF16)
            if r in HKSUM:
                w = _ld(lt_v, (), T2_ROW + HKSUM.index(r) * TS + q * (FF // 4) + 128 * fs[0], 128 * len(fs))
            else:
                k, n, _ = HK[r][1][0]
                w = jnp.concatenate([_ld(w2_v, (4 * q + n,), 512 * f + 128 * k, 128) for f in fs], axis=0)
            accumulate(q, r, _dot(memo[fs, HK[r][0]], w))

        def finish(q, n):
            c0 = (4 * q + n) * 128
            for m in range(2):
                y = (_collect({HK[r][2]: acc[q][HK[r][2]] for r in HKCOL}, m, n) + bias_v[0:1, FF + c0:FF + c0 + 128]) * mod_v[0:1, 5 * D + c0:5 * D + c0 + 128]
                o = (resid1(r0, m * HB, HB, c0, 128) + y).reshape(HB // 8, 8, 128).astype(BF16)
                x_v[pl.ds((r0 >> 3) + m * (HB // 8), HB // 8), :, c0:c0 + 128] = o
            if n % 2:
                out_copy(i, 2 * q + n // 2).start()

        work = [(fs, q, r) for fs in ((0, 1), (2, 3), (4, 5)) for r in range(len(HK)) for q in range(2)]
        piece = 0
        for f in range(FF // 512):
            for lo, hi in ((0, 14), (14, len(HK))):
                up(f, lo, hi)
                ready = [x for x in work[:14] if x[0][-1] < f]
                if ready and piece * LNP < HB:
                    ln2(h2_nxt, rn, piece * LNP)
                    piece += 1
                for x in ready:
                    down(*x)
                work = work[len(ready):]
        assert piece * LNP == HB
        for x in work:
            down(*x)
        for q in range(2):
            for idx, r in enumerate(HKCOL):
                down((6,), q, r)
                for n in range(4):
                    if idx == max(j for j, rr in enumerate(HKCOL) if any(t[1] == n for t in HK[rr][2])):
                        finish(q, n)
        return carry

    with _scope("ffn"):
        lax.fori_loop(0, S // FB, ffn_body, 0)
    with _scope("wait_out"):
        for i in range(S // FB):
            for q in range(4):
                out_copy(i, q).wait()


@jax.jit
def pallas_adaLN_cond__memory_aug_recurrent_mem_tr__dense_activation_gelu__prompt_kernel(
    A_x, A_mem0, A_Wq, A_Wk, A_Wv, A_Wo, A_seg_len, B_x, B_w1, B_b1, B_w2, B_b2, c, w_mod,
):
    del A_seg_len, B_x
    assert A_x.shape == (1, S, D)
    hbm = pl.BlockSpec(memory_space=pl.ANY)
    out = pl.pallas_call(
        _kernel,
        out_shape=jax.ShapeDtypeStruct((NSEG, 4, 8, D), BF16),
        in_specs=[hbm] * 12,
        out_specs=hbm,
        scratch_shapes=[
            pltpu.VMEM((4 * NSEG, 8, D), BF16),
            pltpu.VMEM((8, T0, 128), BF16),
            pltpu.VMEM((TPS, D), F32),
            pltpu.VMEM((2 * H2_SLOT, 128), BF16),
            pltpu.VMEM((S, D), F32),
            pltpu.VMEM((32, D, 128), BF16),
            pltpu.VMEM((8, 6 * D), F32),
            pltpu.VMEM((8, D), BF16),
            pltpu.VMEM((6 * NP + 1, D // 2, 128), U32),
            pltpu.VMEM((8, H * DH, 128), BF16),
            pltpu.VMEM((FF // 128, D, 128), BF16),
            pltpu.VMEM((D // 128, FF, 128), BF16),
            pltpu.VMEM((LT_ROWS, 128), BF16),
            pltpu.VMEM((3 * NP, 64, 128), BF16),
            pltpu.VMEM((H, 32, 128), BF16),
            pltpu.VMEM((NP, 80, 128), BF16),
            pltpu.VMEM((80, 128), F32),
            pltpu.VMEM((1, FF + D), F32),
            pltpu.VMEM((8, T0, 128), F32),
            pltpu.VMEM((M, D), BF16),
            pltpu.VMEM((FF,), BF16),
            pltpu.VMEM((D,), BF16),
            pltpu.VMEM((1, D), BF16),
            pltpu.VMEM((len(HKLS), 2, TH, 128), BF16),
            pltpu.VMEM((7, NP, T0 // 2, 128), BF16),
            pltpu.VMEM((NP, 16, 128), F32),
            pltpu.VMEM((D, 128), F32),
            pltpu.SemaphoreType.DMA((SEM_N,)),
        ],
        compiler_params=pltpu.CompilerParams(vmem_limit_bytes=122 * 1024 * 1024, disable_bounds_checks=True,
                                             disable_semaphore_checks=True),
    )(
        A_x.reshape(NSEG, 4, 8, D), A_mem0.reshape(M, D),
        A_Wq.reshape(D // 2, 2, H, DH), A_Wk.reshape(D // 2, 2, H, DH), A_Wv.reshape(D // 2, 2, H, DH),
        A_Wo.reshape(H * DH, D), B_w1, B_b1, B_w2, B_b2, c, w_mod,
    )
    return out.reshape(1, S, D)
```

```python
import contextlib

import jax
import jax.numpy as jnp
from jax import lax
import jax.experimental.pallas as pl
import jax.experimental.pallas.tpu as pltpu

F32 = jnp.float32
BF16 = jnp.bfloat16
U32 = jnp.uint32

S = 2048
D = 1024
H = 32
DH = 128
M = 8
SEG = 32
FF = 3584
EPS = 1e-5
LOG2E = 1.4426950408889634

NSEG = S // SEG
NP = H // 2
TPS = SEG - 8
T0 = 8 * NSEG
TH = T0 // 2
UA = 8
P1N = 4
NEARLY = 4
FB = 256
HB = FB // 2
MROWS = (0, 336, 688, 1024)
LNP = 16

SORD = (1, 4, 3, 2, 0, 6, 5)

HK = (
    (((0, 0, 1), (1, 0, -1)), ((0, 0, 1), (0, 1, 1), (2, 0, -1)), ((0, 0, 1),)),
    (((1, 0, 1),), ((0, 0, 1), (0, 2, 1), (1, 0, -1)), ((0, 0, 1), (1, 0, 1))),
    (((0, 1, 1),), ((1, 1, 1), (1, 2, 1), (0, 1, -1), (3, 1, -1)), ((0, 1, 1), (1, 1, 1))),
    (((1, 1, 1), (0, 1, -1)), ((1, 0, 1), (1, 1, 1), (1, 3, 1), (2, 1, -1)), ((1, 1, 1),)),
    (((0, 2, 1),), ((2, 1, 1), (2, 2, 1), (0, 2, -1), (3, 2, -1)), ((0, 2, 1),)),
    (((1, 2, 1),), ((2, 0, 1), (2, 2, 1), (2, 3, 1), (1, 2, -1)), ((1, 2, 1),)),
    (((0, 3, 1), (1, 3, -1)), ((3, 1, 1), (3, 3, 1), (2, 3, -1)), ((0, 3, 1),)),
    (((1, 3, 1),), ((3, 2, 1), (3, 3, 1), (1, 3, -1)), ((0, 3, 1), (1, 3, 1))),
    (((0, 1, 1), (1, 0, 1)), ((0, 1, 1), (1, 0, 1)), ((0, 0, 1), (1, 1, 1))),
    (((0, 0, 1), (0, 1, 1)), ((0, 1, 1),), ((0, 0, -1), (0, 1, 1))),
    (((1, 0, 1), (1, 1, 1)), ((1, 0, 1),), ((1, 0, 1), (1, 1, -1))),
    (((0, 0, 1), (0, 2, 1), (1, 0, -1)), ((0, 2, 1), (2, 0, 1)), ((0, 0, 1), (1, 0, 1), (1, 2, -1))),
    (((0, 0, 1), (0, 2, 1)), ((0, 2, 1),), ((0, 0, -1), (0, 2, 1), (1, 0, -1), (1, 2, 1))),
    (((0, 0, 1), (0, 2, 1), (1, 0, -1), (1, 2, -1)), ((2, 0, 1),), ((1, 0, -1), (1, 2, 1))),
    (((0, 3, 1),), ((3, 0, 1),), ((0, 0, 1),)),
    (((1, 3, 1),), ((3, 0, 1),), ((1, 0, 1),)),
    (((0, 0, 1),), ((0, 3, 1),), ((0, 3, 1),)),
    (((1, 0, 1),), ((0, 3, 1),), ((1, 3, 1),)),
    (((1, 1, 1), (1, 2, 1), (0, 1, -1)), ((1, 2, 1), (2, 1, 1)), ((0, 1, 1), (0, 2, -1), (1, 1, 1))),
    (((1, 1, 1), (1, 2, 1)), ((1, 2, 1),), ((0, 1, -1), (0, 2, 1), (1, 1, -1), (1, 2, 1))),
    (((1, 1, 1), (1, 2, 1), (0, 1, -1), (0, 2, -1)), ((2, 1, 1),), ((0, 1, -1), (0, 2, 1))),
    (((0, 1, 1), (1, 3, 1)), ((1, 3, 1), (3, 1, 1)), ((0, 3, 1), (1, 1, 1))),
    (((1, 1, 1), (1, 3, 1)), ((1, 3, 1),), ((1, 1, -1), (1, 3, 1))),
    (((0, 1, 1), (0, 3, 1)), ((3, 1, 1),), ((0, 1, 1), (0, 3, -1))),
    (((0, 2, 1), (0, 3, 1), (1, 3, -1)), ((2, 3, 1), (3, 2, 1)), ((0, 3, 1), (1, 2, -1), (1, 3, 1))),
    (((0, 2, 1), (0, 3, 1), (1, 3, -1), (1, 2, -1)), ((2, 3, 1),), ((1, 2, 1), (1, 3, -1))),
    (((0, 2, 1), (0, 3, 1)), ((3, 2, 1),), ((0, 2, 1), (0, 3, -1), (1, 2, 1), (1, 3, -1))),
)
HKSUM = tuple(r for r, t in enumerate(HK) if len(t[1]) > 1)
HKCOL = tuple(sorted(range(len(HK)), key=lambda r: min(n for _, n, _ in HK[r][2])))
HKBLK = (7, 17, 22, 24, 25, 26, 6, 16, 21, 23, 5, 11, 12, 13, 19, 4, 18, 20, 2, 9, 3, 8, 10, 1, 15, 0, 14)
HKL = tuple(dict.fromkeys(t[0] for t in HK))
HKLS = tuple(t for t in HKL if len(t) > 1)
P1ORD = (9, 10, 14, 15, 13, 12, 1, 11, 0, 8, 19, 20, 23, 2, 18, 22, 3, 21, 25, 5, 24, 17, 7, 26, 16, 6, 4)
TS = FF // 2

T1_ROW = 3 * NP * 2 * T0
T2_ROW = T1_ROW + len(HKSUM) * TS
LT_ROWS = T2_ROW + len(HKSUM) * TS + 16

H2_SLOT = len(HKL) * 2 * HB

SEM_W, SEM_A, SEM_M, SEM_MISC, SEM_OUT = 0, 48, 56, 64, 72
SEM_N = SEM_OUT + S // FB


def _make_sched(h1=24, n1=1, n2=4):
    out = []

    def pairs(a):
        return tuple(p for p in (a, a + 1) if 0 <= p < NP)

    nxt = 0
    for p in range(NP):
        out.append(("proj", p))
        if p >= 2 and p % 2 == 0:
            out.append(("attn", pairs(nxt - 2), pairs(nxt)))
            nxt += 2
    out += [("wo", j, 0, h1) for j in range(n1)]
    out.append(("attn", pairs(nxt - 2), pairs(nxt)))
    out += [("wo", j, 0, h1) for j in range(n1, n2)]
    out.append(("attn", pairs(nxt), ()))
    out += [("wo", j, 0, h1) for j in range(n2, 8)]
    out += [("wo", j, h1, H) for j in range(8)]
    return out


SCHED = _make_sched()
_SCOPES = False


def _scope(name):
    return jax.named_scope(name) if _SCOPES else contextlib.nullcontext()


def _dot(a, b):
    return jnp.dot(a, b, preferred_element_type=F32)


def _bf(x):
    return pltpu.bitcast(x, BF16)


def _unit(p, j):
    return 6 * (p // 2) + 2 * j + p % 2


def _ld(ref, idx, r0, n):
    return _bf(ref.at[(*idx, pl.ds(r0, n), slice(None))].bitcast(U32)[...])


def _ln(x):
    m = jnp.mean(x, axis=-1, keepdims=True)
    xc = x - m
    v = jnp.mean(xc * xc, axis=-1, keepdims=True)
    return xc * lax.rsqrt(v + EPS)


def _gelu(x):
    c = 0.7978845608028654
    hx = 0.5 * x
    return hx + hx * jnp.tanh(x * (c + (c * 0.044715) * (x * x)))


def _strassen_lhs(a11, a12, a21, a22):
    return [a11 + a22, a21 + a22, a11, a22, a11 + a12, a21 - a11, a12 - a22]


def _strassen_rhs(b11, b12, b21, b22):
    return [b11 + b22, b11, b12 - b22, b21 - b11, b22, b11 + b12, b21 + b22]


def _strassen_out(m):
    return (m[0] + m[3] - m[4] + m[6], m[2] + m[4], m[1] + m[3], m[0] - m[1] + m[2] + m[5])


def _comb(terms, blocks, memo=None):
    memo = {} if memo is None else memo
    for n in range(1, len(terms) + 1):
        key = terms[:n]
        if key not in memo:
            i, j, sg = terms[n - 1]
            b = blocks[i, j]
            memo[key] = b if n == 1 else (memo[terms[:n - 1]] + b if sg > 0 else memo[terms[:n - 1]] - b)
    return memo[terms]


def _collect(acc, m, n):
    c = None
    for pat, y in acc.items():
        for mm, nn, sg in pat:
            if (mm, nn) == (m, n):
                c = (y if sg > 0 else -y) if c is None else (c + y if sg > 0 else c - y)
    return c


def _interleave(a, b):
    n = a.shape[0] // 8
    parts = []
    for g in range(n):
        parts.append(a[8 * g:8 * g + 8])
        parts.append(b[8 * g:8 * g + 8])
    return jnp.concatenate(parts, axis=0)


def _deinterleave(v):
    n = v.shape[0] // 16
    a = jnp.concatenate([v[16 * g:16 * g + 8] for g in range(n)], axis=0)
    b = jnp.concatenate([v[16 * g + 8:16 * g + 16] for g in range(n)], axis=0)
    return a, b


def _kernel(x_hbm, mem0_hbm, wq_hbm, wk_hbm, wv_hbm, wo_hbm, w1_hbm, b1_hbm, w2_hbm, b2_hbm,
            c_hbm, wmod_hbm, out_hbm,
            x_v, h_v, hn_v, h2_v, x1_v, wmod_v, mod_v, sc_v, w_v, wo_v, w1_v, w2_v,
            lt_v, fr_v, lo_v, pr_v, fill_v, bias_v, n_v,
            mem0_ref, b1_ref, b2_ref, c_ref, hs_v, so_v, ev_v, st_v,
            sems):
    w32 = [r.bitcast(U32) for r in (wq_hbm, wk_hbm, wv_hbm)]

    def w_copies(c, js=range(3)):
        return [pltpu.make_async_copy(w32[j].at[:, par, 2 * c + e, :], w_v.at[2 * (6 * c + 2 * j + e) + par],
                                      sems.at[SEM_W + 6 * c + 2 * j + e])
                for j in js for e in range(2) for par in range(2)]

    def w_wait(u):
        both = w_v.at[pl.ds(2 * u, 2)]
        pltpu.make_async_copy(both, both, sems.at[SEM_W + u]).wait()

    def _mult(i, m):
        return i * m if isinstance(i, int) else pl.multiple_of(i * m, m)

    def wa_copies(k, units=range(UA)):
        r = pl.ds(_mult(k, 64), 64)
        return [pltpu.make_async_copy(w32[u % 6 // 2].at[r, par, u // 6 * 2 + u % 2, :], w_v.at[2 * u + par, r],
                                      sems.at[SEM_A + k]) for u in units for par in range(2)]

    def m_copies(k):
        return [pltpu.make_async_copy(wmod_hbm.at[:, pl.ds(_mult(k + 8 * t, 128), 128)], wmod_v.at[16 + k + 8 * t],
                                      sems.at[SEM_M + k]) for t in range(2)]

    def start(cps):
        for cp in cps:
            cp.start()

    def wait(cps):
        for cp in cps:
            cp.wait()

    cp_x0 = pltpu.make_async_copy(x_hbm.at[:, 0], x_v.at[3 * NSEG:4 * NSEG], sems.at[SEM_MISC + 1])

    def x_pairs(s0, s1):
        return [(x_hbm.at[s0:s1, g + 1], x_v.at[g * NSEG + s0:g * NSEG + s1]) for g in range(3)]

    def wo_copy(j):
        return pltpu.make_async_copy(wo_hbm.at[:, pl.ds(_mult(j, 128), 128)], wo_v.at[j], sems.at[SEM_MISC + 3])

    def late_copies(first):
        sem = sems.at[SEM_MISC + (4 if first else 5)]
        cps = x_pairs(1, 2 * NEARLY + 1) if first else x_pairs(2 * NEARLY + 1, NSEG)
        cps += [(wmod_hbm.at[:, (16 + j) * 128:(17 + j) * 128], wmod_v.at[j])
                for j in (range(NEARLY) if first else range(NEARLY, 32))]
        for src, dst, nt, nr in ((w1_hbm, w1_v, FF // 128, D), (w2_hbm, w2_v, D // 128, 512)):
            for j in range(nt):
                if j < 4:
                    rows = slice(0, nr) if first else slice(nr, src.shape[0])
                else:
                    rows = slice(0, 0) if first else slice(0, src.shape[0])
                if rows.stop > rows.start:
                    cps.append((src.at[rows, j * 128:(j + 1) * 128], dst.at[j, rows]))
        return [pltpu.make_async_copy(src, dst, sem) for src, dst in cps]

    cp_small = [pltpu.make_async_copy(src, dst, sems.at[SEM_MISC])
                for src, dst in [(c_hbm, c_ref), (mem0_hbm, mem0_ref), (b1_hbm, b1_ref), (b2_hbm, b2_ref)]
                + x_pairs(0, 1)]

    start(cp_small)
    cp_x0.start()
    start(m_copies(0))
    for k in range(2):
        start(m_copies(k + 1))
        start(wa_copies(k))

    scale = DH ** -0.5
    ri = lax.broadcasted_iota(jnp.int32, (80, 128), 0)
    ci = lax.broadcasted_iota(jnp.int32, (80, 128), 1)
    same_head = (((ri >> 3) & 1) == ((ci >> 3) & 1)) & (ci < 80)
    rpos = (((ri >> 4) & 3) << 3) + (ri & 7)
    cpos = (((ci >> 4) & 3) << 3) + (ci & 7)
    keep = (ri < 16) | (ci < 16) | (rpos >= cpos)
    fill_v[...] = jnp.where(same_head, jnp.where(keep, 0.0, -1e9 / scale), -jnp.inf).astype(F32)

    wait(cp_small)
    c = c_ref[...].astype(F32)
    sc = jnp.broadcast_to(c * jax.nn.sigmoid(c), (8, D)).astype(BF16)

    sc_v[...] = sc
    for k in range(8):
        st_v[k * 128:(k + 1) * 128, :] = jnp.broadcast_to(sc[0:1, k * 128:(k + 1) * 128].astype(F32), (128, 128)).T
    bias_v[:, 0:FF] = b1_ref[...].astype(F32).reshape(1, FF)
    bias_v[:, FF:FF + D] = b2_ref[...].astype(F32).reshape(1, D)

    def zero_body(i, carry):
        x1_v[pl.ds(pl.multiple_of(i * 64, 64), 64), :] = jnp.zeros((64, D), F32)
        return carry

    lax.fori_loop(0, -(-UA // 4) * 8, zero_body, 0)

    def relayout(c, rows):
        a = w_v[c, rows, :]
        b = w_v[c + 1, rows, :]
        lo = (a & jnp.uint32(0xFFFF)) | (b << 16)
        hi = (a >> 16) | (b & jnp.uint32(0xFFFF0000))
        w_v[c, rows, :] = lo
        w_v[c + 1, rows, :] = hi
        return _bf(lo), _bf(hi)

    def store_lead(u, a, b):
        lt_v[pl.ds(_mult(u, 2 * T0), 2 * T0), :] = _interleave(a, b).astype(BF16)

    def mod_tile(ct):
        m = _dot(sc_v[...], _ld(wmod_v, (16 + ct,), 0, D))
        mod_v[:, pl.ds(_mult(ct, 128), 128)] = m
        return m[0:1]

    with _scope("wait_x0"):
        cp_x0.wait()

    def ln1_body(i, carry):
        r = pl.multiple_of(i * 128, 128)
        n = _ln(x_v[pl.ds(3 * NSEG + i * 16, 16)].astype(F32).reshape(128, D))
        for k in range(8):
            n_v[k, pl.ds(r, 128), :] = n[:, k * 128:(k + 1) * 128]
        return carry

    with _scope("ln1"):
        lax.fori_loop(0, T0 // 128, ln1_body, 0)
    start(m_copies(3))
    start(wa_copies(2))
    with _scope("wait_m0"):
        wait(m_copies(0))
    h_v[0] = (n_v[0] * (1.0 + mod_tile(8)) + mod_tile(0)).astype(BF16)

    def hs_piece(j, r):
        blocks = {(m, k): _ld(h_v, (2 * k + j,), m * TH + r, 16).astype(F32) for m in range(2) for k in range(4)}
        memo = {}
        for i, terms in enumerate(HKLS):
            hs_v[i, j, r:r + 16, :] = _comb(terms, blocks, memo).astype(BF16)

    def sa_body(k, carry):
        last = isinstance(k, int)
        with _scope("wait_a"):
            wait(wa_copies(k))
            if not last:
                wait(m_copies(k + 1))

        rows = pl.ds(_mult(k, 64), 64)
        hk = _ld(h_v, (k,), 0, T0)
        macc = [None, None]
        for u in range(UA):
            res = []
            for t, w in enumerate(relayout(2 * u, rows)):
                c = 2 * u + t
                acc = x1_v.at[c // 8 * T0:(c // 8 + 1) * T0, c % 8 * 128:(c % 8 + 1) * 128]
                r = _dot(hk, w) + acc[...]
                if not last:
                    acc[...] = r
                res.append(r)
            if last:
                store_lead(u, *res)
                for e in range(4 * u, 4 * u + 4):
                    hs_piece(e % 2, (e // 2) * 16)
                continue
            if u in (1, 3, 5):
                r0, nr = MROWS[u // 2], MROWS[u // 2 + 1] - MROWS[u // 2]
                sb = st_v[r0:r0 + nr, :]
                for t in range(2):
                    pr = _ld(wmod_v, (17 + k + 8 * t,), r0, nr).astype(F32) * sb
                    for g in range(nr // 8):
                        macc[t] = pr[8 * g:8 * g + 8] if macc[t] is None else macc[t] + pr[8 * g:8 * g + 8]
                    w_v[6 * NP, 8 * t:8 * t + 8, :] = pltpu.bitcast(macc[t], U32)
            if u == 5:
                sh, sc1 = [jnp.sum(m_, axis=0, keepdims=True) for m_ in macc]
                mod_v[0:1, pl.ds(_mult(k + 1, 128), 128)] = sh
                mod_v[0:1, pl.ds(_mult(k + 9, 128), 128)] = sc1
            if u == 6:
                @pl.when(k + 4 < 8)
                def _():
                    start(m_copies(k + 4))

            if u >= 4 and u % 2 == 0:
                @pl.when(k + 3 < 8)
                def _():
                    start(wa_copies(k + 3, range((u - 4) * 2, (u - 4) * 2 + 4)))

        if last:
            start(w_copies(3))
            return carry
        h_v[k + 1] = (n_v[k + 1] * (1.0 + sc1) + sh).astype(BF16)

        @pl.when(k == 4)
        def _():
            start(w_copies(1, range(1, 3)))

        @pl.when(k == 5)
        def _():
            start(w_copies(2))

        return carry

    with _scope("stageA"):
        lax.fori_loop(0, 7, sa_body, 0)
        sa_body(7, 0)

    def ln1(seg):
        xb = jnp.concatenate([x_v[g * NSEG + seg].astype(F32) for g in range(3)], axis=0)
        return _ln(xb) * (1.0 + mod_v[0:1, D:2 * D]) + mod_v[0:1, 0:D]

    def lhs1(terms):
        if len(terms) == 1:
            m, k, _ = terms[0]
            tiles = [_ld(h_v, (2 * k + j,), m * TH, TH) for j in range(2)]
        else:
            tiles = [_ld(hs_v, (HKLS.index(terms), j), 0, TH) for j in range(2)]
        return jnp.concatenate(tiles, axis=1)

    NP1 = (3 * NP - UA) // P1N
    late = late_copies(False)
    nl = -(-len(late) // 6)

    def p1_body(i, carry):
        u0 = UA + P1N * i
        with _scope("wait_w"):
            for q in range(P1N):
                w_wait(u0 + q)

        def dma_slot(q):
            if q == 0:
                @pl.when(i < 4)
                def _():
                    start(w_copies(4 + i))
            elif q == 2:
                @pl.when(jnp.logical_and(i >= 3, i < 7))
                def _():
                    start([wo_copy(2 * (i - 3) + r) for r in range(2)])
            elif q == 3:
                @pl.when(i == 6)
                def _():
                    start(late_copies(True))

            @pl.when(i == NP1 - 1)
            def _():
                start(late[q * nl:(q + 1) * nl])

        for g in range(P1N // 2):
            u = u0 + 2 * g
            tiles = relayout(2 * u, slice(None)) + relayout(2 * u + 2, slice(None))
            b = {(k, n): tiles[n][256 * k:256 * (k + 1)] for k in range(4) for n in range(4)}
            bf = {key: x.astype(F32) for key, x in b.items()}
            acc = {}
            for idx, r in enumerate(P1ORD):
                terms = HK[r][1]
                w = b[terms[0][0:2]] if len(terms) == 1 else _comb(terms, bf).astype(BF16)
                y = _dot(lhs1(HK[r][0]), w)
                acc[HK[r][2]] = y + acc[HK[r][2]] if HK[r][2] in acc else y
                if idx % 9 == 8:
                    dma_slot(3 * g + idx // 9)
            c = {(m, n): _collect(acc, m, n) for m in range(2) for n in range(4)}
            col = [jnp.concatenate([c[0, n], c[1, n]], axis=0) for n in range(4)]
            store_lead(u, col[0], col[1])
            store_lead(u + 1, col[2], col[3])

        hn_v[...] = ln1(0)
        return carry

    with _scope("phase1"):
        lax.fori_loop(0, NP1, p1_body, 0)

    with _scope("wait_wo"):
        wait([wo_copy(j) for j in range(8)])
        wait(late_copies(True))

    def prep_views(odd, pc):
        f = pc >> 2
        if odd:
            q, half = (pc >> 1) & 1, pc & 1
            kb, w, tile0, r0 = 128, w2_v, 4 * q, 512 * f + 64 * half
            d0 = T2_ROW + q * (FF // 4) + 128 * f + 64 * half
        else:
            kb, w, tile0, r0 = 256, w1_v, 4 * f, 64 * (pc & 3)
            d0 = T1_ROW + 64 * pc
        src = w.at[pl.ds(tile0, 4), pl.ds(pl.multiple_of(r0, 64), 3 * kb + 64), :]
        dst = lt_v.at[pl.ds(pl.multiple_of(d0, 64), (len(HKSUM) - 1) * TS + 64), :]
        return src, dst, kb

    def prep(views, piece):
        src, dst, kb = views
        r0 = (piece // 2) * 16
        sel = HKSUM[:6] if piece % 2 == 0 else HKSUM[6:]
        need = sorted({(k, n) for r in sel for k, n, _ in HK[r][1]})
        blocks = {(k, n): _ld(src, (n,), k * kb + r0, 16).astype(F32) for k, n in need}
        for r in sel:
            o = HKSUM.index(r) * TS + r0
            dst[o:o + 16, :] = _comb(HK[r][1], blocks).astype(BF16)

    def step(it, odd, mem, macc):
        s = 2 * it + int(odd)
        lead = lt_v.at[pl.ds(pl.multiple_of(16 * s, 16), T1_ROW), :]
        lhs = jnp.concatenate([mem, hn_v[...]], axis=0).astype(BF16)
        hn_v[...] = ln1(jnp.minimum(s + 1, NSEG - 1))

        def proj(p):
            if p == 0:
                ct = [2 * _unit(0, j) + t for j in range(3) for t in range(2)]
                half = [_dot(lhs[:, 0:D // 2], _bf(w_v[c, 0:D // 4, :])) for c in ct]
                cols = [_dot(lhs[:, D // 2:D], _bf(w_v[c, D // 4:D // 2, :])) + h for c, h in zip(ct, half)]
            for j in range(3):
                u = _unit(p, j)
                if p == 0:
                    r = _interleave(cols[j * 2], cols[j * 2 + 1])
                else:
                    r = _interleave(_dot(lhs, _bf(w_v[2 * u])), _dot(lhs, _bf(w_v[2 * u + 1])))
                fr_v[u] = r.astype(BF16)

        def stack(p, j):
            u = _unit(p, j)
            return jnp.concatenate([fr_v[u], _ld(lead, (), u * 2 * T0, 16)], axis=0)

        def attn(pvs, qks):
            os_ = [_dot(pr_v[p, :, 0:80], stack(p, 2)) for p in pvs]
            ss = [lax.dot_general(stack(p, 0), stack(p, 1), (((1,), (1,)), ((), ())),
                                  preferred_element_type=F32) for p in qks]
            for p, o in zip(pvs, os_):
                for t, oh in enumerate(_deinterleave(o[0:64])):
                    lo_v[2 * p + t] = oh.astype(BF16)
                if odd:
                    ev = ev_v[p]
                    for k, sk in enumerate(_strassen_lhs(ev[0:8], ev[8:16], o[64:72], o[72:80])):
                        so_v[k, p, pl.ds(pl.multiple_of(8 * it, 8), 8), :] = sk.astype(BF16)
                else:
                    ev_v[p] = o[64:80]
            for p, sc_ in zip(qks, ss):
                fill = fill_v[...]
                sc_ = jnp.concatenate([sc_, jnp.zeros((80, 48), F32)], axis=1)
                sc_ = jnp.where(fill == 0.0, sc_, fill)
                mx = jnp.max(sc_, axis=-1, keepdims=True)
                e = jnp.exp2((sc_ - mx) * (scale * LOG2E))
                l = jnp.sum(e, axis=-1, keepdims=True)
                r = pl.reciprocal(l, approx=True)
                pr_v[p] = (e * (r * (2.0 - l * r))).astype(BF16)

        part = {}

        def wo(j, h0, h1):
            lo = jnp.concatenate([lo_v[h] for h in range(h0, h1)], axis=1)
            r = _dot(lo, _ld(wo_v, (j,), h0 * DH, (h1 - h0) * DH))
            part[j] = r + part[j] if j in part else r

        pc = jnp.maximum(it - NEARLY, 0)
        views = prep_views(odd, pc)
        npiece = 0
        for op in SCHED:
            if op[0] == "proj":
                proj(op[1])
            elif op[0] == "attn":
                attn(op[1], op[2])
                if npiece < 8:
                    prep(views, npiece)
                    k0 = (8 * int(odd) + npiece) * 64
                    pr = _ld(wmod_v, (it,), k0, 64).astype(F32) * st_v[k0:k0 + 64, :]
                    for g in range(8):
                        macc = pr[8 * g:8 * g + 8] if macc is None else macc + pr[8 * g:8 * g + 8]
                    lt_v[LT_ROWS - 16:LT_ROWS, :] = _bf(macc)
                    npiece += 1
            else:
                wo(*op[1:])
        res = jnp.concatenate([part[j] for j in range(8)], axis=1)
        for g in range(3):
            x1_v[pl.ds(pl.multiple_of(g * T0 + 8 * s, 8), 8), :] = res[8 * g + 8:8 * g + 16]
        return res[0:8], macc

    with _scope("main"):
        def steps(i, mem):
            @pl.when(i == NEARLY)
            def _():
                wait(late)

            with _scope("iter"):
                mem, macc = step(i, True, *step(i, False, mem, None))
                mod_v[0:1, pl.ds(pl.multiple_of((16 + i) * 128, 128), 128)] = jnp.sum(macc, axis=0, keepdims=True)

            return mem

        lax.fori_loop(0, NSEG // 2, steps, mem0_ref[...].astype(F32))

    def resid1(r, k0, n, c0=0, nc=D):
        xb = x_v[pl.ds((r >> 3) + k0 // 8, n // 8), :, c0:c0 + nc].astype(F32).reshape(n, nc)
        return xb + mod_v[0:1, 2 * D + c0:2 * D + c0 + nc] * x1_v[pl.ds(r + k0, n), c0:c0 + nc]

    def h2_view(slot, k0=0):
        r = slot * H2_SLOT + k0
        return h2_v.at[pl.ds(pl.multiple_of(r, LNP), H2_SLOT - HB + (HB if isinstance(k0, int) else LNP)), :]

    def ln2(dst, r, k0):
        hm = [_ln(resid1(r, k0 + m * HB, LNP)) * (1.0 + mod_v[0:1, 4 * D:5 * D])
              + mod_v[0:1, 3 * D:4 * D] for m in range(2)]
        for j in range(2):
            blocks = {(m, k): hm[m][:, k * 256 + j * 128:k * 256 + (j + 1) * 128]
                      for m in range(2) for k in range(4)}
            memo = {}
            for i, terms in enumerate(HKL):
                o = (2 * i + j) * HB + k0
                dst[o:o + LNP, :] = _comb(terms, blocks, memo).astype(BF16)

    def wo_body(j, carry):
        acc = {}
        for kc in range(4):
            b = [jnp.concatenate([_ld(wo_v, (j + 4 * n,), (2 * p + t) * DH, DH)
                                  for p in range(4 * kc, 4 * kc + 4)], axis=0)
                 for t in range(2) for n in range(2)]
            tt = _strassen_rhs(*[x.astype(F32) for x in b])
            tt = [b[0] if k == 1 else b[3] if k == 4 else tt[k].astype(BF16) for k in range(7)]
            for k in SORD:
                sk = jnp.concatenate([_ld(so_v, (k, p), 0, TH) for p in range(4 * kc, 4 * kc + 4)], axis=1)
                y = _dot(sk, tt[k])
                acc[k] = y + acc[k] if kc else y
        for e in range(2):
            k0 = (2 * j + e) * LNP
            ln2(h2_view(0, k0), pl.multiple_of(k0, LNP), 0)
        for t, c in enumerate(_strassen_out(acc)):
            cs = pl.ds(pl.multiple_of((j + 4 * (t % 2)) * 128, 128), 128)
            for g in range(NSEG // 2):
                r0 = 3 * T0 + (2 * g + t // 2) * 8
                x1_v[r0:r0 + 8, cs] = c[8 * g:8 * g + 8]
        return carry

    with _scope("p3a"):
        lax.fori_loop(0, 4, wo_body, 0)

    def out_copy(i, q):
        cols = pl.ds(q * 256, 256)
        return pltpu.make_async_copy(x_v.at[pl.ds(i * (FB // 8), FB // 8), :, cols],
                                     out_hbm.at[pl.ds((i & 1) * (FB // 8), FB // 8), ((i >> 1) + 1) & 3, :, cols],
                                     sems.at[SEM_OUT + i])

    def ffn_body(i, carry):
        r0 = pl.multiple_of(i * FB, FB)
        rn = pl.multiple_of(jnp.minimum(r0 + FB, S - FB), FB)
        h2_cur, h2_nxt = h2_view(i & 1), h2_view(1 - (i & 1))
        acc = {}
        act = {}
        memo = {}

        def accumulate(key, r, y):
            a = acc.setdefault(key, {})
            a[HK[r][2]] = y + a[HK[r][2]] if HK[r][2] in a else y

        def up(f, lo, hi):
            for idx in range(lo, hi):
                r = HKBLK[idx]
                lhs = jnp.concatenate([_ld(h2_cur, (), (2 * HKL.index(HK[r][0]) + j) * HB, HB) for j in range(2)], axis=1)
                if r in HKSUM:
                    w = _ld(lt_v, (), T1_ROW + HKSUM.index(r) * TS + 256 * f, 256)
                else:
                    k, n, _ = HK[r][1][0]
                    w = _ld(w1_v, (4 * f + n,), 256 * k, 256)
                accumulate(("up", f), r, _dot(lhs, w))
                for m, n, _ in HK[r][2]:
                    if not any((m, n) == t[0:2] for rr in HKBLK[idx + 1:] for t in HK[rr][2]):
                        c0 = (4 * f + n) * 128
                        act.setdefault(f, {})[m, n] = _gelu(
                            _collect(acc["up", f], m, n) + bias_v[0:1, c0:c0 + 128])

        def down(fs, q, r):
            if (fs, HK[r][0]) not in memo:
                memo[fs, HK[r][0]] = jnp.concatenate(
                    [_comb(HK[r][0], act[f], memo.setdefault(f, {})) for f in fs], axis=1).astype(BF16)
            if r in HKSUM:
                w = _ld(lt_v, (), T2_ROW + HKSUM.index(r) * TS + q * (FF // 4) + 128 * fs[0], 128 * len(fs))
            else:
                k, n, _ = HK[r][1][0]
                w = jnp.concatenate([_ld(w2_v, (4 * q + n,), 512 * f + 128 * k, 128) for f in fs], axis=0)
            accumulate(q, r, _dot(memo[fs, HK[r][0]], w))

        def finish(q, n):
            c0 = (4 * q + n) * 128
            for m in range(2):
                y = _collect({HK[r][2]: acc[q][HK[r][2]] for r in HKCOL}, m, n)
                y = (y + bias_v[0:1, FF + c0:FF + c0 + 128]) * mod_v[0:1, 5 * D + c0:5 * D + c0 + 128]
                o = (resid1(r0, m * HB, HB, c0, 128) + y).reshape(HB // 8, 8, 128).astype(BF16)
                x_v[pl.ds((r0 >> 3) + m * (HB // 8), HB // 8), :, c0:c0 + 128] = o
            if n % 2:
                out_copy(i, 2 * q + n // 2).start()

        work = [(fs, q, r) for fs in ((0, 1), (2, 3), (4, 5)) for r in range(len(HK)) for q in range(2)]
        piece = 0
        for f in range(FF // 512):
            for lo, hi in ((0, 14), (14, len(HK))):
                up(f, lo, hi)
                ready = [x for x in work[:14] if x[0][-1] < f]
                if ready and piece * LNP < HB:
                    ln2(h2_nxt, rn, piece * LNP)
                    piece += 1
                for x in ready:
                    down(*x)
                work = work[len(ready):]
        assert piece * LNP == HB
        for x in work:
            down(*x)
        for q in range(2):
            for idx, r in enumerate(HKCOL):
                down((6,), q, r)
                for n in range(4):
                    if idx == max(j for j, rr in enumerate(HKCOL) if any(t[1] == n for t in HK[rr][2])):
                        finish(q, n)
        return carry

    with _scope("ffn"):
        lax.fori_loop(0, S // FB, ffn_body, 0)
    with _scope("wait_out"):
        for i in range(S // FB):
            for q in range(4):
                out_copy(i, q).wait()


@jax.jit
def pallas_adaLN_cond__memory_aug_recurrent_mem_tr__dense_activation_gelu__prompt_kernel(
    A_x, A_mem0, A_Wq, A_Wk, A_Wv, A_Wo, A_seg_len, B_x, B_w1, B_b1, B_w2, B_b2, c, w_mod,
):
    del A_seg_len, B_x
    assert A_x.shape == (1, S, D)
    hbm = pl.BlockSpec(memory_space=pl.ANY)
    out = pl.pallas_call(
        _kernel,
        out_shape=jax.ShapeDtypeStruct((NSEG, 4, 8, D), BF16),
        in_specs=[hbm] * 12,
        out_specs=hbm,
        scratch_shapes=[
            pltpu.VMEM((4 * NSEG, 8, D), BF16),
            pltpu.VMEM((8, T0, 128), BF16),
            pltpu.VMEM((TPS, D), F32),
            pltpu.VMEM((2 * H2_SLOT, 128), BF16),
            pltpu.VMEM((S, D), F32),
            pltpu.VMEM((32, D, 128), BF16),
            pltpu.VMEM((8, 6 * D), F32),
            pltpu.VMEM((8, D), BF16),
            pltpu.VMEM((6 * NP + 1, D // 2, 128), U32),
            pltpu.VMEM((8, H * DH, 128), BF16),
            pltpu.VMEM((FF // 128, D, 128), BF16),
            pltpu.VMEM((D // 128, FF, 128), BF16),
            pltpu.VMEM((LT_ROWS, 128), BF16),
            pltpu.VMEM((3 * NP, 64, 128), BF16),
            pltpu.VMEM((H, 32, 128), BF16),
            pltpu.VMEM((NP, 80, 128), BF16),
            pltpu.VMEM((80, 128), F32),
            pltpu.VMEM((1, FF + D), F32),
            pltpu.VMEM((8, T0, 128), F32),
            pltpu.VMEM((M, D), BF16),
            pltpu.VMEM((FF,), BF16),
            pltpu.VMEM((D,), BF16),
            pltpu.VMEM((1, D), BF16),
            pltpu.VMEM((len(HKLS), 2, TH, 128), BF16),
            pltpu.VMEM((7, NP, T0 // 2, 128), BF16),
            pltpu.VMEM((NP, 16, 128), F32),
            pltpu.VMEM((D, 128), F32),
            pltpu.SemaphoreType.DMA((SEM_N,)),
        ],
        compiler_params=pltpu.CompilerParams(vmem_limit_bytes=122 * 1024 * 1024, disable_bounds_checks=True,
                                             disable_semaphore_checks=True),
    )(
        A_x.reshape(NSEG, 4, 8, D), A_mem0.reshape(M, D),
        A_Wq.reshape(D // 2, 2, H, DH), A_Wk.reshape(D // 2, 2, H, DH), A_Wv.reshape(D // 2, 2, H, DH),
        A_Wo.reshape(H * DH, D), B_w1, B_b1, B_w2, B_b2, c, w_mod,
    )
    return out.reshape(1, S, D)
```
